```python
import jax
import jax.numpy as jnp

def _softmax(x, axis=-1):
    return jax.nn.softmax(x, axis=axis)

def _gelu(x):
    return jax.nn.gelu(x, approximate=True)

def _silu(x):
    return jax.nn.silu(x)

def _sigmoid(x):
    return jax.nn.sigmoid(x)

def _layernorm(x, axis=-1, eps=1e-05):
    m = jnp.mean(x, axis=axis, keepdims=True)
    v = jnp.var(x, axis=axis, keepdims=True)
    return (x - m) / jnp.sqrt(v + eps)

def _scatter_add(tgt, idx, src, axis=0):
    return tgt.at[idx].add(src)

def _segment_sum(src, seg, n):
    return jax.ops.segment_sum(src, seg, n)

class _Rng:

    def __init__(self, key):
        self._k = key

    def _next(self):
        self._k, sub = jax.random.split(self._k)
        return sub

    def normal(self, shape):
        return jax.random.normal(self._next(), shape, dtype=jnp.bfloat16)

    def randint(self, lo, hi, shape):
        return jax.random.randint(self._next(), shape, lo, hi, dtype=jnp.int32)

    def uniform(self, shape, lo=0.0, hi=1.0):
        return jax.random.uniform(self._next(), shape, jnp.bfloat16, lo, hi)

    def permutation(self, n):
        return jax.random.permutation(self._next(), n)
kernel_name = 'standalone__window_attn_davit__vision'

def setup_inputs():
    _rng = _Rng(jax.random.key(int.from_bytes(__import__("os").urandom(4), "little")))
    _w = lambda a: (lambda t: t.astype(jnp.bfloat16) if jnp.issubdtype(t.dtype, jnp.floating) else t)(jnp.asarray(a))
    HW = 512
    C0 = 192
    ws = 7
    nh = 4
    H = W = max(HW // ws * ws, ws)
    C = max(C0 // nh * nh, nh)
    k = 3
    return {'x': _w((lambda *s: _rng.normal(s) * 0.05)(1, H, W, C)), 'dw_pe': _w((lambda *s: _rng.normal(s) * 0.05)(k, k, C) * 0.1), 'w_qkv': _w((lambda *s: _rng.normal(s) * 0.05)(C, 3 * C) * C ** (-0.5)), 'w_o': _w((lambda *s: _rng.normal(s) * 0.05)(C, C) * C ** (-0.5))}

def reference(x, dw_pe, w_qkv, w_o):
    B, H, W, C = x.shape
    ws = 7
    nh = 4
    dh = C // nh
    kk = dw_pe.shape[0]
    pad = kk // 2
    xp = jnp.pad(x, ((0, 0), (pad, pad), (pad, pad), (0, 0)))
    pe = jnp.zeros_like(x)
    for i in range(kk):
        for j in range(kk):
            pe = pe + xp[:, i:i + H, j:j + W, :] * dw_pe[i, j][None, None, None, :]
    x0 = x + pe
    h = _layernorm(x0, axis=-1)
    hw = h.reshape(B, H // ws, ws, W // ws, ws, C)
    hw = (lambda x, *d: x.transpose(*d))(hw, 0, 1, 3, 2, 4, 5)
    hw = hw.reshape(-1, ws * ws, C)
    qkv = (hw @ w_qkv).reshape(-1, ws * ws, 3, nh, dh)
    q = qkv[:, :, 0].copy()
    k = qkv[:, :, 1].copy()
    v = qkv[:, :, 2].copy()
    scale = dh ** (-0.5)
    attn = jnp.einsum('wnhd,wmhd->whnm', q, k) * scale
    attn = _softmax(attn, axis=-1)
    out = jnp.einsum('whnm,wmhd->wnhd', attn, v)
    out = out.reshape(-1, ws * ws, C) @ w_o
    out = out.reshape(B, H // ws, W // ws, ws, ws, C)
    out = (lambda x, *d: x.transpose(*d))(out, 0, 1, 3, 2, 4, 5)
    out = out.reshape(B, H, W, C)
    return x0 + out
```

```python
import functools
import math

import jax
import jax.numpy as jnp
from jax import lax
import jax.experimental.pallas as pl
import jax.experimental.pallas.tpu as pltpu

WS = 7
NH = 4
C = 192
DH = C // NH
LANES = 128
WP = 512
NT = WP // LANES
SLOTS = 8 * WS
EPS = 1e-5
F32 = jnp.float32
BF16 = jnp.bfloat16
U32 = jnp.uint32

_NT_DIMS = (((1,), (1,)), ((), ()))


def _dot(a, b):
    return jnp.dot(a, b, preferred_element_type=F32)


def _dot_nt(a, b):
    return lax.dot_general(a, b, _NT_DIMS, preferred_element_type=F32)


def _kernel(xm_ref, xt_ref, xb_ref, dw_ref, wqkv_ref, wot_ref, o_ref,
            dws_ref, ws_ref, wos_ref, x0_ref, qkv_ref, ob_ref, *, W, nwin, nstrip):
    s = pl.program_id(0)

    @pl.when(s == 0)
    def _():
        for k in range(9):
            w = dw_ref[k]
            dws_ref[k] = w + 1.0 if k == 4 else w
        lane = lax.broadcasted_iota(jnp.int32, (C, LANES), 1)
        qs = (DH ** -0.5) * math.log2(math.e)
        for n in range(5):
            w = wqkv_ref[:, n * LANES:(n + 1) * LANES].astype(F32)
            if n == 0:
                w = jnp.where(lane >= 32, w * qs, w)
            elif n == 1:
                w = jnp.where((lane >= 32) & (lane < 64), w, w * qs)
            w = w.astype(BF16)
            ws_ref[0, n] = w[0:128]
            ws_ref[1, n] = w[64:192]
            ws_ref[2, n] = jnp.concatenate([w[128:192], w[0:64]], axis=0)
        wos_ref[...] = wot_ref[...]
        ob_ref[...] = jnp.zeros(ob_ref.shape, ob_ref.dtype)

    lane_w = lax.broadcasted_iota(jnp.int32, (8, WP), 1)
    valid_col = lane_w < W
    top_ok = s > 0
    bot_ok = s < nstrip - 1

    def conv_group(g):
        c0 = g * 8
        wts = [jnp.concatenate([dws_ref[k, pl.ds(c0, 8), :]] * NT, axis=1) for k in range(9)]

        def load_row(i):
            if i == 0:
                v = xt_ref[0, pl.ds(c0, 8), :].astype(F32)
                return jnp.where(valid_col & top_ok, v, 0.0)
            if i == WS + 1:
                v = xb_ref[0, pl.ds(c0, 8), :].astype(F32)
                return jnp.where(valid_col & bot_ok, v, 0.0)
            v = xm_ref[i - 1, pl.ds(c0, 8), :].astype(F32)
            last = jnp.where(valid_col[:, WP - LANES:], v[:, WP - LANES:], 0.0)
            return jnp.concatenate([v[:, :WP - LANES], last], axis=1)

        rows = [load_row(i) for i in range(WS + 2)]
        for r in range(WS):
            a = rows[r] * wts[0] + rows[r + 1] * wts[3] + rows[r + 2] * wts[6]
            b = rows[r] * wts[1] + rows[r + 1] * wts[4] + rows[r + 2] * wts[7]
            c = rows[r] * wts[2] + rows[r + 1] * wts[5] + rows[r + 2] * wts[8]
            x0 = pltpu.roll(a, 1, 1) + b + pltpu.roll(c, WP - 1, 1)
            x0_ref[r, pl.ds(c0, 8), :] = x0

    def conv_body(g, carry):
        conv_group(pl.multiple_of(g, 1))
        return carry

    for g in range(C // 8):
        conv_group(g)

    def layernorm_tile(r, t):
        x0 = x0_ref[r, :, t * LANES:(t + 1) * LANES]
        m = jnp.sum(x0, axis=0, keepdims=True) * (1.0 / C)
        d = x0 - m
        v = jnp.sum(d * d, axis=0, keepdims=True) * (1.0 / C)
        return d * lax.rsqrt(v + EPS)

    for r in range(WS):
        for tp in range(NT // 2):
            ta, tb = 2 * tp, 2 * tp + 1
            ha = layernorm_tile(r, ta)
            hb = layernorm_tile(r, tb)
            t1 = jnp.concatenate([ha[0:64] - hb[0:64], ha[64:128]], axis=0).astype(BF16).T
            t2 = jnp.concatenate([hb[64:128], hb[128:192] - ha[128:192]], axis=0).astype(BF16).T
            t3 = jnp.concatenate([ha[128:192], hb[0:64]], axis=0).astype(BF16).T
            for n in range(5):
                p1 = _dot(t1, ws_ref[0, n])
                p2 = _dot(t2, ws_ref[1, n])
                p3 = _dot(t3, ws_ref[2, n])
                qkv_ref[n, r, ta * LANES:(ta + 1) * LANES, :] = p1 + p3
                qkv_ref[n, r, tb * LANES:(tb + 1) * LANES, :] = p2 + p3

    lane = lax.broadcasted_iota(jnp.int32, (SLOTS, LANES), 1)
    head_lo = [(lane >= 32) & (lane < 80), (lane < 32) | ((lane >= 64) & (lane < 80))]
    head_hi = lane >= 80
    lane2 = lax.broadcasted_iota(jnp.int32, (2 * SLOTS, LANES), 1)
    sl = lax.broadcasted_iota(jnp.int32, (SLOTS, 2 * SLOTS), 0)
    ql = lax.broadcasted_iota(jnp.int32, (SLOTS, 2 * SLOTS), 1)
    key_ok = (sl & 7) < WS
    keep_a = key_ok & (ql < SLOTS)
    keep_b = key_ok & (ql >= SLOTS)
    key_ok8 = lax.broadcasted_iota(jnp.int32, (8, 2 * SLOTS), 0) < WS
    ql1 = lax.broadcasted_iota(jnp.int32, (1, 2 * SLOTS), 1)

    def gather(n, off):
        return jnp.concatenate([qkv_ref[n, r, pl.ds(off, 8), :] for r in range(WS)], axis=0)

    def softmax_t(st):
        m8 = st[0:8]
        for r in range(1, WS):
            m8 = jnp.maximum(m8, st[8 * r:8 * r + 8])
        m = jnp.max(jnp.where(key_ok8, m8, -jnp.inf), axis=0, keepdims=True)
        p = jnp.exp2(st - m)
        s8 = p[0:8]
        for r in range(1, WS):
            s8 = s8 + p[8 * r:8 * r + 8]
        den = jnp.sum(jnp.where(key_ok8, s8, 0.0), axis=0, keepdims=True)
        return p, den

    def attn_pair(offa):
        offb = offa + WS
        ta = [gather(n, offa) for n in range(5)]
        tb = [gather(n, offb) for n in range(5)]
        both = [jnp.concatenate([ta[n], tb[n]], axis=0) for n in range(5)]
        u2 = jnp.where(lane2 < 16, both[0],
                       jnp.where(lane2 < 32, both[2],
                                 jnp.where(lane2 < 48, both[1], both[3])))
        u1t = both[4].astype(BF16).T
        u2t = u2.astype(BF16)[:, 0:64].T
        vt = [u1t[0:48], u1t[48:96],
              jnp.concatenate([u1t[96:128], u2t[0:16]], axis=0), u2t[16:64]]
        outs = []
        for hp in range(2):
            qa, qb, ka, kb = ta[hp], tb[hp], ta[2 + hp], tb[2 + hp]
            lo = head_lo[hp]
            q1 = jnp.concatenate([jnp.where(lo, qa, 0.0), jnp.where(head_hi, qb, 0.0)], axis=0)
            q2 = jnp.concatenate([jnp.where(head_hi, qa, 0.0), jnp.where(lo, qb, 0.0)], axis=0)
            k1 = jnp.where(head_hi, kb, ka)
            k2 = jnp.where(head_hi, ka, kb)
            p1, d1 = softmax_t(_dot_nt(k1, q1))
            p2, d2 = softmax_t(_dot_nt(k2, q2))
            plo = jnp.concatenate([jnp.where(keep_a, p1, 0.0), jnp.where(keep_b, p2, 0.0)], axis=0)
            phi = jnp.concatenate([jnp.where(keep_a, p2, 0.0), jnp.where(keep_b, p1, 0.0)], axis=0)
            r1 = 1.0 / d1
            r2 = 1.0 / d2
            rlo = jnp.where(ql1 < SLOTS, r1, r2)
            rhi = jnp.where(ql1 < SLOTS, r2, r1)
            outs.append(_dot(vt[2 * hp], plo) * rlo)
            outs.append(_dot(vt[2 * hp + 1], phi) * rhi)
        lo96 = jnp.concatenate(outs[0:2], axis=0)
        hi96 = jnp.concatenate(outs[2:4], axis=0)
        w = pltpu.pack_elementwise([lo96, hi96], packed_dtype=BF16)
        wt = w.T
        for i, off in enumerate((offa, offb)):
            for r in range(WS):
                base = i * SLOTS + 8 * r
                ob_ref[r, pl.ds(off, WS), 0:96] = wt[base:base + WS]

    npair = (nwin + 1) // 2
    for p in range(npair):
        attn_pair(min(2 * p, nwin - 2) * WS)

    for r in range(WS):
        for t in range(NT):
            w = ob_ref[r, t * LANES:(t + 1) * LANES, 0:96]
            lo = pltpu.unpack_elementwise(w, index=0, packed_dtype=BF16, unpacked_dtype=F32)
            hi = pltpu.unpack_elementwise(w, index=1, packed_dtype=BF16, unpacked_dtype=F32)
            y = (_dot_nt(wos_ref[0], lo) + _dot_nt(wos_ref[1], hi)
                 + x0_ref[r, :, t * LANES:(t + 1) * LANES])
            o_ref[r, :, t * LANES:(t + 1) * LANES] = y.astype(o_ref.dtype)


@jax.jit
def pallas_standalone__window_attn_davit__vision_kernel(
    x: jax.Array,
    dw_pe: jax.Array,
    w_qkv: jax.Array,
    w_o: jax.Array,
):
    B, H, W, Cx = x.shape
    assert B == 1 and Cx == C and H % WS == 0 and W % WS == 0 and WP - LANES < W < WP
    nstrip = H // WS
    nwin = W // WS

    xt = jnp.transpose(x[0], (0, 2, 1))
    dwb = jnp.broadcast_to(dw_pe.reshape(9, C, 1), (9, C, LANES)).astype(F32)
    wq, wk, wv = w_qkv[:, 0:C], w_qkv[:, C:2 * C], w_qkv[:, 2 * C:3 * C]
    z16 = jnp.zeros((C, 16), w_qkv.dtype)
    wperm = jnp.concatenate([
        wv[:, 128:144], z16, wq[:, 0:96],
        wq[:, 96:128], wv[:, 160:176], z16, wq[:, 128:192],
        z16, wv[:, 144:160], wk[:, 0:96],
        wk[:, 96:128], z16, wv[:, 176:192], wk[:, 128:192],
        wv[:, 0:128]], axis=1)
    wot = jnp.transpose(w_o.reshape(2, 96, C), (0, 2, 1))

    kernel = functools.partial(_kernel, W=W, nwin=nwin, nstrip=nstrip)
    yt = pl.pallas_call(
        kernel,
        grid=(nstrip,),
        in_specs=[
            pl.BlockSpec((WS, C, WP), lambda s: (s, 0, 0)),
            pl.BlockSpec((1, C, WP), lambda s: (jnp.maximum(s * WS - 1, 0), 0, 0)),
            pl.BlockSpec((1, C, WP), lambda s: (jnp.minimum(s * WS + WS, H - 1), 0, 0)),
            pl.BlockSpec((9, C, LANES), lambda s: (0, 0, 0)),
            pl.BlockSpec((C, 5 * LANES), lambda s: (0, 0)),
            pl.BlockSpec((2, C, 96), lambda s: (0, 0, 0)),
        ],
        out_specs=pl.BlockSpec((WS, C, WP), lambda s: (s, 0, 0)),
        out_shape=jax.ShapeDtypeStruct((H, C, W), x.dtype),
        scratch_shapes=[
            pltpu.VMEM((9, C, LANES), F32),
            pltpu.VMEM((3, 5, LANES, LANES), BF16),
            pltpu.VMEM((2, C, 96), BF16),
            pltpu.VMEM((WS, C, WP), F32),
            pltpu.VMEM((5, WS, WP, LANES), F32),
            pltpu.VMEM((WS, WP, LANES), U32),
        ],
        compiler_params=pltpu.CompilerParams(
            dimension_semantics=("arbitrary",),
            vmem_limit_bytes=64 * 1024 * 1024,
        ),
        name="davit_window_attn",
    )(xt, xt, xt, dwb, wperm, wot)
    return jnp.transpose(yt, (0, 2, 1))[None]
```

```python
import functools
import math

import jax
import jax.numpy as jnp
from jax import lax
import jax.experimental.pallas as pl
import jax.experimental.pallas.tpu as pltpu

WS = 7
NH = 4
C = 192
DH = C // NH
LANES = 128
WP = 512
NT = WP // LANES
SLOTS = 8 * WS
EPS = 1e-5
F32 = jnp.float32
BF16 = jnp.bfloat16
U32 = jnp.uint32

_NT_DIMS = (((1,), (1,)), ((), ()))


def _dot(a, b):
    return jnp.dot(a, b, preferred_element_type=F32)


def _dot_nt(a, b):
    return lax.dot_general(a, b, _NT_DIMS, preferred_element_type=F32)


def _cat(xs):
    return jnp.concatenate(xs, axis=0)


def _merge(main, fill):
    out, j = [], 0
    for i, item in enumerate(main):
        out.append(item)
        while j < len(fill) and (j + 1) * len(main) <= (i + 1) * len(fill):
            out.append(fill[j])
            j += 1
    return out + fill[j:]


def _kernel(x0m_ref, x0b_ref, xm_ref, xt_ref, xb_ref, dw_ref, wqkv_ref, wot_ref, o_ref,
            dws_ref, ws_ref, wos_ref, x0_ref, qkv_ref, ob_ref, *, W, nwin, nstrip):
    s = pl.program_id(0)
    cur = s % 2
    nxt = 1 - cur

    lane_w = lax.broadcasted_iota(jnp.int32, (8, WP), 1)
    valid_col = lane_w < W
    valid_last = lax.broadcasted_iota(jnp.int32, (8, LANES), 1) < W - (WP - LANES)

    def conv_group(c0, m_ref, t_ref, b_ref, bot_ok, slot):
        wts = [jnp.concatenate([dws_ref[k, pl.ds(c0, 8), :]] * NT, axis=1) for k in range(9)]

        def load(ref, i):
            v = ref[i, pl.ds(c0, 8), :].astype(F32)
            last = jnp.where(valid_last, v[:, WP - LANES:], 0.0)
            return jnp.concatenate([v[:, :WP - LANES], last], axis=1)

        rows = [None if t_ref is None else load(t_ref, 0)]
        rows += [load(m_ref, i) for i in range(WS)]
        if bot_ok is None:
            rows.append(load(b_ref, 0))
        else:
            rows.append(jnp.where(valid_col & bot_ok, b_ref[0, pl.ds(c0, 8), :].astype(F32), 0.0))
        for r in range(WS):
            abc = []
            for j in range(3):
                acc = rows[r + 1] * wts[3 + j] + rows[r + 2] * wts[6 + j]
                if rows[r] is not None:
                    acc = acc + rows[r] * wts[j]
                abc.append(acc)
            x0 = pltpu.roll(abc[0], 1, 1) + abc[1] + pltpu.roll(abc[2], WP - 1, 1)
            x0_ref[slot, r, pl.ds(c0, 8), :] = x0

    @pl.when(s == 0)
    def _():
        for k in range(9):
            w = dw_ref[k]
            dws_ref[k] = w + 1.0 if k == 4 else w
        lane = lax.broadcasted_iota(jnp.int32, (C, LANES), 1)
        qs = (DH ** -0.5) * math.log2(math.e)
        for n in range(5):
            w = wqkv_ref[:, n * LANES:(n + 1) * LANES].astype(F32)
            if n == 0:
                w = jnp.where(lane >= 32, w * qs, w)
            elif n == 1:
                w = jnp.where((lane >= 32) & (lane < 64), w, w * qs)
            ws_ref[0, n] = pltpu.bitcast(w[0:128].astype(BF16), U32)
            ws_ref[1, n] = pltpu.bitcast(w[64:192].astype(BF16), U32)
            ws_ref[2, n] = pltpu.bitcast(_cat([w[128:192], w[0:64]]).astype(BF16), U32)
        for i in range(2):
            wos_ref[i] = pltpu.bitcast(wot_ref[i].astype(F32).astype(BF16), U32)
        ob_ref[...] = jnp.zeros(ob_ref.shape, ob_ref.dtype)

        def body(g, carry):
            conv_group(pl.multiple_of(g * 8, 8), x0m_ref, None, x0b_ref, None, 0)
            return carry
        lax.fori_loop(0, C // 8, body, 0)

    bot_ok = s + 1 < nstrip - 1
    conv_items = [functools.partial(conv_group, 8 * g, xm_ref, xt_ref, xb_ref, bot_ok, nxt)
                  for g in range(C // 8)]

    def layernorm_tile(r, t):
        x0 = x0_ref[cur, r, :, t * LANES:(t + 1) * LANES]
        m = jnp.sum(x0, axis=0, keepdims=True) * (1.0 / C)
        d = x0 - m
        v = jnp.sum(d * d, axis=0, keepdims=True) * (1.0 / C)
        return d * lax.rsqrt(v + EPS)

    def s1_unit(a, b):
        st = {}

        def chunk(n):
            if n == 0:
                ha = layernorm_tile(*a)
                hb = layernorm_tile(*b)
                st["t"] = [
                    _cat([ha[0:64] - hb[0:64], ha[64:128]]).astype(BF16).T,
                    _cat([hb[64:128], hb[128:192] - ha[128:192]]).astype(BF16).T,
                    _cat([ha[128:192], hb[0:64]]).astype(BF16).T]
            p = [_dot(st["t"][i], pltpu.bitcast(ws_ref[i, n], BF16)) for i in range(3)]
            qkv_ref[n, a[0], a[1] * LANES:(a[1] + 1) * LANES, :] = p[0] + p[2]
            qkv_ref[n, b[0], b[1] * LANES:(b[1] + 1) * LANES, :] = p[1] + p[2]

        return [functools.partial(chunk, n) for n in range(5)]

    s1 = []
    for t in (0, 2):
        units = [((0, t), (1, t)), ((2, t), (3, t)), ((4, t), (5, t)), ((6, t), (6, t + 1)),
                 ((0, t + 1), (1, t + 1)), ((2, t + 1), (3, t + 1)), ((4, t + 1), (5, t + 1))]
        s1 += [s1_unit(*u) for u in units]

    lane8 = lax.broadcasted_iota(jnp.int32, (8, LANES), 1)
    sub8 = lax.broadcasted_iota(jnp.int32, (8, LANES), 0)
    hi_l = lane8 >= 80
    lo_l = lane8 < 80
    v_l = lane8 < 32
    key_ok = sub8 < WS
    left = lane8 < SLOTS
    keep_a = key_ok & left
    keep_b = key_ok & (lane8 >= SLOTS)
    zero8 = jnp.zeros((8, LANES), F32)

    def gather(n, off):
        return [qkv_ref[n, r, pl.ds(off, 8), :] for r in range(WS)]

    def allred(x, op):
        for sh in (4, 2, 1):
            x = op(x, pltpu.roll(x, sh, 0))
        return x

    def softmax_t(st):
        rows = [st[8 * r:8 * r + 8] for r in range(WS)]
        m = functools.reduce(jnp.maximum, rows)
        m = allred(jnp.where(key_ok, m, -jnp.inf), jnp.maximum)
        p = [jnp.exp2(x - m) for x in rows]
        return p, functools.reduce(jnp.add, p)

    def s2_pair(offa):
        offb = offa + WS
        st = {}

        def scores():
            st["s"] = []
            for hp in range(2):
                qa, qb = gather(hp, offa), gather(hp, offb)
                ka, kb = gather(2 + hp, offa), gather(2 + hp, offb)
                q1 = _cat([jnp.where(lo_l, v, 0.0) for v in qa] + [jnp.where(hi_l, v, 0.0) for v in qb]
                          + [zero8, zero8])
                q2 = _cat([jnp.where(hi_l, v, 0.0) for v in qa] + [jnp.where(lo_l, v, 0.0) for v in qb]
                          + [zero8, zero8])
                k1 = _cat([jnp.where(hi_l, y, x) for x, y in zip(ka, kb)])
                k2 = _cat([jnp.where(hi_l, x, y) for x, y in zip(ka, kb)])
                st["s"] += [_dot_nt(k1, q1), _dot_nt(k2, q2)]
            u1 = _cat(gather(4, offa) + gather(4, offb) + [zero8, zero8])
            u2 = _cat([jnp.where(v_l, x, y) for x, y in
                       zip(gather(0, offa) + gather(0, offb), gather(1, offa) + gather(1, offb))]
                      + [zero8, zero8])
            u1t = pltpu.bitcast(u1.astype(BF16).T, U32)
            u2t = pltpu.bitcast(u2[:, 0:64].astype(BF16).T, U32)
            vt = _cat([u1t, u2t])
            st["vt"] = [pltpu.bitcast(vt[24 * h:24 * h + 24], BF16) for h in range(NH)]

        def values():
            outs = []
            for hp in range(2):
                p1, s1_ = softmax_t(st["s"][2 * hp])
                p2, s2_ = softmax_t(st["s"][2 * hp + 1])
                plo = _cat([jnp.where(keep_a, v, 0.0) for v in p1]
                           + [jnp.where(keep_b, v, 0.0) for v in p2] + [zero8, zero8])
                phi = _cat([jnp.where(keep_a, v, 0.0) for v in p2]
                           + [jnp.where(keep_b, v, 0.0) for v in p1] + [zero8, zero8])
                for pm, sa, sb, h in ((plo, s1_, s2_, 2 * hp), (phi, s2_, s1_, 2 * hp + 1)):
                    den = allred(jnp.where(key_ok, jnp.where(left, sa, sb), 0.0), jnp.add)
                    rec = pl.reciprocal(den, approx=True)
                    rec = rec * (2.0 - den * rec)
                    o = _dot(st["vt"][h], pm)
                    outs.append(_cat([o[8 * i:8 * i + 8] * rec for i in range(DH // 8)]))
            w = pltpu.pack_elementwise([_cat(outs[0:2]), _cat(outs[2:4])], packed_dtype=BF16)
            wt = w.T
            for i, off in enumerate((offa, offb)):
                for r in range(WS):
                    base = i * SLOTS + 8 * r
                    ob_ref[r, pl.ds(off, WS), 0:96] = wt[base:base + WS]

        return scores, values

    npair = (nwin + 1) // 2
    pairs = [s2_pair(min(2 * p, nwin - 2) * WS) for p in range(npair)]

    def s3_unit(r, tp):
        ys = []
        for t in (2 * tp, 2 * tp + 1):
            w = ob_ref[r, t * LANES:(t + 1) * LANES, :]
            lo = pltpu.unpack_elementwise(w, index=0, packed_dtype=BF16, unpacked_dtype=F32)
            hi = pltpu.unpack_elementwise(w, index=1, packed_dtype=BF16, unpacked_dtype=F32)
            ys.append(_dot_nt(pltpu.bitcast(wos_ref[0], BF16), lo)
                      + _dot_nt(pltpu.bitcast(wos_ref[1], BF16), hi))
        cols = slice(2 * tp * LANES, (2 * tp + 2) * LANES)
        y = jnp.concatenate(ys, axis=1) + x0_ref[cur, r, :, cols]
        o_ref[r, :, cols] = y.astype(o_ref.dtype)

    s3 = [[functools.partial(s3_unit, r, tp) for r in range(WS)] for tp in range(2)]

    def s2_items(lo, hi):
        items = []
        for p in range(lo, hi):
            items.append(pairs[p][0])
            if p > 0:
                items.append(pairs[p - 1][1])
        return items

    flat = lambda us: [c for u in us for c in u]
    prog = flat(s1[0:4])
    prog += _merge(flat(s1[4:7]), s2_items(0, 9))
    prog += _merge(flat(s1[7:11]), s2_items(9, 18))
    prog += _merge(flat(s1[11:14]), s2_items(18, 27))
    prog += _merge(s2_items(27, npair), s3[0])
    prog += [pairs[npair - 1][1]]
    prog += s3[1]
    prog = _merge(prog, conv_items)
    for item in prog:
        item()


@jax.jit
def pallas_standalone__window_attn_davit__vision_kernel(
    x: jax.Array,
    dw_pe: jax.Array,
    w_qkv: jax.Array,
    w_o: jax.Array,
):
    B, H, W, Cx = x.shape
    assert B == 1 and Cx == C and H % WS == 0 and W % WS == 0 and WP - LANES < W < WP
    nstrip = H // WS
    nwin = W // WS

    xt = jnp.transpose(x[0], (0, 2, 1))
    dwb = jnp.broadcast_to(dw_pe.reshape(9, C, 1), (9, C, LANES)).astype(F32)
    wq, wk, wv = w_qkv[:, 0:C], w_qkv[:, C:2 * C], w_qkv[:, 2 * C:3 * C]
    z32 = jnp.zeros((C, 32), w_qkv.dtype)
    wperm = jnp.concatenate([
        wv[:, 128:160], wq[:, 0:96],
        wq[:, 96:128], wv[:, 160:192], wq[:, 128:192],
        z32, wk[:, 0:96],
        wk[:, 96:128], z32, wk[:, 128:192],
        wv[:, 0:128]], axis=1)
    wot = jnp.transpose(w_o.reshape(2, 96, C), (0, 2, 1))
    wot = jnp.pad(wot, ((0, 0), (0, 0), (0, LANES - 96)))

    nx = lambda s: jnp.minimum(s + 1, nstrip - 1)
    kernel = functools.partial(_kernel, W=W, nwin=nwin, nstrip=nstrip)
    yt = pl.pallas_call(
        kernel,
        grid=(nstrip,),
        in_specs=[
            pl.BlockSpec((WS, C, WP), lambda s: (0, 0, 0)),
            pl.BlockSpec((1, C, WP), lambda s: (WS, 0, 0)),
            pl.BlockSpec((WS, C, WP), lambda s: (nx(s), 0, 0)),
            pl.BlockSpec((1, C, WP), lambda s: (nx(s) * WS - 1, 0, 0)),
            pl.BlockSpec((1, C, WP), lambda s: (jnp.minimum(nx(s) * WS + WS, H - 1), 0, 0)),
            pl.BlockSpec((9, C, LANES), lambda s: (0, 0, 0)),
            pl.BlockSpec((C, 5 * LANES), lambda s: (0, 0)),
            pl.BlockSpec((2, C, LANES), lambda s: (0, 0, 0)),
        ],
        out_specs=pl.BlockSpec((WS, C, WP), lambda s: (s, 0, 0)),
        out_shape=jax.ShapeDtypeStruct((H, C, W), x.dtype),
        scratch_shapes=[
            pltpu.VMEM((9, C, LANES), F32),
            pltpu.VMEM((3, 5, LANES // 2, LANES), U32),
            pltpu.VMEM((2, C // 2, LANES), U32),
            pltpu.VMEM((2, WS, C, WP), F32),
            pltpu.VMEM((5, WS, WP, LANES), F32),
            pltpu.VMEM((WS, WP, LANES), U32),
        ],
        compiler_params=pltpu.CompilerParams(
            dimension_semantics=("arbitrary",),
            vmem_limit_bytes=64 * 1024 * 1024,
        ),
        name="davit_window_attn",
    )(xt, xt, xt, xt, xt, dwb, wperm, wot)
    return jnp.transpose(yt, (0, 2, 1))[None]
```

```python
import functools
import math
import os

import jax
import jax.numpy as jnp
from jax import lax
import jax.experimental.pallas as pl
import jax.experimental.pallas.tpu as pltpu

WS = 7
NH = 4
C = 192
DH = C // NH
LANES = 128
WP = 512
NT = WP // LANES
SLOTS = 8 * WS
EPS = 1e-5
F32 = jnp.float32
BF16 = jnp.bfloat16
U32 = jnp.uint32

_NT_DIMS = (((1,), (1,)), ((), ()))

X0_SLOT = WS * NT * C
DW_OFF = 2 * X0_SLOT
R_ROWS = DW_OFF + 2 * C


def _dot(a, b):
    return jnp.dot(a, b, preferred_element_type=F32)


def _dot_nt(a, b):
    return lax.dot_general(a, b, _NT_DIMS, preferred_element_type=F32)


def _cat(xs):
    return jnp.concatenate(xs, axis=0)


def _env(name, default):
    return type(default)(os.environ.get(name, default))


def _kernel(x0m_ref, x0b_ref, xm_ref, xt_ref, xb_ref, dw_ref, wqkv_ref, wot_ref, o_ref,
            ra_ref, rb_ref, oba_ref, obb_ref, dws_ref, ws_ref, wos_ref, qkv_ref,
            *, W, nwin, nstrip):
    s = pl.program_id(0)
    KS3 = _env("KS3", 1)

    def rows_at(base, off, n):
        if isinstance(base, int):
            return pl.ds(base + off, n)
        return pl.ds(pl.multiple_of(base + off, 8), n)

    lane_w = lax.broadcasted_iota(jnp.int32, (8, WP), 1)
    valid_col = lane_w < W
    lane8 = lax.broadcasted_iota(jnp.int32, (8, LANES), 1)
    sub8 = lax.broadcasted_iota(jnp.int32, (8, LANES), 0)
    valid_last = lane8 < W - (WP - LANES)

    def conv_group(c0, m_ref, t_ref, b_ref, bot_ok, r_ref, slot):
        st = {}

        def load(ref, i):
            v = ref[i, pl.ds(c0, 8), :].astype(F32)
            last = jnp.where(valid_last, v[:, WP - LANES:], 0.0)
            return jnp.concatenate([v[:, :WP - LANES], last], axis=1)

        def row(i):
            if i not in st:
                if i == 0:
                    st[i] = None if t_ref is None else load(t_ref, 0)
                elif i <= WS:
                    st[i] = load(m_ref, i - 1)
                elif bot_ok is None:
                    st[i] = load(b_ref, 0)
                else:
                    st[i] = jnp.where(valid_col & bot_ok, b_ref[0, pl.ds(c0, 8), :].astype(F32), 0.0)
            return st[i]

        def bc(v):
            return jnp.concatenate([v] * NT, axis=1)

        def taps(r):
            st["tw", r] = [bc(r_ref[rows_at(c0, DW_OFF + k * C, 8), :]) for k in range(2)]

        def piece(r):
            if "w" not in st:
                st["w"] = [bc(dws_ref[k, pl.ds(c0, 8), :]) for k in range(9)]
            wts = list(st["w"])
            if ("tw", r) in st:
                wts[6], wts[8] = st["tw", r]
            abc = []
            for j in range(3):
                acc = row(r + 1) * wts[3 + j]
                if row(r) is not None:
                    acc = acc + row(r) * wts[j]
                abc.append(acc + row(r + 2) * wts[6 + j])
            x0 = pltpu.roll(abc[0], 1, 1) + abc[1] + pltpu.roll(abc[2], WP - 1, 1)
            for t in range(NT):
                r_ref[rows_at(slot + c0, (r * NT + t) * C, 8), :] = x0[:, t * LANES:(t + 1) * LANES]

        return taps, piece

    @pl.when(s == 0)
    def _():
        for k in range(9):
            w = dw_ref[k]
            dws_ref[k] = w + 1.0 if k == 4 else w
            if k in (6, 8):
                for r_ref in (ra_ref, rb_ref):
                    r_ref[pl.ds(DW_OFF + (k - 6) // 2 * C, C), :] = w
        lane = lax.broadcasted_iota(jnp.int32, (C, LANES), 1)
        qs = (DH ** -0.5) * math.log2(math.e)
        for n in range(5):
            w = wqkv_ref[:, n * LANES:(n + 1) * LANES].astype(F32)
            if n == 0:
                w = jnp.where(lane >= 32, w * qs, w)
            elif n == 1:
                w = jnp.where((lane >= 32) & (lane < 64), w, w * qs)
            for i, wi in enumerate((w[0:128], w[64:192], _cat([w[128:192], w[0:64]]))):
                ws_ref[i, n] = pltpu.bitcast(wi.astype(BF16), U32)
        for i in range(3):
            wos_ref[i] = pltpu.bitcast(wot_ref[i].astype(F32).astype(BF16), U32)

        def zero(i, carry):
            z = jnp.zeros((64, LANES), F32)
            rb_ref[pl.ds(pl.multiple_of(X0_SLOT + i * 96, 8), 96), :] = jnp.zeros((96, LANES), F32)
            oba_ref[pl.ds(pl.multiple_of(i * 64, 8), 64), :] = z
            obb_ref[pl.ds(pl.multiple_of(i * 64, 8), 64), :] = z
            return carry
        lax.fori_loop(0, WS * 8, zero, 0)

        def body(g, carry):
            _, piece = conv_group(pl.multiple_of(g * 8, 8), x0m_ref, None, x0b_ref, None, ra_ref, 0)
            for r in range(WS):
                piece(r)
            return carry
        lax.fori_loop(0, C // 8, body, 0)

    left64 = lane8 < 64

    def s3_unit(ob_ref, x_ref, base, r, tp):
        st = {}

        def unpack(t):
            w = pltpu.bitcast(ob_ref[pl.ds(r * WP + t * LANES, LANES), :], U32)
            return [pltpu.unpack_elementwise(w, index=i, packed_dtype=BF16, unpacked_dtype=F32)
                    for i in range(2)]

        def wo(i):
            return pltpu.bitcast(wos_ref[i], BF16)

        def finish(ya, yb):
            ys = [y + x_ref[rows_at(base, (r * NT + 2 * tp + i) * C, C), :]
                  for i, y in enumerate((ya, yb))]
            cols = slice(2 * tp * LANES, (2 * tp + 2) * LANES)
            o_ref[r, :, cols] = jnp.concatenate(ys, axis=1).astype(o_ref.dtype)

        def blocks(v):
            return [v[8 * i:8 * i + 8] for i in range(LANES // 8)]

        def all_dots():
            (la, ha), (lb, hb) = unpack(2 * tp), unpack(2 * tp + 1)
            if KS3:
                t3 = _cat([jnp.where(left64, x, y) for x, y in zip(blocks(lb), blocks(ha))])
                t1 = _cat([x - jnp.where(left64, y, 0.0) for x, y in zip(blocks(la), blocks(lb))])
                t2 = _cat([jnp.where(left64, x - y, z)
                           for x, y, z in zip(blocks(hb), blocks(ha), blocks(lb))])
                p3 = _dot_nt(wo(2), t3)
                finish(_dot_nt(wo(0), t1) + p3, _dot_nt(wo(1), t2) + p3)
            else:
                finish(_dot_nt(wo(0), la) + _dot_nt(wo(1), ha), _dot_nt(wo(0), lb) + _dot_nt(wo(1), hb))

        return [C] * (3 if KS3 else 4), all_dots

    def main(c_ref, r_ref, obw_ref, obr_ref):
        cur = ((s // 2) % 2) * X0_SLOT
        nxt = (((s + 1) // 2) % 2) * X0_SLOT
        prv = X0_SLOT - nxt
        bot_ok = s + 1 < nstrip - 1
        groups = [conv_group(8 * g, xm_ref, xt_ref, xb_ref, bot_ok, r_ref, nxt) for g in range(C // 8)]
        WLEAD = _env("WLEAD", 3)
        plist = [(g, r) for g in range(C // 8) for r in range(WS)]
        conv_items = []
        for k, (g, r) in enumerate(plist):
            fs = []
            if k + WLEAD < len(plist):
                g2, r2 = plist[k + WLEAD]
                fs.append(functools.partial(groups[g2][0], r2))
            fs.append(functools.partial(groups[g][1], r))
            conv_items.append(fs)

        def layernorm_tile(r, t):
            x0 = c_ref[rows_at(cur, (r * NT + t) * C, C), :]
            m = jnp.sum(x0, axis=0, keepdims=True) * (1.0 / C)
            d = x0 - m
            v = jnp.sum(d * d, axis=0, keepdims=True) * (1.0 / C)
            return d * lax.rsqrt(v + EPS)

        def s1_unit(a, b):
            st = {}

            def prep():
                ha = layernorm_tile(*a)
                hb = layernorm_tile(*b)
                st["t"] = [
                    _cat([ha[0:64] - hb[0:64], ha[64:128]]).astype(BF16).T,
                    _cat([hb[64:128], hb[128:192] - ha[128:192]]).astype(BF16).T,
                    _cat([ha[128:192], hb[0:64]]).astype(BF16).T]

            def chunk(n):
                p = {i: _dot(st["t"][i], pltpu.bitcast(ws_ref[i, n], BF16)) for i in (2, 0, 1)}
                qkv_ref[n, a[0], a[1] * LANES:(a[1] + 1) * LANES, :] = p[0] + p[2]
                qkv_ref[n, b[0], b[1] * LANES:(b[1] + 1) * LANES, :] = p[1] + p[2]

            return prep, [functools.partial(chunk, n) for n in range(5)]

        s1 = []
        for t in (0, 2):
            units = [((0, t), (1, t)), ((2, t), (3, t)), ((4, t), (5, t)), ((6, t), (6, t + 1)),
                     ((0, t + 1), (1, t + 1)), ((2, t + 1), (3, t + 1)), ((4, t + 1), (5, t + 1))]
            s1 += [s1_unit(*u) for u in units]
        tile_done_unit = {0: 3, 1: 6, 2: 10, 3: 13}

        hi_l = lane8 >= 80
        lo_l = lane8 < 80
        v_l = lane8 < 32
        key_ok = sub8 < WS
        left = lane8 < SLOTS
        keep_a = key_ok & left
        keep_b = key_ok & (lane8 >= SLOTS)
        zero8 = jnp.zeros((8, LANES), F32)

        def gather(n, off):
            return [qkv_ref[n, r, pl.ds(off, 8), :] for r in range(WS)]

        def allred(x, op):
            for sh in (4, 2, 1):
                x = op(x, pltpu.roll(x, sh, 0))
            return x

        def softmax_t(st):
            rows = [st[8 * r:8 * r + 8] for r in range(WS)]
            m = functools.reduce(jnp.maximum, rows)
            m = allred(jnp.where(key_ok, m, -jnp.inf), jnp.maximum)
            p = [jnp.exp2(x - m) for x in rows]
            return p, functools.reduce(jnp.add, p)

        def s2_pair(offa):
            offb = offa + WS
            st = {}

            def vprep():
                u1 = _cat(gather(4, offa) + gather(4, offb) + [zero8, zero8])
                u2 = _cat([jnp.where(v_l, x, y) for x, y in
                           zip(gather(0, offa) + gather(0, offb), gather(1, offa) + gather(1, offb))]
                          + [zero8, zero8])
                u1t = pltpu.bitcast(u1.astype(BF16).T, U32)
                u2t = pltpu.bitcast(u2[:, 0:64].astype(BF16).T, U32)
                vt = _cat([u1t, u2t])
                st["vt"] = [pltpu.bitcast(vt[24 * h:24 * h + 24], BF16) for h in range(NH)]

            def score(i):
                hp, sw = divmod(i, 2)
                ma, mb = (lo_l, hi_l) if sw == 0 else (hi_l, lo_l)
                q = _cat([jnp.where(ma, v, 0.0) for v in gather(hp, offa)]
                         + [jnp.where(mb, v, 0.0) for v in gather(hp, offb)] + [zero8, zero8])
                k = _cat([jnp.where(ma, x, y)
                          for x, y in zip(gather(2 + hp, offa), gather(2 + hp, offb))])
                st["p", i] = softmax_t(_dot_nt(k, q))

            def value(h):
                hp, sw = divmod(h, 2)
                (pa, sa), (pb, sb) = st["p", 2 * hp + sw], st["p", 2 * hp + 1 - sw]
                pm = _cat([jnp.where(keep_a, v, 0.0) for v in pa]
                          + [jnp.where(keep_b, v, 0.0) for v in pb] + [zero8, zero8])
                den = allred(jnp.where(key_ok, jnp.where(left, sa, sb), 0.0), jnp.add)
                rec = pl.reciprocal(den, approx=True)
                rec = rec * (2.0 - den * rec)
                o = _dot(st["vt"][h], pm)
                st["o", h] = [o[8 * i:8 * i + 8] * rec for i in range(DH // 8)]

            def finish():
                o = [b for h in range(NH) for b in st["o", h]]
                if KS3:
                    lo, hi = o[0:16], o[16:24] + o[16:24]
                else:
                    lo, hi = o[0:12], o[12:24]
                w = pltpu.pack_elementwise([_cat(lo), _cat(hi)], packed_dtype=BF16)
                wt = pltpu.bitcast(w, F32).T
                for i, off in enumerate((offa, offb)):
                    for r in range(WS):
                        base = i * SLOTS + 8 * r
                        obw_ref[pl.ds(r * WP + off, WS), 0:wt.shape[1]] = wt[base:base + WS]

            return vprep, score, value, finish

        npair = (nwin + 1) // 2
        offs = [min(2 * p, nwin - 2) * WS for p in range(npair)]
        pairs = [s2_pair(o) for o in offs]
        s3 = [s3_unit(obr_ref, r_ref, prv, r, tp) for r in range(WS) for tp in range(2)]

        LSM = _env("LSM", 240)
        LQKV = _env("LQKV", 250)
        LFIN = _env("LFIN", 200)
        PREP = _env("PREP", 600)
        VLEAD = _env("VLEAD", 0)
        HEAD = _env("HEAD", 3)
        MID = _env("MID", 3)
        CONVEND = _env("CONVEND", 1.0)
        SGRP = _env("SGRP", 4)
        VGRP = _env("VGRP", 2)

        load = [0] * 4
        tm = [0] * 4
        prog, extra = [], []

        def emit(rows_list, fn, ready=0):
            start = min(tm)
            ends = []
            for rows in rows_list:
                m = load.index(min(load))
                load[m] += rows
                tm[m] = max(tm[m], ready) + rows
                ends.append(tm[m])
            prog.append((start, fn))
            return ends

        fillers = [("s3", u) for u in s3[:HEAD]]
        s1_list = [("s1", (u, n)) for u in range(14) for n in range(5)]
        mids = s3[HEAD:HEAD + MID]
        for i, it in enumerate(s1_list):
            fillers.append(it)
            if mids and (i + 1) % (len(s1_list) // (MID + 1)) == 0:
                fillers.append(("s3", mids.pop(0)))
        fillers += [("s3", u) for u in mids + s3[HEAD + MID:]]
        total = (70 * 384 + npair * 416 + sum(sum(u[0]) for u in s3)) / 4
        tile_ready = {}
        next_s = 0
        s_end = {}
        pend_v = []
        v_end = {}
        first_t = None
        while fillers or next_s < 4 * npair or pend_v:
            now = tm[load.index(min(load))]
            p = next_s // 4
            s_ok = False
            if next_s < 4 * npair:
                tneed = (offs[p] + 2 * WS) // LANES
                if tneed in tile_ready:
                    if first_t is None:
                        first_t = tile_ready[0]
                    target = first_t + (total - _env("TAILGAP", 500) - first_t) * next_s / (4 * npair)
                    s_ok = now >= tile_ready[tneed] and now >= target
            v_ok = pend_v and all(now >= x[0] for x in pend_v[:VGRP // 2]) and len(pend_v) >= VGRP // 2
            if not fillers and not s_ok and not v_ok:
                if pend_v and (next_s >= 4 * npair or len(pend_v) >= 4):
                    v_ok = True
                else:
                    s_ok = True
            if v_ok:
                for rdy, pv, hp in pend_v[:VGRP // 2]:
                    for h in (2 * hp, 2 * hp + 1):
                        v_end[pv, h] = emit([DH], functools.partial(pairs[pv][2], h), rdy)[0]
                    if hp == 1:
                        extra.append((max(v_end[pv, h] for h in range(NH)) + LFIN, [pairs[pv][3]]))
                pend_v = pend_v[VGRP // 2:]
            elif s_ok:
                for _ in range(SGRP):
                    p, i = divmod(next_s, 4)
                    if i == 0:
                        prog.append((min(tm), pairs[p][0]))
                    s_end[p, i] = emit([SLOTS], functools.partial(pairs[p][1], i))[0]
                    if i % 2 == 1:
                        pend_v.append((max(s_end[p, i], s_end[p, i - 1]) + LSM, p, i // 2))
                    next_s += 1
            else:
                kind, it = fillers.pop(0)
                if kind == "s3":
                    emit(it[0], it[1])
                else:
                    u, n = it
                    if n == 0:
                        extra.append((min(tm) - PREP, [s1[u][0]]))
                    ends = emit([LANES] * 3, s1[u][1][n])
                    if n == 4:
                        for t, du in tile_done_unit.items():
                            if du == u:
                                tile_ready[t] = max(ends) + LQKV
        if _env("VERB", 0):
            print("planned makespan", max(tm), "ideal", total)
        for j, fs in enumerate(conv_items):
            extra.append(((j + 1) * CONVEND * max(tm) / len(conv_items), fs))
        extra.sort(key=lambda e: e[0])
        j = 0
        for t0, fn in prog:
            while j < len(extra) and extra[j][0] <= t0:
                for f in extra[j][1]:
                    f()
                j += 1
            fn()
        for e in extra[j:]:
            for f in e[1]:
                f()

    pl.when((s % 2 == 0) & (s < nstrip))(functools.partial(main, ra_ref, rb_ref, oba_ref, obb_ref))
    if not _env("ONE", 0):
        pl.when((s % 2 == 1) & (s < nstrip))(functools.partial(main, rb_ref, ra_ref, obb_ref, oba_ref))

    @pl.when(s == nstrip)
    def _():
        last = nstrip - 1
        x_ref, ob_ref = (ra_ref, oba_ref) if last % 2 == 0 else (rb_ref, obb_ref)
        for r in range(WS):
            for tp in range(2):
                s3_unit(ob_ref, x_ref, ((last // 2) % 2) * X0_SLOT, r, tp)[1]()


@jax.jit
def pallas_standalone__window_attn_davit__vision_kernel(
    x: jax.Array,
    dw_pe: jax.Array,
    w_qkv: jax.Array,
    w_o: jax.Array,
):
    B, H, W, Cx = x.shape
    assert B == 1 and Cx == C and H % WS == 0 and W % WS == 0 and WP - LANES < W < WP
    nstrip = H // WS
    nwin = W // WS

    xt = jnp.transpose(x[0], (0, 2, 1))
    dwb = jnp.broadcast_to(dw_pe.reshape(9, C, 1), (9, C, LANES)).astype(F32)
    wq, wk, wv = w_qkv[:, 0:C], w_qkv[:, C:2 * C], w_qkv[:, 2 * C:3 * C]
    z32 = jnp.zeros((C, 32), w_qkv.dtype)
    wperm = jnp.concatenate([
        wv[:, 128:160], wq[:, 0:96],
        wq[:, 96:128], wv[:, 160:192], wq[:, 128:192],
        z32, wk[:, 0:96],
        wk[:, 96:128], z32, wk[:, 128:192],
        wv[:, 0:128]], axis=1)
    wt = w_o.T
    if _env("KS3", 1):
        wx, wy, wz = wt[:, 0:64], wt[:, 64:128], wt[:, 128:192]
        wot = jnp.stack([jnp.concatenate(p, axis=1) for p in ((wx, wy), (wz, wy), (wx, wz))])
    else:
        wot = jnp.stack([jnp.concatenate(p, axis=1)
                         for p in ((wt[:, 0:96], z32), (wt[:, 96:192], z32), (wt[:, 0:96], z32))])

    nx = lambda s: jnp.minimum(s + 1, nstrip - 1)
    kernel = functools.partial(_kernel, W=W, nwin=nwin, nstrip=nstrip)
    yt = pl.pallas_call(
        kernel,
        grid=(nstrip + 1,),
        in_specs=[
            pl.BlockSpec((WS, C, WP), lambda s: (0, 0, 0)),
            pl.BlockSpec((1, C, WP), lambda s: (WS, 0, 0)),
            pl.BlockSpec((WS, C, WP), lambda s: (nx(s), 0, 0)),
            pl.BlockSpec((1, C, WP), lambda s: (nx(s) * WS - 1, 0, 0)),
            pl.BlockSpec((1, C, WP), lambda s: (jnp.minimum(nx(s) * WS + WS, H - 1), 0, 0)),
            pl.BlockSpec((9, C, LANES), lambda s: (0, 0, 0)),
            pl.BlockSpec((C, 5 * LANES), lambda s: (0, 0)),
            pl.BlockSpec((3, C, LANES), lambda s: (0, 0, 0)),
        ],
        out_specs=pl.BlockSpec((WS, C, WP), lambda s: (jnp.maximum(s - 1, 0), 0, 0)),
        out_shape=jax.ShapeDtypeStruct((H, C, W), x.dtype),
        scratch_shapes=[
            pltpu.VMEM((R_ROWS, LANES), F32),
            pltpu.VMEM((R_ROWS, LANES), F32),
            pltpu.VMEM((WS * WP, LANES), F32),
            pltpu.VMEM((WS * WP, LANES), F32),
            pltpu.VMEM((9, C, LANES), F32),
            pltpu.VMEM((3, 5, LANES // 2, LANES), U32),
            pltpu.VMEM((3, C // 2, LANES), U32),
            pltpu.VMEM((5, WS, WP, LANES), F32),
        ],
        compiler_params=pltpu.CompilerParams(
            dimension_semantics=("arbitrary",),
            vmem_limit_bytes=64 * 1024 * 1024,
        ),
        name="davit_window_attn",
    )(xt, xt, xt, xt, xt, dwb, wperm, wot)
    return jnp.transpose(yt, (0, 2, 1))[None]
```

```python
import functools
import math
import os

import jax
import jax.numpy as jnp
from jax import lax
import jax.experimental.pallas as pl
import jax.experimental.pallas.tpu as pltpu

WS = 7
NH = 4
C = 192
DH = C // NH
LANES = 128
WP = 512
NT = WP // LANES
SLOTS = 8 * WS
EPS = 1e-5
F32 = jnp.float32
BF16 = jnp.bfloat16
U32 = jnp.uint32

_NT_DIMS = (((1,), (1,)), ((), ()))

X0_SLOT = WS * NT * C
DW_OFF = 2 * X0_SLOT
BAR_OFF = DW_OFF + 2 * C
R_ROWS = BAR_OFF + 8
OB_ROWS = WS * WP + 8


def _dot(a, b):
    return jnp.dot(a, b, preferred_element_type=F32)


def _dot_nt(a, b):
    return lax.dot_general(a, b, _NT_DIMS, preferred_element_type=F32)


def _dot_tn(a, b):
    return lax.dot_general(a, b, (((0,), (0,)), ((), ())), preferred_element_type=F32)


def _cat(xs):
    return jnp.concatenate(xs, axis=0)


def _env(name, default):
    return type(default)(os.environ.get(name, default))


def _kernel(x0m_ref, x0b_ref, xm_ref, xt_ref, xb_ref, dw_ref, wqkv_ref, wot_ref, o_ref,
            ra_ref, rb_ref, oba_ref, obb_ref, dws_ref, ws_ref, wos_ref, qkv_ref, t_ref,
            *, W, nwin, nstrip):
    s = pl.program_id(0)
    KS3 = _env("KS3", 1)
    dyn0 = jnp.minimum(s, 0)
    last = {}

    def barrier(ref, row):
        if "v" in last:
            ref[pl.ds(pl.multiple_of(row + dyn0 * 8, 8), 8), :] = last["v"]

    def rows_at(base, off, n):
        if isinstance(base, int):
            return pl.ds(base + off, n)
        return pl.ds(pl.multiple_of(base + off, 8), n)

    lane_w = lax.broadcasted_iota(jnp.int32, (8, WP), 1)
    valid_col = lane_w < W
    lane8 = lax.broadcasted_iota(jnp.int32, (8, LANES), 1)
    sub8 = lax.broadcasted_iota(jnp.int32, (8, LANES), 0)
    valid_last = lane8 < W - (WP - LANES)

    def conv_group(c0, m_ref, t_ref, b_ref, bot_ok, r_ref, slot):
        st = {}

        def load(ref, i):
            v = ref[i, pl.ds(c0, 8), :].astype(F32)
            last = jnp.where(valid_last, v[:, WP - LANES:], 0.0)
            return jnp.concatenate([v[:, :WP - LANES], last], axis=1)

        def row(i):
            if i not in st:
                if i == 0:
                    st[i] = None if t_ref is None else load(t_ref, 0)
                elif i <= WS:
                    st[i] = load(m_ref, i - 1)
                elif bot_ok is None:
                    st[i] = load(b_ref, 0)
                else:
                    st[i] = jnp.where(valid_col & bot_ok, b_ref[0, pl.ds(c0, 8), :].astype(F32), 0.0)
            return st[i]

        def bc(v):
            return jnp.concatenate([v] * NT, axis=1)

        def taps(r):
            st["tw", r] = [bc(r_ref[rows_at(c0, DW_OFF + k * C, 8), :]) for k in range(2)]

        def piece(r):
            if _env("REUNP", 0):
                for i in range(WS + 2):
                    st.pop(i, None)
            if "w" not in st or _env("REW", 0):
                st["w"] = [bc(dws_ref[k, pl.ds(c0, 8), :]) for k in range(9)]
            wts = list(st["w"])
            if ("tw", r) in st:
                wts[6], wts[8] = st["tw", r]
            abc = []
            for j in range(3):
                acc = row(r + 1) * wts[3 + j]
                if row(r) is not None:
                    acc = acc + row(r) * wts[j]
                abc.append(acc + row(r + 2) * wts[6 + j])
            x0 = pltpu.roll(abc[0], 1, 1) + abc[1] + pltpu.roll(abc[2], WP - 1, 1)
            for t in range(NT):
                r_ref[rows_at(slot + c0, (r * NT + t) * C, 8), :] = x0[:, t * LANES:(t + 1) * LANES]

        return taps, piece

    @pl.when(s == 0)
    def _():
        for k in range(9):
            w = dw_ref[k]
            dws_ref[k] = w + 1.0 if k == 4 else w
            if k in (6, 8):
                for r_ref in (ra_ref, rb_ref):
                    r_ref[pl.ds(DW_OFF + (k - 6) // 2 * C, C), :] = w
        lane = lax.broadcasted_iota(jnp.int32, (C, LANES), 1)
        qs = (DH ** -0.5) * math.log2(math.e)
        for n in range(5):
            w = wqkv_ref[:, n * LANES:(n + 1) * LANES].astype(F32)
            if n == 0:
                w = jnp.where(lane >= 32, w * qs, w)
            elif n == 1:
                w = jnp.where((lane >= 32) & (lane < 64), w, w * qs)
            for i, wi in enumerate((w[0:128], w[64:192], _cat([w[128:192], w[0:64]]))):
                ws_ref[i, n] = pltpu.bitcast(wi.astype(BF16), U32)
        for i in range(3):
            wos_ref[i] = pltpu.bitcast(wot_ref[i].astype(F32).astype(BF16), U32)

        def zero(i, carry):
            z = jnp.zeros((64, LANES), F32)
            rb_ref[pl.ds(pl.multiple_of(X0_SLOT + i * 96, 8), 96), :] = jnp.zeros((96, LANES), F32)
            oba_ref[pl.ds(pl.multiple_of(i * 64, 8), 64), :] = z
            obb_ref[pl.ds(pl.multiple_of(i * 64, 8), 64), :] = z
            return carry
        lax.fori_loop(0, WS * 8, zero, 0)

        def body(g, carry):
            _, piece = conv_group(pl.multiple_of(g * 8, 8), x0m_ref, None, x0b_ref, None, ra_ref, 0)
            for r in range(WS):
                piece(r)
            return carry
        lax.fori_loop(0, C // 8, body, 0)

    left64 = lane8 < 64

    def s3_unit(ob_ref, x_ref, base, r, tp):
        st = {}

        def unpack(t):
            w = pltpu.bitcast(ob_ref[pl.ds(r * WP + t * LANES, LANES), :], U32)
            return [pltpu.unpack_elementwise(w, index=i, packed_dtype=BF16, unpacked_dtype=F32)
                    for i in range(2)]

        def wo(i):
            return pltpu.bitcast(wos_ref[i], BF16)

        def finish(ya, yb):
            ys = [y + x_ref[rows_at(base, (r * NT + 2 * tp + i) * C, C), :]
                  for i, y in enumerate((ya, yb))]
            cols = slice(2 * tp * LANES, (2 * tp + 2) * LANES)
            o_ref[r, :, cols] = jnp.concatenate(ys, axis=1).astype(o_ref.dtype)

        def blocks(v):
            return [v[8 * i:8 * i + 8] for i in range(LANES // 8)]

        def prep():
            if _env("G3", 0):
                barrier(ob_ref, WS * WP)
            (la, ha), (lb, hb) = unpack(2 * tp), unpack(2 * tp + 1)
            if KS3:
                t3 = _cat([jnp.where(left64, x, y) for x, y in zip(blocks(lb), blocks(ha))])
                t1 = _cat([x - jnp.where(left64, y, 0.0) for x, y in zip(blocks(la), blocks(lb))])
                t2 = _cat([jnp.where(left64, x - y, z)
                           for x, y, z in zip(blocks(hb), blocks(ha), blocks(lb))])
                st["t"] = (t1, t2, t3)
            else:
                st["t"] = (la, ha, lb, hb)

        def all_dots():
            if KS3:
                t1, t2, t3 = st["t"]
                p3 = _dot_nt(wo(2), t3)
                last["v"] = p3[0:8]
                finish(_dot_nt(wo(0), t1) + p3, _dot_nt(wo(1), t2) + p3)
            else:
                la, ha, lb, hb = st["t"]
                finish(_dot_nt(wo(0), la) + _dot_nt(wo(1), ha), _dot_nt(wo(0), lb) + _dot_nt(wo(1), hb))

        return [C] * (3 if KS3 else 4), all_dots, prep

    def main(c_ref, r_ref, obw_ref, obr_ref):
        last.clear()
        cur = ((s // 2) % 2) * X0_SLOT
        nxt = (((s + 1) // 2) % 2) * X0_SLOT
        prv = X0_SLOT - nxt
        bot_ok = s + 1 < nstrip - 1
        groups = [conv_group(8 * g, xm_ref, xt_ref, xb_ref, bot_ok, r_ref, nxt) for g in range(C // 8)]
        WLEAD = _env("WLEAD", 3)

        def conv_items(gs):
            plist = [(g, r) for g in gs for r in range(WS)]
            items = []
            for k, (g, r) in enumerate(plist):
                fs = []
                if k + WLEAD < len(plist):
                    g2, r2 = plist[k + WLEAD]
                    fs.append(functools.partial(groups[g2][0], r2))
                fs.append(functools.partial(groups[g][1], r))
                items.append(fs)
            return items

        def tree(xs, op=jnp.add):
            xs = list(xs)
            while len(xs) > 1:
                xs = [op(xs[i], xs[i + 1]) if i + 1 < len(xs) else xs[i] for i in range(0, len(xs), 2)]
            return xs[0]

        def chains(xs, k, op=jnp.add):
            return tree([functools.reduce(op, xs[i::k]) for i in range(k)], op)

        def allred(x, op):
            for sh in (4, 2, 1):
                x = op(x, pltpu.roll(x, sh, 0))
            return x

        LNMODE = _env("LNMODE", 1)
        LMR = _env("LMR", 0)

        def layernorm_tile(r, t):
            if LNMODE == 0:
                x0 = c_ref[rows_at(cur, (r * NT + t) * C, C), :]
                m = jnp.sum(x0, axis=0, keepdims=True) * (1.0 / C)
                d = x0 - m
                v = jnp.sum(d * d, axis=0, keepdims=True) * (1.0 / C)
                return d * lax.rsqrt(v + EPS)
            ld = lambda: [c_ref[rows_at(cur, (r * NT + t) * C + 8 * g, 8), :] for g in range(C // 8)]
            m = allred(chains(ld(), 3), jnp.add) * (1.0 / C)
            d = [x - m for x in ld()]
            v = allred(chains([x * x for x in d], 3), jnp.add) * (1.0 / C)
            rs = lax.rsqrt(v + EPS)
            if LNMODE == 2:
                d = [x - m for x in ld()]
            return _cat([x * rs for x in d])

        def s1_unit(uid, a, b):
            st = {}

            def prep():
                if _env("G1", 0):
                    barrier(c_ref, BAR_OFF)
                ha = layernorm_tile(*a)
                hb = layernorm_tile(*b)
                ts = [_cat([ha[0:64] - hb[0:64], ha[64:128]]),
                      _cat([hb[64:128], hb[128:192] - ha[128:192]]),
                      _cat([ha[128:192], hb[0:64]])]
                if LMR == 0:
                    st["t"] = [t.astype(BF16).T for t in ts]
                else:
                    st["t"] = [t.astype(BF16) for t in ts]
                for i in range(3):
                    t_ref[uid, i] = pltpu.bitcast(st["t"][i], U32)

            def chunk(n, order=(2, 0, 1)):
                dot = _dot_tn if LMR else _dot
                if LMR and n == 0:
                    st["t"] = [pltpu.bitcast(t_ref[uid, i], BF16) for i in range(3)]
                p = {i: dot(st["t"][i] if LMR else pltpu.bitcast(t_ref[uid, i], BF16),
                            pltpu.bitcast(ws_ref[i, n], BF16)) for i in order}
                last["v"] = p[2][0:8]
                for i in range(0, LANES, 8):
                    qkv_ref[n, a[0], pl.ds(a[1] * LANES + i, 8), :] = p[0][i:i + 8] + p[2][i:i + 8]
                    qkv_ref[n, b[0], pl.ds(b[1] * LANES + i, 8), :] = p[1][i:i + 8] + p[2][i:i + 8]

            return prep, [functools.partial(chunk, n) for n in range(5)]

        s1 = []
        for t in (0, 2):
            units = [((0, t), (1, t)), ((2, t), (3, t)), ((4, t), (5, t)), ((6, t), (6, t + 1)),
                     ((0, t + 1), (1, t + 1)), ((2, t + 1), (3, t + 1)), ((4, t + 1), (5, t + 1))]
            s1 += [s1_unit(len(s1) + i, *u) for i, u in enumerate(units)]
        tile_done_unit = {0: 3, 1: 6, 2: 10, 3: 13}

        key_ok = sub8 < WS
        left = lane8 < SLOTS
        keep_a = key_ok & left
        keep_b = key_ok & (lane8 >= SLOTS)
        zero8 = jnp.zeros((8, LANES), F32)

        def gather(n, off):
            return [qkv_ref[n, r, pl.ds(off, 8), :] for r in range(WS)]

        def softmax_t(st):
            rows = [st[8 * r:8 * r + 8] for r in range(WS)]
            m = functools.reduce(jnp.maximum, rows)
            m = allred(jnp.where(key_ok, m, -jnp.inf), jnp.maximum)
            p = [jnp.exp2(x - m) for x in rows]
            return p, functools.reduce(jnp.add, p)

        never = lane8 < dyn0
        fin = {}
        GK = _env("GK", 0)

        def s2_pair(pi, offa):
            offb = offa + WS
            st = {}

            def vprep():
                ln = lane8
                if GK and pi - GK in fin:
                    ln = jnp.where(never, pltpu.bitcast(fin[pi - GK], jnp.int32), lane8)
                st["lo"], st["hi"], v_l = ln < 80, ln >= 80, ln < 32
                u1 = _cat(gather(4, offa) + gather(4, offb) + [zero8, zero8])
                u2 = _cat([jnp.where(v_l, x, y) for x, y in
                           zip(gather(0, offa) + gather(0, offb), gather(1, offa) + gather(1, offb))]
                          + [zero8, zero8])
                u1t = pltpu.bitcast(u1.astype(BF16).T, U32)
                u2t = pltpu.bitcast(u2[:, 0:64].astype(BF16).T, U32)
                vt = _cat([u1t, u2t])
                st["vt"] = [pltpu.bitcast(vt[24 * h:24 * h + 24], BF16) for h in range(NH)]

            def score(i):
                hp, sw = divmod(i, 2)
                ma, mb = (st["lo"], st["hi"]) if sw == 0 else (st["hi"], st["lo"])
                q = _cat([jnp.where(ma, v, 0.0) for v in gather(hp, offa)]
                         + [jnp.where(mb, v, 0.0) for v in gather(hp, offb)] + [zero8, zero8])
                k = _cat([jnp.where(ma, x, y)
                          for x, y in zip(gather(2 + hp, offa), gather(2 + hp, offb))])
                st["p", i] = softmax_t(_dot_nt(k, q))

            def value(h):
                hp, sw = divmod(h, 2)
                (pa, sa), (pb, sb) = st["p", 2 * hp + sw], st["p", 2 * hp + 1 - sw]
                pm = _cat([jnp.where(keep_a, v, 0.0) for v in pa]
                          + [jnp.where(keep_b, v, 0.0) for v in pb] + [zero8, zero8])
                den = allred(jnp.where(key_ok, jnp.where(left, sa, sb), 0.0), jnp.add)
                rec = pl.reciprocal(den, approx=True)
                rec = rec * (2.0 - den * rec)
                o = _dot(st["vt"][h], pm)
                st["o", h] = [o[8 * i:8 * i + 8] * rec for i in range(DH // 8)]

            def finish():
                o = [b for h in range(NH) for b in st["o", h]]
                if KS3:
                    lo, hi = o[0:16], o[16:24] + o[16:24]
                else:
                    lo, hi = o[0:12], o[12:24]
                w = pltpu.pack_elementwise([_cat(lo), _cat(hi)], packed_dtype=BF16)
                wt = pltpu.bitcast(w, F32).T
                fin[pi] = wt[104:112]
                for i, off in enumerate((offa, offb)):
                    for r in range(WS):
                        base = i * SLOTS + 8 * r
                        obw_ref[pl.ds(r * WP + off, WS), 0:wt.shape[1]] = wt[base:base + WS]

            return vprep, score, value, finish

        npair = (nwin + 1) // 2
        offs = [min(2 * p, nwin - 2) * WS for p in range(npair)]
        pairs = [s2_pair(i, o) for i, o in enumerate(offs)]
        s3 = [s3_unit(obr_ref, r_ref, prv, r, tp) for r in range(WS) for tp in range(2)]

        LSM = _env("LSM", 240)
        LQKV = _env("LQKV", 250)
        LFIN = _env("LFIN", 200)
        PREP = _env("PREP", 600)
        CONVEND = _env("CONVEND", 1.0)
        SGRP = _env("SGRP", 4)
        VGRP = _env("VGRP", 2)
        TAILGAP = _env("TAILGAP", 800)

        def segment(units, pids, s3u, gs, preps, own_preps, head):
            last.clear()
            fin.clear()
            load = [0] * 4
            tm = [0] * 4
            prog, extra = [], []

            def emit(rows_list, fn, ready=0):
                start = min(tm)
                ends = []
                for rows in rows_list:
                    m = load.index(min(load))
                    load[m] += rows
                    tm[m] = max(tm[m], ready) + rows
                    ends.append(tm[m])
                prog.append((start, fn))
                return ends

            fillers = [("s3", u) for u in s3u[:head]]
            fillers += [("s1", (u, n)) for u in units for n in range(5)]
            fillers += [("s3", u) for u in s3u[head:]]
            total = (len(units) * 5 * 384 + len(pids) * 416 + sum(sum(u[0]) for u in s3u)) / 4
            nsc = 4 * len(pids)
            next_s = 0
            s_end, v_end, pend_v, held = {}, {}, [], {}
            while fillers or next_s < nsc or pend_v:
                now = tm[load.index(min(load))]
                s_ok = next_s < nsc and now >= (total - TAILGAP) * next_s / max(nsc - 4, 1)
                v_ok = len(pend_v) >= VGRP // 2 and all(now >= x[0] for x in pend_v[:VGRP // 2])
                if not fillers and not s_ok and not v_ok:
                    if pend_v and (next_s >= nsc or len(pend_v) >= 4):
                        v_ok = True
                    else:
                        s_ok = True
                if v_ok:
                    for rdy, pv, hp in pend_v[:VGRP // 2]:
                        for h in (2 * hp, 2 * hp + 1):
                            v_end[pv, h] = emit([DH], functools.partial(pairs[pv][2], h), rdy)[0]
                        if hp == 1:
                            extra.append((max(v_end[pv, h] for h in range(NH)) + LFIN, [pairs[pv][3]]))
                    pend_v = pend_v[VGRP // 2:]
                elif s_ok:
                    for _ in range(SGRP):
                        p, i = pids[next_s // 4], next_s % 4
                        if i == 0:
                            prog.append((min(tm), pairs[p][0]))
                        s_end[p, i] = emit([SLOTS], functools.partial(pairs[p][1], i))[0]
                        if i % 2 == 1:
                            pend_v.append((max(s_end[p, i], s_end[p, i - 1]) + LSM, p, i // 2))
                        next_s += 1
                else:
                    kind, it = fillers.pop(0)
                    if kind == "s3":
                        extra.append((min(tm) - _env("PREP3", 350), [it[2]]))
                        emit(it[0], it[1])
                    else:
                        u, n = it
                        if n == 0:
                            held = {}
                            if u in own_preps:
                                extra.append((min(tm) - PREP, [s1[u][0]]))
                        ld, tgt = list(load), []
                        for _ in range(3):
                            m = ld.index(min(ld))
                            ld[m] += LANES
                            tgt.append(m)
                        order = [held.get(m) if tgt.index(m) == j else None for j, m in enumerate(tgt)]
                        for j in range(3):
                            if order[j] is not None and order[j] in order[:j]:
                                order[j] = None
                        rest = [i for i in (2, 0, 1) if i not in order]
                        order = [o if o is not None else rest.pop(0) for o in order]
                        held.update(zip(tgt, order))
                        if not LMR:
                            order = (2, 0, 1)
                        emit([LANES] * 3, functools.partial(s1[u][1][n], tuple(order)))
            if _env("VERB", 0):
                print("planned makespan", max(tm), "ideal", total)
            ci = conv_items(gs)
            for j, fs in enumerate(ci):
                extra.append(((j + 1) * CONVEND * max(tm) / len(ci), fs))
            for j, u in enumerate(preps):
                extra.append(((j + 0.3) * max(tm) / len(preps), [s1[u][0]]))
            extra.sort(key=lambda e: e[0])
            j = 0
            for t0, fn in prog:
                while j < len(extra) and extra[j][0] <= t0:
                    for f in extra[j][1]:
                        f()
                    j += 1
                fn()
            for e in extra[j:]:
                for f in e[1]:
                    f()

        spec = [tuple(int(v) for v in x.split(",")) for x in
                _env("SEGS", "14,0,3,24;0,37,11,0").split(";")]
        STAGE = _env("STAGE", 1)
        pos = [0, 0, 0, 0]
        segs = []
        for sp in spec:
            segs.append([list(range(a, a + n)) for a, n in zip(pos, sp)])
            pos = [a + n for a, n in zip(pos, sp)]
        assert pos == [14, npair, 14, C // 8], pos
        for k, (units, pids, s3i, gs) in enumerate(segs):
            ahead = segs[k + 1][0][:STAGE] if k + 1 < len(segs) else []
            own = units if k == 0 else units[STAGE:]
            fn = functools.partial(segment, units, pids, [s3[i] for i in s3i], gs, ahead, own,
                                   _env("HEAD", 3) if k == 0 else 0)
            pl.when(dyn0 != k + 1)(fn)

    pl.when((s % 2 == 0) & (s < nstrip))(functools.partial(main, ra_ref, rb_ref, oba_ref, obb_ref))
    if not _env("ONE", 0):
        pl.when((s % 2 == 1) & (s < nstrip))(functools.partial(main, rb_ref, ra_ref, obb_ref, oba_ref))

    @pl.when(s == nstrip)
    def _():
        lst = nstrip - 1
        x_ref, ob_ref = (ra_ref, oba_ref) if lst % 2 == 0 else (rb_ref, obb_ref)
        for r in range(WS):
            for tp in range(2):
                u = s3_unit(ob_ref, x_ref, ((lst // 2) % 2) * X0_SLOT, r, tp)
                last.clear()
                u[2]()
                u[1]()


@jax.jit
def pallas_standalone__window_attn_davit__vision_kernel(
    x: jax.Array,
    dw_pe: jax.Array,
    w_qkv: jax.Array,
    w_o: jax.Array,
):
    B, H, W, Cx = x.shape
    assert B == 1 and Cx == C and H % WS == 0 and W % WS == 0 and WP - LANES < W < WP
    nstrip = H // WS
    nwin = W // WS

    xt = jnp.transpose(x[0], (0, 2, 1))
    dwb = jnp.broadcast_to(dw_pe.reshape(9, C, 1), (9, C, LANES)).astype(F32)
    wq, wk, wv = w_qkv[:, 0:C], w_qkv[:, C:2 * C], w_qkv[:, 2 * C:3 * C]
    z32 = jnp.zeros((C, 32), w_qkv.dtype)
    wperm = jnp.concatenate([
        wv[:, 128:160], wq[:, 0:96],
        wq[:, 96:128], wv[:, 160:192], wq[:, 128:192],
        z32, wk[:, 0:96],
        wk[:, 96:128], z32, wk[:, 128:192],
        wv[:, 0:128]], axis=1)
    wt = w_o.T
    if _env("KS3", 1):
        wx, wy, wz = wt[:, 0:64], wt[:, 64:128], wt[:, 128:192]
        wot = jnp.stack([jnp.concatenate(p, axis=1) for p in ((wx, wy), (wz, wy), (wx, wz))])
    else:
        wot = jnp.stack([jnp.concatenate(p, axis=1)
                         for p in ((wt[:, 0:96], z32), (wt[:, 96:192], z32), (wt[:, 0:96], z32))])

    nx = lambda s: jnp.minimum(s + 1, nstrip - 1)
    kernel = functools.partial(_kernel, W=W, nwin=nwin, nstrip=nstrip)
    yt = pl.pallas_call(
        kernel,
        grid=(nstrip + 1,),
        in_specs=[
            pl.BlockSpec((WS, C, WP), lambda s: (0, 0, 0)),
            pl.BlockSpec((1, C, WP), lambda s: (WS, 0, 0)),
            pl.BlockSpec((WS, C, WP), lambda s: (nx(s), 0, 0)),
            pl.BlockSpec((1, C, WP), lambda s: (nx(s) * WS - 1, 0, 0)),
            pl.BlockSpec((1, C, WP), lambda s: (jnp.minimum(nx(s) * WS + WS, H - 1), 0, 0)),
            pl.BlockSpec((9, C, LANES), lambda s: (0, 0, 0)),
            pl.BlockSpec((C, 5 * LANES), lambda s: (0, 0)),
            pl.BlockSpec((3, C, LANES), lambda s: (0, 0, 0)),
        ],
        out_specs=pl.BlockSpec((WS, C, WP), lambda s: (jnp.maximum(s - 1, 0), 0, 0)),
        out_shape=jax.ShapeDtypeStruct((H, C, W), x.dtype),
        scratch_shapes=[
            pltpu.VMEM((R_ROWS, LANES), F32),
            pltpu.VMEM((R_ROWS, LANES), F32),
            pltpu.VMEM((OB_ROWS, LANES), F32),
            pltpu.VMEM((OB_ROWS, LANES), F32),
            pltpu.VMEM((9, C, LANES), F32),
            pltpu.VMEM((3, 5, LANES // 2, LANES), U32),
            pltpu.VMEM((3, C // 2, LANES), U32),
            pltpu.VMEM((5, WS, WP, LANES), F32),
            pltpu.VMEM((14, 3, LANES // 2, LANES), U32),
        ],
        compiler_params=pltpu.CompilerParams(
            dimension_semantics=("arbitrary",),
            vmem_limit_bytes=64 * 1024 * 1024,
            fuse_transposed_lhs_in_matmul=True,
        ),
        name="davit_window_attn",
    )(xt, xt, xt, xt, xt, dwb, wperm, wot)
    return jnp.transpose(yt, (0, 2, 1))[None]
```

```python
import functools
import math
import os

import jax
import jax.numpy as jnp
from jax import lax
import jax.experimental.pallas as pl
import jax.experimental.pallas.tpu as pltpu

WS = 7
NH = 4
C = 192
DH = C // NH
NG = C // 8
LANES = 128
WP = 512
NT = WP // LANES
NU = WS * NT // 2
SLOTS = 8 * WS
EPS = 1e-5
F32 = jnp.float32
BF16 = jnp.bfloat16
U32 = jnp.uint32

X0_SLOT = WS * NT * C
DW_OFF = 3 * X0_SLOT
X0_ROWS = DW_OFF + 2 * C


def _dot(a, b):
    return jnp.dot(a, b, preferred_element_type=F32)


def _dot_nt(a, b):
    return lax.dot_general(a, b, (((1,), (1,)), ((), ())), preferred_element_type=F32)


def _cat(xs):
    return jnp.concatenate(xs, axis=0)


def _blocks(v):
    return [v[i:i + 8] for i in range(0, v.shape[0], 8)]


def _allred(x, op):
    for sh in (4, 2, 1):
        x = op(x, pltpu.roll(x, sh, 0))
    return x


def _sum3(xs):
    a, b, c = (functools.reduce(jnp.add, xs[i::3]) for i in range(3))
    return (a + b) + c


def _env(name, default):
    return type(default)(os.environ.get(name, default))


def _kernel(x0m_ref, x0b_ref, xm_ref, xt_ref, xb_ref, dw_ref, wqkv_ref, wot_ref, o_ref,
            x0_ref, ob_ref, dws_ref, ws_ref, wos_ref, qkv_ref, t_ref, *, W, nwin, nstrip):
    s = pl.program_id(0)
    dyn0 = jnp.minimum(s, 0)

    def rows_at(base, off, n):
        if isinstance(base, int):
            return pl.ds(base + off, n)
        return pl.ds(pl.multiple_of(base + off, 8), n)

    valid_col = lax.broadcasted_iota(jnp.int32, (8, WP), 1) < W
    lane8 = lax.broadcasted_iota(jnp.int32, (8, LANES), 1)
    sub8 = lax.broadcasted_iota(jnp.int32, (8, LANES), 0)
    valid_last = lane8 < W - (WP - LANES)

    def conv_group(c0, m_ref, top_ref, b_ref, bot_ok, slot):
        st = {}

        def load(ref, i):
            v = ref[i, pl.ds(c0, 8), :].astype(F32)
            last = jnp.where(valid_last, v[:, WP - LANES:], 0.0)
            return jnp.concatenate([v[:, :WP - LANES], last], axis=1)

        def row(i):
            if i not in st:
                if i == 0:
                    st[i] = None if top_ref is None else load(top_ref, 0)
                elif i <= WS:
                    st[i] = load(m_ref, i - 1)
                elif bot_ok is None:
                    st[i] = load(b_ref, 0)
                else:
                    st[i] = jnp.where(valid_col & bot_ok, b_ref[0, pl.ds(c0, 8), :].astype(F32), 0.0)
            return st[i]

        def bc(v):
            return jnp.concatenate([v] * NT, axis=1)

        def taps(r):
            st["tw", r] = [bc(x0_ref[rows_at(c0, DW_OFF + k * C, 8), :]) for k in range(2)]

        def piece(r):
            if "w" not in st:
                st["w"] = [bc(dws_ref[k, pl.ds(c0, 8), :]) for k in range(9)]
            wts = list(st["w"])
            if ("tw", r) in st:
                wts[6], wts[8] = st["tw", r]
            abc = []
            for j in range(3):
                acc = row(r + 1) * wts[3 + j]
                if row(r) is not None:
                    acc = acc + row(r) * wts[j]
                abc.append(acc + row(r + 2) * wts[6 + j])
            x0 = pltpu.roll(abc[0], 1, 1) + abc[1] + pltpu.roll(abc[2], WP - 1, 1)
            for t in range(NT):
                x0_ref[rows_at(slot + c0, (r * NT + t) * C, 8), :] = x0[:, t * LANES:(t + 1) * LANES]

        return taps, piece

    @pl.when(s == 0)
    def _():
        for k in range(9):
            w = dw_ref[k]
            dws_ref[k] = w + 1.0 if k == 4 else w
            if k in (6, 8):
                x0_ref[pl.ds(DW_OFF + (k - 6) // 2 * C, C), :] = w
        lane = lax.broadcasted_iota(jnp.int32, (C, LANES), 1)
        qs = (DH ** -0.5) * math.log2(math.e)
        for n in range(5):
            w = wqkv_ref[:, n * LANES:(n + 1) * LANES].astype(F32)
            if n == 0:
                w = jnp.where(lane >= 32, w * qs, w)
            elif n == 1:
                w = jnp.where((lane >= 32) & (lane < 64), w, w * qs)
            for i, wi in enumerate((w[0:128], w[64:192], _cat([w[128:192], w[0:64]]))):
                ws_ref[i, n] = pltpu.bitcast(wi.astype(BF16), U32)
        for i in range(3):
            wos_ref[i] = pltpu.bitcast(wot_ref[i].astype(F32).astype(BF16), U32)

        def zero(i, carry):
            x0_ref[pl.ds(pl.multiple_of(2 * X0_SLOT + i * 96, 8), 96), :] = jnp.zeros((96, LANES), F32)
            for k in range(2):
                ob_ref[k, pl.ds(pl.multiple_of(i * 64, 8), 64), :] = jnp.zeros((64, LANES), F32)
            return carry
        lax.fori_loop(0, WS * 8, zero, 0)

        def body(g, carry):
            _, piece = conv_group(pl.multiple_of(g * 8, 8), x0m_ref, None, x0b_ref, None, 0)
            for r in range(WS):
                piece(r)
            return carry
        lax.fori_loop(0, NG, body, 0)

    cur = (s % 3) * X0_SLOT
    nxt = ((s + 1) % 3) * X0_SLOT
    prv = ((s + 2) % 3) * X0_SLOT
    obw = s % 2
    obr = 1 - obw

    bot_ok = s + 1 < nstrip - 1
    groups = [conv_group(8 * g, xm_ref, xt_ref, xb_ref, bot_ok, nxt) for g in range(NG)]
    WLEAD = _env("WLEAD", 4)

    def conv_items(gs):
        plist = [(g, r) for g in gs for r in range(WS)]
        items = []
        for k, (g, r) in enumerate(plist):
            fs = []
            if k + WLEAD < len(plist):
                g2, r2 = plist[k + WLEAD]
                fs.append(functools.partial(groups[g2][0], r2))
            fs.append(functools.partial(groups[g][1], r))
            items.append(fs)
        return items

    LNP = _env("LNP", 3)

    def layernorm_tile(r, t):
        def ld(k):
            return [x0_ref[rows_at(cur + dyn0 * (8 * k), (r * NT + t) * C + 8 * g, 8), :]
                    for g in range(NG)]
        xs = ld(0)
        m = _allred(_sum3(xs), jnp.add) * (1.0 / C)
        if LNP == 2:
            v = _allred(_sum3([x * x for x in xs]), jnp.add) * (1.0 / C)
            v = jnp.maximum(v - m * m, 0.0)
        else:
            d = [x - m for x in ld(1)]
            v = _allred(_sum3([x * x for x in d]), jnp.add) * (1.0 / C)
        rs = lax.rsqrt(v + EPS)
        return _cat([(x - m) * rs for x in ld(2)])

    def ln_prep(u):
        r, tp = divmod(u, 2)
        ha = layernorm_tile(r, 2 * tp)
        hb = layernorm_tile(r, 2 * tp + 1)
        ts = [_cat([ha[0:64] - hb[0:64], ha[64:128]]),
              _cat([hb[64:128], hb[128:192] - ha[128:192]]),
              _cat([ha[128:192], hb[0:64]])]
        for i, t in enumerate(ts):
            t_ref[u, i] = pltpu.bitcast(t.astype(BF16).T, U32)

    def qkv_chunk(u, n):
        r, tp = divmod(u, 2)
        p = {i: _dot(pltpu.bitcast(t_ref[u, i], BF16), pltpu.bitcast(ws_ref[i, n], BF16))
             for i in (2, 0, 1)}
        for j in range(2):
            qkv_ref[n, r, pl.ds((2 * tp + j) * LANES, LANES), :] = p[j] + p[2]

    lo_l = lane8 < 80
    hi_l = lane8 >= 80
    v_l = lane8 < 32
    key_ok = sub8 < WS
    left = lane8 < SLOTS
    keep_a = key_ok & left
    keep_b = key_ok & (lane8 >= SLOTS)
    zero8 = jnp.zeros((8, LANES), F32)

    def gather(n, off):
        return [qkv_ref[n, r, pl.ds(off, 8), :] for r in range(WS)]

    def softmax_t(st):
        rows = _blocks(st)
        m = functools.reduce(jnp.maximum, rows)
        m = _allred(jnp.where(key_ok, m, -jnp.inf), jnp.maximum)
        p = [jnp.exp2(x - m) for x in rows]
        return p, functools.reduce(jnp.add, p)

    def s2_pair(offa):
        offb = offa + WS
        st = {}

        def vprep():
            u1 = _cat(gather(4, offa) + gather(4, offb) + [zero8, zero8])
            u2 = _cat([jnp.where(v_l, x, y) for x, y in
                       zip(gather(0, offa) + gather(0, offb), gather(1, offa) + gather(1, offb))]
                      + [zero8, zero8])
            u1t = pltpu.bitcast(u1.astype(BF16).T, U32)
            u2t = pltpu.bitcast(u2[:, 0:64].astype(BF16).T, U32)
            vt = _cat([u1t, u2t])
            st["vt"] = [pltpu.bitcast(vt[24 * h:24 * h + 24], BF16) for h in range(NH)]

        def score(i):
            hp, sw = divmod(i, 2)
            ma, mb = (lo_l, hi_l) if sw == 0 else (hi_l, lo_l)
            q = _cat([jnp.where(ma, v, 0.0) for v in gather(hp, offa)]
                     + [jnp.where(mb, v, 0.0) for v in gather(hp, offb)] + [zero8, zero8])
            k = _cat([jnp.where(ma, x, y)
                      for x, y in zip(gather(2 + hp, offa), gather(2 + hp, offb))])
            st["p", i] = softmax_t(_dot_nt(k, q))

        def value(h):
            hp, sw = divmod(h, 2)
            (pa, sa), (pb, sb) = st["p", 2 * hp + sw], st["p", 2 * hp + 1 - sw]
            pm = _cat([jnp.where(keep_a, v, 0.0) for v in pa]
                      + [jnp.where(keep_b, v, 0.0) for v in pb] + [zero8, zero8])
            den = _allred(jnp.where(key_ok, jnp.where(left, sa, sb), 0.0), jnp.add)
            rec = pl.reciprocal(den, approx=True)
            rec = rec * (2.0 - den * rec)
            st["o", h] = [b * rec for b in _blocks(_dot(st["vt"][h], pm))]

        def finish():
            o = [b for h in range(NH) for b in st["o", h]]
            w = pltpu.pack_elementwise([_cat(o[0:16]), _cat(o[16:24] + o[16:24])], packed_dtype=BF16)
            wt = pltpu.bitcast(w, F32).T
            for i, off in enumerate((offa, offb)):
                for r in range(WS):
                    base = i * SLOTS + 8 * r
                    ob_ref[obw, pl.ds(r * WP + off, WS), :] = wt[base:base + WS]

        return vprep, score, value, finish

    npair = (nwin + 1) // 2
    pairs = [s2_pair(min(2 * p, nwin - 2) * WS) for p in range(npair)]

    left64 = lane8 < 64

    def s3_unit(r, tp):
        def unpack(t):
            w = pltpu.bitcast(ob_ref[obr, pl.ds(r * WP + t * LANES, LANES), :], U32)
            return [_blocks(pltpu.unpack_elementwise(w, index=i, packed_dtype=BF16, unpacked_dtype=F32))
                    for i in range(2)]

        (la, ha), (lb, hb) = unpack(2 * tp), unpack(2 * tp + 1)
        t3 = _cat([jnp.where(left64, x, y) for x, y in zip(lb, ha)])
        t1 = _cat([x - jnp.where(left64, y, 0.0) for x, y in zip(la, lb)])
        t2 = _cat([jnp.where(left64, x - y, z) for x, y, z in zip(hb, ha, lb)])
        p3 = _dot_nt(pltpu.bitcast(wos_ref[2], BF16), t3)
        ys = [_dot_nt(pltpu.bitcast(wos_ref[i], BF16), t) + p3
              + x0_ref[rows_at(prv, (r * NT + 2 * tp + i) * C, C), :] for i, t in enumerate((t1, t2))]
        o_ref[r, :, pl.ds(2 * tp * LANES, 2 * LANES)] = jnp.concatenate(ys, axis=1).astype(o_ref.dtype)

    s3_all = [functools.partial(s3_unit, r, tp) for tp in (1, 0) for r in range(WS)]

    LSM = _env("LSM", 240)
    LFIN = _env("LFIN", 200)
    PREP = _env("PREP", 600)
    SGRP = _env("SGRP", 4)
    VGRP = _env("VGRP", 2)
    TAILGAP = _env("TAILGAP", 800)

    def segment(units, pids, s3u, gs, lns, head):
        load = [0] * 4
        tm = [0] * 4
        prog, extra = [], []

        def emit(rows_list, fn, ready=0):
            prog.append((min(tm), fn))
            ends = []
            for rows in rows_list:
                m = load.index(min(load))
                load[m] += rows
                tm[m] = max(tm[m], ready) + rows
                ends.append(tm[m])
            return ends

        fillers = [([C] * 3, f) for f in s3u[:head]]
        fillers += [([LANES] * 3, functools.partial(qkv_chunk, u, n)) for u in units for n in range(5)]
        fillers += [([C] * 3, f) for f in s3u[head:]]
        total = (sum(sum(f[0]) for f in fillers) + len(pids) * 4 * (SLOTS + DH)) / 4
        nsc = 4 * len(pids)
        next_s = 0
        s_end, v_end, pend_v = {}, {}, []
        while fillers or next_s < nsc or pend_v:
            now = tm[load.index(min(load))]
            s_ok = next_s < nsc and now >= (total - TAILGAP) * next_s / max(nsc - 4, 1)
            v_ok = len(pend_v) >= VGRP // 2 and all(now >= x[0] for x in pend_v[:VGRP // 2])
            if not fillers and not s_ok and not v_ok:
                if pend_v and (next_s >= nsc or len(pend_v) >= 4):
                    v_ok = True
                else:
                    s_ok = True
            if v_ok:
                for rdy, pv, hp in pend_v[:VGRP // 2]:
                    for h in (2 * hp, 2 * hp + 1):
                        v_end[pv, h] = emit([DH], functools.partial(pairs[pv][2], h), rdy)[0]
                    if hp == 1:
                        extra.append((max(v_end[pv, h] for h in range(NH)) + LFIN, [pairs[pv][3]]))
                pend_v = pend_v[VGRP // 2:]
            elif s_ok:
                for _ in range(SGRP):
                    p, i = pids[next_s // 4], next_s % 4
                    if i == 0:
                        prog.append((min(tm), pairs[p][0]))
                    s_end[p, i] = emit([SLOTS], functools.partial(pairs[p][1], i))[0]
                    if i % 2 == 1:
                        pend_v.append((max(s_end[p, i], s_end[p, i - 1]) + LSM, p, i // 2))
                    next_s += 1
            else:
                emit(*fillers.pop(0))
        ci = conv_items(gs)
        for j, fs in enumerate(ci):
            extra.append(((j + 1) * max(tm) / len(ci), fs))
        for j, u in enumerate(lns):
            extra.append((j * _env("LNSTEP", 150) - 1, [functools.partial(ln_prep, u)]))
        extra.sort(key=lambda e: e[0])
        j = 0
        for t0, fn in prog:
            while j < len(extra) and extra[j][0] <= t0:
                for f in extra[j][1]:
                    f()
                j += 1
            fn()
        for e in extra[j:]:
            for f in e[1]:
                f()

    spec = [[int(v) for v in x.split(",")] for x in
            _env("SEGS", "4,0,3,0,14;10,0,0,24,0;0,37,11,0,0").split(";")]
    pos = [0] * 5
    for k, sp in enumerate(spec):
        units, pids, s3i, gs, lns = [list(range(a, a + n)) for a, n in zip(pos, sp)]
        pos = [a + n for a, n in zip(pos, sp)]
        fn = functools.partial(segment, units, pids, [s3_all[i] for i in s3i], gs, lns,
                               _env("HEAD", 3) if k == 0 else 0)
        pl.when(s + dyn0 * k < nstrip)(fn)
    assert pos == [NU, npair, NU, NG, NU], pos

    @pl.when(s == nstrip)
    def _():
        for f in s3_all:
            f()


@jax.jit
def pallas_standalone__window_attn_davit__vision_kernel(
    x: jax.Array,
    dw_pe: jax.Array,
    w_qkv: jax.Array,
    w_o: jax.Array,
):
    B, H, W, Cx = x.shape
    assert B == 1 and Cx == C and H % WS == 0 and W % WS == 0 and WP - LANES < W < WP
    nstrip = H // WS
    nwin = W // WS

    xt = jnp.transpose(x[0], (0, 2, 1))
    dwb = jnp.broadcast_to(dw_pe.reshape(9, C, 1), (9, C, LANES)).astype(F32)
    wq, wk, wv = w_qkv[:, 0:C], w_qkv[:, C:2 * C], w_qkv[:, 2 * C:3 * C]
    z32 = jnp.zeros((C, 32), w_qkv.dtype)
    wperm = jnp.concatenate([
        wv[:, 128:160], wq[:, 0:96],
        wq[:, 96:128], wv[:, 160:192], wq[:, 128:192],
        z32, wk[:, 0:96],
        wk[:, 96:128], z32, wk[:, 128:192],
        wv[:, 0:128]], axis=1)
    wt = w_o.T
    wx, wy, wz = wt[:, 0:64], wt[:, 64:128], wt[:, 128:192]
    wot = jnp.stack([jnp.concatenate(p, axis=1) for p in ((wx, wy), (wz, wy), (wx, wz))])

    nx = lambda s: jnp.minimum(s + 1, nstrip - 1)
    kernel = functools.partial(_kernel, W=W, nwin=nwin, nstrip=nstrip)
    yt = pl.pallas_call(
        kernel,
        grid=(nstrip + 1,),
        in_specs=[
            pl.BlockSpec((WS, C, WP), lambda s: (0, 0, 0)),
            pl.BlockSpec((1, C, WP), lambda s: (WS, 0, 0)),
            pl.BlockSpec((WS, C, WP), lambda s: (nx(s), 0, 0)),
            pl.BlockSpec((1, C, WP), lambda s: (nx(s) * WS - 1, 0, 0)),
            pl.BlockSpec((1, C, WP), lambda s: (jnp.minimum(nx(s) * WS + WS, H - 1), 0, 0)),
            pl.BlockSpec((9, C, LANES), lambda s: (0, 0, 0)),
            pl.BlockSpec((C, 5 * LANES), lambda s: (0, 0)),
            pl.BlockSpec((3, C, LANES), lambda s: (0, 0, 0)),
        ],
        out_specs=pl.BlockSpec((WS, C, WP), lambda s: (jnp.maximum(s - 1, 0), 0, 0)),
        out_shape=jax.ShapeDtypeStruct((H, C, W), x.dtype),
        scratch_shapes=[
            pltpu.VMEM((X0_ROWS, LANES), F32),
            pltpu.VMEM((2, WS * WP, LANES), F32),
            pltpu.VMEM((9, C, LANES), F32),
            pltpu.VMEM((3, 5, LANES // 2, LANES), U32),
            pltpu.VMEM((3, C // 2, LANES), U32),
            pltpu.VMEM((5, WS, WP, LANES), F32),
            pltpu.VMEM((NU, 3, LANES // 2, LANES), U32),
        ],
        compiler_params=pltpu.CompilerParams(
            dimension_semantics=("arbitrary",),
            vmem_limit_bytes=64 * 1024 * 1024,
        ),
        name="davit_window_attn",
    )(xt, xt, xt, xt, xt, dwb, wperm, wot)
    return jnp.transpose(yt, (0, 2, 1))[None]
```

```python
import functools
import math
import os

import jax
import jax.numpy as jnp
from jax import lax
import jax.experimental.pallas as pl
import jax.experimental.pallas.tpu as pltpu

WS = 7
NH = 4
C = 192
DH = C // NH
NG = C // 8
LANES = 128
WP = 512
NT = WP // LANES
NU = WS * NT // 2
SLOTS = 8 * WS
EPS = 1e-5
F32 = jnp.float32
BF16 = jnp.bfloat16
U32 = jnp.uint32

X0_SLOT = WS * NT * C
DW_OFF = 3 * X0_SLOT
X0_ROWS = DW_OFF + 2 * C


def _dot(a, b):
    return jnp.dot(a, b, preferred_element_type=F32)


def _dot_nt(a, b):
    return lax.dot_general(a, b, (((1,), (1,)), ((), ())), preferred_element_type=F32)


def _cat(xs):
    return jnp.concatenate(xs, axis=0)


def _blocks(v):
    return [v[i:i + 8] for i in range(0, v.shape[0], 8)]


def _allred(x, op):
    for sh in (4, 2, 1):
        x = op(x, pltpu.roll(x, sh, 0))
    return x


def _sum3(xs):
    k = _env("NCH", 1)
    return functools.reduce(jnp.add, [functools.reduce(jnp.add, xs[i::k]) for i in range(k)])


def _env(name, default):
    return type(default)(os.environ.get(name, default))


def _kernel(x0m_ref, x0b_ref, xm_ref, xt_ref, xb_ref, dw_ref, wqkv_ref, wot_ref, o_ref,
            x0_ref, ob_ref, dws_ref, ws_ref, wos_ref, qkv_ref, t_ref, *, W, nwin, nstrip):
    s = pl.program_id(0)
    dyn0 = jnp.minimum(s, 0)

    def rows_at(base, off, n):
        if isinstance(base, int):
            return pl.ds(base + off, n)
        return pl.ds(pl.multiple_of(base + off, 8), n)

    valid_col = lax.broadcasted_iota(jnp.int32, (8, WP), 1) < W
    lane8 = lax.broadcasted_iota(jnp.int32, (8, LANES), 1)
    sub8 = lax.broadcasted_iota(jnp.int32, (8, LANES), 0)
    valid_last = lane8 < W - (WP - LANES)

    def conv_group(c0, m_ref, top_ref, b_ref, bot_ok, slot):
        st = {}

        def load(ref, i):
            v = ref[i, pl.ds(c0, 8), :].astype(F32)
            last = jnp.where(valid_last, v[:, WP - LANES:], 0.0)
            return jnp.concatenate([v[:, :WP - LANES], last], axis=1)

        def row(i):
            if i not in st:
                if i == 0:
                    st[i] = None if top_ref is None else load(top_ref, 0)
                elif i <= WS:
                    st[i] = load(m_ref, i - 1)
                elif bot_ok is None:
                    st[i] = load(b_ref, 0)
                else:
                    st[i] = jnp.where(valid_col & bot_ok, b_ref[0, pl.ds(c0, 8), :].astype(F32), 0.0)
            return st[i]

        def bc(v):
            return jnp.concatenate([v] * NT, axis=1)

        def taps(r):
            st["tw", r] = [bc(x0_ref[rows_at(c0, DW_OFF + k * C, 8), :]) for k in range(2)]

        def piece(r):
            if "w" not in st:
                st["w"] = [bc(dws_ref[k, pl.ds(c0, 8), :]) for k in range(9)]
            wts = list(st["w"])
            if ("tw", r) in st:
                wts[6], wts[8] = st["tw", r]
            abc = []
            for j in range(3):
                acc = row(r + 1) * wts[3 + j]
                if row(r) is not None:
                    acc = acc + row(r) * wts[j]
                abc.append(acc + row(r + 2) * wts[6 + j])
            x0 = pltpu.roll(abc[0], 1, 1) + abc[1] + pltpu.roll(abc[2], WP - 1, 1)
            for t in range(NT):
                x0_ref[rows_at(slot + c0, (r * NT + t) * C, 8), :] = x0[:, t * LANES:(t + 1) * LANES]

        return taps, piece

    @pl.when(s == 0)
    def _():
        for k in range(9):
            w = dw_ref[k]
            dws_ref[k] = w + 1.0 if k == 4 else w
            if k in (6, 8):
                x0_ref[pl.ds(DW_OFF + (k - 6) // 2 * C, C), :] = w
        lane = lax.broadcasted_iota(jnp.int32, (C, LANES), 1)
        qs = (DH ** -0.5) * math.log2(math.e)
        for n in range(5):
            w = wqkv_ref[:, n * LANES:(n + 1) * LANES].astype(F32)
            if n == 0:
                w = jnp.where(lane >= 32, w * qs, w)
            elif n == 1:
                w = jnp.where((lane >= 32) & (lane < 64), w, w * qs)
            for i, wi in enumerate((w[0:128], w[64:192], _cat([w[128:192], w[0:64]]))):
                ws_ref[i, n] = pltpu.bitcast(wi.astype(BF16), U32)
        for i in range(3):
            wos_ref[i] = pltpu.bitcast(wot_ref[i].astype(F32).astype(BF16), U32)

        def zero(i, carry):
            x0_ref[pl.ds(pl.multiple_of(2 * X0_SLOT + i * 96, 8), 96), :] = jnp.zeros((96, LANES), F32)
            for k in range(2):
                ob_ref[k, pl.ds(pl.multiple_of(i * 64, 8), 64), :] = jnp.zeros((64, LANES), F32)
            return carry
        lax.fori_loop(0, WS * 8, zero, 0)

        def body(g, carry):
            _, piece = conv_group(pl.multiple_of(g * 8, 8), x0m_ref, None, x0b_ref, None, 0)
            for r in range(WS):
                piece(r)
            return carry
        lax.fori_loop(0, NG, body, 0)

    cur = (s % 3) * X0_SLOT
    nxt = ((s + 1) % 3) * X0_SLOT
    prv = ((s + 2) % 3) * X0_SLOT
    obw = s % 2
    obr = 1 - obw

    bot_ok = s + 1 < nstrip - 1
    groups = [conv_group(8 * g, xm_ref, xt_ref, xb_ref, bot_ok, nxt) for g in range(NG)]
    WLEAD = _env("WLEAD", 5)

    def conv_items(gs):
        plist = [(g, r) for g in gs for r in range(WS)]
        items = []
        for k, (g, r) in enumerate(plist):
            fs = []
            if k + WLEAD < len(plist):
                g2, r2 = plist[k + WLEAD]
                fs.append(functools.partial(groups[g2][0], r2))
            fs.append(functools.partial(groups[g][1], r))
            items.append(fs)
        return items

    LNP = _env("LNP", 3)
    never = lane8 < dyn0
    tokens = {}

    def layernorm_tile(r, t, gates):
        def ld(k):
            return [x0_ref[rows_at(cur + dyn0 * (8 * k), (r * NT + t) * C + 8 * g, 8), :]
                    for g in range(NG)]
        xs = ld(0)
        for g in gates:
            for i in range(_env("NCH", 1)):
                xs[i] = jnp.where(never, g, xs[i])
        m = _allred(_sum3(xs), jnp.add) * (1.0 / C)
        if LNP == 2:
            v = _allred(_sum3([x * x for x in xs]), jnp.add) * (1.0 / C)
            v = jnp.maximum(v - m * m, 0.0)
        else:
            d = [x - m for x in ld(1)]
            v = _allred(_sum3([x * x for x in d]), jnp.add) * (1.0 / C)
        rs = lax.rsqrt(v + EPS)
        tokens["rs", r * NT + t] = (m, v, rs)[_env("CHAT", 2)]
        return _cat([(x - m) * rs for x in ld(2)])

    def ln_prep(u):
        r, tp = divmod(u, 2)
        hs = []
        for j in range(2):
            gates = []
            k = 2 * u + j - _env("CH1", 2)
            if _env("CH1", 2) and ("rs", k) in tokens:
                gates.append(tokens["rs", k])
            k = u - _env("CH2", 4)
            if _env("CH2", 4) and k in tokens:
                gates += [pltpu.bitcast(x, F32) for x in (tokens[k][0:2] if j == 0 else tokens[k][2:3])]
            hs.append(layernorm_tile(r, 2 * tp + j, gates))
        ha, hb = hs
        ts = [_cat([ha[0:64] - hb[0:64], ha[64:128]]),
              _cat([hb[64:128], hb[128:192] - ha[128:192]]),
              _cat([ha[128:192], hb[0:64]])]
        toks = []
        for i, t in enumerate(ts):
            t = pltpu.bitcast(t.astype(BF16).T, U32)
            t_ref[u, i] = t
            toks.append(t[56:64])
        tokens[u] = toks

    def qkv_chunk(u, n, after=None):
        r, tp = divmod(u, 2)
        p = {}
        for i in (2, 0, 1):
            lhs = t_ref[u, i]
            if after is not None:
                lhs = _cat([jnp.where(never, tokens[after][i], lhs[0:8]), lhs[8:]])
            p[i] = _dot(pltpu.bitcast(lhs, BF16), pltpu.bitcast(ws_ref[i, n], BF16))
        if _env("BLK", 0):
            for i in range(0, LANES, 8):
                for j in range(2):
                    qkv_ref[n, r, pl.ds((2 * tp + j) * LANES + i, 8), :] = p[j][i:i + 8] + p[2][i:i + 8]
            return
        for j in range(2):
            qkv_ref[n, r, pl.ds((2 * tp + j) * LANES, LANES), :] = p[j] + p[2]

    lo_l = lane8 < 80
    hi_l = lane8 >= 80
    v_l = lane8 < 32
    key_ok = sub8 < WS
    left = lane8 < SLOTS
    keep_a = key_ok & left
    keep_b = key_ok & (lane8 >= SLOTS)
    zero8 = jnp.zeros((8, LANES), F32)

    def gather(n, off):
        return [qkv_ref[n, r, pl.ds(off, 8), :] for r in range(WS)]

    def softmax_t(st):
        rows = _blocks(st)
        m = functools.reduce(jnp.maximum, rows)
        m = _allred(jnp.where(key_ok, m, -jnp.inf), jnp.maximum)
        p = [jnp.exp2(x - m) for x in rows]
        return p, functools.reduce(jnp.add, p)

    def s2_pair(offa):
        offb = offa + WS
        st = {}

        def vprep():
            u1 = _cat(gather(4, offa) + gather(4, offb) + [zero8, zero8])
            u2 = _cat([jnp.where(v_l, x, y) for x, y in
                       zip(gather(0, offa) + gather(0, offb), gather(1, offa) + gather(1, offb))]
                      + [zero8, zero8])
            u1t = pltpu.bitcast(u1.astype(BF16).T, U32)
            u2t = pltpu.bitcast(u2[:, 0:64].astype(BF16).T, U32)
            vt = _cat([u1t, u2t])
            st["vt"] = [pltpu.bitcast(vt[24 * h:24 * h + 24], BF16) for h in range(NH)]

        def score(i):
            hp, sw = divmod(i, 2)
            ma, mb = (lo_l, hi_l) if sw == 0 else (hi_l, lo_l)
            q = _cat([jnp.where(ma, v, 0.0) for v in gather(hp, offa)]
                     + [jnp.where(mb, v, 0.0) for v in gather(hp, offb)] + [zero8, zero8])
            k = _cat([jnp.where(ma, x, y)
                      for x, y in zip(gather(2 + hp, offa), gather(2 + hp, offb))])
            st["p", i] = softmax_t(_dot_nt(k, q))

        def value(h):
            hp, sw = divmod(h, 2)
            (pa, sa), (pb, sb) = st["p", 2 * hp + sw], st["p", 2 * hp + 1 - sw]
            pm = _cat([jnp.where(keep_a, v, 0.0) for v in pa]
                      + [jnp.where(keep_b, v, 0.0) for v in pb] + [zero8, zero8])
            den = _allred(jnp.where(key_ok, jnp.where(left, sa, sb), 0.0), jnp.add)
            rec = pl.reciprocal(den, approx=True)
            rec = rec * (2.0 - den * rec)
            st["o", h] = [b * rec for b in _blocks(_dot(st["vt"][h], pm))]

        def finish():
            o = [b for h in range(NH) for b in st["o", h]]
            w = pltpu.pack_elementwise([_cat(o[0:16]), _cat(o[16:24] + o[16:24])], packed_dtype=BF16)
            wt = pltpu.bitcast(w, F32).T
            for i, off in enumerate((offa, offb)):
                for r in range(WS):
                    base = i * SLOTS + 8 * r
                    ob_ref[obw, pl.ds(r * WP + off, WS), :] = wt[base:base + WS]

        return vprep, score, value, finish

    npair = (nwin + 1) // 2
    pairs = [s2_pair(min(2 * p, nwin - 2) * WS) for p in range(npair)]

    left64 = lane8 < 64

    def s3_unit(r, tp):
        def unpack(t):
            w = pltpu.bitcast(ob_ref[obr, pl.ds(r * WP + t * LANES, LANES), :], U32)
            return [_blocks(pltpu.unpack_elementwise(w, index=i, packed_dtype=BF16, unpacked_dtype=F32))
                    for i in range(2)]

        (la, ha), (lb, hb) = unpack(2 * tp), unpack(2 * tp + 1)
        t3 = _cat([jnp.where(left64, x, y) for x, y in zip(lb, ha)])
        t1 = _cat([x - jnp.where(left64, y, 0.0) for x, y in zip(la, lb)])
        t2 = _cat([jnp.where(left64, x - y, z) for x, y, z in zip(hb, ha, lb)])
        p3 = _dot_nt(pltpu.bitcast(wos_ref[2], BF16), t3)
        ys = [_dot_nt(pltpu.bitcast(wos_ref[i], BF16), t) + p3
              + x0_ref[rows_at(prv, (r * NT + 2 * tp + i) * C, C), :] for i, t in enumerate((t1, t2))]
        o_ref[r, :, pl.ds(2 * tp * LANES, 2 * LANES)] = jnp.concatenate(ys, axis=1).astype(o_ref.dtype)

    H0 = _env("H0", 2)
    s3_all = [functools.partial(s3_unit, r, tp) for r, tp in
              [(r, 0) for r in range(H0)] + [(r, 1) for r in range(WS)] + [(r, 0) for r in range(H0, WS)]]

    LSM = _env("LSM", 240)
    LFIN = _env("LFIN", 200)
    PREP = _env("PREP", 600)
    SGRP = _env("SGRP", 4)
    VGRP = _env("VGRP", 2)
    TAILGAP = _env("TAILGAP", 800)

    def segment(units, pids, s3u, gs, lns, head):
        load = [0] * 4
        tm = [0] * 4
        prog, extra = [], []

        def emit(rows_list, fn, ready=0):
            prog.append((min(tm), fn))
            ends = []
            for rows in rows_list:
                m = load.index(min(load))
                load[m] += rows
                tm[m] = max(tm[m], ready) + rows
                ends.append(tm[m])
            return ends

        fillers = [([C] * 3, f) for f in s3u[:head]]
        chunks = [(u, n) for u in units for n in range(5)]
        late = [u for u in lns if u not in units]
        dl = {}
        if _env("DL", 0):
            c0 = _env("DL0", 3)
            for j, u in enumerate(late):
                k = c0 + j * (len(chunks) + _env("DLX", 0) - c0) // len(late)
                if k < len(chunks):
                    dl[k] = u
        fillers += [([LANES] * 3, functools.partial(qkv_chunk, u, n, dl.get(k)))
                    for k, (u, n) in enumerate(chunks)]
        fillers += [([C] * 3, f) for f in s3u[head:]]
        total = (sum(sum(f[0]) for f in fillers) + len(pids) * 4 * (SLOTS + DH)) / 4
        nsc = 4 * len(pids)
        next_s = 0
        s_end, v_end, pend_v = {}, {}, []
        while fillers or next_s < nsc or pend_v:
            now = tm[load.index(min(load))]
            s_ok = next_s < nsc and now >= (total - TAILGAP) * next_s / max(nsc - 4, 1)
            v_ok = len(pend_v) >= VGRP // 2 and all(now >= x[0] for x in pend_v[:VGRP // 2])
            if not fillers and not s_ok and not v_ok:
                if pend_v and (next_s >= nsc or len(pend_v) >= 4):
                    v_ok = True
                else:
                    s_ok = True
            if v_ok:
                for rdy, pv, hp in pend_v[:VGRP // 2]:
                    for h in (2 * hp, 2 * hp + 1):
                        v_end[pv, h] = emit([DH], functools.partial(pairs[pv][2], h), rdy)[0]
                    if hp == 1:
                        extra.append((max(v_end[pv, h] for h in range(NH)) + LFIN, [pairs[pv][3]]))
                pend_v = pend_v[VGRP // 2:]
            elif s_ok:
                for _ in range(SGRP):
                    p, i = pids[next_s // 4], next_s % 4
                    if i == 0:
                        prog.append((min(tm), pairs[p][0]))
                    s_end[p, i] = emit([SLOTS], functools.partial(pairs[p][1], i))[0]
                    if i % 2 == 1:
                        pend_v.append((max(s_end[p, i], s_end[p, i - 1]) + LSM, p, i // 2))
                    next_s += 1
            else:
                emit(*fillers.pop(0))
        ci = conv_items(gs)
        for j, fs in enumerate(ci):
            extra.append(((j + 1) * max(tm) / len(ci), fs))
        for j, u in enumerate(lns):
            extra.append((-1, [functools.partial(ln_prep, u)]))
        extra.sort(key=lambda e: e[0])
        j = 0
        for t0, fn in prog:
            while j < len(extra) and extra[j][0] <= t0:
                for f in extra[j][1]:
                    f()
                j += 1
            fn()
        for e in extra[j:]:
            for f in e[1]:
                f()

    spec = [[int(v) for v in x.split(",")] for x in
            _env("SEGS", "4,0,3,0,14;10,0,0,24,0;0,37,11,0,0").split(";")]
    pos = [0] * 5
    for k, sp in enumerate(spec):
        units, pids, s3i, gs, lns = [list(range(a, a + n)) for a, n in zip(pos, sp)]
        pos = [a + n for a, n in zip(pos, sp)]
        fn = functools.partial(segment, units, pids, [s3_all[i] for i in s3i], gs, lns,
                               _env("HEAD", 3) if k == 0 else 0)
        pl.when(s + dyn0 * k < nstrip)(fn)
    assert pos == [NU, npair, NU, NG, NU], pos

    @pl.when(s == nstrip)
    def _():
        for f in s3_all:
            f()


@jax.jit
def pallas_standalone__window_attn_davit__vision_kernel(
    x: jax.Array,
    dw_pe: jax.Array,
    w_qkv: jax.Array,
    w_o: jax.Array,
):
    B, H, W, Cx = x.shape
    assert B == 1 and Cx == C and H % WS == 0 and W % WS == 0 and WP - LANES < W < WP
    nstrip = H // WS
    nwin = W // WS

    xt = jnp.transpose(x[0], (0, 2, 1))
    dwb = jnp.broadcast_to(dw_pe.reshape(9, C, 1), (9, C, LANES)).astype(F32)
    wq, wk, wv = w_qkv[:, 0:C], w_qkv[:, C:2 * C], w_qkv[:, 2 * C:3 * C]
    z32 = jnp.zeros((C, 32), w_qkv.dtype)
    wperm = jnp.concatenate([
        wv[:, 128:160], wq[:, 0:96],
        wq[:, 96:128], wv[:, 160:192], wq[:, 128:192],
        z32, wk[:, 0:96],
        wk[:, 96:128], z32, wk[:, 128:192],
        wv[:, 0:128]], axis=1)
    wt = w_o.T
    wx, wy, wz = wt[:, 0:64], wt[:, 64:128], wt[:, 128:192]
    wot = jnp.stack([jnp.concatenate(p, axis=1) for p in ((wx, wy), (wz, wy), (wx, wz))])

    nx = lambda s: jnp.minimum(s + 1, nstrip - 1)
    kernel = functools.partial(_kernel, W=W, nwin=nwin, nstrip=nstrip)
    yt = pl.pallas_call(
        kernel,
        grid=(nstrip + 1,),
        in_specs=[
            pl.BlockSpec((WS, C, WP), lambda s: (0, 0, 0)),
            pl.BlockSpec((1, C, WP), lambda s: (WS, 0, 0)),
            pl.BlockSpec((WS, C, WP), lambda s: (nx(s), 0, 0)),
            pl.BlockSpec((1, C, WP), lambda s: (nx(s) * WS - 1, 0, 0)),
            pl.BlockSpec((1, C, WP), lambda s: (jnp.minimum(nx(s) * WS + WS, H - 1), 0, 0)),
            pl.BlockSpec((9, C, LANES), lambda s: (0, 0, 0)),
            pl.BlockSpec((C, 5 * LANES), lambda s: (0, 0)),
            pl.BlockSpec((3, C, LANES), lambda s: (0, 0, 0)),
        ],
        out_specs=pl.BlockSpec((WS, C, WP), lambda s: (jnp.maximum(s - 1, 0), 0, 0)),
        out_shape=jax.ShapeDtypeStruct((H, C, W), x.dtype),
        scratch_shapes=[
            pltpu.VMEM((X0_ROWS, LANES), F32),
            pltpu.VMEM((2, WS * WP, LANES), F32),
            pltpu.VMEM((9, C, LANES), F32),
            pltpu.VMEM((3, 5, LANES // 2, LANES), U32),
            pltpu.VMEM((3, C // 2, LANES), U32),
            pltpu.VMEM((5, WS, WP, LANES), F32),
            pltpu.VMEM((NU, 3, LANES // 2, LANES), U32),
        ],
        compiler_params=pltpu.CompilerParams(
            dimension_semantics=("arbitrary",),
            vmem_limit_bytes=64 * 1024 * 1024,
        ),
        name="davit_window_attn",
    )(xt, xt, xt, xt, xt, dwb, wperm, wot)
    return jnp.transpose(yt, (0, 2, 1))[None]
```

```python
import functools
import math
import os

import jax
import jax.numpy as jnp
from jax import lax
import jax.experimental.pallas as pl
import jax.experimental.pallas.tpu as pltpu

WS = 7
NH = 4
C = 192
DH = C // NH
NG = C // 8
LANES = 128
WP = 512
NT = WP // LANES
NU = WS * NT // 2
SLOTS = 8 * WS
EPS = 1e-5
F32 = jnp.float32
BF16 = jnp.bfloat16
U32 = jnp.uint32

X0_SLOT = WS * NT * C
DW_OFF = 3 * X0_SLOT
X0_ROWS = DW_OFF + 2 * C


def _dot(a, b):
    return jnp.dot(a, b, preferred_element_type=F32)


def _dot_nt(a, b):
    return lax.dot_general(a, b, (((1,), (1,)), ((), ())), preferred_element_type=F32)


def _cat(xs):
    return jnp.concatenate(xs, axis=0)


def _blocks(v):
    return [v[i:i + 8] for i in range(0, v.shape[0], 8)]


def _allred(x, op):
    for sh in (4, 2, 1):
        x = op(x, pltpu.roll(x, sh, 0))
    return x


def _sum3(xs):
    k = _env("NCH", 1)
    return functools.reduce(jnp.add, [functools.reduce(jnp.add, xs[i::k]) for i in range(k)])


def _env(name, default):
    return type(default)(os.environ.get(name, default))


def _kernel(xm_ref, xt_ref, xb_ref, dw_ref, wqkv_ref, wot_ref, o_ref,
            x0_ref, ob_ref, dws_ref, ws_ref, wos_ref, qkv_ref, t_ref, *, W, nwin, nstrip):
    k_ = pl.program_id(0)
    dyn0 = jnp.minimum(k_, 0)

    def rows_at(base, off, n):
        if isinstance(base, int):
            return pl.ds(base + off, n)
        return pl.ds(pl.multiple_of(base + off, 8), n)

    mk = {}

    def new_masks():
        lane = lax.broadcasted_iota(jnp.int32, (8, LANES), 1)
        sub = lax.broadcasted_iota(jnp.int32, (8, LANES), 0)
        nlast = W - (WP - LANES)
        key_ok = sub < WS
        mk.update(
            last=lane < nlast,
            top=lane < jnp.where(k_ > 0, LANES, 0), top_last=lane < jnp.where(k_ > 0, nlast, 0),
            bot=lane < jnp.where(k_ < nstrip - 1, LANES, 0),
            bot_last=lane < jnp.where(k_ < nstrip - 1, nlast, 0),
            never=lane < dyn0, lo=lane < 80, hi=lane >= 80, v=lane < 32, key=key_ok,
            left=lane < SLOTS, keep_a=key_ok & (lane < SLOTS), keep_b=key_ok & (lane >= SLOTS),
            left64=lane < 64)

    nxt = (k_ % 3) * X0_SLOT
    cur = ((k_ + 2) % 3) * X0_SLOT
    prv = ((k_ + 1) % 3) * X0_SLOT
    obw = k_ % 2
    obr = 1 - obw

    def conv_group(c0):
        st = {}

        def row(i):
            if i not in st:
                if i == 0:
                    v, m, ml = xt_ref[0, c0:c0 + 8, :], mk["top"], mk["top_last"]
                elif i == WS + 1:
                    v, m, ml = xb_ref[0, c0:c0 + 8, :], mk["bot"], mk["bot_last"]
                else:
                    v, m, ml = xm_ref[i - 1, c0:c0 + 8, :], None, mk["last"]
                v = v.astype(F32)
                ts = [v[:, t * LANES:(t + 1) * LANES] for t in range(NT)]
                ts = [t if m is None else jnp.where(m, t, 0.0) for t in ts[:-1]] + [jnp.where(ml, ts[-1], 0.0)]
                st[i] = jnp.concatenate(ts, axis=1)
            return st[i]

        def bc(v):
            return jnp.concatenate([v] * NT, axis=1)

        def taps(r):
            st["tw", r] = [bc(x0_ref[rows_at(c0, DW_OFF + k * C, 8), :]) for k in range(2)]

        def piece(r):
            if "w" not in st:
                st["w"] = [bc(dws_ref[k, pl.ds(c0, 8), :]) for k in range(9)]
            wts = list(st["w"])
            if ("tw", r) in st:
                wts[6], wts[8] = st["tw", r]
            abc = [row(r + 1) * wts[3 + j] + row(r) * wts[j] + row(r + 2) * wts[6 + j] for j in range(3)]
            x0 = pltpu.roll(abc[0], 1, 1) + abc[1] + pltpu.roll(abc[2], WP - 1, 1)
            for t in range(NT):
                x0_ref[rows_at(nxt, (r * NT + t) * C + c0, 8), :] = x0[:, t * LANES:(t + 1) * LANES]

        return taps, piece

    @pl.when(k_ == 0)
    def _():
        for k in range(9):
            w = dw_ref[k]
            dws_ref[k] = w + 1.0 if k == 4 else w
            if k in (6, 8):
                x0_ref[pl.ds(DW_OFF + (k - 6) // 2 * C, C), :] = w
        lane = lax.broadcasted_iota(jnp.int32, (C, LANES), 1)
        qs = (DH ** -0.5) * math.log2(math.e)
        for n in range(5):
            w = wqkv_ref[:, n * LANES:(n + 1) * LANES].astype(F32)
            if n == 0:
                w = jnp.where(lane >= 32, w * qs, w)
            elif n == 1:
                w = jnp.where((lane >= 32) & (lane < 64), w, w * qs)
            for i, wi in enumerate((w[0:128], w[64:192], _cat([w[128:192], w[0:64]]))):
                ws_ref[i, n] = pltpu.bitcast(wi.astype(BF16), U32)
        for i in range(3):
            wos_ref[i] = pltpu.bitcast(wot_ref[i].astype(F32).astype(BF16), U32)

        def zero(i, carry):
            x0_ref[pl.ds(pl.multiple_of(2 * X0_SLOT + i * 768, 8), 768), :] = jnp.zeros((768, LANES), F32)
            ob_ref[0, pl.ds(pl.multiple_of(i * WP, 8), WP), :] = jnp.zeros((WP, LANES), F32)
            ob_ref[1, pl.ds(pl.multiple_of(i * WP + WP - 8, 8), 8), :] = jnp.zeros((8, LANES), F32)
            for j in range(2):
                t_ref[2 * i + j] = jnp.zeros(t_ref.shape[1:], U32)
            return carry
        lax.fori_loop(0, WS, zero, 0)

    groups = [conv_group(8 * g) for g in range(NG)]
    WLEAD = _env("WLEAD", 5)

    def conv_items(gs):
        plist = [(g, r) for g in gs for r in range(WS)]
        items = []
        for k, (g, r) in enumerate(plist):
            fs = []
            if k + WLEAD < len(plist):
                g2, r2 = plist[k + WLEAD]
                fs.append(functools.partial(groups[g2][0], r2))
            fs.append(functools.partial(groups[g][1], r))
            items.append(fs)
        return items

    LNP = _env("LNP", 3)
    tokens = {}

    def layernorm_tile(r, t, gates):
        def ld(k):
            return [x0_ref[rows_at(cur + dyn0 * (8 * k), (r * NT + t) * C + 8 * g, 8), :]
                    for g in range(NG)]
        xs = ld(0)
        for g in gates:
            for i in range(_env("NCH", 1)):
                xs[i] = jnp.where(mk["never"], g, xs[i])
        m = _allred(_sum3(xs), jnp.add) * (1.0 / C)
        if LNP == 2:
            v = _allred(_sum3([x * x for x in xs]), jnp.add) * (1.0 / C)
            v = jnp.maximum(v - m * m, 0.0)
        else:
            d = [x - m for x in ld(1)]
            v = _allred(_sum3([x * x for x in d]), jnp.add) * (1.0 / C)
        rs = lax.rsqrt(v + EPS)
        tokens["rs", r * NT + t] = (m, v, rs)[_env("CHAT", 2)]
        return _cat([(x - m) * rs for x in ld(2)])

    def ln_prep(u):
        r, tp = divmod(u, 2)
        hs = []
        for j in range(2):
            gates = []
            k = 2 * u + j - _env("CH1", 2)
            if _env("CH1", 2) and ("rs", k) in tokens:
                gates.append(tokens["rs", k])
            k = u - _env("CH2", 4)
            if _env("CH2", 4) and k in tokens:
                gates += [pltpu.bitcast(x, F32) for x in (tokens[k][0:2] if j == 0 else tokens[k][2:3])]
            hs.append(layernorm_tile(r, 2 * tp + j, gates))
        ha, hb = hs
        ts = [_cat([ha[0:64] - hb[0:64], ha[64:128]]),
              _cat([hb[64:128], hb[128:192] - ha[128:192]]),
              _cat([ha[128:192], hb[0:64]])]
        toks = []
        for i, t in enumerate(ts):
            t = pltpu.bitcast(t.astype(BF16).T, U32)
            t_ref[u, i] = t
            toks.append(t[56:64])
        tokens[u] = toks

    def qkv_chunk(u, n, after=None):
        r, tp = divmod(u, 2)
        p = {}
        for i in (2, 0, 1):
            lhs = t_ref[u, i]
            if after is not None:
                lhs = _cat([jnp.where(mk["never"], tokens[after][i], lhs[0:8]), lhs[8:]])
            p[i] = _dot(pltpu.bitcast(lhs, BF16), pltpu.bitcast(ws_ref[i, n], BF16))
        if _env("BLK", 0):
            for i in range(0, LANES, 8):
                for j in range(2):
                    qkv_ref[n, r, pl.ds((2 * tp + j) * LANES + i, 8), :] = p[j][i:i + 8] + p[2][i:i + 8]
            return
        for j in range(2):
            qkv_ref[n, r, pl.ds((2 * tp + j) * LANES, LANES), :] = p[j] + p[2]

    zero8 = jnp.zeros((8, LANES), F32)

    def gather(n, off):
        return [qkv_ref[n, r, pl.ds(off, 8), :] for r in range(WS)]

    def softmax_t(st):
        rows = _blocks(st)
        m = functools.reduce(jnp.maximum, rows)
        m = _allred(jnp.where(mk["key"], m, -jnp.inf), jnp.maximum)
        p = [jnp.exp2(x - m) for x in rows]
        return p, functools.reduce(jnp.add, p)

    def s2_pair(offa):
        offb = offa + WS
        st = {}

        def vprep():
            u1 = _cat(gather(4, offa) + gather(4, offb) + [zero8, zero8])
            u2 = _cat([jnp.where(mk["v"], x, y) for x, y in
                       zip(gather(0, offa) + gather(0, offb), gather(1, offa) + gather(1, offb))]
                      + [zero8, zero8])
            u1t = pltpu.bitcast(u1.astype(BF16).T, U32)
            u2t = pltpu.bitcast(u2[:, 0:64].astype(BF16).T, U32)
            vt = _cat([u1t, u2t])
            st["vt"] = [pltpu.bitcast(vt[24 * h:24 * h + 24], BF16) for h in range(NH)]

        def score(i):
            hp, sw = divmod(i, 2)
            ma, mb = (mk["lo"], mk["hi"]) if sw == 0 else (mk["hi"], mk["lo"])
            q = _cat([jnp.where(ma, v, 0.0) for v in gather(hp, offa)]
                     + [jnp.where(mb, v, 0.0) for v in gather(hp, offb)] + [zero8, zero8])
            k = _cat([jnp.where(ma, x, y)
                      for x, y in zip(gather(2 + hp, offa), gather(2 + hp, offb))])
            st["p", i] = softmax_t(_dot_nt(k, q))

        def value(h):
            hp, sw = divmod(h, 2)
            (pa, sa), (pb, sb) = st["p", 2 * hp + sw], st["p", 2 * hp + 1 - sw]
            pm = _cat([jnp.where(mk["keep_a"], v, 0.0) for v in pa]
                      + [jnp.where(mk["keep_b"], v, 0.0) for v in pb] + [zero8, zero8])
            den = _allred(jnp.where(mk["key"], jnp.where(mk["left"], sa, sb), 0.0), jnp.add)
            rec = pl.reciprocal(den, approx=True)
            rec = rec * (2.0 - den * rec)
            st["o", h] = [b * rec for b in _blocks(_dot(st["vt"][h], pm))]

        def finish():
            o = [b for h in range(NH) for b in st["o", h]]
            w = pltpu.pack_elementwise([_cat(o[0:16]), _cat(o[16:24] + o[16:24])], packed_dtype=BF16)
            wt = pltpu.bitcast(w, F32).T
            for i, off in enumerate((offa, offb)):
                for r in range(WS):
                    base = i * SLOTS + 8 * r
                    ob_ref[obw, pl.ds(r * WP + off, WS), :] = wt[base:base + WS]

        return vprep, score, value, finish

    npair = (nwin + 1) // 2
    pairs = [s2_pair(min(2 * p, nwin - 2) * WS) for p in range(npair)]

    def s3_unit(r, tp):
        def unpack(t):
            w = pltpu.bitcast(ob_ref[obr, pl.ds(r * WP + t * LANES, LANES), :], U32)
            return [_blocks(pltpu.unpack_elementwise(w, index=i, packed_dtype=BF16, unpacked_dtype=F32))
                    for i in range(2)]

        (la, ha), (lb, hb) = unpack(2 * tp), unpack(2 * tp + 1)
        t3 = _cat([jnp.where(mk["left64"], x, y) for x, y in zip(lb, ha)])
        t1 = _cat([x - jnp.where(mk["left64"], y, 0.0) for x, y in zip(la, lb)])
        t2 = _cat([jnp.where(mk["left64"], x - y, z) for x, y, z in zip(hb, ha, lb)])
        p3 = _dot_nt(pltpu.bitcast(wos_ref[2], BF16), t3)
        ys = [_dot_nt(pltpu.bitcast(wos_ref[i], BF16), t) + p3
              + x0_ref[rows_at(prv, (r * NT + 2 * tp + i) * C, C), :] for i, t in enumerate((t1, t2))]
        o_ref[r, :, pl.ds(2 * tp * LANES, 2 * LANES)] = jnp.concatenate(ys, axis=1).astype(o_ref.dtype)

    H0 = _env("H0", 2)
    s3_all = [functools.partial(s3_unit, r, tp) for r, tp in
              [(r, 0) for r in range(H0)] + [(r, 1) for r in range(WS)] + [(r, 0) for r in range(H0, WS)]]

    LSM = _env("LSM", 240)
    LFIN = _env("LFIN", 200)
    PREP = _env("PREP", 600)
    SGRP = _env("SGRP", 4)
    VGRP = _env("VGRP", 2)
    TAILGAP = _env("TAILGAP", 800)

    def segment(units, pids, s3u, gs, lns, head):
        new_masks()
        load = [0] * 4
        tm = [0] * 4
        prog, extra = [], []

        def emit(rows_list, fn, ready=0):
            prog.append((min(tm), fn))
            ends = []
            for rows in rows_list:
                m = load.index(min(load))
                load[m] += rows
                tm[m] = max(tm[m], ready) + rows
                ends.append(tm[m])
            return ends

        fillers = [([C] * 3, f) for f in s3u[:head]]
        chunks = [(u, n) for u in units for n in range(5)]
        late = [u for u in lns if u not in units]
        dl = {}
        if _env("DL", 0):
            c0 = _env("DL0", 3)
            for j, u in enumerate(late):
                k = c0 + j * (len(chunks) + _env("DLX", 0) - c0) // len(late)
                if k < len(chunks):
                    dl[k] = u
        fillers += [([LANES] * 3, functools.partial(qkv_chunk, u, n, dl.get(k)))
                    for k, (u, n) in enumerate(chunks)]
        fillers += [([C] * 3, f) for f in s3u[head:]]
        total = (sum(sum(f[0]) for f in fillers) + len(pids) * 4 * (SLOTS + DH)) / 4
        nsc = 4 * len(pids)
        next_s = 0
        s_end, v_end, pend_v = {}, {}, []
        while fillers or next_s < nsc or pend_v:
            now = tm[load.index(min(load))]
            s_ok = next_s < nsc and now >= (total - TAILGAP) * next_s / max(nsc - 4, 1)
            v_ok = len(pend_v) >= VGRP // 2 and all(now >= x[0] for x in pend_v[:VGRP // 2])
            if not fillers and not s_ok and not v_ok:
                if pend_v and (next_s >= nsc or len(pend_v) >= 4):
                    v_ok = True
                else:
                    s_ok = True
            if v_ok:
                for rdy, pv, hp in pend_v[:VGRP // 2]:
                    for h in (2 * hp, 2 * hp + 1):
                        v_end[pv, h] = emit([DH], functools.partial(pairs[pv][2], h), rdy)[0]
                    if hp == 1:
                        extra.append((max(v_end[pv, h] for h in range(NH)) + LFIN, [pairs[pv][3]]))
                pend_v = pend_v[VGRP // 2:]
            elif s_ok:
                for _ in range(SGRP):
                    p, i = pids[next_s // 4], next_s % 4
                    if i == 0:
                        prog.append((min(tm), pairs[p][0]))
                    s_end[p, i] = emit([SLOTS], functools.partial(pairs[p][1], i))[0]
                    if i % 2 == 1:
                        pend_v.append((max(s_end[p, i], s_end[p, i - 1]) + LSM, p, i // 2))
                    next_s += 1
            else:
                emit(*fillers.pop(0))
        ci = conv_items(gs)
        for j, fs in enumerate(ci):
            extra.append(((j + 1) * max(tm) / len(ci), fs))
        for j, u in enumerate(lns):
            extra.append((-1, [functools.partial(ln_prep, u)]))
        extra.sort(key=lambda e: e[0])
        j = 0
        for t0, fn in prog:
            while j < len(extra) and extra[j][0] <= t0:
                for f in extra[j][1]:
                    f()
                j += 1
            fn()
        for e in extra[j:]:
            for f in e[1]:
                f()

    spec = [[int(v) for v in x.split(",")] for x in
            _env("SEGS", "4,0,3,0,14;10,0,0,24,0;0,37,11,0,0").split(";")]
    pos = [0] * 5
    for k, sp in enumerate(spec):
        units, pids, s3i, gs, lns = [list(range(a, a + n)) for a, n in zip(pos, sp)]
        pos = [a + n for a, n in zip(pos, sp)]
        fn = functools.partial(segment, units, pids, [s3_all[i] for i in s3i], gs, lns,
                               _env("HEAD", 3) if k == 0 else 0)
        pl.when((k_ + dyn0 * k <= nstrip) & (k_ >= (0 if gs else 1)))(fn)
    assert pos == [NU, npair, NU, NG, NU], pos

    @pl.when(k_ == nstrip + 1)
    def _():
        new_masks()
        for f in s3_all:
            f()


@jax.jit
def pallas_standalone__window_attn_davit__vision_kernel(
    x: jax.Array,
    dw_pe: jax.Array,
    w_qkv: jax.Array,
    w_o: jax.Array,
):
    B, H, W, Cx = x.shape
    assert B == 1 and Cx == C and H % WS == 0 and W % WS == 0 and WP - LANES < W < WP
    nstrip = H // WS
    nwin = W // WS

    xt = jnp.transpose(x[0], (0, 2, 1))
    dwb = jnp.broadcast_to(dw_pe.reshape(9, C, 1), (9, C, LANES)).astype(F32)
    wq, wk, wv = w_qkv[:, 0:C], w_qkv[:, C:2 * C], w_qkv[:, 2 * C:3 * C]
    z32 = jnp.zeros((C, 32), w_qkv.dtype)
    wperm = jnp.concatenate([
        wv[:, 128:160], wq[:, 0:96],
        wq[:, 96:128], wv[:, 160:192], wq[:, 128:192],
        z32, wk[:, 0:96],
        wk[:, 96:128], z32, wk[:, 128:192],
        wv[:, 0:128]], axis=1)
    wt = w_o.T
    wx, wy, wz = wt[:, 0:64], wt[:, 64:128], wt[:, 128:192]
    wot = jnp.stack([jnp.concatenate(p, axis=1) for p in ((wx, wy), (wz, wy), (wx, wz))])

    nx = lambda s: jnp.minimum(s, nstrip - 1)
    kernel = functools.partial(_kernel, W=W, nwin=nwin, nstrip=nstrip)
    yt = pl.pallas_call(
        kernel,
        grid=(nstrip + 2,),
        in_specs=[
            pl.BlockSpec((WS, C, WP), lambda s: (nx(s), 0, 0)),
            pl.BlockSpec((1, C, WP), lambda s: (jnp.maximum(nx(s) * WS - 1, 0), 0, 0)),
            pl.BlockSpec((1, C, WP), lambda s: (jnp.minimum(nx(s) * WS + WS, H - 1), 0, 0)),
            pl.BlockSpec((9, C, LANES), lambda s: (0, 0, 0)),
            pl.BlockSpec((C, 5 * LANES), lambda s: (0, 0)),
            pl.BlockSpec((3, C, LANES), lambda s: (0, 0, 0)),
        ],
        out_specs=pl.BlockSpec((WS, C, WP), lambda s: (jnp.maximum(s - 2, 0), 0, 0)),
        out_shape=jax.ShapeDtypeStruct((H, C, W), x.dtype),
        scratch_shapes=[
            pltpu.VMEM((X0_ROWS, LANES), F32),
            pltpu.VMEM((2, WS * WP, LANES), F32),
            pltpu.VMEM((9, C, LANES), F32),
            pltpu.VMEM((3, 5, LANES // 2, LANES), U32),
            pltpu.VMEM((3, C // 2, LANES), U32),
            pltpu.VMEM((5, WS, WP, LANES), F32),
            pltpu.VMEM((NU, 3, LANES // 2, LANES), U32),
        ],
        compiler_params=pltpu.CompilerParams(
            dimension_semantics=("arbitrary",),
            vmem_limit_bytes=64 * 1024 * 1024,
        ),
        name="davit_window_attn",
    )(xt, xt, xt, dwb, wperm, wot)
    return jnp.transpose(yt, (0, 2, 1))[None]
```

```python
import functools
import math
import os

import jax
import jax.numpy as jnp
from jax import lax
import jax.experimental.pallas as pl
import jax.experimental.pallas.tpu as pltpu

WS = 7
NH = 4
C = 192
DH = C // NH
NG = C // 8
LANES = 128
WP = 512
NT = WP // LANES
NU = WS * NT // 2
SLOTS = 8 * WS
EPS = 1e-5
F32 = jnp.float32
BF16 = jnp.bfloat16
U32 = jnp.uint32

X0_SLOT = WS * NT * C
DW_OFF = 3 * X0_SLOT
X0_ROWS = DW_OFF + 2 * C


def _dot(a, b):
    return jnp.dot(a, b, preferred_element_type=F32)


def _dot_nt(a, b):
    return lax.dot_general(a, b, (((1,), (1,)), ((), ())), preferred_element_type=F32)


def _cat(xs):
    return jnp.concatenate(xs, axis=0)


def _blocks(v):
    return [v[i:i + 8] for i in range(0, v.shape[0], 8)]


def _allred(x, op):
    for sh in (4, 2, 1):
        x = op(x, pltpu.roll(x, sh, 0))
    return x


def _sum3(xs):
    k = _env("NCH", 1)
    return functools.reduce(jnp.add, [functools.reduce(jnp.add, xs[i::k]) for i in range(k)])


def _env(name, default):
    return type(default)(os.environ.get(name, default))


def _kernel(xm_ref, xt_ref, xb_ref, dw_ref, wqkv_ref, wot_ref, o_ref,
            x0_ref, ob_ref, dws_ref, ws_ref, wos_ref, qkv_ref, t_ref, stg_ref, *, W, nwin, nstrip):
    k_ = pl.program_id(0)
    dyn0 = jnp.minimum(k_, 0)

    def rows_at(base, off, n):
        if isinstance(base, int):
            return pl.ds(base + off, n)
        return pl.ds(pl.multiple_of(base + off, 8), n)

    mk = {}

    def new_masks():
        lane = lax.broadcasted_iota(jnp.int32, (8, LANES), 1)
        sub = lax.broadcasted_iota(jnp.int32, (8, LANES), 0)
        nlast = W - (WP - LANES)
        key_ok = sub < WS
        mk.update(
            last=lane < nlast,
            top=lane < jnp.where(k_ > 0, LANES, 0), top_last=lane < jnp.where(k_ > 0, nlast, 0),
            bot=lane < jnp.where(k_ < nstrip - 1, LANES, 0),
            bot_last=lane < jnp.where(k_ < nstrip - 1, nlast, 0),
            never=lane < dyn0, lo=lane < 80, hi=lane >= 80, v=lane < 32, key=key_ok,
            left=lane < SLOTS, keep_a=key_ok & (lane < SLOTS), keep_b=key_ok & (lane >= SLOTS),
            left64=lane < 64)

    nxt = (k_ % 3) * X0_SLOT
    prv = ((k_ + 1) % 3) * X0_SLOT

    def conv_group(c0):
        st = {}

        def row(i):
            if i not in st:
                if i == 0:
                    v, m, ml = xt_ref[0, c0:c0 + 8, :], mk["top"], mk["top_last"]
                elif i == WS + 1:
                    v, m, ml = xb_ref[0, c0:c0 + 8, :], mk["bot"], mk["bot_last"]
                else:
                    v, m, ml = xm_ref[i - 1, c0:c0 + 8, :], None, mk["last"]
                v = v.astype(F32)
                ts = [v[:, t * LANES:(t + 1) * LANES] for t in range(NT)]
                ts = [t if m is None else jnp.where(m, t, 0.0) for t in ts[:-1]] + [jnp.where(ml, ts[-1], 0.0)]
                st[i] = jnp.concatenate(ts, axis=1)
            return st[i]

        def bc(v):
            return jnp.concatenate([v] * NT, axis=1)

        def taps(r):
            st["tw", r] = [bc(x0_ref[rows_at(c0, DW_OFF + k * C, 8), :]) for k in range(2)]

        def piece(r):
            if "w" not in st:
                st["w"] = [bc(dws_ref[k, pl.ds(c0, 8), :]) for k in range(9)]
            wts = list(st["w"])
            if ("tw", r) in st:
                wts[6], wts[8] = st["tw", r]
            abc = [row(r + 1) * wts[3 + j] + row(r) * wts[j] + row(r + 2) * wts[6 + j] for j in range(3)]
            x0 = pltpu.roll(abc[0], 1, 1) + abc[1] + pltpu.roll(abc[2], WP - 1, 1)
            for t in range(NT):
                x0_ref[rows_at(nxt, (r * NT + t) * C + c0, 8), :] = x0[:, t * LANES:(t + 1) * LANES]

        return taps, piece

    @pl.when(k_ == 0)
    def _():
        for k in range(9):
            w = dw_ref[k]
            dws_ref[k] = w + 1.0 if k == 4 else w
            if k in (6, 8):
                x0_ref[pl.ds(DW_OFF + (k - 6) // 2 * C, C), :] = w
        lane = lax.broadcasted_iota(jnp.int32, (C, LANES), 1)
        qs = (DH ** -0.5) * math.log2(math.e)
        for n in range(5):
            w = wqkv_ref[:, n * LANES:(n + 1) * LANES].astype(F32)
            if n == 0:
                w = jnp.where(lane >= 32, w * qs, w)
            elif n == 1:
                w = jnp.where((lane >= 32) & (lane < 64), w, w * qs)
            for i, wi in enumerate((w[0:128], w[64:192], _cat([w[128:192], w[0:64]]))):
                ws_ref[i, n] = pltpu.bitcast(wi.astype(BF16), U32)
        for i in range(3):
            wos_ref[i] = pltpu.bitcast(wot_ref[i].astype(F32).astype(BF16), U32)

        def zero(i, carry):
            x0_ref[pl.ds(pl.multiple_of(X0_SLOT + i * 1536, 8), 1536), :] = jnp.zeros((1536, LANES), F32)
            ob_ref[pl.ds(pl.multiple_of(i * WP, 8), WP), :] = jnp.zeros((WP, LANES), F32)
            for j in range(2):
                t_ref[2 * i + j] = jnp.zeros(t_ref.shape[1:], U32)
            for j in range(6):
                stg_ref[6 * i + j] = jnp.zeros(stg_ref.shape[1:], F32)
            return carry
        lax.fori_loop(0, WS, zero, 0)

    groups = [conv_group(8 * g) for g in range(NG)]
    WLEAD = _env("WLEAD", 5)

    def conv_items(gs):
        plist = [(g, r) for g in gs for r in range(WS)]
        items = []
        for k, (g, r) in enumerate(plist):
            fs = []
            if k + WLEAD < len(plist):
                g2, r2 = plist[k + WLEAD]
                fs.append(functools.partial(groups[g2][0], r2))
            fs.append(functools.partial(groups[g][1], r))
            items.append(fs)
        return items

    LNP = _env("LNP", 3)
    tokens = {}

    def layernorm_tile(r, t, gates):
        def ld(k):
            return [x0_ref[rows_at(nxt + dyn0 * (8 * k), (r * NT + t) * C + 8 * g, 8), :]
                    for g in range(NG)]
        xs = ld(0)
        for g in gates:
            for i in range(_env("NCH", 1)):
                xs[i] = jnp.where(mk["never"], g, xs[i])
        m = _allred(_sum3(xs), jnp.add) * (1.0 / C)
        if LNP == 2:
            v = _allred(_sum3([x * x for x in xs]), jnp.add) * (1.0 / C)
            v = jnp.maximum(v - m * m, 0.0)
        else:
            d = [x - m for x in ld(1)]
            v = _allred(_sum3([x * x for x in d]), jnp.add) * (1.0 / C)
        rs = lax.rsqrt(v + EPS)
        tokens["rs", r * NT + t] = (m, v, rs)[_env("CHAT", 2)]
        return _cat([(x - m) * rs for x in ld(2)])

    def ln_prep(u):
        r, tp = divmod(u, 2)
        hs = []
        for j in range(2):
            gates = []
            k = 2 * u + j - _env("CH1", 2)
            if _env("CH1", 2) and ("rs", k) in tokens:
                gates.append(tokens["rs", k])
            k = u - _env("CH2", 4)
            if _env("CH2", 4) and k in tokens:
                gates += [pltpu.bitcast(x, F32) for x in (tokens[k][0:2] if j == 0 else tokens[k][2:3])]
            hs.append(layernorm_tile(r, 2 * tp + j, gates))
        ha, hb = hs
        ts = [_cat([ha[0:64] - hb[0:64], ha[64:128]]),
              _cat([hb[64:128], hb[128:192] - ha[128:192]]),
              _cat([ha[128:192], hb[0:64]])]
        toks = []
        for i, t in enumerate(ts):
            t = pltpu.bitcast(t.astype(BF16).T, U32)
            t_ref[u, i] = t
            toks.append(t[56:64])
        tokens[u] = toks

    def qkv_chunk(u, n, after=None):
        r, tp = divmod(u, 2)
        p = {}
        for i in (2, 0, 1):
            lhs = t_ref[u, i]
            if after is not None:
                lhs = _cat([jnp.where(mk["never"], tokens[after][i], lhs[0:8]), lhs[8:]])
            p[i] = _dot(pltpu.bitcast(lhs, BF16), pltpu.bitcast(ws_ref[i, n], BF16))
        if _env("BLK", 0):
            for i in range(0, LANES, 8):
                for j in range(2):
                    qkv_ref[n, r, pl.ds((2 * tp + j) * LANES + i, 8), :] = p[j][i:i + 8] + p[2][i:i + 8]
            return
        for j in range(2):
            qkv_ref[n, r, pl.ds((2 * tp + j) * LANES, LANES), :] = p[j] + p[2]

    zero8 = jnp.zeros((8, LANES), F32)

    def gather(n, off):
        return [qkv_ref[n, r, pl.ds(off, 8), :] for r in range(WS)]

    def softmax_t(st):
        rows = _blocks(st)
        m = functools.reduce(jnp.maximum, rows)
        m = _allred(jnp.where(mk["key"], m, -jnp.inf), jnp.maximum)
        p = [jnp.exp2(x - m) for x in rows]
        return p, functools.reduce(jnp.add, p)

    def s2_pair(pi, offa):
        offb = offa + WS
        st = {}

        def vprep():
            u1 = _cat(gather(4, offa) + gather(4, offb) + [zero8, zero8])
            u2 = _cat([jnp.where(mk["v"], x, y) for x, y in
                       zip(gather(0, offa) + gather(0, offb), gather(1, offa) + gather(1, offb))]
                      + [zero8, zero8])
            VM = _env("VM", 0)
            if VM == 0:
                u1t = pltpu.bitcast(u1.astype(BF16).T, U32)
                u2t = pltpu.bitcast(u2[:, 0:64].astype(BF16).T, U32)
                vt = _cat([u1t, u2t])
            elif VM == 1:
                vt = _cat([pltpu.bitcast(u.astype(BF16).T, U32) for u in (u1, u2)])
            else:
                vt = pltpu.bitcast(jnp.concatenate([u1, u2], axis=1).astype(BF16).T, U32)
            st["vt"] = [pltpu.bitcast(vt[24 * h:24 * h + 24], BF16) for h in range(NH)]

        def score(i):
            hp, sw = divmod(i, 2)
            ma, mb = (mk["lo"], mk["hi"]) if sw == 0 else (mk["hi"], mk["lo"])
            q = _cat([jnp.where(ma, v, 0.0) for v in gather(hp, offa)]
                     + [jnp.where(mb, v, 0.0) for v in gather(hp, offb)] + [zero8, zero8])
            k = _cat([jnp.where(ma, x, y)
                      for x, y in zip(gather(2 + hp, offa), gather(2 + hp, offb))])
            st["p", i] = softmax_t(_dot_nt(k, q))

        def value(h):
            hp, sw = divmod(h, 2)
            (pa, sa), (pb, sb) = st["p", 2 * hp + sw], st["p", 2 * hp + 1 - sw]
            pm = _cat([jnp.where(mk["keep_a"], v, 0.0) for v in pa]
                      + [jnp.where(mk["keep_b"], v, 0.0) for v in pb] + [zero8, zero8])
            den = _allred(jnp.where(mk["key"], jnp.where(mk["left"], sa, sb), 0.0), jnp.add)
            rec = pl.reciprocal(den, approx=True)
            if _env("NR", 1):
                rec = rec * (2.0 - den * rec)
            st["o", h] = [b * rec for b in _blocks(_dot(st["vt"][h], pm))]

        def finish():
            if _env("PH", 0):
                xs, ys, zs = ([b for h in range(NH) for b in st["o", h][2 * j:2 * j + 2]] for j in range(3))
                o = xs + ys + zs
            else:
                o = [b for h in range(NH) for b in st["o", h]]
            w = pltpu.pack_elementwise([_cat(o[0:16]), _cat(o[16:24] + o[16:24])], packed_dtype=BF16)
            stg_ref[pi] = pltpu.bitcast(w, F32)

        def scatter():
            wt = stg_ref[pi].T
            for i, off in enumerate((offa, offb)):
                for r in range(WS):
                    base = i * SLOTS + 8 * r
                    ob_ref[pl.ds(r * WP + off, WS), :] = wt[base:base + WS]

        return vprep, score, value, finish, scatter

    npair = (nwin + 1) // 2
    pairs = [s2_pair(p, min(2 * p, nwin - 2) * WS) for p in range(npair)]

    def s3_unit(r, tp):
        def unpack(t):
            w = pltpu.bitcast(ob_ref[pl.ds(r * WP + t * LANES, LANES), :], U32)
            return [_blocks(pltpu.unpack_elementwise(w, index=i, packed_dtype=BF16, unpacked_dtype=F32))
                    for i in range(2)]

        (la, ha), (lb, hb) = unpack(2 * tp), unpack(2 * tp + 1)
        t3 = _cat([jnp.where(mk["left64"], x, y) for x, y in zip(lb, ha)])
        t1 = _cat([x - jnp.where(mk["left64"], y, 0.0) for x, y in zip(la, lb)])
        t2 = _cat([jnp.where(mk["left64"], x - y, z) for x, y, z in zip(hb, ha, lb)])
        p3 = _dot_nt(pltpu.bitcast(wos_ref[2], BF16), t3)
        ys = [_dot_nt(pltpu.bitcast(wos_ref[i], BF16), t) + p3
              + x0_ref[rows_at(prv, (r * NT + 2 * tp + i) * C, C), :] for i, t in enumerate((t1, t2))]
        o_ref[r, :, pl.ds(2 * tp * LANES, 2 * LANES)] = jnp.concatenate(ys, axis=1).astype(o_ref.dtype)

    s3_all = [functools.partial(s3_unit, r, tp) for r in range(WS) for tp in range(2)]

    LSM = _env("LSM", 240)
    LFIN = _env("LFIN", 200)
    PREP = _env("PREP", 600)
    SGRP = _env("SGRP", 4)
    VGRP = _env("VGRP", 2)
    TAILGAP = _env("TAILGAP", 800)

    def segment(units, pids, s3u, gs, lns, head, scat=()):
        load = [0] * 4
        tm = [0] * 4
        prog, extra = [], []

        def emit(rows_list, fn, ready=0):
            prog.append((min(tm), fn))
            ends = []
            for rows in rows_list:
                m = load.index(min(load))
                load[m] += rows
                tm[m] = max(tm[m], ready) + rows
                ends.append(tm[m])
            return ends

        fillers = [([C] * 3, f) for f in s3u[:head]]
        chunks = [(u, n) for u in units for n in range(5)]
        late = [u for u in lns if u not in units]
        dl = {}
        if _env("DL", 0):
            c0 = _env("DL0", 3)
            for j, u in enumerate(late):
                k = c0 + j * (len(chunks) + _env("DLX", 0) - c0) // len(late)
                if k < len(chunks):
                    dl[k] = u
        fillers += [([LANES] * 3, functools.partial(qkv_chunk, u, n, dl.get(k)))
                    for k, (u, n) in enumerate(chunks)]
        fillers += [([C] * 3, f) for f in s3u[head:]]
        total = (sum(sum(f[0]) for f in fillers) + len(pids) * 4 * (SLOTS + DH)) / 4
        nsc = 4 * len(pids)
        next_s = 0
        s_end, v_end, pend_v = {}, {}, []
        while fillers or next_s < nsc or pend_v:
            now = tm[load.index(min(load))]
            s_ok = next_s < nsc and now >= (total - TAILGAP) * next_s / max(nsc - 4, 1)
            v_ok = len(pend_v) >= VGRP // 2 and all(now >= x[0] for x in pend_v[:VGRP // 2])
            if not fillers and not s_ok and not v_ok:
                if pend_v and (next_s >= nsc or len(pend_v) >= 4):
                    v_ok = True
                else:
                    s_ok = True
            if v_ok:
                for rdy, pv, hp in pend_v[:VGRP // 2]:
                    for h in (2 * hp, 2 * hp + 1):
                        v_end[pv, h] = emit([DH], functools.partial(pairs[pv][2], h), rdy)[0]
                    if hp == 1:
                        extra.append((max(v_end[pv, h] for h in range(NH)) + LFIN, [pairs[pv][3]]))
                pend_v = pend_v[VGRP // 2:]
            elif s_ok:
                for _ in range(SGRP):
                    p, i = pids[next_s // 4], next_s % 4
                    if i == 0:
                        prog.append((min(tm), pairs[p][0]))
                    s_end[p, i] = emit([SLOTS], functools.partial(pairs[p][1], i))[0]
                    if i % 2 == 1:
                        pend_v.append((max(s_end[p, i], s_end[p, i - 1]) + LSM, p, i // 2))
                    next_s += 1
            else:
                emit(*fillers.pop(0))
        ci = conv_items(gs)
        if ci:
            for j, p in enumerate(scat):
                ci[_env("SC0", 0) + 4 * j].insert(0, pairs[p][4])
            scat = ()
        for j, fs in enumerate(ci):
            extra.append(((j + 1) * max(tm) / len(ci), fs))
        for j, u in enumerate(lns):
            extra.append((-1, [functools.partial(ln_prep, u)]))
        for j, p in enumerate(scat):
            t0 = head * 3 * C / 4
            extra.append((t0 + j * _env("SCEND", 0.8) * (max(tm) - t0) / len(scat), [pairs[p][4]]))
        extra.sort(key=lambda e: e[0])
        j = 0
        for t0, fn in prog:
            while j < len(extra) and extra[j][0] <= t0:
                for f in extra[j][1]:
                    f()
                j += 1
            fn()
        for e in extra[j:]:
            for f in e[1]:
                f()

    NB = _env("NB", 4)
    NSC = _env("NSC", 24)
    HEAD = _env("HEAD", 3)
    blocks = [
        (0, functools.partial(segment, list(range(NB, NU)), [], [], list(range(NG)), [], 0,
                              list(range(NSC, npair)))),
        (1, functools.partial(segment, [], list(range(npair)), s3_all[HEAD:], [], [], 0)),
        (0, functools.partial(segment, list(range(NB)), [], s3_all[:HEAD], [], list(range(NU)), HEAD,
                              list(range(NSC)))),
    ]
    for k, (first, fn) in enumerate(blocks):
        if str(k) in _env("ONLY", "012"):
            new_masks()
            pl.when((k_ + dyn0 * k <= nstrip) & (k_ >= first))(fn)

    @pl.when(k_ == nstrip + 1)
    def _():
        new_masks()
        for p in range(NSC, npair):
            pairs[p][4]()
        for f in s3_all[:1 if "ONLY" in os.environ else NU]:
            f()


@jax.jit
def pallas_standalone__window_attn_davit__vision_kernel(
    x: jax.Array,
    dw_pe: jax.Array,
    w_qkv: jax.Array,
    w_o: jax.Array,
):
    B, H, W, Cx = x.shape
    assert B == 1 and Cx == C and H % WS == 0 and W % WS == 0 and WP - LANES < W < WP
    nstrip = H // WS
    nwin = W // WS

    xt = jnp.transpose(x[0], (0, 2, 1))
    dwb = jnp.broadcast_to(dw_pe.reshape(9, C, 1), (9, C, LANES)).astype(F32)
    wq, wk, wv = w_qkv[:, 0:C], w_qkv[:, C:2 * C], w_qkv[:, 2 * C:3 * C]
    z32 = jnp.zeros((C, 32), w_qkv.dtype)
    wperm = jnp.concatenate([
        wv[:, 128:160], wq[:, 0:96],
        wq[:, 96:128], wv[:, 160:192], wq[:, 128:192],
        z32, wk[:, 0:96],
        wk[:, 96:128], z32, wk[:, 128:192],
        wv[:, 0:128]], axis=1)
    wt = w_o.T
    wx, wy, wz = wt[:, 0:64], wt[:, 64:128], wt[:, 128:192]
    if _env("PH", 0):
        wx, wy, wz = (jnp.concatenate([wt[:, DH * h + 16 * j:DH * h + 16 * j + 16] for h in range(NH)], axis=1)
                      for j in range(3))
    wot = jnp.stack([jnp.concatenate(p, axis=1) for p in ((wx, wy), (wz, wy), (wx, wz))])

    nx = lambda s: jnp.minimum(s, nstrip - 1)
    kernel = functools.partial(_kernel, W=W, nwin=nwin, nstrip=nstrip)
    yt = pl.pallas_call(
        kernel,
        grid=(nstrip + 2,),
        in_specs=[
            pl.BlockSpec((WS, C, WP), lambda s: (nx(s), 0, 0)),
            pl.BlockSpec((1, C, WP), lambda s: (jnp.maximum(nx(s) * WS - 1, 0), 0, 0)),
            pl.BlockSpec((1, C, WP), lambda s: (jnp.minimum(nx(s) * WS + WS, H - 1), 0, 0)),
            pl.BlockSpec((9, C, LANES), lambda s: (0, 0, 0)),
            pl.BlockSpec((C, 5 * LANES), lambda s: (0, 0)),
            pl.BlockSpec((3, C, LANES), lambda s: (0, 0, 0)),
        ],
        out_specs=pl.BlockSpec((WS, C, WP), lambda s: (jnp.maximum(s - 2, 0), 0, 0)),
        out_shape=jax.ShapeDtypeStruct((H, C, W), x.dtype),
        scratch_shapes=[
            pltpu.VMEM((X0_ROWS, LANES), F32),
            pltpu.VMEM((WS * WP, LANES), F32),
            pltpu.VMEM((9, C, LANES), F32),
            pltpu.VMEM((3, 5, LANES // 2, LANES), U32),
            pltpu.VMEM((3, C // 2, LANES), U32),
            pltpu.VMEM((5, WS, WP, LANES), F32),
            pltpu.VMEM((NU, 3, LANES // 2, LANES), U32),
            pltpu.VMEM((42, LANES, LANES), F32),
        ],
        compiler_params=pltpu.CompilerParams(
            dimension_semantics=("arbitrary",),
            vmem_limit_bytes=64 * 1024 * 1024,
        ),
        name="davit_window_attn",
    )(xt, xt, xt, dwb, wperm, wot)
    return jnp.transpose(yt, (0, 2, 1))[None]
```

```python
import functools
import math
import os

import jax
import jax.numpy as jnp
from jax import lax
import jax.experimental.pallas as pl
import jax.experimental.pallas.tpu as pltpu

WS = 7
NH = 4
C = 192
DH = C // NH
NG = C // 8
LANES = 128
WP = 512
NT = WP // LANES
NU = WS * NT // 2
SLOTS = 8 * WS
EPS = 1e-5
F32 = jnp.float32
BF16 = jnp.bfloat16
U32 = jnp.uint32

X0_SLOT = WS * NT * C
DW_OFF = 3 * X0_SLOT
X0_ROWS = DW_OFF + 2 * C


def _dot(a, b):
    return jnp.dot(a, b, preferred_element_type=F32)


def _dot_nt(a, b):
    return lax.dot_general(a, b, (((1,), (1,)), ((), ())), preferred_element_type=F32)


def _cat(xs):
    return jnp.concatenate(xs, axis=0)


def _blocks(v):
    return [v[i:i + 8] for i in range(0, v.shape[0], 8)]


def _allred(x, op):
    for sh in (4, 2, 1):
        x = op(x, pltpu.roll(x, sh, 0))
    return x


def _sum3(xs):
    k = _env("NCH", 1)
    return functools.reduce(jnp.add, [functools.reduce(jnp.add, xs[i::k]) for i in range(k)])


def _env(name, default):
    return type(default)(os.environ.get(name, default))


def _kernel(xm_ref, xt_ref, xb_ref, dw_ref, wqkv_ref, wo_ref, o_ref,
            x0_ref, ob_ref, dws_ref, ws_ref, wos_ref, qkv_ref, t_ref, stg_ref, ms_ref, *, W, nwin, nstrip):
    k_ = pl.program_id(0)
    dyn0 = jnp.minimum(k_, 0)

    def rows_at(base, off, n):
        if isinstance(base, int):
            return pl.ds(base + off, n)
        return pl.ds(pl.multiple_of(base + off, 8), n)

    mk = {}

    def new_masks():
        lane = lax.broadcasted_iota(jnp.int32, (8, LANES), 1)
        sub = lax.broadcasted_iota(jnp.int32, (8, LANES), 0)
        nlast = W - (WP - LANES)
        key_ok = sub < WS
        mk.update(
            last=lane < nlast,
            top=lane < jnp.where(k_ > 0, LANES, 0), top_last=lane < jnp.where(k_ > 0, nlast, 0),
            bot=lane < jnp.where(k_ < nstrip - 1, LANES, 0),
            bot_last=lane < jnp.where(k_ < nstrip - 1, nlast, 0),
            never=lane < dyn0, lo=lane < 80, hi=lane >= 80, v=lane < 32, key=key_ok,
            left=lane < SLOTS, keep_a=key_ok & (lane < SLOTS), keep_b=key_ok & (lane >= SLOTS),
            left64=lane < 64)

    nxt = (k_ % 3) * X0_SLOT
    prv = ((k_ + 1) % 3) * X0_SLOT

    def conv_group(c0):
        st = {}

        def row(i):
            if i not in st:
                if i == 0:
                    v, m, ml = xt_ref[0, c0:c0 + 8, :], mk["top"], mk["top_last"]
                elif i == WS + 1:
                    v, m, ml = xb_ref[0, c0:c0 + 8, :], mk["bot"], mk["bot_last"]
                else:
                    v, m, ml = xm_ref[i - 1, c0:c0 + 8, :], None, mk["last"]
                v = v.astype(F32)
                ts = [v[:, t * LANES:(t + 1) * LANES] for t in range(NT)]
                ts = [t if m is None else jnp.where(m, t, 0.0) for t in ts[:-1]] + [jnp.where(ml, ts[-1], 0.0)]
                st[i] = jnp.concatenate(ts, axis=1)
            return st[i]

        def bc(v):
            return jnp.concatenate([v] * NT, axis=1)

        def taps(r):
            st["tw", r] = [bc(x0_ref[rows_at(c0, DW_OFF + k * C, 8), :]) for k in range(2)]

        def piece(r):
            if "w" not in st:
                st["w"] = [bc(dws_ref[k, pl.ds(c0, 8), :]) for k in range(9)]
            wts = list(st["w"])
            if ("tw", r) in st:
                wts[6], wts[8] = st["tw", r]
            abc = [row(r + 1) * wts[3 + j] + row(r) * wts[j] + row(r + 2) * wts[6 + j] for j in range(3)]
            x0 = pltpu.roll(abc[0], 1, 1) + abc[1] + pltpu.roll(abc[2], WP - 1, 1)
            for t in range(NT):
                x0_ref[rows_at(nxt, (r * NT + t) * C + c0, 8), :] = x0[:, t * LANES:(t + 1) * LANES]

        return taps, piece

    @pl.when(k_ == 0)
    def _():
        for k in range(9):
            w = dw_ref[k // 3].astype(F32)[k % 3:k % 3 + 1, :]
            w = jnp.broadcast_to(w, (LANES, C)).T
            dws_ref[k] = w + 1.0 if k == 4 else w
            if k in (6, 8):
                x0_ref[pl.ds(DW_OFF + (k - 6) // 2 * C, C), :] = w
        w = wqkv_ref[...].astype(F32)
        wq = w[:, 0:C] * ((DH ** -0.5) * math.log2(math.e))
        wk, wv = w[:, C:2 * C], w[:, 2 * C:3 * C]
        z32 = jnp.zeros((C, 32), F32)
        tiles = [(wv[:, 128:160], wq[:, 0:96]),
                 (wq[:, 96:128], wv[:, 160:192], wq[:, 128:192]),
                 (z32, wk[:, 0:96]),
                 (wk[:, 96:128], z32, wk[:, 128:192]),
                 (wv[:, 0:128],)]
        for n, parts in enumerate(tiles):
            w = jnp.concatenate(parts, axis=1)
            for i, wi in enumerate((w[0:128], w[64:192], _cat([w[128:192], w[0:64]]))):
                ws_ref[i, n] = pltpu.bitcast(wi.astype(BF16), U32)
        w = wo_ref[...].astype(F32)
        wx, wy, wz = w[0:64], w[64:128], w[128:192]
        for i, parts in enumerate(((wx, wy), (wz, wy), (wx, wz))):
            wos_ref[i] = pltpu.bitcast(_cat(parts).T.astype(BF16), U32)

        def zero(i, carry):
            x0_ref[pl.ds(pl.multiple_of(X0_SLOT + i * 1536, 8), 1536), :] = jnp.zeros((1536, LANES), F32)
            ob_ref[pl.ds(pl.multiple_of(i * WP, 8), WP), :] = jnp.zeros((WP, LANES), F32)
            for j in range(2):
                t_ref[2 * i + j] = jnp.zeros(t_ref.shape[1:], U32)
            for j in range(6):
                stg_ref[6 * i + j] = jnp.zeros(stg_ref.shape[1:], F32)
            return carry
        lax.fori_loop(0, WS, zero, 0)

    groups = [conv_group(8 * g) for g in range(NG)]
    WLEAD = _env("WLEAD", 5)

    def conv_items(gs):
        plist = [(g, r) for g in gs for r in range(WS)]
        items = []
        for k, (g, r) in enumerate(plist):
            fs = []
            if k + WLEAD < len(plist):
                g2, r2 = plist[k + WLEAD]
                fs.append(functools.partial(groups[g2][0], r2))
            fs.append(functools.partial(groups[g][1], r))
            items.append(fs)
        return items

    LNP = _env("LNP", 3)
    tokens = {}

    NST = _env("NST", 0)

    def ld_x0(j, k):
        return [x0_ref[rows_at(nxt + dyn0 * (8 * k), j * C + 8 * g, 8), :] for g in range(NG)]

    def ln_stats(j, gates):
        xs = ld_x0(j, 0)
        for g in gates:
            for i in range(_env("NCH", 1)):
                xs[i] = jnp.where(mk["never"], g, xs[i])
        m = _allred(_sum3(xs), jnp.add) * (1.0 / C)
        if LNP == 2:
            v = _allred(_sum3([x * x for x in xs]), jnp.add) * (1.0 / C)
            v = jnp.maximum(v - m * m, 0.0)
        else:
            d = [x - m for x in ld_x0(j, 1)]
            v = _allred(_sum3([x * x for x in d]), jnp.add) * (1.0 / C)
            tokens["d"] = d
        rs = lax.rsqrt(v + EPS)
        if isinstance(j, int):
            tokens["rs", j] = rs
        return m, rs

    def early_stats(j):
        k = j - _env("CHS", 100)
        m, rs = ln_stats(j, [tokens["rs", k]] if ("rs", k) in tokens else [])
        ms_ref[j] = _cat([m, rs])

    def layernorm_tile(r, t, gates):
        j = r * NT + t
        if j < NST:
            m, rs = ms_ref[j, 0:8, :], ms_ref[j, 8:16, :]
            for g in gates:
                m = jnp.where(mk["never"], g, m)
        else:
            m, rs = ln_stats(j, gates)
            if LNP == 4:
                return _cat([x * rs for x in tokens["d"]])
        return _cat([(x - m) * rs for x in ld_x0(j, 2)])

    def ln_prep(u):
        r, tp = divmod(u, 2)
        hs = []
        for j in range(2):
            gates = []
            k = 2 * u + j - _env("CH1", 2)
            if _env("CH1", 2) and ("rs", k) in tokens:
                gates.append(tokens["rs", k])
            k = u - _env("CH2", 4)
            if _env("CH2", 4) and k in tokens:
                gates += [pltpu.bitcast(x, F32) for x in (tokens[k][0:2] if j == 0 else tokens[k][2:3])]
            hs.append(layernorm_tile(r, 2 * tp + j, gates))
        ha, hb = hs
        ts = [_cat([ha[0:64] - hb[0:64], ha[64:128]]),
              _cat([hb[64:128], hb[128:192] - ha[128:192]]),
              _cat([ha[128:192], hb[0:64]])]
        toks = []
        for i, t in enumerate(ts):
            t = pltpu.bitcast(t.astype(BF16).T, U32)
            t_ref[u, i] = t
            toks.append(t[56:64])
        tokens[u] = toks

    def qkv_chunk(u, n, after=None):
        r, tp = divmod(u, 2)
        p = {}
        for i in (2, 0, 1):
            lhs = t_ref[u, i]
            if after is not None:
                lhs = _cat([jnp.where(mk["never"], tokens[after][i], lhs[0:8]), lhs[8:]])
            p[i] = _dot(pltpu.bitcast(lhs, BF16), pltpu.bitcast(ws_ref[i, n], BF16))
        if _env("BLK", 0):
            for i in range(0, LANES, 8):
                for j in range(2):
                    qkv_ref[n, r, pl.ds((2 * tp + j) * LANES + i, 8), :] = p[j][i:i + 8] + p[2][i:i + 8]
            return
        for j in range(2):
            qkv_ref[n, r, pl.ds((2 * tp + j) * LANES, LANES), :] = p[j] + p[2]

    zero8 = jnp.zeros((8, LANES), F32)

    def gather(n, off):
        return [qkv_ref[n, r, pl.ds(off, 8), :] for r in range(WS)]

    def softmax_t(st):
        rows = _blocks(st)
        m = functools.reduce(jnp.maximum, rows)
        m = _allred(jnp.where(mk["key"], m, -jnp.inf), jnp.maximum)
        p = [jnp.exp2(x - m) for x in rows]
        return p, functools.reduce(jnp.add, p)

    def s2_pair(pi, offa):
        offb = offa + WS
        st = {}

        def vprep():
            u1 = _cat(gather(4, offa) + gather(4, offb) + [zero8, zero8])
            u2 = _cat([jnp.where(mk["v"], x, y) for x, y in
                       zip(gather(0, offa) + gather(0, offb), gather(1, offa) + gather(1, offb))]
                      + [zero8, zero8])
            VM = _env("VM", 0)
            if VM == 0:
                u1t = pltpu.bitcast(u1.astype(BF16).T, U32)
                u2t = pltpu.bitcast(u2[:, 0:64].astype(BF16).T, U32)
                vt = _cat([u1t, u2t])
            elif VM == 1:
                vt = _cat([pltpu.bitcast(u.astype(BF16).T, U32) for u in (u1, u2)])
            else:
                vt = pltpu.bitcast(jnp.concatenate([u1, u2], axis=1).astype(BF16).T, U32)
            st["vt"] = [pltpu.bitcast(vt[24 * h:24 * h + 24], BF16) for h in range(NH)]

        def score(i):
            hp, sw = divmod(i, 2)
            ma, mb = (mk["lo"], mk["hi"]) if sw == 0 else (mk["hi"], mk["lo"])
            q = _cat([jnp.where(ma, v, 0.0) for v in gather(hp, offa)]
                     + [jnp.where(mb, v, 0.0) for v in gather(hp, offb)] + [zero8, zero8])
            k = _cat([jnp.where(ma, x, y)
                      for x, y in zip(gather(2 + hp, offa), gather(2 + hp, offb))])
            st["p", i] = softmax_t(_dot_nt(k, q))

        def value(h):
            hp, sw = divmod(h, 2)
            (pa, sa), (pb, sb) = st["p", 2 * hp + sw], st["p", 2 * hp + 1 - sw]
            pm = _cat([jnp.where(mk["keep_a"], v, 0.0) for v in pa]
                      + [jnp.where(mk["keep_b"], v, 0.0) for v in pb] + [zero8, zero8])
            den = _allred(jnp.where(mk["key"], jnp.where(mk["left"], sa, sb), 0.0), jnp.add)
            rec = pl.reciprocal(den, approx=True)
            if _env("NR", 1):
                rec = rec * (2.0 - den * rec)
            st["o", h] = [b * rec for b in _blocks(_dot(st["vt"][h], pm))]

        def finish():
            o = [b for h in range(NH) for b in st["o", h]]
            w = pltpu.pack_elementwise([_cat(o[0:16]), _cat(o[16:24] + o[16:24])], packed_dtype=BF16)
            stg_ref[pi] = pltpu.bitcast(w, F32)

        def scatter():
            wt = stg_ref[pi].T
            for i, off in enumerate((offa, offb)):
                for r in range(WS):
                    base = i * SLOTS + 8 * r
                    ob_ref[pl.ds(r * WP + off, WS), :] = wt[base:base + WS]

        return vprep, score, value, finish, scatter

    npair = (nwin + 1) // 2
    pairs = [s2_pair(p, min(2 * p, nwin - 2) * WS) for p in range(npair)]

    def s3_unit(r, tp):
        def unpack(t):
            w = pltpu.bitcast(ob_ref[pl.ds(r * WP + t * LANES, LANES), :], U32)
            return [_blocks(pltpu.unpack_elementwise(w, index=i, packed_dtype=BF16, unpacked_dtype=F32))
                    for i in range(2)]

        (la, ha), (lb, hb) = unpack(2 * tp), unpack(2 * tp + 1)
        t3 = _cat([jnp.where(mk["left64"], x, y) for x, y in zip(lb, ha)])
        t1 = _cat([x - jnp.where(mk["left64"], y, 0.0) for x, y in zip(la, lb)])
        t2 = _cat([jnp.where(mk["left64"], x - y, z) for x, y, z in zip(hb, ha, lb)])
        p3 = _dot_nt(pltpu.bitcast(wos_ref[2], BF16), t3)
        ys = [_dot_nt(pltpu.bitcast(wos_ref[i], BF16), t) + p3
              + x0_ref[rows_at(prv, (r * NT + 2 * tp + i) * C, C), :] for i, t in enumerate((t1, t2))]
        o_ref[r, :, pl.ds(2 * tp * LANES, 2 * LANES)] = jnp.concatenate(ys, axis=1).astype(o_ref.dtype)

    s3_all = [functools.partial(s3_unit, r, tp) for r in range(WS) for tp in range(2)]

    LSM = _env("LSM", 240)
    LFIN = _env("LFIN", 200)
    PREP = _env("PREP", 600)
    SGRP = _env("SGRP", 4)
    VGRP = _env("VGRP", 2)
    TAILGAP = _env("TAILGAP", 800)

    def segment(units, pids, s3u, gs, lns, head, scat=()):
        tokens.clear()
        load = [0] * 4
        tm = [0] * 4
        prog, extra = [], []

        def emit(rows_list, fn, ready=0):
            prog.append((min(tm), fn))
            ends = []
            for rows in rows_list:
                m = load.index(min(load))
                load[m] += rows
                tm[m] = max(tm[m], ready) + rows
                ends.append(tm[m])
            return ends

        fillers = [([C] * 3, f) for f in s3u[:head]]
        chunks = [(u, n) for u in units for n in range(5)]
        late = [u for u in lns if u not in units]
        dl = {}
        if _env("DL", 0):
            c0 = _env("DL0", 3)
            for j, u in enumerate(late):
                k = c0 + j * (len(chunks) + _env("DLX", 0) - c0) // len(late)
                if k < len(chunks):
                    dl[k] = u
        fillers += [([LANES] * 3, functools.partial(qkv_chunk, u, n, dl.get(k)))
                    for k, (u, n) in enumerate(chunks)]
        fillers += [([C] * 3, f) for f in s3u[head:]]
        total = (sum(sum(f[0]) for f in fillers) + len(pids) * 4 * (SLOTS + DH)) / 4
        nsc = 4 * len(pids)
        next_s = 0
        s_end, v_end, pend_v = {}, {}, []
        while fillers or next_s < nsc or pend_v:
            now = tm[load.index(min(load))]
            s_ok = next_s < nsc and now >= (total - TAILGAP) * next_s / max(nsc - 4, 1)
            v_ok = len(pend_v) >= VGRP // 2 and all(now >= x[0] for x in pend_v[:VGRP // 2])
            if not fillers and not s_ok and not v_ok:
                if pend_v and (next_s >= nsc or len(pend_v) >= 4):
                    v_ok = True
                else:
                    s_ok = True
            if v_ok:
                for rdy, pv, hp in pend_v[:VGRP // 2]:
                    for h in (2 * hp, 2 * hp + 1):
                        v_end[pv, h] = emit([DH], functools.partial(pairs[pv][2], h), rdy)[0]
                    if hp == 1:
                        extra.append((max(v_end[pv, h] for h in range(NH)) + LFIN, [pairs[pv][3]]))
                pend_v = pend_v[VGRP // 2:]
            elif s_ok:
                for _ in range(SGRP):
                    p, i = pids[next_s // 4], next_s % 4
                    if i == 0:
                        prog.append((min(tm), pairs[p][0]))
                    s_end[p, i] = emit([SLOTS], functools.partial(pairs[p][1], i))[0]
                    if i % 2 == 1:
                        pend_v.append((max(s_end[p, i], s_end[p, i - 1]) + LSM, p, i // 2))
                    next_s += 1
            else:
                emit(*fillers.pop(0))
        ci = conv_items(gs)
        if ci:
            for j, p in enumerate(scat):
                ci[_env("SC0", 0) + 4 * j].insert(0, pairs[p][4])
            scat = ()
        for j, fs in enumerate(ci):
            extra.append(((j + 1) * max(tm) / len(ci), fs))
        if pids:
            for j in range(NST):
                extra.append((j * max(tm) / NST, [functools.partial(early_stats, j)]))
        for j, u in enumerate(lns):
            extra.append((-1, [functools.partial(ln_prep, u)]))
        for j, p in enumerate(scat):
            t0 = head * 3 * C / 4
            extra.append((t0 + j * _env("SCEND", 0.8) * (max(tm) - t0) / len(scat), [pairs[p][4]]))
        extra.sort(key=lambda e: e[0])
        j = 0
        for t0, fn in prog:
            while j < len(extra) and extra[j][0] <= t0:
                for f in extra[j][1]:
                    f()
                j += 1
            fn()
        for e in extra[j:]:
            for f in e[1]:
                f()

    NB = _env("NB", 4)
    NSC = _env("NSC", 16)
    HEAD = _env("HEAD", 3)
    blocks = [
        (0, functools.partial(segment, list(range(NB, NU)), [], [], list(range(NG)), [], 0,
                              list(range(NSC, npair)))),
        (1, functools.partial(segment, [], list(range(npair)), s3_all[HEAD:], [], [], 0)),
        (0, functools.partial(segment, list(range(NB)), [], s3_all[:HEAD], [], list(range(NU)), HEAD,
                              list(range(NSC)))),
    ]
    for k, (first, fn) in enumerate(blocks):
        if k == 2 and NST:
            @pl.when(k_ == 0)
            def _():
                def body(j, carry):
                    tokens.clear()
                    m, rs = ln_stats(j, [])
                    ms_ref[j] = _cat([m, rs])
                    return carry
                lax.fori_loop(0, NST, body, 0)
        if str(k) in _env("ONLY", "012"):
            new_masks()
            pl.when((k_ + dyn0 * k <= nstrip) & (k_ >= first))(fn)

    @pl.when(k_ == nstrip + 1)
    def _():
        new_masks()
        for p in range(NSC, npair):
            pairs[p][4]()
        for f in s3_all[:1 if "ONLY" in os.environ else NU]:
            f()


@jax.jit
def pallas_standalone__window_attn_davit__vision_kernel(
    x: jax.Array,
    dw_pe: jax.Array,
    w_qkv: jax.Array,
    w_o: jax.Array,
):
    B, H, W, Cx = x.shape
    assert B == 1 and Cx == C and H % WS == 0 and W % WS == 0 and WP - LANES < W < WP
    nstrip = H // WS
    nwin = W // WS

    xt = jnp.transpose(x[0], (0, 2, 1))

    nx = lambda s: jnp.minimum(s, nstrip - 1)
    kernel = functools.partial(_kernel, W=W, nwin=nwin, nstrip=nstrip)
    yt = pl.pallas_call(
        kernel,
        grid=(nstrip + 2,),
        in_specs=[
            pl.BlockSpec((WS, C, WP), lambda s: (nx(s), 0, 0)),
            pl.BlockSpec((1, C, WP), lambda s: (jnp.maximum(nx(s) * WS - 1, 0), 0, 0)),
            pl.BlockSpec((1, C, WP), lambda s: (jnp.minimum(nx(s) * WS + WS, H - 1), 0, 0)),
            pl.BlockSpec((3, 3, C), lambda s: (0, 0, 0)),
            pl.BlockSpec((C, 3 * C), lambda s: (0, 0)),
            pl.BlockSpec((C, C), lambda s: (0, 0)),
        ],
        out_specs=pl.BlockSpec((WS, C, WP), lambda s: (jnp.maximum(s - 2, 0), 0, 0)),
        out_shape=jax.ShapeDtypeStruct((H, C, W), x.dtype),
        scratch_shapes=[
            pltpu.VMEM((X0_ROWS, LANES), F32),
            pltpu.VMEM((WS * WP, LANES), F32),
            pltpu.VMEM((9, C, LANES), F32),
            pltpu.VMEM((3, 5, LANES // 2, LANES), U32),
            pltpu.VMEM((3, C // 2, LANES), U32),
            pltpu.VMEM((5, WS, WP, LANES), F32),
            pltpu.VMEM((NU, 3, LANES // 2, LANES), U32),
            pltpu.VMEM((42, LANES, LANES), F32),
            pltpu.VMEM((WS * NT, 16, LANES), F32),
        ],
        compiler_params=pltpu.CompilerParams(
            dimension_semantics=("arbitrary",),
            vmem_limit_bytes=64 * 1024 * 1024,
        ),
        name="davit_window_attn",
    )(xt, xt, xt, dw_pe, w_qkv, w_o)
    return jnp.transpose(yt, (0, 2, 1))[None]
```

```python
import functools
import math
import os

import jax
import jax.numpy as jnp
from jax import lax
import jax.experimental.pallas as pl
import jax.experimental.pallas.tpu as pltpu

WS = 7
NH = 4
C = 192
DH = C // NH
NG = C // 8
LANES = 128
WP = 512
NT = WP // LANES
NU = WS * NT // 2
SLOTS = 8 * WS
EPS = 1e-5
F32 = jnp.float32
BF16 = jnp.bfloat16
U32 = jnp.uint32

X0_SLOT = WS * NT * C
DW_OFF = 3 * X0_SLOT
X0_ROWS = DW_OFF + 2 * C


def _dot(a, b):
    return jnp.dot(a, b, preferred_element_type=F32)


def _dot_nt(a, b):
    return lax.dot_general(a, b, (((1,), (1,)), ((), ())), preferred_element_type=F32)


def _cat(xs):
    return jnp.concatenate(xs, axis=0)


def _blocks(v):
    return [v[i:i + 8] for i in range(0, v.shape[0], 8)]


def _allred(x, op):
    for sh in (4, 2, 1):
        x = op(x, pltpu.roll(x, sh, 0))
    return x


def _sum3(xs):
    k = _env("NCH", 1)
    return functools.reduce(jnp.add, [functools.reduce(jnp.add, xs[i::k]) for i in range(k)])


def _env(name, default):
    return type(default)(os.environ.get(name, default))


def _kernel(xm_ref, xb_ref, dw_ref, wqkv_ref, wo_ref, o_ref,
            x0_ref, ob_ref, dws_ref, ws_ref, wos_ref, qkv_ref, t_ref, stg_ref, ms_ref, top_ref, *, W, nwin, nstrip):
    k_ = pl.program_id(0)
    dyn0 = jnp.minimum(k_, 0)

    def rows_at(base, off, n):
        if isinstance(base, int):
            return pl.ds(base + off, n)
        return pl.ds(pl.multiple_of(base + off, 8), n)

    mk = {}

    def new_masks():
        lane = lax.broadcasted_iota(jnp.int32, (8, LANES), 1)
        sub = lax.broadcasted_iota(jnp.int32, (8, LANES), 0)
        nlast = W - (WP - LANES)
        key_ok = sub < WS
        mk.update(
            last=lane < nlast,
            bot=lane < jnp.where(k_ < nstrip - 1, LANES, 0),
            bot_last=lane < jnp.where(k_ < nstrip - 1, nlast, 0),
            never=lane < dyn0, lo=lane < 80, hi=lane >= 80, v=lane < 32, key=key_ok,
            left=lane < SLOTS, keep_a=key_ok & (lane < SLOTS), keep_b=key_ok & (lane >= SLOTS),
            left64=lane < 64)

    k3 = k_ - 3 * ((k_ * 171) >> 9)
    nxt = k3 * X0_SLOT
    prv = jnp.where(k3 == 2, 0, nxt + X0_SLOT)

    def conv_group(c0):
        st = {}

        def row(i):
            if i == 0 and i not in st:
                st[i] = top_ref[c0:c0 + 8, :]
            if i not in st:
                if i == WS + 1:
                    v, m, ml = xb_ref[0, c0:c0 + 8, :], mk["bot"], mk["bot_last"]
                else:
                    v, m, ml = xm_ref[i - 1, c0:c0 + 8, :], None, mk["last"]
                v = v.astype(F32)
                ts = [v[:, t * LANES:(t + 1) * LANES] for t in range(NT)]
                ts = [t if m is None else jnp.where(m, t, 0.0) for t in ts[:-1]] + [jnp.where(ml, ts[-1], 0.0)]
                st[i] = jnp.concatenate(ts, axis=1)
                if i == WS:
                    top_ref[c0:c0 + 8, :] = st[i]
            return st[i]

        def bc(v):
            return jnp.concatenate([v] * NT, axis=1)

        def taps(r):
            st["tw", r] = [bc(x0_ref[rows_at(c0, DW_OFF + k * C, 8), :]) for k in range(2)]

        def piece(r):
            if "w" not in st:
                st["w"] = [bc(dws_ref[k, pl.ds(c0, 8), :]) for k in range(9)]
            wts = list(st["w"])
            if ("tw", r) in st:
                wts[6], wts[8] = st["tw", r]
            abc = [row(r + 1) * wts[3 + j] + row(r) * wts[j] + row(r + 2) * wts[6 + j] for j in range(3)]
            x0 = pltpu.roll(abc[0], 1, 1) + abc[1] + pltpu.roll(abc[2], WP - 1, 1)
            for t in range(NT):
                x0_ref[rows_at(nxt, (r * NT + t) * C + c0, 8), :] = x0[:, t * LANES:(t + 1) * LANES]

        return taps, piece

    @pl.when(k_ == 0)
    def _():
        for k in range(9):
            w = dw_ref[k // 3].astype(F32)[k % 3:k % 3 + 1, :]
            w = jnp.broadcast_to(w, (LANES, C)).T
            dws_ref[k] = w + 1.0 if k == 4 else w
            if k in (6, 8):
                x0_ref[pl.ds(DW_OFF + (k - 6) // 2 * C, C), :] = w
        w = wqkv_ref[...].astype(F32)
        wq = w[:, 0:C] * ((DH ** -0.5) * math.log2(math.e))
        wk, wv = w[:, C:2 * C], w[:, 2 * C:3 * C]
        z32 = jnp.zeros((C, 32), F32)
        tiles = [(wv[:, 128:160], wq[:, 0:96]),
                 (wq[:, 96:128], wv[:, 160:192], wq[:, 128:192]),
                 (z32, wk[:, 0:96]),
                 (wk[:, 96:128], z32, wk[:, 128:192]),
                 (wv[:, 0:128],)]
        for n, parts in enumerate(tiles):
            w = jnp.concatenate(parts, axis=1)
            for i, wi in enumerate((w[0:128], w[64:192], _cat([w[128:192], w[0:64]]))):
                ws_ref[i, n] = pltpu.bitcast(wi.astype(BF16), U32)
        w = wo_ref[...].astype(F32)
        wx, wy, wz = w[0:64], w[64:128], w[128:192]
        for i, parts in enumerate(((wx, wy), (wz, wy), (wx, wz))):
            wos_ref[i] = pltpu.bitcast(_cat(parts).T.astype(BF16), U32)

        top_ref[...] = jnp.zeros(top_ref.shape, F32)

        def zero(i, carry):
            x0_ref[pl.ds(pl.multiple_of(X0_SLOT + i * 1536, 8), 1536), :] = jnp.zeros((1536, LANES), F32)
            ob_ref[pl.ds(pl.multiple_of(i * WP, 8), WP), :] = jnp.zeros((WP, LANES), F32)
            for j in range(2):
                t_ref[2 * i + j] = jnp.zeros(t_ref.shape[1:], U32)
            for j in range(6):
                stg_ref[6 * i + j] = jnp.zeros(stg_ref.shape[1:], F32)
            return carry
        lax.fori_loop(0, WS, zero, 0)

    groups = [conv_group(8 * g) for g in range(NG)]
    WLEAD = _env("WLEAD", 5)

    def conv_items(gs):
        plist = [(g, r) for g in gs for r in range(WS)]
        items = []
        for k, (g, r) in enumerate(plist):
            fs = []
            if k + WLEAD < len(plist):
                g2, r2 = plist[k + WLEAD]
                fs.append(functools.partial(groups[g2][0], r2))
            fs.append(functools.partial(groups[g][1], r))
            items.append(fs)
        return items

    LNP = _env("LNP", 3)
    tokens = {}

    NST = _env("NST", 0)

    def ld_x0(j, k):
        return [x0_ref[rows_at(nxt + dyn0 * (8 * k), j * C + 8 * g, 8), :] for g in range(NG)]

    def ln_stats(j, gates):
        xs = ld_x0(j, 0)
        for g in gates:
            for i in range(_env("NCH", 1)):
                xs[i] = jnp.where(mk["never"], g, xs[i])
        m = _allred(_sum3(xs), jnp.add) * (1.0 / C)
        if LNP == 2:
            v = _allred(_sum3([x * x for x in xs]), jnp.add) * (1.0 / C)
            v = jnp.maximum(v - m * m, 0.0)
        else:
            d = [x - m for x in ld_x0(j, 1)]
            v = _allred(_sum3([x * x for x in d]), jnp.add) * (1.0 / C)
            tokens["d"] = d
        rs = lax.rsqrt(v + EPS)
        if isinstance(j, int):
            tokens["rs", j] = rs
        return m, rs

    def early_stats(j):
        k = j - _env("CHS", 100)
        m, rs = ln_stats(j, [tokens["rs", k]] if ("rs", k) in tokens else [])
        ms_ref[j] = _cat([m, rs])

    def layernorm_tile(r, t, gates):
        j = r * NT + t
        if j < NST:
            m, rs = ms_ref[j, 0:8, :], ms_ref[j, 8:16, :]
            for g in gates:
                m = jnp.where(mk["never"], g, m)
        else:
            m, rs = ln_stats(j, gates)
            if LNP == 4:
                return _cat([x * rs for x in tokens["d"]])
        return _cat([(x - m) * rs for x in ld_x0(j, 2)])

    def ln_prep(u):
        r, tp = divmod(u, 2)
        hs = []
        for j in range(2):
            gates = []
            k = 2 * u + j - _env("CH1", 2)
            if _env("CH1", 2) and ("rs", k) in tokens:
                gates.append(tokens["rs", k])
            k = u - _env("CH2", 4)
            if _env("CH2", 4) and k in tokens:
                gates += [pltpu.bitcast(x, F32) for x in (tokens[k][0:2] if j == 0 else tokens[k][2:3])]
            hs.append(layernorm_tile(r, 2 * tp + j, gates))
        ha, hb = hs
        ts = [_cat([ha[0:64] - hb[0:64], ha[64:128]]),
              _cat([hb[64:128], hb[128:192] - ha[128:192]]),
              _cat([ha[128:192], hb[0:64]])]
        toks = []
        for i, t in enumerate(ts):
            t = pltpu.bitcast(t.astype(BF16).T, U32)
            t_ref[u, i] = t
            toks.append(t[56:64])
        tokens[u] = toks

    def qkv_chunk(u, n, after=None):
        r, tp = divmod(u, 2)
        p = {}
        for i in (2, 0, 1):
            lhs = t_ref[u, i]
            if after is not None:
                lhs = _cat([jnp.where(mk["never"], tokens[after][i], lhs[0:8]), lhs[8:]])
            p[i] = _dot(pltpu.bitcast(lhs, BF16), pltpu.bitcast(ws_ref[i, n], BF16))
        if _env("BLK", 0):
            for i in range(0, LANES, 8):
                for j in range(2):
                    qkv_ref[n, r, pl.ds((2 * tp + j) * LANES + i, 8), :] = p[j][i:i + 8] + p[2][i:i + 8]
            return
        for j in range(2):
            qkv_ref[n, r, pl.ds((2 * tp + j) * LANES, LANES), :] = p[j] + p[2]

    zero8 = jnp.zeros((8, LANES), F32)

    def gather(n, off):
        return [qkv_ref[n, r, pl.ds(off, 8), :] for r in range(WS)]

    def softmax_t(st):
        rows = _blocks(st)
        m = functools.reduce(jnp.maximum, rows)
        m = _allred(jnp.where(mk["key"], m, -jnp.inf), jnp.maximum)
        p = [jnp.exp2(x - m) for x in rows]
        return p, functools.reduce(jnp.add, p)

    def s2_pair(pi, offa):
        offb = offa + WS
        st = {}

        def vprep():
            u1 = _cat(gather(4, offa) + gather(4, offb) + [zero8, zero8])
            u2 = _cat([jnp.where(mk["v"], x, y) for x, y in
                       zip(gather(0, offa) + gather(0, offb), gather(1, offa) + gather(1, offb))]
                      + [zero8, zero8])
            VM = _env("VM", 0)
            if VM == 0:
                u1t = pltpu.bitcast(u1.astype(BF16).T, U32)
                u2t = pltpu.bitcast(u2[:, 0:64].astype(BF16).T, U32)
                vt = _cat([u1t, u2t])
            elif VM == 1:
                vt = _cat([pltpu.bitcast(u.astype(BF16).T, U32) for u in (u1, u2)])
            else:
                vt = pltpu.bitcast(jnp.concatenate([u1, u2], axis=1).astype(BF16).T, U32)
            st["vt"] = [pltpu.bitcast(vt[24 * h:24 * h + 24], BF16) for h in range(NH)]

        def score(i):
            hp, sw = divmod(i, 2)
            ma, mb = (mk["lo"], mk["hi"]) if sw == 0 else (mk["hi"], mk["lo"])
            q = _cat([jnp.where(ma, v, 0.0) for v in gather(hp, offa)]
                     + [jnp.where(mb, v, 0.0) for v in gather(hp, offb)] + [zero8, zero8])
            k = _cat([jnp.where(ma, x, y)
                      for x, y in zip(gather(2 + hp, offa), gather(2 + hp, offb))])
            st["p", i] = softmax_t(_dot_nt(k, q))

        def value(h):
            hp, sw = divmod(h, 2)
            (pa, sa), (pb, sb) = st["p", 2 * hp + sw], st["p", 2 * hp + 1 - sw]
            pm = _cat([jnp.where(mk["keep_a"], v, 0.0) for v in pa]
                      + [jnp.where(mk["keep_b"], v, 0.0) for v in pb] + [zero8, zero8])
            den = _allred(jnp.where(mk["key"], jnp.where(mk["left"], sa, sb), 0.0), jnp.add)
            rec = pl.reciprocal(den, approx=True)
            if _env("NR", 1):
                rec = rec * (2.0 - den * rec)
            st["o", h] = [b * rec for b in _blocks(_dot(st["vt"][h], pm))]

        def finish():
            o = [b for h in range(NH) for b in st["o", h]]
            w = pltpu.pack_elementwise([_cat(o[0:16]), _cat(o[16:24] + o[16:24])], packed_dtype=BF16)
            stg_ref[pi] = pltpu.bitcast(w, F32)

        def scatter():
            wt = stg_ref[pi].T
            for i, off in enumerate((offa, offb)):
                for r in range(WS):
                    base = i * SLOTS + 8 * r
                    ob_ref[pl.ds(r * WP + off, WS), :] = wt[base:base + WS]

        return vprep, score, value, finish, scatter

    npair = (nwin + 1) // 2
    pairs = [s2_pair(p, min(2 * p, nwin - 2) * WS) for p in range(npair)]

    def s3_unit(r, tp):
        def unpack(t):
            w = pltpu.bitcast(ob_ref[pl.ds(r * WP + t * LANES, LANES), :], U32)
            return [_blocks(pltpu.unpack_elementwise(w, index=i, packed_dtype=BF16, unpacked_dtype=F32))
                    for i in range(2)]

        (la, ha), (lb, hb) = unpack(2 * tp), unpack(2 * tp + 1)
        t3 = _cat([jnp.where(mk["left64"], x, y) for x, y in zip(lb, ha)])
        t1 = _cat([x - jnp.where(mk["left64"], y, 0.0) for x, y in zip(la, lb)])
        t2 = _cat([jnp.where(mk["left64"], x - y, z) for x, y, z in zip(hb, ha, lb)])
        p3 = _dot_nt(pltpu.bitcast(wos_ref[2], BF16), t3)
        ys = [_dot_nt(pltpu.bitcast(wos_ref[i], BF16), t) + p3
              + x0_ref[rows_at(prv, (r * NT + 2 * tp + i) * C, C), :] for i, t in enumerate((t1, t2))]
        o_ref[r, :, pl.ds(2 * tp * LANES, 2 * LANES)] = jnp.concatenate(ys, axis=1).astype(o_ref.dtype)

    s3_all = [functools.partial(s3_unit, r, tp) for r in range(WS) for tp in range(2)]

    LSM = _env("LSM", 240)
    LFIN = _env("LFIN", 200)
    PREP = _env("PREP", 600)
    SGRP = _env("SGRP", 4)
    VGRP = _env("VGRP", 2)
    TAILGAP = _env("TAILGAP", 800)

    def segment(units, pids, s3u, gs, lns, head, scat=()):
        tokens.clear()
        load = [0] * 4
        tm = [0] * 4
        prog, extra = [], []

        def emit(rows_list, fn, ready=0):
            prog.append((min(tm), fn))
            ends = []
            for rows in rows_list:
                m = load.index(min(load))
                load[m] += rows
                tm[m] = max(tm[m], ready) + rows
                ends.append(tm[m])
            return ends

        fillers = [([C] * 3, f) for f in s3u[:head]]
        chunks = [(u, n) for u in units for n in range(5)]
        late = [u for u in lns if u not in units]
        dl = {}
        if _env("DL", 0):
            c0 = _env("DL0", 3)
            for j, u in enumerate(late):
                k = c0 + j * (len(chunks) + _env("DLX", 0) - c0) // len(late)
                if k < len(chunks):
                    dl[k] = u
        fillers += [([LANES] * 3, functools.partial(qkv_chunk, u, n, dl.get(k)))
                    for k, (u, n) in enumerate(chunks)]
        fillers += [([C] * 3, f) for f in s3u[head:]]
        total = (sum(sum(f[0]) for f in fillers) + len(pids) * 4 * (SLOTS + DH)) / 4
        nsc = 4 * len(pids)
        next_s = 0
        s_end, v_end, pend_v = {}, {}, []
        while fillers or next_s < nsc or pend_v:
            now = tm[load.index(min(load))]
            s_ok = next_s < nsc and now >= (total - TAILGAP) * next_s / max(nsc - 4, 1)
            v_ok = len(pend_v) >= VGRP // 2 and all(now >= x[0] for x in pend_v[:VGRP // 2])
            if not fillers and not s_ok and not v_ok:
                if pend_v and (next_s >= nsc or len(pend_v) >= 4):
                    v_ok = True
                else:
                    s_ok = True
            if v_ok:
                for rdy, pv, hp in pend_v[:VGRP // 2]:
                    for h in (2 * hp, 2 * hp + 1):
                        v_end[pv, h] = emit([DH], functools.partial(pairs[pv][2], h), rdy)[0]
                    if hp == 1:
                        extra.append((max(v_end[pv, h] for h in range(NH)) + LFIN, [pairs[pv][3]]))
                pend_v = pend_v[VGRP // 2:]
            elif s_ok:
                for _ in range(SGRP):
                    p, i = pids[next_s // 4], next_s % 4
                    if i == 0:
                        prog.append((min(tm), pairs[p][0]))
                    s_end[p, i] = emit([SLOTS], functools.partial(pairs[p][1], i))[0]
                    if i % 2 == 1:
                        pend_v.append((max(s_end[p, i], s_end[p, i - 1]) + LSM, p, i // 2))
                    next_s += 1
            else:
                emit(*fillers.pop(0))
        ci = conv_items(gs)
        if ci:
            for j, p in enumerate(scat):
                ci[_env("SC0", 0) + 4 * j].insert(0, pairs[p][4])
            scat = ()
        for j, fs in enumerate(ci):
            extra.append(((j + 1) * max(tm) / len(ci), fs))
        if pids:
            for j in range(NST):
                extra.append((j * max(tm) / NST, [functools.partial(early_stats, j)]))
        for j, u in enumerate(lns):
            extra.append((-1, [functools.partial(ln_prep, u)]))
        for j, p in enumerate(scat):
            t0 = head * 3 * C / 4
            extra.append((t0 + j * _env("SCEND", 0.8) * (max(tm) - t0) / len(scat), [pairs[p][4]]))
        extra.sort(key=lambda e: e[0])
        j = 0
        for t0, fn in prog:
            while j < len(extra) and extra[j][0] <= t0:
                for f in extra[j][1]:
                    f()
                j += 1
            fn()
        for e in extra[j:]:
            for f in e[1]:
                f()

    NB = _env("NB", 4)
    NSC = _env("NSC", 16)
    HEAD = _env("HEAD", 3)
    blocks = [
        (0, functools.partial(segment, list(range(NB, NU)), [], [], list(range(NG)), [], 0,
                              list(range(NSC, npair)))),
        (1, functools.partial(segment, [], list(range(npair)), s3_all[HEAD:], [], [], 0)),
        (0, functools.partial(segment, list(range(NB)), [], s3_all[:HEAD], [], list(range(NU)), HEAD,
                              list(range(NSC)))),
    ]
    for k, (first, fn) in enumerate(blocks):
        if k == 2 and NST:
            @pl.when(k_ == 0)
            def _():
                def body(j, carry):
                    tokens.clear()
                    m, rs = ln_stats(j, [])
                    ms_ref[j] = _cat([m, rs])
                    return carry
                lax.fori_loop(0, NST, body, 0)
        if str(k) in _env("ONLY", "012"):
            new_masks()
            pl.when((k_ + dyn0 * k <= nstrip) & (k_ >= first))(fn)

    @pl.when(k_ == nstrip + 1)
    def _():
        new_masks()
        for p in range(NSC, npair):
            pairs[p][4]()
        for f in s3_all[:1 if "ONLY" in os.environ else NU]:
            f()


@jax.jit
def pallas_standalone__window_attn_davit__vision_kernel(
    x: jax.Array,
    dw_pe: jax.Array,
    w_qkv: jax.Array,
    w_o: jax.Array,
):
    B, H, W, Cx = x.shape
    assert B == 1 and Cx == C and H % WS == 0 and W % WS == 0 and WP - LANES < W < WP
    nstrip = H // WS
    nwin = W // WS

    xt = jnp.transpose(x[0], (0, 2, 1))

    assert nstrip + 2 <= 256
    kernel = functools.partial(_kernel, W=W, nwin=nwin, nstrip=nstrip)
    yt = pl.pallas_call(
        kernel,
        grid=(nstrip + 2,),
        in_specs=[
            pl.BlockSpec((WS, C, WP), lambda s: (jnp.minimum(s, nstrip - 1), 0, 0)),
            pl.BlockSpec((1, C, WP), lambda s: (jnp.minimum(s * WS + WS, H - 1), 0, 0)),
            pl.BlockSpec((3, 3, C), lambda s: (0, 0, 0)),
            pl.BlockSpec((C, 3 * C), lambda s: (0, 0)),
            pl.BlockSpec((C, C), lambda s: (0, 0)),
        ],
        out_specs=pl.BlockSpec((WS, C, WP), lambda s: (jnp.maximum(s - 2, 0), 0, 0)),
        out_shape=jax.ShapeDtypeStruct((H, C, W), x.dtype),
        scratch_shapes=[
            pltpu.VMEM((X0_ROWS, LANES), F32),
            pltpu.VMEM((WS * WP, LANES), F32),
            pltpu.VMEM((9, C, LANES), F32),
            pltpu.VMEM((3, 5, LANES // 2, LANES), U32),
            pltpu.VMEM((3, C // 2, LANES), U32),
            pltpu.VMEM((5, WS, WP, LANES), F32),
            pltpu.VMEM((NU, 3, LANES // 2, LANES), U32),
            pltpu.VMEM((42, LANES, LANES), F32),
            pltpu.VMEM((WS * NT, 16, LANES), F32),
            pltpu.VMEM((C, WP), F32),
        ],
        compiler_params=pltpu.CompilerParams(
            dimension_semantics=("arbitrary",),
            vmem_limit_bytes=64 * 1024 * 1024,
            disable_bounds_checks=bool(_env("NOBC", 1)),
        ),
        name="davit_window_attn",
    )(xt, xt, dw_pe, w_qkv, w_o)
    return jnp.transpose(yt, (0, 2, 1))[None]
```

```python
import functools
import math
import os

import jax
import jax.numpy as jnp
from jax import lax
import jax.experimental.pallas as pl
import jax.experimental.pallas.tpu as pltpu

WS = 7
NH = 4
C = 192
DH = C // NH
NG = C // 8
LANES = 128
WP = 512
NT = WP // LANES
NU = WS * NT // 2
SLOTS = 8 * WS
EPS = 1e-5
F32 = jnp.float32
BF16 = jnp.bfloat16
U32 = jnp.uint32

X0_SLOT = WS * NT * C
DW_OFF = 3 * X0_SLOT
X0_ROWS = DW_OFF + 2 * C


def _dot(a, b):
    return jnp.dot(a, b, preferred_element_type=F32)


def _dot_nt(a, b):
    return lax.dot_general(a, b, (((1,), (1,)), ((), ())), preferred_element_type=F32)


def _cat(xs):
    return jnp.concatenate(xs, axis=0)


def _blocks(v):
    return [v[i:i + 8] for i in range(0, v.shape[0], 8)]


def _allred(x, op):
    for sh in (4, 2, 1):
        x = op(x, pltpu.roll(x, sh, 0))
    return x


def _env(name, default):
    return type(default)(os.environ.get(name, default))


def _kernel(xm_ref, xb_ref, dw_ref, wqkv_ref, wo_ref, o_ref,
            x0_ref, ob_ref, dws_ref, ws_ref, wos_ref, qkv_ref, t_ref, stg_ref, ms_ref, top_ref, *, W, nwin, nstrip):
    k_ = pl.program_id(0)
    dyn0 = jnp.minimum(k_, 0)

    def rows_at(base, off, n):
        if isinstance(base, int):
            return pl.ds(base + off, n)
        return pl.ds(pl.multiple_of(base + off, 8), n)

    mk = {}

    def new_masks():
        lane = lax.broadcasted_iota(jnp.int32, (8, LANES), 1)
        sub = lax.broadcasted_iota(jnp.int32, (8, LANES), 0)
        nlast = W - (WP - LANES)
        key_ok = sub < WS
        mk.update(
            last=lane < nlast,
            bot=lane < jnp.where(k_ < nstrip - 1, LANES, 0),
            bot_last=lane < jnp.where(k_ < nstrip - 1, nlast, 0),
            never=lane < dyn0, lo=lane < 80, hi=lane >= 80, v=lane < 32, key=key_ok,
            left=lane < SLOTS, keep_a=key_ok & (lane < SLOTS), keep_b=key_ok & (lane >= SLOTS),
            left64=lane < 64)

    k3 = k_ - 3 * ((k_ * 171) >> 9)
    nxt = k3 * X0_SLOT
    prv = jnp.where((k3 == 2) | (k_ < 2), 0, nxt + X0_SLOT)

    def conv_group(c0):
        st = {}

        def row(i):
            if i == 0 and i not in st:
                st[i] = top_ref[c0:c0 + 8, :]
            if i not in st:
                if i == WS + 1:
                    v, m, ml = xb_ref[0, c0:c0 + 8, :], mk["bot"], mk["bot_last"]
                else:
                    v, m, ml = xm_ref[i - 1, c0:c0 + 8, :], None, mk["last"]
                v = v.astype(F32)
                ts = [v[:, t * LANES:(t + 1) * LANES] for t in range(NT)]
                ts = [t if m is None else jnp.where(m, t, 0.0) for t in ts[:-1]] + [jnp.where(ml, ts[-1], 0.0)]
                st[i] = jnp.concatenate(ts, axis=1)
                if i == WS:
                    top_ref[c0:c0 + 8, :] = st[i]
            return st[i]

        def bc(v):
            return jnp.concatenate([v] * NT, axis=1)

        def taps(r):
            st["tw", r] = [bc(x0_ref[rows_at(c0, DW_OFF + k * C, 8), :]) for k in range(2)]

        def piece(r):
            if "w" not in st:
                st["w"] = [bc(dws_ref[k, pl.ds(c0, 8), :]) for k in range(9)]
            wts = list(st["w"])
            if ("tw", r) in st:
                wts[6], wts[8] = st["tw", r]
            abc = [row(r + 1) * wts[3 + j] + row(r) * wts[j] + row(r + 2) * wts[6 + j] for j in range(3)]
            x0 = pltpu.roll(abc[0], 1, 1) + abc[1] + pltpu.roll(abc[2], WP - 1, 1)
            for t in range(NT):
                x0_ref[rows_at(nxt, (r * NT + t) * C + c0, 8), :] = x0[:, t * LANES:(t + 1) * LANES]

        return taps, piece

    @pl.when(k_ == 0)
    def _():
        for k in range(9):
            w = dw_ref[k // 3].astype(F32)[k % 3:k % 3 + 1, :]
            w = jnp.broadcast_to(w, (LANES, C)).T
            dws_ref[k] = w + 1.0 if k == 4 else w
            if k in (6, 8):
                x0_ref[pl.ds(DW_OFF + (k - 6) // 2 * C, C), :] = w
        w = wqkv_ref[...].astype(F32)
        wq = w[:, 0:C] * ((DH ** -0.5) * math.log2(math.e))
        wk, wv = w[:, C:2 * C], w[:, 2 * C:3 * C]
        z32 = jnp.zeros((C, 32), F32)
        tiles = [(wv[:, 128:160], wq[:, 0:96]),
                 (wq[:, 96:128], wv[:, 160:192], wq[:, 128:192]),
                 (z32, wk[:, 0:96]),
                 (wk[:, 96:128], z32, wk[:, 128:192]),
                 (wv[:, 0:128],)]
        for n, parts in enumerate(tiles):
            w = jnp.concatenate(parts, axis=1)
            for i, wi in enumerate((w[0:128], w[64:192], _cat([w[0:64], w[128:192]]))):
                ws_ref[i, n] = pltpu.bitcast(wi.astype(BF16), U32)
        w = wo_ref[...].astype(F32)
        wx, wy, wz = w[0:64], w[64:128], w[128:192]
        for i, parts in enumerate(((wx, wy), (wz, wy), (wx, wz))):
            wos_ref[i] = pltpu.bitcast(_cat(parts).T.astype(BF16), U32)

        top_ref[...] = jnp.zeros(top_ref.shape, F32)

        def zero(i, carry):
            ob_ref[pl.ds(pl.multiple_of(i * WP, 8), WP), :] = jnp.zeros((WP, LANES), F32)
            for j in range(6):
                stg_ref[6 * i + j] = jnp.zeros(stg_ref.shape[1:], F32)
            for j in range(2):
                t_ref[2 * i + j] = jnp.zeros(t_ref.shape[1:], U32)
            return carry
        lax.fori_loop(0, WS, zero, 0)

    groups = [conv_group(8 * g) for g in range(NG)]
    WLEAD = _env("WLEAD", 5)

    def conv_items(gs):
        plist = [(g, r) for g in gs for r in range(WS)]
        items = []
        for k, (g, r) in enumerate(plist):
            fs = []
            if k + WLEAD < len(plist):
                g2, r2 = plist[k + WLEAD]
                fs.append(functools.partial(groups[g2][0], r2))
            fs.append(functools.partial(groups[g][1], r))
            items.append(fs)
        return items

    def ld_x0(j, k, gs=range(NG)):
        return [x0_ref[rows_at(nxt + dyn0 * (8 * k), j * C + 8 * g, 8), :] for g in gs]

    def add2(acc, xs):
        a = functools.reduce(jnp.add, xs[0::2])
        b = functools.reduce(jnp.add, xs[1::2])
        return a + b if acc is None else (acc + a) + b

    def stats_steps(j):
        st = {"s": None, "q": None}
        n1, n2 = _env("SEG1", 12), _env("SEG2", 6)

        def sum_step(g0):
            st["s"] = add2(st["s"], ld_x0(j, 0, range(g0, g0 + n1)))
            if g0 + n1 == NG:
                st["s"] = _allred(st["s"], jnp.add) * (1.0 / C)
            return st["s"]

        def var_step(g0):
            d = [x - st["s"] for x in ld_x0(j, 1, range(g0, g0 + n2))]
            st["q"] = add2(st["q"], [x * x for x in d])
            return st["q"]

        def last_step():
            rs = lax.rsqrt(_allred(st["q"], jnp.add) * (1.0 / C) + EPS)
            ms_ref[j] = _cat([st["s"], rs])
            return rs

        return ([functools.partial(sum_step, g) for g in range(0, NG, n1)]
                + [functools.partial(var_step, g) for g in range(0, NG, n2)] + [last_step])

    def normed(j, blk, k):
        m, rs = ms_ref[j, 0:8, :], ms_ref[j, 8:16, :]
        return _cat([(x - m) * rs for x in ld_x0(j, k, range(8 * blk, 8 * blk + 8))])

    def put_t(dst, tiles):
        tt = pltpu.bitcast(jnp.concatenate(tiles, axis=1).astype(BF16).T, U32)
        for i, (u, e) in enumerate(dst):
            t_ref[u, e] = tt[64 * i:64 * i + 64]

    def t_first(u):
        ja, jb = 2 * u, 2 * u + 1
        bx = normed(jb, 0, 0)
        put_t([(u, 0), (u, 2)], [_cat([normed(ja, 0, 0) - bx, normed(ja, 1, 0)]),
                                 _cat([bx, normed(ja, 2, 0)])])

    def t_second(r):
        put_t([(u, 1) for u in (2 * r, 2 * r + 1)],
              [_cat([normed(2 * u + 1, 1, 0), normed(2 * u + 1, 2, 0) - normed(2 * u, 2, _env("RECOMP", 1))])
               for u in (2 * r, 2 * r + 1)])

    t_items = []
    for r in range(WS):
        t_items += [functools.partial(t_first, 2 * r), functools.partial(t_first, 2 * r + 1),
                    functools.partial(t_second, r)]

    def qkv_chunk(u, n, steps=()):
        r, tp = divmod(u, 2)
        ops = {i: [_blocks(t_ref[u, i]), _blocks(ws_ref[i, n])] for i in range(3)}
        side = 1 if _env("ATT", "w") == "w" else 0
        for q, step in enumerate(steps):
            tok = pltpu.bitcast(step(), U32)
            q = q * 24 // len(steps)
            blks = ops[(2, 0, 1)[q % 3]][side]
            e = 7 - q // 3 if side else q // 3
            blks[e] = jnp.where(mk["never"], tok, blks[e])
        p = {i: _dot(*[pltpu.bitcast(_cat(x), BF16) for x in ops[i]]) for i in (2, 0, 1)}
        for j in range(2):
            qkv_ref[n, r, pl.ds((2 * tp + j) * LANES, LANES), :] = p[j] + p[2]

    zero8 = jnp.zeros((8, LANES), F32)

    def gather(n, off):
        return [qkv_ref[n, r, pl.ds(off, 8), :] for r in range(WS)]

    def softmax_t(st):
        rows = _blocks(st)
        m = functools.reduce(jnp.maximum, rows)
        m = _allred(jnp.where(mk["key"], m, -jnp.inf), jnp.maximum)
        p = [jnp.exp2(x - m) for x in rows]
        return p, functools.reduce(jnp.add, p)

    def s2_pair(pi, offa):
        offb = offa + WS
        st = {}

        def vprep():
            u1 = _cat(gather(4, offa) + gather(4, offb) + [zero8, zero8])
            u2 = _cat([jnp.where(mk["v"], x, y) for x, y in
                       zip(gather(0, offa) + gather(0, offb), gather(1, offa) + gather(1, offb))]
                      + [zero8, zero8])
            VM = _env("VM", 2)
            if VM == 0:
                u1t = pltpu.bitcast(u1.astype(BF16).T, U32)
                u2t = pltpu.bitcast(u2[:, 0:64].astype(BF16).T, U32)
                vt = _cat([u1t, u2t])
            elif VM == 1:
                vt = _cat([pltpu.bitcast(u.astype(BF16).T, U32) for u in (u1, u2)])
            else:
                vt = pltpu.bitcast(jnp.concatenate([u1, u2], axis=1).astype(BF16).T, U32)
            st["vt"] = [pltpu.bitcast(vt[24 * h:24 * h + 24], BF16) for h in range(NH)]

        def score(i):
            hp, sw = divmod(i, 2)
            ma, mb = (mk["lo"], mk["hi"]) if sw == 0 else (mk["hi"], mk["lo"])
            q = _cat([jnp.where(ma, v, 0.0) for v in gather(hp, offa)]
                     + [jnp.where(mb, v, 0.0) for v in gather(hp, offb)] + [zero8, zero8])
            k = _cat([jnp.where(ma, x, y)
                      for x, y in zip(gather(2 + hp, offa), gather(2 + hp, offb))])
            st["p", i] = softmax_t(_dot_nt(k, q))

        def value(h):
            hp, sw = divmod(h, 2)
            (pa, sa), (pb, sb) = st["p", 2 * hp + sw], st["p", 2 * hp + 1 - sw]
            pm = _cat([jnp.where(mk["keep_a"], v, 0.0) for v in pa]
                      + [jnp.where(mk["keep_b"], v, 0.0) for v in pb] + [zero8, zero8])
            den = _allred(jnp.where(mk["key"], jnp.where(mk["left"], sa, sb), 0.0), jnp.add)
            rec = pl.reciprocal(den, approx=True)
            if _env("NR", 1):
                rec = rec * (2.0 - den * rec)
            st["o", h] = [b * rec for b in _blocks(_dot(st["vt"][h], pm))]

        def finish():
            o = [b for h in range(NH) for b in st["o", h]]
            w = pltpu.pack_elementwise([_cat(o[0:16]), _cat(o[16:24] + o[16:24])], packed_dtype=BF16)
            stg_ref[pi] = pltpu.bitcast(w, F32)

        def scatter():
            wt = stg_ref[pi].T
            for i, off in enumerate((offa, offb)):
                for r in range(WS):
                    base = i * SLOTS + 8 * r
                    ob_ref[pl.ds(r * WP + off, WS), :] = wt[base:base + WS]

        return vprep, score, value, finish, scatter

    npair = (nwin + 1) // 2
    pairs = [s2_pair(p, min(2 * p, nwin - 2) * WS) for p in range(npair)]

    def s3_unit(r, tp):
        def unpack(t):
            w = pltpu.bitcast(ob_ref[pl.ds(r * WP + t * LANES, LANES), :], U32)
            return [_blocks(pltpu.unpack_elementwise(w, index=i, packed_dtype=BF16, unpacked_dtype=F32))
                    for i in range(2)]

        (la, ha), (lb, hb) = unpack(2 * tp), unpack(2 * tp + 1)
        t3 = _cat([jnp.where(mk["left64"], x, y) for x, y in zip(lb, ha)])
        t1 = _cat([x - jnp.where(mk["left64"], y, 0.0) for x, y in zip(la, lb)])
        t2 = _cat([jnp.where(mk["left64"], x - y, z) for x, y, z in zip(hb, ha, lb)])
        p3 = _dot_nt(pltpu.bitcast(wos_ref[2], BF16), t3)
        ys = [_dot_nt(pltpu.bitcast(wos_ref[i], BF16), t) + p3
              + x0_ref[rows_at(prv, (r * NT + 2 * tp + i) * C, C), :] for i, t in enumerate((t1, t2))]
        o_ref[r, :, pl.ds(2 * tp * LANES, 2 * LANES)] = jnp.concatenate(ys, axis=1).astype(o_ref.dtype)

    s3_all = [functools.partial(s3_unit, r, tp) for tp in range(2) for r in range(WS)]

    def run(prog, extra):
        extra = sorted(extra, key=lambda e: e[0])
        j = 0
        for t0, fn in prog:
            while j < len(extra) and extra[j][0] <= t0:
                extra[j][1]()
                j += 1
            fn()
        for e in extra[j:]:
            e[1]()

    NX3 = _env("NX3", 0)

    def block_x():
        NSC = _env("NSC", 37)
        NSTC = _env("NSTC", 15)
        WAVE = _env("WAVE", 4)
        chunks = [(u, n) for u in range(NU) for n in range(5)]
        steps = []
        for j0 in range(0, WS * NT, WAVE):
            for grp in zip(*[stats_steps(j) for j in range(j0, j0 + WAVE)]):
                steps += grp
        c0 = len(chunks) - NSTC - _env("STOFF", 0)
        prog = []
        for k, (u, n) in enumerate(chunks):
            mine = steps[(k - c0) * len(steps) // NSTC:(k - c0 + 1) * len(steps) // NSTC] if k >= c0 else []
            prog.append((k, functools.partial(qkv_chunk, u, n, mine)))
        prog += [(len(chunks), f) for f in s3_all[:NX3]]
        ci = conv_items(range(NG))
        for p in range(NSC):
            ci[4 * p].insert(0, pairs[p][4])
        extra = [((j + 1) * c0 / len(ci), f) for j, fs in enumerate(ci) for f in fs]
        extra += [(c0 + (p - NSC) * 0.5, pairs[p][4]) for p in range(NSC, npair)]
        run(prog, extra)

    def block_y():
        LSM = _env("LSM", 200)
        LFIN = _env("LFIN", 200)
        SGRP = _env("SGRP", 2)
        VGRP = _env("VGRP", 2)
        TAILGAP = _env("TAILGAP", 500)
        load = [0] * 4
        tm = [0] * 4
        prog, extra = [], []

        def emit(rows_list, fn, ready=0):
            prog.append((min(tm), fn))
            ends = []
            for rows in rows_list:
                m = load.index(min(load))
                load[m] += rows
                tm[m] = max(tm[m], ready) + rows
                ends.append(tm[m])
            return ends

        fillers = list(s3_all[NX3:])
        total = len(fillers) * 3 * C / 4 + npair * (SLOTS + DH)
        nsc = 4 * npair
        next_s = 0
        s_end, v_end, pend_v = {}, {}, []
        while fillers or next_s < nsc or pend_v:
            now = tm[load.index(min(load))]
            s_ok = next_s < nsc and now >= (total - TAILGAP) * next_s / (nsc - 4)
            v_ok = len(pend_v) >= VGRP // 2 and all(now >= x[0] for x in pend_v[:VGRP // 2])
            if not fillers and not s_ok and not v_ok:
                if pend_v and (next_s >= nsc or len(pend_v) >= 4):
                    v_ok = True
                else:
                    s_ok = True
            if v_ok:
                for rdy, pv, hp in pend_v[:VGRP // 2]:
                    for h in (2 * hp, 2 * hp + 1):
                        v_end[pv, h] = emit([DH], functools.partial(pairs[pv][2], h), rdy)[0]
                    if hp == 1:
                        extra.append((max(v_end[pv, h] for h in range(NH)) + LFIN, pairs[pv][3]))
                pend_v = pend_v[VGRP // 2:]
            elif s_ok:
                for _ in range(SGRP):
                    p, i = divmod(next_s, 4)
                    if i == 0:
                        prog.append((min(tm), pairs[p][0]))
                    s_end[p, i] = emit([SLOTS], functools.partial(pairs[p][1], i))[0]
                    if i % 2 == 1:
                        pend_v.append((max(s_end[p, i], s_end[p, i - 1]) + LSM, p, i // 2))
                    next_s += 1
            else:
                emit([C] * 3, fillers.pop(0))
        for j, f in enumerate(t_items):
            extra.append(((j + _env("TY0", 0.5)) * _env("TYF", 0.9) * max(tm) / len(t_items), f))
        run(prog, extra)

    only = _env("ONLY", "01")
    if "0" in only:
        new_masks()
        pl.when(k_ <= nstrip)(block_x)
    if "1" in only:
        new_masks()
        pl.when((k_ <= nstrip) & (k_ >= 1))(block_y)

    @pl.when(k_ == 0)
    def _():
        for f in t_items:
            f()

    @pl.when(k_ == nstrip + 1)
    def _():
        new_masks()
        for p in range(npair):
            pairs[p][4]()
        for f in s3_all:
            f()
        if only != "01":
            i = pl.multiple_of(dyn0 * 8, 8)
            ob_ref[0:8, :] = (qkv_ref[dyn0, dyn0, pl.ds(i, 8), :]
                              + pltpu.bitcast(t_ref[dyn0, dyn0, pl.ds(i, 8), :], F32))


@jax.jit
def pallas_standalone__window_attn_davit__vision_kernel(
    x: jax.Array,
    dw_pe: jax.Array,
    w_qkv: jax.Array,
    w_o: jax.Array,
):
    B, H, W, Cx = x.shape
    assert B == 1 and Cx == C and H % WS == 0 and W % WS == 0 and WP - LANES < W < WP
    nstrip = H // WS
    nwin = W // WS

    xt = jnp.transpose(x[0], (0, 2, 1))

    assert nstrip + 2 <= 256
    kernel = functools.partial(_kernel, W=W, nwin=nwin, nstrip=nstrip)
    yt = pl.pallas_call(
        kernel,
        grid=(nstrip + 2,),
        in_specs=[
            pl.BlockSpec((WS, C, WP), lambda s: (jnp.minimum(s, nstrip - 1), 0, 0)),
            pl.BlockSpec((1, C, WP), lambda s: (jnp.minimum(s * WS + WS, H - 1), 0, 0)),
            pl.BlockSpec((3, 3, C), lambda s: (0, 0, 0)),
            pl.BlockSpec((C, 3 * C), lambda s: (0, 0)),
            pl.BlockSpec((C, C), lambda s: (0, 0)),
        ],
        out_specs=pl.BlockSpec((WS, C, WP), lambda s: (jnp.maximum(s - 2, 0), 0, 0)),
        out_shape=jax.ShapeDtypeStruct((H, C, W), x.dtype),
        scratch_shapes=[
            pltpu.VMEM((X0_ROWS, LANES), F32),
            pltpu.VMEM((WS * WP, LANES), F32),
            pltpu.VMEM((9, C, LANES), F32),
            pltpu.VMEM((3, 5, LANES // 2, LANES), U32),
            pltpu.VMEM((3, C // 2, LANES), U32),
            pltpu.VMEM((5, WS, WP, LANES), F32),
            pltpu.VMEM((NU, 3, LANES // 2, LANES), U32),
            pltpu.VMEM((42, LANES, LANES), F32),
            pltpu.VMEM((WS * NT, 16, LANES), F32),
            pltpu.VMEM((C, WP), F32),
        ],
        compiler_params=pltpu.CompilerParams(
            dimension_semantics=("arbitrary",),
            vmem_limit_bytes=64 * 1024 * 1024,
            disable_bounds_checks=bool(_env("NOBC", 1)),
        ),
        name="davit_window_attn",
    )(xt, xt, dw_pe, w_qkv, w_o)
    return jnp.transpose(yt, (0, 2, 1))[None]
```

```python
import functools
import math
import os

import jax
import jax.numpy as jnp
from jax import lax
import jax.experimental.pallas as pl
import jax.experimental.pallas.tpu as pltpu

WS = 7
NH = 4
C = 192
DH = C // NH
NG = C // 8
LANES = 128
WP = 512
NT = WP // LANES
NU = WS * NT // 2
SLOTS = 8 * WS
EPS = 1e-5
F32 = jnp.float32
BF16 = jnp.bfloat16
U32 = jnp.uint32

X0_SLOT = WS * NT * C
DW_OFF = 3 * X0_SLOT
X0_ROWS = DW_OFF + 2 * C


def _dot(a, b):
    return jnp.dot(a, b, preferred_element_type=F32)


def _dot_nt(a, b):
    return lax.dot_general(a, b, (((1,), (1,)), ((), ())), preferred_element_type=F32)


def _cat(xs):
    return jnp.concatenate(xs, axis=0)


def _blocks(v):
    return [v[i:i + 8] for i in range(0, v.shape[0], 8)]


def _allred(x, op):
    for sh in (4, 2, 1):
        x = op(x, pltpu.roll(x, sh, 0))
    return x


def _env(name, default):
    return type(default)(os.environ.get(name, default))


def _kernel(xm_ref, xb_ref, dw_ref, wqkv_ref, wo_ref, o_ref,
            x0_ref, ob_ref, dws_ref, ws_ref, wos_ref, qkv_ref, t_ref, stg_ref, ms_ref, top_ref, *, W, nwin, nstrip):
    k_ = pl.program_id(0)
    dyn0 = jnp.minimum(k_, 0)

    def rows_at(base, off, n):
        if isinstance(base, int):
            return pl.ds(base + off, n)
        return pl.ds(pl.multiple_of(base + off, 8), n)

    mk = {}

    def new_masks():
        lane = lax.broadcasted_iota(jnp.int32, (8, LANES), 1)
        sub = lax.broadcasted_iota(jnp.int32, (8, LANES), 0)
        nlast = W - (WP - LANES)
        key_ok = sub < WS
        mk.update(
            last=lane < nlast,
            bot=lane < jnp.where(k_ < nstrip - 1, LANES, 0),
            bot_last=lane < jnp.where(k_ < nstrip - 1, nlast, 0),
            never=lane < dyn0, lo=lane < 80, hi=lane >= 80, v=lane < 32, key=key_ok,
            left=lane < SLOTS, keep_a=key_ok & (lane < SLOTS), keep_b=key_ok & (lane >= SLOTS),
            left64=lane < 64)

    k3 = k_ - 3 * ((k_ * 171) >> 9)
    nxt = k3 * X0_SLOT
    prv = jnp.where((k3 == 2) | (k_ < 2), 0, nxt + X0_SLOT)

    def conv_group(c0):
        st = {}

        def row(i):
            if i == 0 and i not in st:
                st[i] = top_ref[c0:c0 + 8, :]
            if i not in st:
                if i == WS + 1:
                    v, m, ml = xb_ref[0, c0:c0 + 8, :], mk["bot"], mk["bot_last"]
                else:
                    v, m, ml = xm_ref[i - 1, c0:c0 + 8, :], None, mk["last"]
                v = v.astype(F32)
                ts = [v[:, t * LANES:(t + 1) * LANES] for t in range(NT)]
                ts = [t if m is None else jnp.where(m, t, 0.0) for t in ts[:-1]] + [jnp.where(ml, ts[-1], 0.0)]
                st[i] = jnp.concatenate(ts, axis=1)
                if i == WS:
                    top_ref[c0:c0 + 8, :] = st[i]
            return st[i]

        def bc(v):
            return jnp.concatenate([v] * NT, axis=1)

        def taps(r):
            st["tw", r] = [bc(x0_ref[rows_at(c0, DW_OFF + k * C, 8), :]) for k in range(2)]

        def piece(r):
            if "w" not in st:
                st["w"] = [bc(dws_ref[k, pl.ds(c0, 8), :]) for k in range(9)]
            wts = list(st["w"])
            if ("tw", r) in st:
                wts[6], wts[8] = st["tw", r]
            abc = [row(r + 1) * wts[3 + j] + row(r) * wts[j] + row(r + 2) * wts[6 + j] for j in range(3)]
            x0 = pltpu.roll(abc[0], 1, 1) + abc[1] + pltpu.roll(abc[2], WP - 1, 1)
            for t in range(NT):
                x0_ref[rows_at(nxt, (r * NT + t) * C + c0, 8), :] = x0[:, t * LANES:(t + 1) * LANES]

        return taps, piece

    @pl.when(k_ == 0)
    def _():
        for k in range(9):
            w = dw_ref[k // 3].astype(F32)[k % 3:k % 3 + 1, :]
            w = jnp.broadcast_to(w, (LANES, C)).T
            dws_ref[k] = w + 1.0 if k == 4 else w
            if k in (6, 8):
                x0_ref[pl.ds(DW_OFF + (k - 6) // 2 * C, C), :] = w
        w = wqkv_ref[...].astype(F32)
        wq = w[:, 0:C] * ((DH ** -0.5) * math.log2(math.e))
        wk, wv = w[:, C:2 * C], w[:, 2 * C:3 * C]
        z32 = jnp.zeros((C, 32), F32)
        tiles = [(wv[:, 128:160], wq[:, 0:96]),
                 (wq[:, 96:128], wv[:, 160:192], wq[:, 128:192]),
                 (z32, wk[:, 0:96]),
                 (wk[:, 96:128], z32, wk[:, 128:192]),
                 (wv[:, 0:128],)]
        for n, parts in enumerate(tiles):
            w = jnp.concatenate(parts, axis=1)
            for i, wi in enumerate((w[0:128], w[64:192], _cat([w[0:64], w[128:192]]))):
                ws_ref[i, n] = pltpu.bitcast(wi.astype(BF16), U32)
        w = wo_ref[...].astype(F32)
        wx, wy, wz = w[0:64], w[64:128], w[128:192]
        for i, parts in enumerate(((wx, wy), (wz, wy), (wx, wz))):
            wos_ref[i] = pltpu.bitcast(_cat(parts).T.astype(BF16), U32)

        top_ref[...] = jnp.zeros(top_ref.shape, F32)

        def zero(i, carry):
            ob_ref[pl.ds(pl.multiple_of(i * WP, 8), WP), :] = jnp.zeros((WP, LANES), F32)
            for j in range(6):
                stg_ref[6 * i + j] = jnp.zeros(stg_ref.shape[1:], F32)
            for j in range(2):
                t_ref[2 * i + j] = jnp.zeros(t_ref.shape[1:], U32)
            return carry
        lax.fori_loop(0, WS, zero, 0)

    groups = [conv_group(8 * g) for g in range(NG)]
    WLEAD = _env("WLEAD", 4)

    def conv_items(gs):
        plist = [(g, r) for g in gs for r in range(WS)]
        items = []
        for k, (g, r) in enumerate(plist):
            fs = []
            if k + WLEAD < len(plist):
                g2, r2 = plist[k + WLEAD]
                fs.append(functools.partial(groups[g2][0], r2))
            fs.append(functools.partial(groups[g][1], r))
            items.append(fs)
        return items

    def ld_x0(j, k, gs=range(NG)):
        return [x0_ref[rows_at(nxt + dyn0 * (8 * k), j * C + 8 * g, 8), :] for g in gs]

    def add2(acc, xs):
        a = functools.reduce(jnp.add, xs[0::2])
        b = functools.reduce(jnp.add, xs[1::2])
        return a + b if acc is None else (acc + a) + b

    def stats_steps(j):
        st = {"s": None, "q": None}
        n1, n2 = _env("SEG1", 8), _env("SEG2", 6)

        def sum_step(g0):
            st["s"] = add2(st["s"], ld_x0(j, 0, range(g0, g0 + n1)))
            if g0 + n1 == NG:
                st["s"] = _allred(st["s"], jnp.add) * (1.0 / C)
            return st["s"]

        def var_step(g0):
            d = [x - st["s"] for x in ld_x0(j, 1, range(g0, g0 + n2))]
            st["q"] = add2(st["q"], [x * x for x in d])
            return st["q"]

        def last_step():
            rs = lax.rsqrt(_allred(st["q"], jnp.add) * (1.0 / C) + EPS)
            ms_ref[j] = _cat([st["s"], rs])
            return rs

        return ([functools.partial(sum_step, g) for g in range(0, NG, n1)]
                + [functools.partial(var_step, g) for g in range(0, NG, n2)] + [last_step])

    def normed(j, blk, k):
        m, rs = ms_ref[j, 0:8, :], ms_ref[j, 8:16, :]
        return _cat([(x - m) * rs for x in ld_x0(j, k, range(8 * blk, 8 * blk + 8))])

    t_done = []

    def put_t(dst, tiles):
        tt = pltpu.bitcast(jnp.concatenate(tiles, axis=1).astype(BF16).T, U32)
        for i, (u, e) in enumerate(dst):
            t_ref[u, e] = tt[64 * i:64 * i + 64]
        t_done.append(pltpu.bitcast(tt[120:128], F32))

    def t_first(u):
        ja, jb = 2 * u, 2 * u + 1
        bx = normed(jb, 0, 0)
        put_t([(u, 0), (u, 2)], [_cat([normed(ja, 0, 0) - bx, normed(ja, 1, 0)]),
                                 _cat([bx, normed(ja, 2, 0)])])

    def t_second(r):
        put_t([(u, 1) for u in (2 * r, 2 * r + 1)],
              [_cat([normed(2 * u + 1, 1, 0), normed(2 * u + 1, 2, 0) - normed(2 * u, 2, _env("RECOMP", 1))])
               for u in (2 * r, 2 * r + 1)])

    t_items = []
    for r in range(WS):
        t_items += [functools.partial(t_first, 2 * r), functools.partial(t_first, 2 * r + 1),
                    functools.partial(t_second, r)]

    def qkv_chunk(u, n, steps=()):
        r, tp = divmod(u, 2)
        ops = {i: [_blocks(t_ref[u, i]), _blocks(ws_ref[i, n])] for i in range(3)}
        side = 1 if _env("ATT", "l") == "w" else 0
        for q, step in enumerate(steps):
            tok = pltpu.bitcast(step(), U32)
            q = q * 24 // len(steps)
            blks = ops[(2, 0, 1)[q % 3]][side]
            e = 7 - q // 3 if side else q // 3
            blks[e] = jnp.where(mk["never"], tok, blks[e])
        p = {i: _dot(*[pltpu.bitcast(_cat(x), BF16) for x in ops[i]]) for i in (2, 0, 1)}
        for j in range(2):
            qkv_ref[n, r, pl.ds((2 * tp + j) * LANES, LANES), :] = p[j] + p[2]

    zero8 = jnp.zeros((8, LANES), F32)

    def gather(n, off):
        return [qkv_ref[n, r, pl.ds(off, 8), :] for r in range(WS)]

    def softmax_t(st):
        rows = _blocks(st)
        m = functools.reduce(jnp.maximum, rows)
        m = _allred(jnp.where(mk["key"], m, -jnp.inf), jnp.maximum)
        p = [jnp.exp2(x - m) for x in rows]
        return p, functools.reduce(jnp.add, p)

    def s2_pair(pi, offa):
        offb = offa + WS
        st = {}

        def vprep():
            u1 = _cat(gather(4, offa) + gather(4, offb) + [zero8, zero8])
            u2 = _cat([jnp.where(mk["v"], x, y) for x, y in
                       zip(gather(0, offa) + gather(0, offb), gather(1, offa) + gather(1, offb))]
                      + [zero8, zero8])
            VM = _env("VM", 2)
            if VM == 0:
                u1t = pltpu.bitcast(u1.astype(BF16).T, U32)
                u2t = pltpu.bitcast(u2[:, 0:64].astype(BF16).T, U32)
                vt = _cat([u1t, u2t])
            elif VM == 1:
                vt = _cat([pltpu.bitcast(u.astype(BF16).T, U32) for u in (u1, u2)])
            else:
                vt = pltpu.bitcast(jnp.concatenate([u1, u2], axis=1).astype(BF16).T, U32)
            st["vt"] = [pltpu.bitcast(vt[24 * h:24 * h + 24], BF16) for h in range(NH)]

        def score(i, after=None):
            hp, sw = divmod(i, 2)
            ma, mb = (mk["lo"], mk["hi"]) if sw == 0 else (mk["hi"], mk["lo"])
            q = _cat([jnp.where(ma, v, 0.0) for v in gather(hp, offa)]
                     + [jnp.where(mb, v, 0.0) for v in gather(hp, offb)] + [zero8, zero8])
            k = [jnp.where(ma, x, y) for x, y in zip(gather(2 + hp, offa), gather(2 + hp, offb))]
            if after is not None:
                k[0] = jnp.where(mk["never"], t_done[after], k[0])
            k = _cat(k)
            st["p", i] = softmax_t(_dot_nt(k, q))

        def value(h):
            hp, sw = divmod(h, 2)
            (pa, sa), (pb, sb) = st["p", 2 * hp + sw], st["p", 2 * hp + 1 - sw]
            pm = _cat([jnp.where(mk["keep_a"], v, 0.0) for v in pa]
                      + [jnp.where(mk["keep_b"], v, 0.0) for v in pb] + [zero8, zero8])
            den = _allred(jnp.where(mk["key"], jnp.where(mk["left"], sa, sb), 0.0), jnp.add)
            rec = pl.reciprocal(den, approx=True)
            if _env("NR", 1):
                rec = rec * (2.0 - den * rec)
            st["o", h] = [b * rec for b in _blocks(_dot(st["vt"][h], pm))]

        def finish():
            o = [b for h in range(NH) for b in st["o", h]]
            w = pltpu.pack_elementwise([_cat(o[0:16]), _cat(o[16:24] + o[16:24])], packed_dtype=BF16)
            stg_ref[pi] = pltpu.bitcast(w, F32)

        def scatter():
            wt = stg_ref[pi].T
            for i, off in enumerate((offa, offb)):
                for r in range(WS):
                    base = i * SLOTS + 8 * r
                    ob_ref[pl.ds(r * WP + off, WS), :] = wt[base:base + WS]

        return vprep, score, value, finish, scatter

    npair = (nwin + 1) // 2
    pairs = [s2_pair(p, min(2 * p, nwin - 2) * WS) for p in range(npair)]

    def s3_unit(r, tp):
        def unpack(t):
            w = pltpu.bitcast(ob_ref[pl.ds(r * WP + t * LANES, LANES), :], U32)
            return [_blocks(pltpu.unpack_elementwise(w, index=i, packed_dtype=BF16, unpacked_dtype=F32))
                    for i in range(2)]

        (la, ha), (lb, hb) = unpack(2 * tp), unpack(2 * tp + 1)
        t3 = _cat([jnp.where(mk["left64"], x, y) for x, y in zip(lb, ha)])
        t1 = _cat([x - jnp.where(mk["left64"], y, 0.0) for x, y in zip(la, lb)])
        t2 = _cat([jnp.where(mk["left64"], x - y, z) for x, y, z in zip(hb, ha, lb)])
        p3 = _dot_nt(pltpu.bitcast(wos_ref[2], BF16), t3)
        ys = [_dot_nt(pltpu.bitcast(wos_ref[i], BF16), t) + p3
              + x0_ref[rows_at(prv, (r * NT + 2 * tp + i) * C, C), :] for i, t in enumerate((t1, t2))]
        o_ref[r, :, pl.ds(2 * tp * LANES, 2 * LANES)] = jnp.concatenate(ys, axis=1).astype(o_ref.dtype)

    s3_all = [functools.partial(s3_unit, r, tp) for tp in range(2) for r in range(WS)]

    def run(prog, extra):
        extra = sorted(extra, key=lambda e: e[0])
        j = 0
        for t0, fn in prog:
            while j < len(extra) and extra[j][0] <= t0:
                extra[j][1]()
                j += 1
            fn()
        for e in extra[j:]:
            e[1]()

    MERGE = _env("MERGE", 0)
    NX3 = _env("NX3", 0)

    def block_x():
        NSC = _env("NSC", 31)
        NSTC = _env("NSTC", 10)
        WAVE = _env("WAVE", 2)
        chunks = [(u, n) for u in range(NU) for n in range(5)]
        steps = []
        for j0 in range(0, WS * NT, WAVE):
            for grp in zip(*[stats_steps(j) for j in range(j0, j0 + WAVE)]):
                steps += grp
        c0 = len(chunks) - NSTC - _env("STOFF", 0)
        prog = []
        for k, (u, n) in enumerate(chunks):
            mine = steps[(k - c0) * len(steps) // NSTC:(k - c0 + 1) * len(steps) // NSTC] if k >= c0 else []
            prog.append((k, functools.partial(qkv_chunk, u, n, mine)))
        prog += [(len(chunks), f) for f in s3_all[:NX3]]
        ci = conv_items(range(NG))
        for p in range(NSC):
            ci[4 * p].insert(0, pairs[p][4])
        extra = [((j + 1) * c0 / len(ci), f) for j, fs in enumerate(ci) for f in fs]
        extra += [(c0 + (p - NSC) * 0.5, pairs[p][4]) for p in range(NSC, npair)]
        run(prog, extra)

    def block_y():
        LSM = _env("LSM", 180)
        LFIN = _env("LFIN", 200)
        SGRP = _env("SGRP", 4)
        VGRP = _env("VGRP", 4)
        TAILGAP = _env("TAILGAP", 600)
        load = [LANES, LANES, 0, 0] if MERGE else [0] * 4
        tm = list(load)
        t_0 = LANES + _env("LQKV", 220) if MERGE else 0
        prog, extra = [], []

        def emit(rows_list, fn, ready=0):
            prog.append((min(tm), fn))
            ends = []
            for rows in rows_list:
                m = load.index(min(load))
                load[m] += rows
                tm[m] = max(tm[m], ready) + rows
                ends.append(tm[m])
            return ends

        fillers = list(s3_all[NX3:])
        total = len(fillers) * 3 * C / 4 + npair * (SLOTS + DH)
        nsc = 4 * npair
        next_s = 0
        s_end, v_end, pend_v = {}, {}, []
        t_done.clear()
        d0, d1 = _env("TD0", 8), _env("TD1", 0)
        dl = {d0 + j * (nsc + d1 - d0) // len(t_items): j for j in range(len(t_items))}
        while fillers or next_s < nsc or pend_v:
            now = tm[load.index(min(load))]
            s_ok = next_s < nsc and now >= t_0 + (total - TAILGAP - t_0) * next_s / (nsc - 4)
            v_ok = len(pend_v) >= VGRP // 2 and all(now >= x[0] for x in pend_v[:VGRP // 2])
            if not fillers and not s_ok and not v_ok:
                if pend_v and (next_s >= nsc or len(pend_v) >= 4):
                    v_ok = True
                else:
                    s_ok = True
            if v_ok:
                for rdy, pv, hp in pend_v[:VGRP // 2]:
                    for h in (2 * hp, 2 * hp + 1):
                        v_end[pv, h] = emit([DH], functools.partial(pairs[pv][2], h), rdy)[0]
                    if hp == 1:
                        extra.append((max(v_end[pv, h] for h in range(NH)) + LFIN, pairs[pv][3]))
                pend_v = pend_v[VGRP // 2:]
            elif s_ok:
                for _ in range(SGRP):
                    p, i = divmod(next_s, 4)
                    if i == 0:
                        prog.append((min(tm), pairs[p][0]))
                    if next_s in dl:
                        extra.append((min(tm) - _env("TLEAD", 450), t_items[dl[next_s]]))
                    s_end[p, i] = emit([SLOTS], functools.partial(pairs[p][1], i, dl.get(next_s)))[0]
                    if i % 2 == 1:
                        pend_v.append((max(s_end[p, i], s_end[p, i - 1]) + LSM, p, i // 2))
                    next_s += 1
            else:
                emit([C] * 3, fillers.pop(0))
        extra += [(max(tm) - 600, t_items[j]) for q, j in dl.items() if q >= nsc]
        run(prog, extra)

    only = _env("ONLY", "01")
    if MERGE:
        new_masks()

        @pl.when(k_ <= nstrip)
        def _():
            block_x()
            block_y()
    else:
        if "0" in only:
            new_masks()
            pl.when(k_ <= nstrip)(block_x)
        if "1" in only:
            new_masks()
            pl.when((k_ <= nstrip) & (k_ >= 1))(block_y)

        @pl.when(k_ == 0)
        def _():
            for f in t_items:
                f()

    @pl.when(k_ == nstrip + 1)
    def _():
        new_masks()
        for p in range(npair):
            pairs[p][4]()
        for f in s3_all:
            f()
        if only != "01":
            i = pl.multiple_of(dyn0 * 8, 8)
            ob_ref[0:8, :] = (qkv_ref[dyn0, dyn0, pl.ds(i, 8), :]
                              + pltpu.bitcast(t_ref[dyn0, dyn0, pl.ds(i, 8), :], F32))


@jax.jit
def pallas_standalone__window_attn_davit__vision_kernel(
    x: jax.Array,
    dw_pe: jax.Array,
    w_qkv: jax.Array,
    w_o: jax.Array,
):
    B, H, W, Cx = x.shape
    assert B == 1 and Cx == C and H % WS == 0 and W % WS == 0 and WP - LANES < W < WP
    nstrip = H // WS
    nwin = W // WS

    xt = jnp.transpose(x[0], (0, 2, 1))

    assert nstrip + 2 <= 256
    kernel = functools.partial(_kernel, W=W, nwin=nwin, nstrip=nstrip)
    yt = pl.pallas_call(
        kernel,
        grid=(nstrip + 2,),
        in_specs=[
            pl.BlockSpec((WS, C, WP), lambda s: (jnp.minimum(s, nstrip - 1), 0, 0)),
            pl.BlockSpec((1, C, WP), lambda s: (jnp.minimum(s * WS + WS, H - 1), 0, 0)),
            pl.BlockSpec((3, 3, C), lambda s: (0, 0, 0)),
            pl.BlockSpec((C, 3 * C), lambda s: (0, 0)),
            pl.BlockSpec((C, C), lambda s: (0, 0)),
        ],
        out_specs=pl.BlockSpec((WS, C, WP), lambda s: (jnp.maximum(s - 2, 0), 0, 0)),
        out_shape=jax.ShapeDtypeStruct((H, C, W), x.dtype),
        scratch_shapes=[
            pltpu.VMEM((X0_ROWS, LANES), F32),
            pltpu.VMEM((WS * WP, LANES), F32),
            pltpu.VMEM((9, C, LANES), F32),
            pltpu.VMEM((3, 5, LANES // 2, LANES), U32),
            pltpu.VMEM((3, C // 2, LANES), U32),
            pltpu.VMEM((5, WS, WP, LANES), F32),
            pltpu.VMEM((NU, 3, LANES // 2, LANES), U32),
            pltpu.VMEM((42, LANES, LANES), F32),
            pltpu.VMEM((WS * NT, 16, LANES), F32),
            pltpu.VMEM((C, WP), F32),
        ],
        compiler_params=pltpu.CompilerParams(
            dimension_semantics=("arbitrary",),
            vmem_limit_bytes=64 * 1024 * 1024,
            disable_bounds_checks=bool(_env("NOBC", 1)),
        ),
        name="davit_window_attn",
    )(xt, xt, dw_pe, w_qkv, w_o)
    return jnp.transpose(yt, (0, 2, 1))[None]
```

```python
import functools
import math
import os

import jax
import jax.numpy as jnp
from jax import lax
import jax.experimental.pallas as pl
import jax.experimental.pallas.tpu as pltpu

WS = 7
NH = 4
C = 192
DH = C // NH
NG = C // 8
LANES = 128
WP = 512
NT = WP // LANES
NU = WS * NT // 2
SLOTS = 8 * WS
EPS = 1e-5
F32 = jnp.float32
BF16 = jnp.bfloat16
U32 = jnp.uint32

X0_SLOT = WS * NT * C
DW_OFF = 3 * X0_SLOT
X0_ROWS = DW_OFF + 2 * C


def _dot(a, b):
    return jnp.dot(a, b, preferred_element_type=F32)


def _dot_nt(a, b):
    return lax.dot_general(a, b, (((1,), (1,)), ((), ())), preferred_element_type=F32)


def _cat(xs):
    return jnp.concatenate(xs, axis=0)


def _blocks(v):
    return [v[i:i + 8] for i in range(0, v.shape[0], 8)]


def _allred(x, op):
    for sh in (4, 2, 1):
        x = op(x, pltpu.roll(x, sh, 0))
    return x


def _env(name, default):
    return type(default)(os.environ.get(name, default))


def _kernel(x_hbm, dw_ref, wqkv_ref, wo_ref, o_hbm, *scratch, H, W):
    step = functools.partial(_step, x_hbm, dw_ref, wqkv_ref, wo_ref, o_hbm, *scratch, H=H, W=W)
    nstrip = H // WS

    def loop(lo, hi, mode):
        def body(k, carry):
            step(k_=k, mode=mode)
            return carry
        lax.fori_loop(lo, hi, body, 0)

    loop(0, 1, "first")
    loop(1, nstrip + 1, "main")
    loop(nstrip + 1, nstrip + 2, "last")


def _step(x_hbm, dw_ref, wqkv_ref, wo_ref, o_hbm,
          x_ref, o_ref, sems, x0_ref, ob_ref, dws_ref, ws_ref, wos_ref, qkv_ref, t_ref, stg_ref, ms_ref,
          top_ref, *, H, W, k_, mode):
    nstrip, nwin = H // WS, W // WS

    def x_copy(k):
        return pltpu.make_async_copy(x_hbm.at[pl.ds(jnp.minimum(k * WS, H - WS - 1), WS + 1)], x_ref,
                                     sems.at[0])

    def o_copy(k):
        return pltpu.make_async_copy(o_ref, o_hbm.at[pl.ds(k * WS, WS)], sems.at[1])

    def when(cond, modes):
        if mode in modes:
            return pl.when(cond)
        return lambda f: None

    xoff = jnp.where(k_ >= nstrip - 1, 1, 0)
    dyn0 = jnp.minimum(k_, 0)

    def rows_at(base, off, n):
        if isinstance(base, int):
            return pl.ds(base + off, n)
        return pl.ds(pl.multiple_of(base + off, 8), n)

    mk = {}

    def new_masks():
        lane = lax.broadcasted_iota(jnp.int32, (8, LANES), 1)
        sub = lax.broadcasted_iota(jnp.int32, (8, LANES), 0)
        key_ok = sub < WS
        mk.update(
            bot=lane < jnp.where(k_ < nstrip - 1, LANES, 0),
            never=lane < dyn0, lo=lane < 80, hi=lane >= 80, v=lane < 32, key=key_ok,
            left=lane < SLOTS, keep_a=key_ok & (lane < SLOTS), keep_b=key_ok & (lane >= SLOTS),
            left64=lane < 64)

    k3 = k_ - 3 * ((k_ * 171) >> 9)
    nxt = k3 * X0_SLOT
    prv = jnp.where((k3 == 2) | (k_ < 2), 0, nxt + X0_SLOT)

    def conv_group(c0):
        st = {}

        def row(i):
            if i == 0 and i not in st:
                st[i] = top_ref[pl.ds(c0, 8), :]
            if i not in st:
                v = x_ref[WS if i == WS + 1 else xoff + (i - 1), pl.ds(c0, 8), :].astype(F32)
                v = jnp.concatenate([v, jnp.zeros((8, WP - W), F32)], axis=1)
                ts = [v[:, t * LANES:(t + 1) * LANES] for t in range(NT)]
                if i == WS + 1:
                    ts = [jnp.where(mk["bot"], t, 0.0) for t in ts]
                st[i] = jnp.concatenate(ts, axis=1)
                if i == WS:
                    top_ref[pl.ds(c0, 8), :] = st[i]
            return st[i]

        def bc(v):
            return jnp.concatenate([v] * NT, axis=1)

        def taps(r):
            st["tw", r] = [bc(x0_ref[rows_at(c0, DW_OFF + k * C, 8), :]) for k in range(2)]

        def piece(r):
            if "w" not in st:
                st["w"] = [bc(dws_ref[k, pl.ds(c0, 8), :]) for k in range(9)]
            wts = list(st["w"])
            if ("tw", r) in st:
                wts[6], wts[8] = st["tw", r]
            abc = [row(r + 1) * wts[3 + j] + row(r) * wts[j] + row(r + 2) * wts[6 + j] for j in range(3)]
            x0 = pltpu.roll(abc[0], 1, 1) + abc[1] + pltpu.roll(abc[2], WP - 1, 1)
            for t in range(NT):
                x0_ref[rows_at(nxt, (r * NT + t) * C + c0, 8), :] = x0[:, t * LANES:(t + 1) * LANES]

        return taps, piece

    @when(k_ == 0, ("first",))
    def _():
        x_copy(0).start()
        for k in range(9):
            w = dw_ref[k // 3].astype(F32)[k % 3:k % 3 + 1, :]
            w = jnp.broadcast_to(w, (LANES, C)).T
            dws_ref[k] = w + 1.0 if k == 4 else w
            if k in (6, 8):
                x0_ref[pl.ds(DW_OFF + (k - 6) // 2 * C, C), :] = w
        w = wqkv_ref[...].astype(F32)
        wq = w[:, 0:C] * ((DH ** -0.5) * math.log2(math.e))
        wk, wv = w[:, C:2 * C], w[:, 2 * C:3 * C]
        z32 = jnp.zeros((C, 32), F32)
        tiles = [(wv[:, 128:160], wq[:, 0:96]),
                 (wq[:, 96:128], wv[:, 160:192], wq[:, 128:192]),
                 (z32, wk[:, 0:96]),
                 (wk[:, 96:128], z32, wk[:, 128:192]),
                 (wv[:, 0:128],)]
        for n, parts in enumerate(tiles):
            w = jnp.concatenate(parts, axis=1)
            for i, wi in enumerate((w[0:128], w[64:192], _cat([w[0:64], w[128:192]]))):
                ws_ref[i, n] = pltpu.bitcast(wi.astype(BF16), U32)
        w = wo_ref[...].astype(F32)
        wx, wy, wz = w[0:64], w[64:128], w[128:192]
        for i, parts in enumerate(((wx, wy), (wz, wy), (wx, wz))):
            wos_ref[i] = pltpu.bitcast(_cat(parts).T.astype(BF16), U32)

        top_ref[...] = jnp.zeros(top_ref.shape, F32)

        for r in range(WS):
            ob_ref[pl.ds(r * WP + WP - 8, 8), :] = jnp.zeros((8, LANES), F32)

    groups = [conv_group(8 * g) for g in range(NG)]
    WLEAD = _env("WLEAD", 4)

    def conv_items(gs):
        plist = [(g, r) for g in gs for r in range(WS)]
        items = []
        for k, (g, r) in enumerate(plist):
            fs = []
            if k + WLEAD < len(plist):
                g2, r2 = plist[k + WLEAD]
                fs.append(functools.partial(groups[g2][0], r2))
            fs.append(functools.partial(groups[g][1], r))
            items.append(fs)
        return items

    def ld_x0(j, k, gs=range(NG)):
        return [x0_ref[rows_at(nxt + dyn0 * (8 * k), j * C + 8 * g, 8), :] for g in gs]

    def add2(acc, xs):
        a = functools.reduce(jnp.add, xs[0::2])
        b = functools.reduce(jnp.add, xs[1::2])
        return a + b if acc is None else (acc + a) + b

    def stats_steps(j):
        st = {"s": None, "q": None}
        n1, n2 = _env("SEG1", 8), _env("SEG2", 6)

        def sum_step(g0):
            st["s"] = add2(st["s"], ld_x0(j, 0, range(g0, g0 + n1)))
            if g0 + n1 == NG:
                st["s"] = _allred(st["s"], jnp.add) * (1.0 / C)
            return st["s"]

        def var_step(g0):
            d = [x - st["s"] for x in ld_x0(j, 1, range(g0, g0 + n2))]
            st["q"] = add2(st["q"], [x * x for x in d])
            return st["q"]

        def last_step():
            rs = lax.rsqrt(_allred(st["q"], jnp.add) * (1.0 / C) + EPS)
            ms_ref[j] = _cat([st["s"], rs])
            return rs

        return ([functools.partial(sum_step, g) for g in range(0, NG, n1)]
                + [functools.partial(var_step, g) for g in range(0, NG, n2)] + [last_step])

    def normed(j, blk, k):
        m, rs = ms_ref[j, 0:8, :], ms_ref[j, 8:16, :]
        return _cat([(x - m) * rs for x in ld_x0(j, k, range(8 * blk, 8 * blk + 8))])

    t_done = []

    def put_t(dst, tiles):
        tt = pltpu.bitcast(jnp.concatenate(tiles, axis=1).astype(BF16).T, U32)
        for i, (u, e) in enumerate(dst):
            t_ref[u, e] = tt[64 * i:64 * i + 64]
        t_done.append(pltpu.bitcast(tt[120:128], F32))

    def t_first(u):
        ja, jb = 2 * u, 2 * u + 1
        bx = normed(jb, 0, 0)
        put_t([(u, 0), (u, 2)], [_cat([normed(ja, 0, 0) - bx, normed(ja, 1, 0)]),
                                 _cat([bx, normed(ja, 2, 0)])])

    def t_second(r):
        put_t([(u, 1) for u in (2 * r, 2 * r + 1)],
              [_cat([normed(2 * u + 1, 1, 0), normed(2 * u + 1, 2, 0) - normed(2 * u, 2, _env("RECOMP", 1))])
               for u in (2 * r, 2 * r + 1)])

    t_items = []
    for r in range(WS):
        t_items += [functools.partial(t_first, 2 * r), functools.partial(t_first, 2 * r + 1),
                    functools.partial(t_second, r)]

    def qkv_chunk(u, n, steps=()):
        r, tp = divmod(u, 2)
        ops = {i: [_blocks(t_ref[u, i]), _blocks(ws_ref[i, n])] for i in range(3)}
        side = 1 if _env("ATT", "l") == "w" else 0
        for q, step in enumerate(steps):
            tok = pltpu.bitcast(step(), U32)
            q = q * 24 // len(steps)
            blks = ops[(2, 0, 1)[q % 3]][side]
            e = 7 - q // 3 if side else q // 3
            blks[e] = jnp.where(mk["never"], tok, blks[e])
        p = {i: _dot(*[pltpu.bitcast(_cat(x), BF16) for x in ops[i]]) for i in (2, 0, 1)}
        for j in range(2):
            qkv_ref[n, r, pl.ds((2 * tp + j) * LANES, LANES), :] = p[j] + p[2]

    zero8 = jnp.zeros((8, LANES), F32)

    def gather(n, off):
        return [qkv_ref[n, r, pl.ds(off, 8), :] for r in range(WS)]

    def softmax_t(st):
        rows = _blocks(st)
        m = functools.reduce(jnp.maximum, rows)
        m = _allred(jnp.where(mk["key"], m, -jnp.inf), jnp.maximum)
        p = [jnp.exp2(x - m) for x in rows]
        return p, functools.reduce(jnp.add, p)

    def s2_pair(pi, offa):
        offb = offa + WS
        st = {}

        def vprep():
            u1 = _cat(gather(4, offa) + gather(4, offb) + [zero8, zero8])
            u2 = _cat([jnp.where(mk["v"], x, y) for x, y in
                       zip(gather(0, offa) + gather(0, offb), gather(1, offa) + gather(1, offb))]
                      + [zero8, zero8])
            VM = _env("VM", 2)
            if VM == 0:
                u1t = pltpu.bitcast(u1.astype(BF16).T, U32)
                u2t = pltpu.bitcast(u2[:, 0:64].astype(BF16).T, U32)
                vt = _cat([u1t, u2t])
            elif VM == 1:
                vt = _cat([pltpu.bitcast(u.astype(BF16).T, U32) for u in (u1, u2)])
            else:
                vt = pltpu.bitcast(jnp.concatenate([u1, u2], axis=1).astype(BF16).T, U32)
            st["vt"] = [pltpu.bitcast(vt[24 * h:24 * h + 24], BF16) for h in range(NH)]

        def score(i, after=None):
            hp, sw = divmod(i, 2)
            ma, mb = (mk["lo"], mk["hi"]) if sw == 0 else (mk["hi"], mk["lo"])
            q = _cat([jnp.where(ma, v, 0.0) for v in gather(hp, offa)]
                     + [jnp.where(mb, v, 0.0) for v in gather(hp, offb)] + [zero8, zero8])
            k = [jnp.where(ma, x, y) for x, y in zip(gather(2 + hp, offa), gather(2 + hp, offb))]
            if after is not None:
                k[0] = jnp.where(mk["never"], t_done[after], k[0])
            k = _cat(k)
            st["p", i] = softmax_t(_dot_nt(k, q))

        def value(h):
            hp, sw = divmod(h, 2)
            (pa, sa), (pb, sb) = st["p", 2 * hp + sw], st["p", 2 * hp + 1 - sw]
            pm = _cat([jnp.where(mk["keep_a"], v, 0.0) for v in pa]
                      + [jnp.where(mk["keep_b"], v, 0.0) for v in pb] + [zero8, zero8])
            den = _allred(jnp.where(mk["key"], jnp.where(mk["left"], sa, sb), 0.0), jnp.add)
            rec = pl.reciprocal(den, approx=True)
            if _env("NR", 1):
                rec = rec * (2.0 - den * rec)
            st["o", h] = [b * rec for b in _blocks(_dot(st["vt"][h], pm))]

        def finish():
            o = [b for h in range(NH) for b in st["o", h]]
            w = pltpu.pack_elementwise([_cat(o[0:16]), _cat(o[16:24] + o[16:24])], packed_dtype=BF16)
            stg_ref[pi] = pltpu.bitcast(w, F32)

        def scatter():
            wt = stg_ref[pi].T
            for i, off in enumerate((offa, offb)):
                for r in range(WS):
                    base = i * SLOTS + 8 * r
                    ob_ref[pl.ds(r * WP + off, WS), :] = wt[base:base + WS]

        return vprep, score, value, finish, scatter

    npair = (nwin + 1) // 2
    pairs = [s2_pair(p, min(2 * p, nwin - 2) * WS) for p in range(npair)]

    def s3_unit(r, tp):
        def unpack(t):
            w = pltpu.bitcast(ob_ref[pl.ds(r * WP + t * LANES, LANES), :], U32)
            return [_blocks(pltpu.unpack_elementwise(w, index=i, packed_dtype=BF16, unpacked_dtype=F32))
                    for i in range(2)]

        (la, ha), (lb, hb) = unpack(2 * tp), unpack(2 * tp + 1)
        t3 = _cat([jnp.where(mk["left64"], x, y) for x, y in zip(lb, ha)])
        t1 = _cat([x - jnp.where(mk["left64"], y, 0.0) for x, y in zip(la, lb)])
        t2 = _cat([jnp.where(mk["left64"], x - y, z) for x, y, z in zip(hb, ha, lb)])
        p3 = _dot_nt(pltpu.bitcast(wos_ref[2], BF16), t3)
        ys = [_dot_nt(pltpu.bitcast(wos_ref[i], BF16), t) + p3
              + x0_ref[rows_at(prv, (r * NT + 2 * tp + i) * C, C), :] for i, t in enumerate((t1, t2))]
        n = min(2 * LANES, W - 2 * tp * LANES)
        o_ref[r, :, pl.ds(2 * tp * LANES, n)] = jnp.concatenate(ys, axis=1).astype(o_ref.dtype)[:, :n]

    s3_all = [functools.partial(s3_unit, r, tp) for tp in range(2) for r in range(WS)]

    def run(prog, extra):
        extra = sorted(extra, key=lambda e: e[0])
        j = 0
        for t0, fn in prog:
            while j < len(extra) and extra[j][0] <= t0:
                extra[j][1]()
                j += 1
            fn()
        for e in extra[j:]:
            e[1]()

    MERGE = _env("MERGE", 0)
    NX3 = _env("NX3", 0)

    def block_x():
        NSC = _env("NSC", 31)
        NSTC = _env("NSTC", 10)
        WAVE = _env("WAVE", 2)
        chunks = [(u, n) for u in range(NU) for n in range(5)]
        steps = []
        for j0 in range(0, WS * NT, WAVE):
            for grp in zip(*[stats_steps(j) for j in range(j0, j0 + WAVE)]):
                steps += grp
        c0 = len(chunks) - NSTC - _env("STOFF", 0)
        prog = []
        for k, (u, n) in enumerate(chunks):
            mine = steps[(k - c0) * len(steps) // NSTC:(k - c0 + 1) * len(steps) // NSTC] if k >= c0 else []
            prog.append((k, functools.partial(qkv_chunk, u, n, mine)))
        prog += [(len(chunks), f) for f in s3_all[:NX3]]
        ci = conv_items(range(NG))
        for p in range(NSC):
            ci[4 * p].insert(0, pairs[p][4])
        extra = [((j + 1) * c0 / len(ci), f) for j, fs in enumerate(ci) for f in fs]
        extra += [(c0 + (p - NSC) * 0.5, pairs[p][4]) for p in range(NSC, npair)]
        run(prog, extra)

    def block_y():
        LSM = _env("LSM", 180)
        LFIN = _env("LFIN", 200)
        SGRP = _env("SGRP", 4)
        VGRP = _env("VGRP", 4)
        TAILGAP = _env("TAILGAP", 600)
        load = [LANES, LANES, 0, 0] if MERGE else [0] * 4
        tm = list(load)
        t_0 = LANES + _env("LQKV", 220) if MERGE else 0
        prog, extra = [], []

        def emit(rows_list, fn, ready=0):
            prog.append((min(tm), fn))
            ends = []
            for rows in rows_list:
                m = load.index(min(load))
                load[m] += rows
                tm[m] = max(tm[m], ready) + rows
                ends.append(tm[m])
            return ends

        fillers = list(s3_all[NX3:])
        total = len(fillers) * 3 * C / 4 + npair * (SLOTS + DH)
        nsc = 4 * npair
        next_s = 0
        s_end, v_end, pend_v = {}, {}, []
        t_done.clear()
        d0, d1 = _env("TD0", 8), _env("TD1", 0)
        dl = {d0 + j * (nsc + d1 - d0) // len(t_items): j for j in range(len(t_items))}
        while fillers or next_s < nsc or pend_v:
            now = tm[load.index(min(load))]
            s_ok = next_s < nsc and now >= t_0 + (total - TAILGAP - t_0) * next_s / (nsc - 4)
            v_ok = len(pend_v) >= VGRP // 2 and all(now >= x[0] for x in pend_v[:VGRP // 2])
            if not fillers and not s_ok and not v_ok:
                if pend_v and (next_s >= nsc or len(pend_v) >= 4):
                    v_ok = True
                else:
                    s_ok = True
            if v_ok:
                for rdy, pv, hp in pend_v[:VGRP // 2]:
                    for h in (2 * hp, 2 * hp + 1):
                        v_end[pv, h] = emit([DH], functools.partial(pairs[pv][2], h), rdy)[0]
                    if hp == 1:
                        extra.append((max(v_end[pv, h] for h in range(NH)) + LFIN, pairs[pv][3]))
                pend_v = pend_v[VGRP // 2:]
            elif s_ok:
                for _ in range(SGRP):
                    p, i = divmod(next_s, 4)
                    if i == 0:
                        prog.append((min(tm), pairs[p][0]))
                    if next_s in dl:
                        extra.append((min(tm) - _env("TLEAD", 450), t_items[dl[next_s]]))
                    s_end[p, i] = emit([SLOTS], functools.partial(pairs[p][1], i, dl.get(next_s)))[0]
                    if i % 2 == 1:
                        pend_v.append((max(s_end[p, i], s_end[p, i - 1]) + LSM, p, i // 2))
                    next_s += 1
            else:
                emit([C] * 3, fillers.pop(0))
        extra += [(max(tm) - 600, t_items[j]) for q, j in dl.items() if q >= nsc]
        run(prog, extra)

    only = _env("ONLY", "01")
    NODMA = _env("NODMA", 0)

    @when(k_ < (1 if NODMA & 1 else nstrip), ("first", "main"))
    def _():
        x_copy(k_).wait()

    if "0" in only:
        new_masks()
        when(k_ <= nstrip, ("main",))(block_x)

    @when(k_ == 0, ("first",))
    def _():
        def body(g, carry):
            for j in range(FG):
                piece = conv_group(pl.multiple_of((g * FG + j) * 8, 8))[1]
                for r in range(WS):
                    piece(r)
            return carry
        FG = _env("FG", 8)
        lax.fori_loop(0, NG // FG, body, 0)

    @when(k_ < (0 if NODMA & 1 else nstrip - 1), ("first", "main"))
    def _():
        x_copy(k_ + 1).start()

    @when(k_ >= (1000 if NODMA & 2 else 3), ("main", "last"))
    def _():
        o_copy(k_ - 3).wait()

    if "1" in only:
        new_masks()
        when((k_ <= nstrip) & (k_ >= 1), ("main",))(block_y)

    @when(k_ == 0, ("first",))
    def _():
        for j in range(WS * NT):
            for f in stats_steps(j):
                f()
        for f in t_items:
            f()

    @when(k_ == nstrip + 1, ("last",))
    def _():
        new_masks()
        for p in range(npair):
            pairs[p][4]()
        for f in s3_all:
            f()
        if only != "01":
            i = pl.multiple_of(dyn0 * 8, 8)
            ob_ref[0:8, :] = (qkv_ref[dyn0, dyn0, pl.ds(i, 8), :]
                              + pltpu.bitcast(t_ref[dyn0, dyn0, pl.ds(i, 8), :], F32))

    @when(k_ >= (nstrip + 1 if NODMA & 2 else 2), ("main", "last"))
    def _():
        o_copy(k_ - 2).start()

    @when(k_ == nstrip + 1, ("last",))
    def _():
        o_copy(k_ - 2).wait()


@jax.jit
def pallas_standalone__window_attn_davit__vision_kernel(
    x: jax.Array,
    dw_pe: jax.Array,
    w_qkv: jax.Array,
    w_o: jax.Array,
):
    B, H, W, Cx = x.shape
    assert B == 1 and Cx == C and H % WS == 0 and W % WS == 0 and WP - LANES < W < WP
    xt = jnp.transpose(x[0], (0, 2, 1))

    assert H // WS + 2 <= 256
    vmem = pl.BlockSpec(memory_space=pltpu.VMEM)
    yt = pl.pallas_call(
        functools.partial(_kernel, H=H, W=W),
        in_specs=[pl.BlockSpec(memory_space=pl.ANY), vmem, vmem, vmem],
        out_specs=pl.BlockSpec(memory_space=pl.ANY),
        out_shape=jax.ShapeDtypeStruct((H, C, W), x.dtype),
        scratch_shapes=[
            pltpu.VMEM((WS + 1, C, W), x.dtype),
            pltpu.VMEM((WS, C, W), x.dtype),
            pltpu.SemaphoreType.DMA((2,)),
            pltpu.VMEM((X0_ROWS, LANES), F32),
            pltpu.VMEM((WS * WP, LANES), F32),
            pltpu.VMEM((9, C, LANES), F32),
            pltpu.VMEM((3, 5, LANES // 2, LANES), U32),
            pltpu.VMEM((3, C // 2, LANES), U32),
            pltpu.VMEM((5, WS, WP, LANES), F32),
            pltpu.VMEM((NU, 3, LANES // 2, LANES), U32),
            pltpu.VMEM((37, LANES, LANES), F32),
            pltpu.VMEM((WS * NT, 16, LANES), F32),
            pltpu.VMEM((C, WP), F32),
        ],
        compiler_params=pltpu.CompilerParams(
            vmem_limit_bytes=64 * 1024 * 1024,
            disable_bounds_checks=bool(_env("NOBC", 1)),
        ),
        name="davit_window_attn",
    )(xt, dw_pe, w_qkv, w_o)
    return jnp.transpose(yt, (0, 2, 1))[None]
```

```python
import functools
import math
import os

import jax
import jax.numpy as jnp
from jax import lax
import jax.experimental.pallas as pl
import jax.experimental.pallas.tpu as pltpu

WS = 7
NH = 4
C = 192
DH = C // NH
NG = C // 8
LANES = 128
WP = 512
NT = WP // LANES
NU = WS * NT // 2
SLOTS = 8 * WS
EPS = 1e-5
F32 = jnp.float32
BF16 = jnp.bfloat16
U32 = jnp.uint32

X0_SLOT = WS * NT * C
DW_OFF = 3 * X0_SLOT
X0_ROWS = DW_OFF + 2 * C


def _dot(a, b):
    return jnp.dot(a, b, preferred_element_type=F32)


def _dot_nt(a, b):
    return lax.dot_general(a, b, (((1,), (1,)), ((), ())), preferred_element_type=F32)


def _cat(xs):
    return jnp.concatenate(xs, axis=0)


def _blocks(v):
    return [v[i:i + 8] for i in range(0, v.shape[0], 8)]


def _allred(x, op):
    for sh in (4, 2, 1):
        x = op(x, pltpu.roll(x, sh, 0))
    return x


def _env(name, default):
    return type(default)(os.environ.get(name, default))


def _kernel(x_hbm, dw_ref, wqkv_ref, wo_ref, o_hbm, *scratch, H, W):
    step = functools.partial(_step, x_hbm, dw_ref, wqkv_ref, wo_ref, o_hbm, *scratch, H=H, W=W)
    nstrip = H // WS

    def loop(lo, hi, mode):
        def body(k, carry):
            step(k_=k, mode=mode)
            return carry
        lax.fori_loop(lo, hi, body, 0)

    loop(0, 1, "first")
    loop(1 + _env("SKIP", 0), nstrip + 1, "main")
    loop(nstrip + 1, nstrip + 2, "last")


def _step(x_hbm, dw_ref, wqkv_ref, wo_ref, o_hbm,
          x_ref, o_ref, sems, x0_ref, ob_ref, dws_ref, ws_ref, wos_ref, qkv_ref, t_ref, stg_ref, ms_ref,
          top_ref, *, H, W, k_, mode):
    nstrip, nwin = H // WS, W // WS

    def x_copy(k):
        return pltpu.make_async_copy(x_hbm.at[pl.ds(jnp.minimum(k * WS, H - WS - 1), WS + 1)], x_ref,
                                     sems.at[0])

    def o_copy(k):
        return pltpu.make_async_copy(o_ref, o_hbm.at[pl.ds(k * WS, WS)], sems.at[1])

    def when(cond, modes):
        if mode in modes:
            return pl.when(cond)
        return lambda f: None

    xoff = jnp.where(k_ >= nstrip - 1, 1, 0)
    dyn0 = jnp.minimum(k_, 0)

    def rows_at(base, off, n):
        if isinstance(base, int):
            return pl.ds(base + off, n)
        return pl.ds(pl.multiple_of(base + off, 8), n)

    mk = {}

    def new_masks():
        lane = lax.broadcasted_iota(jnp.int32, (8, LANES), 1)
        sub = lax.broadcasted_iota(jnp.int32, (8, LANES), 0)
        key_ok = sub < WS
        mk.update(
            bot=lane < jnp.where(k_ < nstrip - 1, LANES, 0),
            never=lane < dyn0, lo=lane < DH, hi0=(lane >= DH) & ((lane < 64) | (lane >= 96)),
            hi1=(lane >= DH) & (lane < 96), v=lane < 96, key=key_ok,
            keep_a=key_ok & (lane < SLOTS), keep_b=key_ok & (lane >= SLOTS),
            left64=lane < 64)

    k3 = k_ - 3 * ((k_ * 171) >> 9)
    nxt = k3 * X0_SLOT
    prv = jnp.where((k3 == 2) | (k_ < 2), 0, nxt + X0_SLOT)

    def conv_group(c0):
        st = {}

        def row(i):
            if i == 0 and i not in st:
                st[i] = top_ref[pl.ds(c0, 8), :]
            if i not in st:
                v = x_ref[WS if i == WS + 1 else xoff + (i - 1), pl.ds(c0, 8), :].astype(F32)
                v = jnp.concatenate([v, jnp.zeros((8, WP - W), F32)], axis=1)
                ts = [v[:, t * LANES:(t + 1) * LANES] for t in range(NT)]
                if i == WS + 1:
                    ts = [jnp.where(mk["bot"], t, 0.0) for t in ts]
                st[i] = jnp.concatenate(ts, axis=1)
                if i == WS:
                    top_ref[pl.ds(c0, 8), :] = st[i]
            return st[i]

        def bc(v):
            return jnp.concatenate([v] * NT, axis=1)

        def taps(r):
            st["tw", r] = [bc(x0_ref[rows_at(c0, DW_OFF + k * C, 8), :]) for k in range(2)]

        def piece(r):
            if "w" not in st:
                st["w"] = [bc(dws_ref[k, pl.ds(c0, 8), :]) for k in range(9)]
            wts = list(st["w"])
            if ("tw", r) in st:
                wts[6], wts[8] = st["tw", r]
            abc = [row(r + 1) * wts[3 + j] + row(r) * wts[j] + row(r + 2) * wts[6 + j] for j in range(3)]
            x0 = pltpu.roll(abc[0], 1, 1) + abc[1] + pltpu.roll(abc[2], WP - 1, 1)
            for t in range(NT):
                x0_ref[rows_at(nxt, (r * NT + t) * C + c0, 8), :] = x0[:, t * LANES:(t + 1) * LANES]

        return taps, piece

    @when(k_ == 0, ("first",))
    def _():
        x_copy(0).start()
        for k in range(9):
            w = dw_ref[k // 3].astype(F32)[k % 3:k % 3 + 1, :]
            w = jnp.broadcast_to(w, (LANES, C)).T
            dws_ref[k] = w + 1.0 if k == 4 else w
            if k in (6, 8):
                x0_ref[pl.ds(DW_OFF + (k - 6) // 2 * C, C), :] = w
        w = wqkv_ref[...].astype(F32)
        wq = w[:, 0:C] * ((DH ** -0.5) * math.log2(math.e))
        wk, wv = w[:, C:2 * C], w[:, 2 * C:3 * C]
        tiles = [(wq[:, 0:64], wv[:, 64:96], wq[:, 64:96]),
                 (wq[:, 96:192], wv[:, 96:128]),
                 (wk[:, 0:64], wv[:, 128:160], wk[:, 64:96]),
                 (wk[:, 96:192], wv[:, 160:192]),
                 (wv[:, 0:128],)]
        for n, parts in enumerate(tiles):
            w = jnp.concatenate(parts, axis=1)
            for i, wi in enumerate((w[0:128], w[64:192], _cat([w[0:64], w[128:192]]))):
                if n == 4:
                    wi = wi.T
                ws_ref[i, n] = pltpu.bitcast(wi.astype(BF16), U32)
        w = wo_ref[...].astype(F32)
        wx, wy, wz = w[0:64], w[64:128], w[128:192]
        for i, parts in enumerate(((wx, wy), (wz, wy), (wx, wz))):
            wos_ref[i] = pltpu.bitcast(_cat(parts).T.astype(BF16), U32)

        top_ref[...] = jnp.zeros(top_ref.shape, F32)

        for r in range(WS):
            ob_ref[pl.ds(r * WP + WP - 8, 8), :] = jnp.zeros((8, LANES), F32)

    groups = [conv_group(8 * g) for g in range(NG)]
    WLEAD = _env("WLEAD", 4)

    def conv_items(nslow):
        plist = [(g, r) for g in range(NG) for r in range(WS)]
        items, nxt_tap = [], WLEAD
        for k, (g, r) in enumerate(plist):
            fs = []
            lead = WLEAD if k < nslow else _env("WLEAD2", 6)
            while nxt_tap <= min(k + lead, len(plist) - 1):
                g2, r2 = plist[nxt_tap]
                fs.append(functools.partial(groups[g2][0], r2))
                nxt_tap += 1
            fs.append(functools.partial(groups[g][1], r))
            items.append(fs)
        return items

    def ld_x0(j, k, gs=range(NG)):
        return [x0_ref[rows_at(nxt + dyn0 * (8 * k), j * C + 8 * g, 8), :] for g in gs]

    def add2(acc, xs):
        a = functools.reduce(jnp.add, xs[0::2])
        b = functools.reduce(jnp.add, xs[1::2])
        return a + b if acc is None else (acc + a) + b

    stats_done = set()

    def stats_steps(j):
        st = {"s": None, "q": None}
        n1, n2 = _env("SEG1", 8), _env("SEG2", 8)

        def sum_step(g0):
            st["s"] = add2(st["s"], ld_x0(j, 0, range(g0, g0 + n1)))
            if g0 + n1 == NG:
                st["s"] = _allred(st["s"], jnp.add) * (1.0 / C)
            return st["s"]

        def var_step(g0):
            d = [x - st["s"] for x in ld_x0(j, 1, range(g0, g0 + n2))]
            st["q"] = add2(st["q"], [x * x for x in d])
            return st["q"]

        def last_step():
            rs = lax.rsqrt(_allred(st["q"], jnp.add) * (1.0 / C) + EPS)
            ms_ref[j] = _cat([st["s"], rs])
            stats_done.add(j)
            return rs

        return ([functools.partial(sum_step, g) for g in range(0, NG, n1)]
                + [functools.partial(var_step, g) for g in range(0, NG, n2)] + [last_step])

    def normed(j, blk, k):
        assert j in stats_done or "ONLY" in os.environ and j < NSTX, j
        m, rs = ms_ref[j, 0:8, :], ms_ref[j, 8:16, :]
        return _cat([(x - m) * rs for x in ld_x0(j, k, range(8 * blk, 8 * blk + 8))])

    t_done = []

    def put_t(dst, tiles):
        tt = pltpu.bitcast(jnp.concatenate(tiles, axis=1).astype(BF16).T, U32)
        for i, (u, e) in enumerate(dst):
            t_ref[u, e] = tt[64 * i:64 * i + 64]
        t_done.append(pltpu.bitcast(tt[120:128], F32))

    def t_first(u):
        ja, jb = 2 * u, 2 * u + 1
        bx = normed(jb, 0, 0)
        put_t([(u, 0), (u, 2)], [_cat([normed(ja, 0, 0) - bx, normed(ja, 1, 0)]),
                                 _cat([bx, normed(ja, 2, 0)])])

    def t_second(r):
        put_t([(u, 1) for u in (2 * r, 2 * r + 1)],
              [_cat([normed(2 * u + 1, 1, 0), normed(2 * u + 1, 2, 0) - normed(2 * u, 2, _env("RECOMP", 1))])
               for u in (2 * r, 2 * r + 1)])

    t_items = []
    for r in range(WS):
        t_items += [functools.partial(t_first, 2 * r), functools.partial(t_first, 2 * r + 1),
                    functools.partial(t_second, r)]

    def qkv_chunk(u, n, steps=()):
        r, tp = divmod(u, 2)
        ops = {i: [_blocks(t_ref[u, i]), _blocks(ws_ref[i, n])] for i in range(3)}
        side = 1 if _env("ATT", "l") == "w" else 0
        for q, step in enumerate(steps):
            tok = pltpu.bitcast(step(), U32)
            q = q * 24 // len(steps)
            blks = ops[(2, 0, 1)[q % 3]][side]
            e = 7 - q // 3 if side else q // 3
            blks[e] = jnp.where(mk["never"], tok, blks[e])
        p = {i: _dot(*[pltpu.bitcast(_cat(x), BF16) for x in ops[i]]) for i in (2, 0, 1)}
        for j in range(2):
            qkv_ref[n, r, pl.ds((2 * tp + j) * LANES, LANES), :] = p[j] + p[2]

    vr_words = {}
    job_done = {}

    def vr_dots(u):
        p = {i: _dot_nt(pltpu.bitcast(ws_ref[i, 4, 0:32, :], BF16), pltpu.bitcast(t_ref[u, i], BF16))
             for i in (2, 0, 1)}
        vr_words[u] = pltpu.pack_elementwise([p[0] + p[2], p[1] + p[2]], packed_dtype=BF16)

    def vr_store(u):
        r, tp = divmod(u, 2)
        w = pltpu.bitcast(vr_words[u], F32)
        wt = pltpu.bitcast(_cat([w, w]).T, U32)
        job_done["v", u] = pltpu.bitcast(wt[120:128], F32)
        for j in range(2):
            qkv_ref[4, r, pl.ds((2 * tp + j) * LANES, LANES), :] = pltpu.unpack_elementwise(
                wt, index=j, packed_dtype=BF16, unpacked_dtype=F32)

    zero8 = jnp.zeros((8, LANES), F32)

    def gather(n, off):
        return [qkv_ref[n, r, pl.ds(off, 8), :] for r in range(WS)]

    def softmax_t(st):
        rows = _blocks(st)
        m = functools.reduce(jnp.maximum, rows)
        m = _allred(jnp.where(mk["key"], m, -jnp.inf), jnp.maximum)
        p = [jnp.exp2(x - m) for x in rows]
        return p, functools.reduce(jnp.add, p)

    def s2_pair(pi, offa):
        offb = offa + WS
        st = {}

        def vprep():
            g = [gather(n, offa) + gather(n, offb) for n in range(5)]
            u1 = [jnp.where(mk["left64"], z, jnp.where(mk["v"], x, y)) for x, y, z in zip(g[0], g[1], g[4])]
            u2 = [jnp.where(mk["v"], x, y) for x, y in zip(g[2], g[3])]
            u = jnp.concatenate([_cat(u1 + [zero8, zero8]), _cat(u2 + [zero8, zero8])], axis=1)
            vt = pltpu.bitcast(u.astype(BF16).T, U32)
            vt = _cat([vt[0:64], vt[96:128]])
            st["vt"] = [pltpu.bitcast(vt[24 * h:24 * h + 24], BF16) for h in range(NH)]

        def score(i, after=None, steps=()):
            hp, sw = divmod(i, 2)
            lo, hi = mk["lo"], mk["hi%d" % hp]
            ma, mb = (lo, hi) if sw == 0 else (hi, lo)
            q = _cat([jnp.where(ma, v, 0.0) for v in gather(hp, offa)]
                     + [jnp.where(mb, v, 0.0) for v in gather(hp, offb)] + [zero8, zero8])
            ka, kb = gather(2 + hp, offa), gather(2 + hp, offb)
            k = [jnp.where(lo, x, y) for x, y in (zip(ka, kb) if sw == 0 else zip(kb, ka))]
            if after is not None:
                k[0] = jnp.where(mk["never"], t_done[after], k[0])
            for q_, step in enumerate(steps):
                e = 1 + (q_ * 6) // len(steps)
                k[e] = jnp.where(mk["never"], step(), k[e])
            k = _cat(k)
            st["p", i] = softmax_t(_dot_nt(k, q))

        def value(h):
            hp, sw = divmod(h, 2)
            (pa, sa), (pb, sb) = st["p", 2 * hp + sw], st["p", 2 * hp + 1 - sw]
            pm = _cat([jnp.where(mk["keep_a"], v, 0.0) for v in pa]
                      + [jnp.where(mk["keep_b"], v, 0.0) for v in pb] + [zero8, zero8])
            den = _allred(jnp.where(mk["keep_a"], sa, jnp.where(mk["keep_b"], sb, 0.0)), jnp.add)
            rec = pl.reciprocal(den, approx=True)
            if _env("NR", 0):
                rec = rec * (2.0 - den * rec)
            st["o", h] = [b * rec for b in _blocks(_dot(st["vt"][h], pm))]

        def finish():
            o = [b for h in range(NH) for b in st["o", h]]
            w = pltpu.pack_elementwise([_cat(o[0:16]), _cat(o[16:24] + o[16:24])], packed_dtype=BF16)
            stg_ref[pi] = pltpu.bitcast(w, F32)

        def scatter():
            wt = stg_ref[pi].T
            job_done["s", pi] = wt[104:112]
            for i, off in enumerate((offa, offb)):
                for r in range(WS):
                    base = i * SLOTS + 8 * r
                    ob_ref[pl.ds(r * WP + off, WS), :] = wt[base:base + WS]

        return vprep, score, value, finish, scatter

    npair = (nwin + 1) // 2
    pairs = [s2_pair(p, min(2 * p, nwin - 2) * WS) for p in range(npair)]

    def s3_unit(r, tp, steps=()):
        def unpack(t):
            w = pltpu.bitcast(ob_ref[pl.ds(r * WP + t * LANES, LANES), :], U32)
            return [_blocks(pltpu.unpack_elementwise(w, index=i, packed_dtype=BF16, unpacked_dtype=F32))
                    for i in range(2)]

        (la, ha), (lb, hb) = unpack(2 * tp), unpack(2 * tp + 1)
        t3 = _cat([jnp.where(mk["left64"], x, y) for x, y in zip(lb, ha)])
        t1 = _cat([x - jnp.where(mk["left64"], y, 0.0) for x, y in zip(la, lb)])
        t2 = _cat([jnp.where(mk["left64"], x - y, z) for x, y, z in zip(hb, ha, lb)])
        wo = [_blocks(wos_ref[i]) for i in range(3)]
        e0, e1 = _env("E0", 0), _env("E1", 12)
        for q, step in enumerate(steps):
            q = q * 3 * (e1 - e0) // len(steps)
            blks = wo[(2, 0, 1)[q % 3]]
            blks[e0 + q // 3] = jnp.where(mk["never"], pltpu.bitcast(step(), U32), blks[e0 + q // 3])
        wo = [pltpu.bitcast(_cat(w), BF16) for w in wo]
        p3 = _dot_nt(wo[2], t3)
        ys = [_dot_nt(wo[i], t) + p3
              + x0_ref[rows_at(prv, (r * NT + 2 * tp + i) * C, C), :] for i, t in enumerate((t1, t2))]
        n = min(2 * LANES, W - 2 * tp * LANES)
        o_ref[r, :, pl.ds(2 * tp * LANES, n)] = jnp.concatenate(ys, axis=1).astype(o_ref.dtype)[:, :n]

    s3_all = [functools.partial(s3_unit, r, tp) for tp in range(2) for r in range(WS)]

    def run(prog, extra):
        extra = sorted(extra, key=lambda e: e[0])
        j = 0
        for t0, fn in prog:
            while j < len(extra) and extra[j][0] <= t0:
                extra[j][1]()
                j += 1
            fn()
        for e in extra[j:]:
            e[1]()

    MERGE = _env("MERGE", 0)
    NX3 = _env("NX3", 0)

    NSY = _env("NSY", 0)

    NSTX = _env("NSTX", 28)

    def wave_steps(lo, hi, wave):
        steps = []
        for j0 in range(lo, hi, wave):
            for grp in zip(*[stats_steps(j) for j in range(j0, min(j0 + wave, hi))]):
                steps += grp
        return steps

    def block_x():
        NJ = _env("NJ", 24)
        NSTC = _env("NSTC", 11)
        WAVE = _env("WAVE", 4)
        VRLAG = _env("VRLAG", 200)
        chunks = [(u, n) for u in range(NU) for n in range(4)]
        steps = wave_steps(0, NSTX, WAVE)
        c0 = len(chunks) - NSTC
        vr_at = {min(u * _env("VRSTEP", 2), len(chunks) - 1): u for u in range(NU)}
        plan, t, vr_ready = [], 0, {}
        for k, (u, n) in enumerate(chunks):
            if k == c0:
                t_conv = t
            if k in vr_at:
                plan.append((t, vr_at[k], None, []))
                t += 48
                vr_ready[vr_at[k]] = t + VRLAG
            mine = steps[(k - c0) * len(steps) // NSTC:(k - c0 + 1) * len(steps) // NSTC] if k >= c0 else []
            plan.append((t, u, n, list(mine)))
            t += 96
        ci = conv_items(4 * NJ)
        slow = _env("SLOW", 32.0)
        fast = (t_conv - 4 * NJ * slow) / max(len(ci) - 4 * NJ, 1)
        t_piece = [min(j, 4 * NJ) * slow + max(j - 4 * NJ, 0) * fast for j in range(len(ci) + 1)]
        scat, vrs = list(range(npair - NSY)), list(range(NU))
        jobs = []
        for q in range(NJ):
            if vrs and vr_ready[vrs[0]] <= t_piece[4 * q + 1]:
                jobs.append((t_piece[4 * q + 1], ("v", vrs[0])))
                ci[4 * q].insert(0, functools.partial(vr_store, vrs.pop(0)))
            elif scat:
                jobs.append((t_piece[4 * q + 1], ("s", scat[0])))
                ci[4 * q].insert(0, pairs[scat.pop(0)][4])
        extra = [(t_piece[j + 1], f) for j, fs in enumerate(ci) for f in fs]
        tail = [(("v", u), functools.partial(vr_store, u)) for u in vrs] + [(("s", p), pairs[p][4]) for p in scat]
        for q, (key, f) in enumerate(tail):
            t_q = max(t_conv + 1 + (q // 3) * 128, vr_ready[key[1]] if key[0] == "v" else 0)
            extra.append((t_q, f))
            jobs.append((t_q, key))
        if _env("JDL", 800):
            for t_q, key in jobs:
                later = [e for e in plan if e[2] is not None and e[0] >= t_q + _env("JDL", 800)]
                if later:
                    later[0][3].insert(0, functools.partial(job_done.get, key))
        prog = [(t0, functools.partial(vr_dots, u) if n is None else functools.partial(qkv_chunk, u, n, st))
                for t0, u, n, st in plan]
        run(prog, extra)

    def block_y():
        LSM = _env("LSM", 170)
        LFIN = _env("LFIN", 0)
        SGRP = _env("SGRP", 4)
        VGRP = _env("VGRP", 2)
        TAILGAP = _env("TAILGAP", 500)
        load = [LANES, LANES, 0, 0] if MERGE else [0] * 4
        tm = list(load)
        t_0 = LANES + _env("LQKV", 220) if MERGE else 0
        prog, extra = [], []

        def emit(rows_list, fn, ready=0):
            prog.append((min(tm), fn))
            ends = []
            for rows in rows_list:
                m = load.index(min(load))
                load[m] += rows
                tm[m] = max(tm[m], ready) + rows
                ends.append(tm[m])
            return ends

        fillers = list(s3_all[NX3:])
        total = len(fillers) * 3 * C / 4 + npair * (SLOTS + DH)
        nsc = 4 * npair
        next_s = 0
        s_end, v_end, pend_v = {}, {}, []
        t_done.clear()
        ysteps = wave_steps(NSTX, WS * NT, _env("WAVEY", 2))
        SQ = _env("SQ", 110)
        sy0, sy1 = _env("SY0", 14), _env("SY1", 70)
        sdl = {sy0 + q * (sy1 - sy0) // max(NSY, 1): npair - NSY + q for q in range(NSY)}
        S3Q = _env("S3Q", 10)
        if S3Q:
            fillers = [functools.partial(f, ysteps[q * len(ysteps) // S3Q:(q + 1) * len(ysteps) // S3Q])
                       for q, f in enumerate(fillers)]
            ysteps = []
        d0, d1 = _env("TD0", 16), _env("TD1", 0)
        dl = {d0 + j * (nsc + d1 - d0) // len(t_items): j for j in range(len(t_items))}
        while fillers or next_s < nsc or pend_v:
            now = tm[load.index(min(load))]
            s_ok = next_s < nsc and now >= t_0 + (total - TAILGAP - t_0) * next_s / (nsc - 4)
            v_ok = len(pend_v) >= VGRP // 2 and all(now >= x[0] for x in pend_v[:VGRP // 2])
            if not fillers and not s_ok and not v_ok:
                if pend_v and (next_s >= nsc or len(pend_v) >= 4):
                    v_ok = True
                else:
                    s_ok = True
            if v_ok:
                for rdy, pv, hp in pend_v[:VGRP // 2]:
                    for h in (2 * hp, 2 * hp + 1):
                        v_end[pv, h] = emit([DH], functools.partial(pairs[pv][2], h), rdy)[0]
                    if hp == 1:
                        extra.append((max(v_end[pv, h] for h in range(NH)) + LFIN, pairs[pv][3]))
                pend_v = pend_v[VGRP // 2:]
            elif s_ok:
                for _ in range(SGRP):
                    p, i = divmod(next_s, 4)
                    if i == 0:
                        prog.append((min(tm), pairs[p][0]))
                    sj = []
                    if next_s in sdl:
                        extra.append((min(tm) - _env("TLEAD", 300), pairs[sdl[next_s]][4]))
                        sj = [functools.partial(job_done.get, ("s", sdl[next_s]))]
                    if next_s in dl:
                        extra.append((min(tm) - _env("TLEAD", 300), t_items[dl[next_s]]))
                    s_end[p, i] = emit([SLOTS], functools.partial(
                        pairs[p][1], i, dl.get(next_s),
                        ysteps[next_s * len(ysteps) // SQ:(next_s + 1) * len(ysteps) // SQ] + sj))[0]
                    if i % 2 == 1:
                        pend_v.append((max(s_end[p, i], s_end[p, i - 1]) + LSM, p, i // 2))
                    next_s += 1
            else:
                emit([C] * 3, fillers.pop(0))
        extra += [(max(tm) - 600, t_items[j]) for q, j in dl.items() if q >= nsc]
        run(prog, extra)

    only = _env("ONLY", "01")
    NODMA = _env("NODMA", 0)

    @when(k_ < (1 if NODMA & 1 else nstrip), ("first", "main"))
    def _():
        x_copy(k_).wait()

    new_masks()
    if "0" in only:
        when(k_ <= nstrip, ("main",))(block_x)

    @when(k_ == 0, ("first",))
    def _():
        def body(g, carry):
            for j in range(FG):
                piece = conv_group(pl.multiple_of((g * FG + j) * 8, 8))[1]
                for r in range(WS):
                    piece(r)
            return carry
        FG = _env("FG", 8)
        lax.fori_loop(0, NG // FG, body, 0)

    @when(k_ < (0 if NODMA & 1 else nstrip - 1), ("first", "main"))
    def _():
        x_copy(k_ + 1).start()

    @when(k_ >= (1000 if NODMA & 2 else 3), ("main", "last"))
    def _():
        o_copy(k_ - 3).wait()

    if "1" in only:
        new_masks()
        when((k_ <= nstrip) & (k_ >= 1), ("main",))(block_y)

    @when(k_ == 0, ("first",))
    def _():
        for j in range(WS * NT):
            for f in stats_steps(j):
                f()
        for f in t_items:
            f()

    @when(k_ == nstrip + 1, ("last",))
    def _():
        new_masks()
        for p in range(npair):
            pairs[p][4]()
        for f in s3_all:
            f()
        if only != "01":
            i = pl.multiple_of(dyn0 * 8, 8)
            ob_ref[0:8, :] = (qkv_ref[dyn0, dyn0, pl.ds(i, 8), :]
                              + pltpu.bitcast(t_ref[dyn0, dyn0, pl.ds(i, 8), :], F32))

    @when(k_ >= (nstrip + 1 if NODMA & 2 else 2), ("main", "last"))
    def _():
        o_copy(k_ - 2).start()

    @when(k_ == nstrip + 1, ("last",))
    def _():
        o_copy(k_ - 2).wait()


@jax.jit
def pallas_standalone__window_attn_davit__vision_kernel(
    x: jax.Array,
    dw_pe: jax.Array,
    w_qkv: jax.Array,
    w_o: jax.Array,
):
    B, H, W, Cx = x.shape
    assert B == 1 and Cx == C and H % WS == 0 and W % WS == 0 and WP - LANES < W < WP
    xt = jnp.transpose(x[0], (0, 2, 1))

    assert H // WS + 2 <= 256
    vmem = pl.BlockSpec(memory_space=pltpu.VMEM)
    yt = pl.pallas_call(
        functools.partial(_kernel, H=H, W=W),
        in_specs=[pl.BlockSpec(memory_space=pl.ANY), vmem, vmem, vmem],
        out_specs=pl.BlockSpec(memory_space=pl.ANY),
        out_shape=jax.ShapeDtypeStruct((H, C, W), x.dtype),
        scratch_shapes=[
            pltpu.VMEM((WS + 1, C, W), x.dtype),
            pltpu.VMEM((WS, C, W), x.dtype),
            pltpu.SemaphoreType.DMA((2,)),
            pltpu.VMEM((X0_ROWS, LANES), F32),
            pltpu.VMEM((WS * WP, LANES), F32),
            pltpu.VMEM((9, C, LANES), F32),
            pltpu.VMEM((3, 5, LANES // 2, LANES), U32),
            pltpu.VMEM((3, C // 2, LANES), U32),
            pltpu.VMEM((5, WS, WP, LANES), F32),
            pltpu.VMEM((NU, 3, LANES // 2, LANES), U32),
            pltpu.VMEM((37, LANES, LANES), F32),
            pltpu.VMEM((WS * NT, 16, LANES), F32),
            pltpu.VMEM((C, WP), F32),
        ],
        compiler_params=pltpu.CompilerParams(
            vmem_limit_bytes=64 * 1024 * 1024,
            disable_bounds_checks=bool(_env("NOBC", 1)),
        ),
        name="davit_window_attn",
    )(xt, dw_pe, w_qkv, w_o)
    return jnp.transpose(yt, (0, 2, 1))[None]
```

```python
import functools
import math
import os

import jax
import jax.numpy as jnp
from jax import lax
import jax.experimental.pallas as pl
import jax.experimental.pallas.tpu as pltpu

WS = 7
NH = 4
C = 192
DH = C // NH
NG = C // 8
LANES = 128
WP = 512
NT = WP // LANES
NU = WS * NT // 2
SLOTS = 8 * WS
EPS = 1e-5
F32 = jnp.float32
BF16 = jnp.bfloat16
U32 = jnp.uint32

X0_SLOT = WS * NT * C
DW_OFF = 3 * X0_SLOT
X0_ROWS = DW_OFF + 2 * C


def _dot(a, b):
    return jnp.dot(a, b, preferred_element_type=F32)


def _dot_nt(a, b):
    return lax.dot_general(a, b, (((1,), (1,)), ((), ())), preferred_element_type=F32)


def _cat(xs):
    return jnp.concatenate(xs, axis=0)


def _blocks(v):
    return [v[i:i + 8] for i in range(0, v.shape[0], 8)]


def _allred(x, op):
    for sh in (4, 2, 1):
        x = op(x, pltpu.roll(x, sh, 0))
    return x


def _env(name, default):
    return type(default)(os.environ.get(name, default))


def _kernel(x_hbm, dw_ref, wqkv_ref, wo_ref, o_hbm, *scratch, H, W):
    step = functools.partial(_step, x_hbm, dw_ref, wqkv_ref, wo_ref, o_hbm, *scratch, H=H, W=W)
    nstrip = H // WS

    def loop(lo, hi, mode):
        def body(k, carry):
            step(k_=k, mode=mode)
            return carry
        lax.fori_loop(lo, hi, body, 0)

    loop(0, 1, "first")
    loop(1 + _env("SKIP", 0), nstrip + 1, "main")
    loop(nstrip + 1, nstrip + 2, "last")


def _step(x_hbm, dw_ref, wqkv_ref, wo_ref, o_hbm,
          x_ref, o_ref, sems, x0_ref, ob_ref, dws_ref, ws_ref, wos_ref, qkv_ref, t_ref, stg_ref, ms_ref,
          top_ref, *, H, W, k_, mode):
    nstrip, nwin = H // WS, W // WS

    def x_copy(k):
        return pltpu.make_async_copy(x_hbm.at[pl.ds(jnp.minimum(k * WS, H - WS - 1), WS + 1)],
                                     x_ref.at[pl.ds(0, WS + 1)], sems.at[0])

    def o_copy(k):
        return pltpu.make_async_copy(o_ref, o_hbm.at[pl.ds(k * WS, WS)], sems.at[1])

    def when(cond, modes):
        if mode in modes:
            return pl.when(cond)
        return lambda f: None

    xoff = jnp.where(k_ >= nstrip - 1, 1, 0)
    dyn0 = jnp.minimum(k_, 0)

    def rows_at(base, off, n):
        if isinstance(base, int):
            return pl.ds(base + off, n)
        return pl.ds(pl.multiple_of(base + off, 8), n)

    mk = {}

    def new_masks(blk):
        lane = lax.broadcasted_iota(jnp.int32, (8, LANES), 1)
        mk.clear()
        mk["never"] = lane < dyn0
        if blk == "x":
            mk["up"] = lax.broadcasted_iota(jnp.int32, (8, LANES), 0) < 4
            return
        key_ok = lax.broadcasted_iota(jnp.int32, (8, LANES), 0) < WS
        mk.update(
            lo=lane < DH, hi0=(lane >= DH) & ((lane < 64) | (lane >= 96)), hi1=(lane >= DH) & (lane < 96),
            v=lane < 96, key=key_ok, keep_a=key_ok & (lane < SLOTS), keep_b=key_ok & (lane >= SLOTS),
            left64=lane < 64)

    k3 = k_ - 3 * ((k_ * 171) >> 9)
    nxt = k3 * X0_SLOT
    prv = jnp.where((k3 == 2) | (k_ < 2), 0, nxt + X0_SLOT)

    def conv_group(c0):
        st = {}

        def row(i):
            if i == 0 and i not in st:
                st[i] = top_ref[pl.ds(c0, 8), :]
            if i not in st:
                v = x_ref[xoff + (i - 1), pl.ds(c0, 8), :].astype(F32)
                st[i] = jnp.concatenate([v, jnp.zeros((8, WP - W), F32)], axis=1)
                if i == WS and i - 2 in st:
                    top_ref[pl.ds(c0, 8), :] = st[i]
            return st[i]

        def bc(v):
            return jnp.concatenate([v] * NT, axis=1)

        def taps(r):
            st["tw", r] = [bc(x0_ref[rows_at(c0, DW_OFF + k * C, 8), :]) for k in range(2)]

        def piece(r):
            if "w" not in st:
                st["w"] = [bc(dws_ref[k, pl.ds(c0, 8), :]) for k in range(9)]
            wts = list(st["w"])
            if ("tw", r) in st:
                wts[6], wts[8] = st["tw", r]
            row(r)
            abc = [row(r + 1) * wts[3 + j] + row(r) * wts[j] + row(r + 2) * wts[6 + j] for j in range(3)]
            x0 = pltpu.roll(abc[0], 1, 1) + abc[1] + pltpu.roll(abc[2], WP - 1, 1)
            for t in range(NT):
                x0_ref[rows_at(nxt, (r * NT + t) * C + c0, 8), :] = x0[:, t * LANES:(t + 1) * LANES]

        return taps, piece

    @when(k_ == 0, ("first",))
    def _():
        x_copy(0).start()
        for k in range(9):
            w = dw_ref[k // 3].astype(F32)[k % 3:k % 3 + 1, :]
            w = jnp.broadcast_to(w, (LANES, C)).T
            dws_ref[k] = w + 1.0 if k == 4 else w
            if k in (6, 8):
                x0_ref[pl.ds(DW_OFF + (k - 6) // 2 * C, C), :] = w
        w = wqkv_ref[...].astype(F32)
        wq = w[:, 0:C] * ((DH ** -0.5) * math.log2(math.e))
        wk, wv = w[:, C:2 * C], w[:, 2 * C:3 * C]
        tiles = [(wq[:, 0:64], wv[:, 64:96], wq[:, 64:96]),
                 (wq[:, 96:192], wv[:, 96:128]),
                 (wk[:, 0:64], wv[:, 128:160], wk[:, 64:96]),
                 (wk[:, 96:192], wv[:, 160:192]),
                 (wv[:, 0:128],)]
        for n, parts in enumerate(tiles):
            w = jnp.concatenate(parts, axis=1)
            for i, wi in enumerate((w[0:128], w[64:192], _cat([w[0:64], w[128:192]]))):
                if n == 4:
                    wi = wi.T
                ws_ref[i, n] = pltpu.bitcast(wi.astype(BF16), U32)
        w = wo_ref[...].astype(F32)
        wx, wy, wz = w[0:64], w[64:128], w[128:192]
        for i, parts in enumerate(((wx, wy), (wz, wy), (wx, wz))):
            wos_ref[i] = pltpu.bitcast(_cat(parts).T.astype(BF16), U32)

        top_ref[...] = jnp.zeros(top_ref.shape, F32)
        x_ref[WS + 1] = jnp.zeros(x_ref.shape[1:], x_ref.dtype)

        for r in range(WS):
            ob_ref[pl.ds(r * WP + WP - 8, 8), :] = jnp.zeros((8, LANES), F32)

    cuts = [int(c) for c in _env("CUTS", "0,7").split(",")]
    bands = list(zip(cuts, cuts[1:]))
    groups = {(b, g): conv_group(8 * g) for b in range(len(bands)) for g in range(NG)}
    WLEAD = _env("WLEAD", 4)

    def conv_items(nslow):
        plist = [((b, g), r) for b, (r0, r1) in enumerate(bands) for g in range(NG) for r in range(r0, r1)]
        items, nxt_tap = [], WLEAD
        for k, (g, r) in enumerate(plist):
            fs = []
            lead = WLEAD if k < nslow else _env("WLEAD2", 6)
            while nxt_tap <= min(k + lead, len(plist) - 1):
                g2, r2 = plist[nxt_tap]
                fs.append(functools.partial(groups[g2][0], r2))
                nxt_tap += 1
            fs.append(functools.partial(groups[g][1], r))
            items.append(fs)
        return items

    def ld_x0(j, k, gs=range(NG)):
        return [x0_ref[rows_at(nxt + dyn0 * (8 * k), j * C + 8 * g, 8), :] for g in gs]

    def add2(acc, xs):
        a = functools.reduce(jnp.add, xs[0::2])
        b = functools.reduce(jnp.add, xs[1::2])
        return a + b if acc is None else (acc + a) + b

    stats_done = set()

    def stats_steps(j):
        st = {"s": None, "q": None}
        n1, n2 = _env("SEG1", 8), _env("SEG2", 8)

        def sum_step(g0):
            st["s"] = add2(st["s"], ld_x0(j, 0, range(g0, g0 + n1)))
            if g0 + n1 == NG:
                st["s"] = _allred(st["s"], jnp.add) * (1.0 / C)
            return st["s"]

        def var_step(g0):
            d = [x - st["s"] for x in ld_x0(j, 1, range(g0, g0 + n2))]
            st["q"] = add2(st["q"], [x * x for x in d])
            return st["q"]

        def last_step():
            rs = lax.rsqrt(_allred(st["q"], jnp.add) * (1.0 / C) + EPS)
            ms_ref[j] = _cat([st["s"], rs])
            stats_done.add(j)
            return rs

        return ([functools.partial(sum_step, g) for g in range(0, NG, n1)]
                + [functools.partial(var_step, g) for g in range(0, NG, n2)] + [last_step])

    def colsum(xs):
        xs = [a + b for a, b in zip(xs[0:8], xs[16:24])] + xs[8:16]
        return _dot(jnp.ones((8, LANES), F32), _cat(xs))

    means = {}

    def mean_dot(j):
        means[j] = colsum(ld_x0(j, 0)) * (1.0 / C)

    def var_dot(j):
        xs = [x0_ref[pl.ds(nxt + (j * C + 8 * g + 4), 8), :] for g in range(NG - 1)]
        xs.append(jnp.where(mk["up"], *ld_x0(j, 0, (0, NG - 1))))
        d = [x - means[j] for x in xs]
        v = colsum([x * x for x in d]) * (1.0 / C) + EPS
        rs = lax.rsqrt(v) if _env("RSQ", 1) else jnp.exp2(jnp.log2(v) * -0.5)
        ms_ref[j] = _cat([means[j], rs])
        stats_done.add(j)

    def normed(j, blk, k):
        assert j in stats_done or "ONLY" in os.environ and j < NSTX, j
        m, rs = ms_ref[j, 0:8, :], ms_ref[j, 8:16, :]
        return _cat([(x - m) * rs for x in ld_x0(j, k, range(8 * blk, 8 * blk + 8))])

    t_done = []

    def put_t(dst, tiles):
        tt = pltpu.bitcast(jnp.concatenate(tiles, axis=1).astype(BF16).T, U32)
        for i, (u, e) in enumerate(dst):
            t_ref[u, e] = tt[64 * i:64 * i + 64]
        t_done.append(pltpu.bitcast(tt[120:128], F32))

    def t_first(u):
        ja, jb = 2 * u, 2 * u + 1
        bx = normed(jb, 0, 0)
        put_t([(u, 0), (u, 2)], [_cat([normed(ja, 0, 0) - bx, normed(ja, 1, 0)]),
                                 _cat([bx, normed(ja, 2, 0)])])

    def t_second(r):
        put_t([(u, 1) for u in (2 * r, 2 * r + 1)],
              [_cat([normed(2 * u + 1, 1, 0), normed(2 * u + 1, 2, 0) - normed(2 * u, 2, _env("RECOMP", 1))])
               for u in (2 * r, 2 * r + 1)])

    t_items = []
    for r in range(WS):
        t_items += [functools.partial(t_first, 2 * r), functools.partial(t_first, 2 * r + 1),
                    functools.partial(t_second, r)]

    def qkv_chunk(u, n, steps=(), tiny=()):
        r, tp = divmod(u, 2)
        ops = {i: [_blocks(t_ref[u, i]), _blocks(ws_ref[i, n])] for i in range(3)}
        side = 1 if _env("ATT", "l") == "w" else 0
        for q, step in enumerate(steps):
            tok = pltpu.bitcast(step(), U32)
            q = q * 24 // len(steps)
            blks = ops[(2, 0, 1)[q % 3]][side]
            e = 7 - q // 3 if side else q // 3
            blks[e] = jnp.where(mk["never"], tok, blks[e])
        p3 = None
        for q, i in enumerate((2, 0, 1)):
            for f in tiny[q * len(tiny) // 3:(q + 1) * len(tiny) // 3]:
                f()
            p = _dot(*[pltpu.bitcast(_cat(x), BF16) for x in ops[i]])
            if p3 is None:
                p3 = p
            else:
                qkv_ref[n, r, pl.ds((2 * tp + i) * LANES, LANES), :] = p + p3

    vr_words = {}
    job_done = {}

    def side_dots(u, n):
        r, tp = divmod(u, 2)
        st = {}

        def one(i, parts=1):
            if parts > 1:
                lhs, rows = t_ref[u, i], 64 // parts
                p = _cat([_dot(pltpu.bitcast(lhs[q * rows:(q + 1) * rows], BF16),
                               pltpu.bitcast(ws_ref[i, n], BF16)) for q in range(parts)])
            elif n == 4:
                p = _dot_nt(pltpu.bitcast(ws_ref[i, 4, 0:32, :], BF16), pltpu.bitcast(t_ref[u, i], BF16))
            else:
                p = _dot(pltpu.bitcast(t_ref[u, i], BF16), pltpu.bitcast(ws_ref[i, n], BF16))
            st[i] = p if i == 2 else p + st[2]
            if n < 4 and i < 2:
                qkv_ref[n, r, pl.ds((2 * tp + i) * LANES, LANES), :] = st[i]
            elif i == 1:
                vr_words[u] = pltpu.pack_elementwise([st[0], st[1]], packed_dtype=BF16)

        return [(64 if n == 4 else LANES, (u, n, i), functools.partial(one, i)) for i in (2, 0, 1)]

    def vr_store(u):
        r, tp = divmod(u, 2)
        w = pltpu.bitcast(vr_words[u], F32)
        wt = pltpu.bitcast(_cat([w, w]).T, U32)
        job_done["v", u] = pltpu.bitcast(wt[120:128], F32)
        for j in range(2):
            qkv_ref[4, r, pl.ds((2 * tp + j) * LANES, LANES), :] = pltpu.unpack_elementwise(
                wt, index=j, packed_dtype=BF16, unpacked_dtype=F32)

    zero8 = jnp.zeros((8, LANES), F32)

    def gather(n, off):
        return [qkv_ref[n, r, pl.ds(off, 8), :] for r in range(WS)]

    def softmax_t(st):
        rows = _blocks(st)
        m = functools.reduce(jnp.maximum, rows)
        m = _allred(jnp.where(mk["key"], m, -jnp.inf), jnp.maximum)
        p = [jnp.exp2(x - m) for x in rows]
        return p, functools.reduce(jnp.add, p)

    def s2_pair(pi, offa):
        offb = offa + WS
        st = {}

        def vprep():
            g = [gather(n, offa) + gather(n, offb) for n in range(5)]
            u1 = [jnp.where(mk["left64"], z, jnp.where(mk["v"], x, y)) for x, y, z in zip(g[0], g[1], g[4])]
            u2 = [jnp.where(mk["v"], x, y) for x, y in zip(g[2], g[3])]
            u = jnp.concatenate([_cat(u1 + [zero8, zero8]), _cat(u2 + [zero8, zero8])], axis=1)
            vt = pltpu.bitcast(u.astype(BF16).T, U32)
            vt = _cat([vt[0:64], vt[96:128]])
            st["vt"] = [pltpu.bitcast(vt[24 * h:24 * h + 24], BF16) for h in range(NH)]

        def score(i, after=None, steps=()):
            hp, sw = divmod(i, 2)
            lo, hi = mk["lo"], mk["hi%d" % hp]
            ma, mb = (lo, hi) if sw == 0 else (hi, lo)
            q = _cat([jnp.where(ma, v, 0.0) for v in gather(hp, offa)]
                     + [jnp.where(mb, v, 0.0) for v in gather(hp, offb)] + [zero8, zero8])
            ka, kb = gather(2 + hp, offa), gather(2 + hp, offb)
            k = [jnp.where(lo, x, y) for x, y in (zip(ka, kb) if sw == 0 else zip(kb, ka))]
            if after is not None:
                k[0] = jnp.where(mk["never"], t_done[after], k[0])
            for q_, step in enumerate(steps):
                e = 1 + (q_ * 6) // len(steps)
                k[e] = jnp.where(mk["never"], step(), k[e])
            k = _cat(k)
            st["p", i] = softmax_t(_dot_nt(k, q))

        def value(h):
            hp, sw = divmod(h, 2)
            (pa, sa), (pb, sb) = st["p", 2 * hp + sw], st["p", 2 * hp + 1 - sw]
            pm = _cat([jnp.where(mk["keep_a"], v, 0.0) for v in pa]
                      + [jnp.where(mk["keep_b"], v, 0.0) for v in pb] + [zero8, zero8])
            den = _allred(jnp.where(mk["keep_a"], sa, jnp.where(mk["keep_b"], sb, 0.0)), jnp.add)
            rec = pl.reciprocal(den, approx=True)
            if _env("NR", 0):
                rec = rec * (2.0 - den * rec)
            st["o", h] = [b * rec for b in _blocks(_dot(st["vt"][h], pm))]

        def finish():
            o = [b for h in range(NH) for b in st["o", h]]
            w = pltpu.pack_elementwise([_cat(o[0:16]), _cat(o[16:24] + o[16:24])], packed_dtype=BF16)
            stg_ref[pi] = pltpu.bitcast(w, F32)

        def scatter():
            wt = stg_ref[pi].T
            job_done["s", pi] = wt[104:112]
            for i, off in enumerate((offa, offb)):
                for r in range(WS):
                    base = i * SLOTS + 8 * r
                    ob_ref[pl.ds(r * WP + off, WS), :] = wt[base:base + WS]

        return vprep, score, value, finish, scatter

    npair = (nwin + 1) // 2
    pairs = [s2_pair(p, min(2 * p, nwin - 2) * WS) for p in range(npair)]

    def s3_unit(r, tp, steps=()):
        def unpack(t):
            w = pltpu.bitcast(ob_ref[pl.ds(r * WP + t * LANES, LANES), :], U32)
            return [_blocks(pltpu.unpack_elementwise(w, index=i, packed_dtype=BF16, unpacked_dtype=F32))
                    for i in range(2)]

        (la, ha), (lb, hb) = unpack(2 * tp), unpack(2 * tp + 1)
        t3 = _cat([jnp.where(mk["left64"], x, y) for x, y in zip(lb, ha)])
        t1 = _cat([x - jnp.where(mk["left64"], y, 0.0) for x, y in zip(la, lb)])
        t2 = _cat([jnp.where(mk["left64"], x - y, z) for x, y, z in zip(hb, ha, lb)])
        wo = [_blocks(wos_ref[i]) for i in range(3)]
        e0, e1 = _env("E0", 0), _env("E1", 12)
        for q, step in enumerate(steps):
            q = q * 3 * (e1 - e0) // len(steps)
            blks = wo[(2, 0, 1)[q % 3]]
            blks[e0 + q // 3] = jnp.where(mk["never"], pltpu.bitcast(step(), U32), blks[e0 + q // 3])
        wo = [pltpu.bitcast(_cat(w), BF16) for w in wo]
        p3 = _dot_nt(wo[2], t3)
        ys = [_dot_nt(wo[i], t) + p3
              + x0_ref[rows_at(prv, (r * NT + 2 * tp + i) * C, C), :] for i, t in enumerate((t1, t2))]
        n = min(2 * LANES, W - 2 * tp * LANES)
        o_ref[r, :, pl.ds(2 * tp * LANES, n)] = jnp.concatenate(ys, axis=1).astype(o_ref.dtype)[:, :n]

    s3_all = [functools.partial(s3_unit, r, tp) for tp in range(2) for r in range(WS)]

    def run(prog, extra):
        extra = sorted(extra, key=lambda e: e[0])
        j = 0
        for t0, fn in prog:
            while j < len(extra) and extra[j][0] <= t0:
                extra[j][1]()
                j += 1
            fn()
        for e in extra[j:]:
            e[1]()

    MERGE = _env("MERGE", 0)
    NX3 = _env("NX3", 0)

    NSY = _env("NSY", 0)

    NSTX = _env("NSTX", 28)

    def wave_steps(lo, hi, wave):
        steps = []
        for j0 in range(lo, hi, wave):
            for grp in zip(*[stats_steps(j) for j in range(j0, min(j0 + wave, hi))]):
                steps += grp
        return steps

    def block_x():
        NJ = _env("NJ", 24)
        NSTC = _env("NSTC", 8)
        WAVE = _env("WAVE", 4)
        VRLAG = _env("VRLAG", 200)
        chunks = [(u, n) for u in range(NU) for n in range(4)]
        MXS = _env("MXS", 0)
        steps = [] if MXS else wave_steps(0, NSTX, WAVE)
        nside = 9
        side, vstep = [], _env("VRSTEP", 1)
        for q in range(NU // 2):
            side += side_dots(2 * q, 4) + side_dots(2 * q + 1, 4)
            for _ in range(vstep):
                if nside:
                    side += side_dots(*chunks.pop())
                    nside -= 1
        for _ in range(nside):
            side += side_dots(*chunks.pop())
        c0 = len(chunks) - NSTC
        plan, t, vr_ready = [], 0, {}
        for k, (u, n) in enumerate(chunks):
            if k == c0:
                t_conv = t
            mine = steps[(k - c0) * len(steps) // NSTC:(k - c0 + 1) * len(steps) // NSTC] if k >= c0 else []
            plan.append((t, u, n, list(mine), []))
            room = LANES
            while side and (room > 0 or k == len(chunks) - 1):
                rows, key, f = side.pop(0)
                plan.append((t, f if room > 0 else functools.partial(f, 4), None, [], []))
                room -= rows
                if key[1:] == (4, 1):
                    vr_ready[key[0]] = t + LANES - room + VRLAG
            t += LANES
        ci = conv_items(4 * NJ)
        slow = _env("SLOW", 32.0)
        fast = (t_conv - 4 * NJ * slow) / max(len(ci) - 4 * NJ, 1)
        t_piece = [min(j, 4 * NJ) * slow + max(j - 4 * NJ, 0) * fast for j in range(len(ci) + 1)]
        scat, vrs = list(range(npair - NSY)), list(range(NU))
        jobs = []
        for q in range(NJ):
            if vrs and vr_ready[vrs[0]] <= t_piece[4 * q + 1]:
                jobs.append((t_piece[4 * q + 1], ("v", vrs[0])))
                ci[4 * q].insert(0, functools.partial(vr_store, vrs.pop(0)))
            elif scat:
                jobs.append((t_piece[4 * q + 1], ("s", scat[0])))
                ci[4 * q].insert(0, pairs[scat.pop(0)][4])
        extra = [(t_piece[j + 1], f) for j, fs in enumerate(ci) for f in fs]
        tail = [(("v", u), functools.partial(vr_store, u)) for u in vrs] + [(("s", p), pairs[p][4]) for p in scat]
        for q, (key, f) in enumerate(tail):
            t_q = max(t_conv + 1 + (q // 3) * 128, vr_ready[key[1]] if key[0] == "v" else 0)
            extra.append((t_q, f))
            jobs.append((t_q, key))
        if MXS:
            todo = []
            for r0, r1 in bands:
                todo += [(t_piece[r1 * NG] + _env("BLAG", 300), 0, j) for j in range(r0 * NT, r1 * NT)]
            for e in plan:
                room = 0 if e[2] is None else _env("ROOM", 3) if e[0] < t_conv else _env("ROOM2", 6)
                fin = e[1:3] == chunks[-1]
                if fin:
                    room = 1000
                while room and todo and (todo[0][0] <= e[0] or fin):
                    _, kind, j = todo.pop(0)
                    e[4].append(functools.partial((mean_dot, var_dot)[kind], j))
                    if kind == 0:
                        todo.append((e[0] + _env("VLAG", 250), 1, j))
                        todo.sort()
                    room -= 1
        if _env("JDL", 800):
            for t_q, key in jobs:
                later = [e for e in plan if e[2] is not None and e[0] >= t_q + _env("JDL", 800)]
                if later:
                    later[0][3].insert(0, functools.partial(job_done.get, key))
        prog = [(t0, u if n is None else functools.partial(qkv_chunk, u, n, st, tn))
                for t0, u, n, st, tn in plan]
        run(prog, extra)

    def block_y():
        LSM = _env("LSM", 170)
        LFIN = _env("LFIN", 0)
        SGRP = _env("SGRP", 4)
        VGRP = _env("VGRP", 2)
        TAILGAP = _env("TAILGAP", 500)
        load = [LANES, LANES, 0, 0] if MERGE else [0] * 4
        tm = list(load)
        t_0 = LANES + _env("LQKV", 220) if MERGE else 0
        prog, extra = [], []

        def emit(rows_list, fn, ready=0):
            prog.append((min(tm), fn))
            ends = []
            for rows in rows_list:
                m = load.index(min(load))
                load[m] += rows
                tm[m] = max(tm[m], ready) + rows
                ends.append(tm[m])
            return ends

        fillers = list(s3_all[NX3:])
        total = len(fillers) * 3 * C / 4 + npair * (SLOTS + DH)
        nsc = 4 * npair
        next_s = 0
        s_end, v_end, pend_v = {}, {}, []
        t_done.clear()
        ysteps = wave_steps(NSTX, WS * NT, _env("WAVEY", 2))
        SQ = _env("SQ", 110)
        sy0, sy1 = _env("SY0", 14), _env("SY1", 70)
        sdl = {sy0 + q * (sy1 - sy0) // max(NSY, 1): npair - NSY + q for q in range(NSY)}
        S3Q = _env("S3Q", 10)
        if S3Q:
            fillers = [functools.partial(f, ysteps[q * len(ysteps) // S3Q:(q + 1) * len(ysteps) // S3Q])
                       for q, f in enumerate(fillers)]
            ysteps = []
        d0, d1 = _env("TD0", 16), _env("TD1", 0)
        dl = {d0 + j * (nsc + d1 - d0) // len(t_items): j for j in range(len(t_items))}
        while fillers or next_s < nsc or pend_v:
            now = tm[load.index(min(load))]
            s_ok = next_s < nsc and now >= t_0 + (total - TAILGAP - t_0) * next_s / (nsc - 4)
            v_ok = len(pend_v) >= VGRP // 2 and all(now >= x[0] for x in pend_v[:VGRP // 2])
            if not fillers and not s_ok and not v_ok:
                if pend_v and (next_s >= nsc or len(pend_v) >= 4):
                    v_ok = True
                else:
                    s_ok = True
            if v_ok:
                for rdy, pv, hp in pend_v[:VGRP // 2]:
                    for h in (2 * hp, 2 * hp + 1):
                        v_end[pv, h] = emit([DH], functools.partial(pairs[pv][2], h), rdy)[0]
                    if hp == 1:
                        extra.append((max(v_end[pv, h] for h in range(NH)) + LFIN, pairs[pv][3]))
                pend_v = pend_v[VGRP // 2:]
            elif s_ok:
                for _ in range(SGRP):
                    p, i = divmod(next_s, 4)
                    if i == 0:
                        prog.append((min(tm), pairs[p][0]))
                    sj = []
                    if next_s in sdl:
                        extra.append((min(tm) - _env("TLEAD", 300), pairs[sdl[next_s]][4]))
                        sj = [functools.partial(job_done.get, ("s", sdl[next_s]))]
                    if next_s in dl:
                        extra.append((min(tm) - _env("TLEAD", 300), t_items[dl[next_s]]))
                    s_end[p, i] = emit([SLOTS], functools.partial(
                        pairs[p][1], i, dl.get(next_s),
                        ysteps[next_s * len(ysteps) // SQ:(next_s + 1) * len(ysteps) // SQ] + sj))[0]
                    if i % 2 == 1:
                        pend_v.append((max(s_end[p, i], s_end[p, i - 1]) + LSM, p, i // 2))
                    next_s += 1
            else:
                emit([C] * 3, fillers.pop(0))
        extra += [(max(tm) - 600, t_items[j]) for q, j in dl.items() if q >= nsc]
        run(prog, extra)

    only = _env("ONLY", "01")
    NODMA = _env("NODMA", 0)

    @when(k_ < (1 if NODMA & 1 else nstrip), ("first", "main"))
    def _():
        x_copy(k_).wait()

    new_masks("x")
    if "0" in only:
        when(k_ <= nstrip, ("main",))(block_x)

    @when(k_ == 0, ("first",))
    def _():
        def body(g, carry):
            for j in range(FG):
                piece = conv_group(pl.multiple_of((g * FG + j) * 8, 8))[1]
                for r in range(WS):
                    piece(r)
            return carry
        FG = _env("FG", 8)
        lax.fori_loop(0, NG // FG, body, 0)

    @when(k_ < (0 if NODMA & 1 else nstrip - 1), ("first", "main"))
    def _():
        x_copy(k_ + 1).start()

    @when(k_ >= (1000 if NODMA & 2 else 3), ("main", "last"))
    def _():
        o_copy(k_ - 3).wait()

    if "1" in only:
        new_masks("y")
        when((k_ <= nstrip) & (k_ >= 1), ("main",))(block_y)

    @when(k_ == 0, ("first",))
    def _():
        for j in range(WS * NT):
            for f in stats_steps(j):
                f()
        for f in t_items:
            f()

    @when(k_ == nstrip + 1, ("last",))
    def _():
        new_masks("y")
        for p in range(npair):
            pairs[p][4]()
        for f in s3_all:
            f()

    if only != "01":
        @when(dyn0 < 0, ("main",))
        def _():
            i = pl.multiple_of(k_ * 8, 8)
            o_ref[0, 0:16, 0:128] = _cat([
                qkv_ref[k3, k3, pl.ds(i, 8), :] + ms_ref[k3, 0:8, :] + stg_ref[k3, pl.ds(i, 8), :],
                pltpu.bitcast(t_ref[k3, k3, pl.ds(i, 8), :], F32) + ob_ref[pl.ds(i, 8), :]]).astype(BF16)
            for rf in (qkv_ref.at[k3, k3], stg_ref.at[k3], ob_ref):
                rf[pl.ds(i, 8), :] = zero8
            t_ref[k3, k3, pl.ds(i, 8), :] = pltpu.bitcast(zero8, U32)

    @when(k_ >= (nstrip + 1 if NODMA & 2 else 2), ("main", "last"))
    def _():
        o_copy(k_ - 2).start()

    @when(k_ == nstrip + 1, ("last",))
    def _():
        o_copy(k_ - 2).wait()


@jax.jit
def pallas_standalone__window_attn_davit__vision_kernel(
    x: jax.Array,
    dw_pe: jax.Array,
    w_qkv: jax.Array,
    w_o: jax.Array,
):
    B, H, W, Cx = x.shape
    assert B == 1 and Cx == C and H % WS == 0 and W % WS == 0 and WP - LANES < W < WP
    xt = jnp.transpose(x[0], (0, 2, 1))

    assert H // WS + 2 <= 256
    vmem = pl.BlockSpec(memory_space=pltpu.VMEM)
    yt = pl.pallas_call(
        functools.partial(_kernel, H=H, W=W),
        in_specs=[pl.BlockSpec(memory_space=pl.ANY), vmem, vmem, vmem],
        out_specs=pl.BlockSpec(memory_space=pl.ANY),
        out_shape=jax.ShapeDtypeStruct((H, C, W), x.dtype),
        scratch_shapes=[
            pltpu.VMEM((WS + 2, C, W), x.dtype),
            pltpu.VMEM((WS, C, W), x.dtype),
            pltpu.SemaphoreType.DMA((2,)),
            pltpu.VMEM((X0_ROWS, LANES), F32),
            pltpu.VMEM((WS * WP, LANES), F32),
            pltpu.VMEM((9, C, LANES), F32),
            pltpu.VMEM((3, 5, LANES // 2, LANES), U32),
            pltpu.VMEM((3, C // 2, LANES), U32),
            pltpu.VMEM((5, WS, WP, LANES), F32),
            pltpu.VMEM((NU, 3, LANES // 2, LANES), U32),
            pltpu.VMEM((37, LANES, LANES), F32),
            pltpu.VMEM((WS * NT, 16, LANES), F32),
            pltpu.VMEM((C, WP), F32),
        ],
        compiler_params=pltpu.CompilerParams(
            vmem_limit_bytes=64 * 1024 * 1024,
            disable_bounds_checks=bool(_env("NOBC", 1)),
        ),
        name="davit_window_attn",
    )(xt, dw_pe, w_qkv, w_o)
    return jnp.transpose(yt, (0, 2, 1))[None]
```

```python
import functools
import math
import os

import jax
import jax.numpy as jnp
from jax import lax
import jax.experimental.pallas as pl
import jax.experimental.pallas.tpu as pltpu

WS = 7
NH = 4
C = 192
DH = C // NH
NG = C // 8
LANES = 128
WP = 512
NT = WP // LANES
NU = WS * NT // 2
SLOTS = 8 * WS
EPS = 1e-5
F32 = jnp.float32
BF16 = jnp.bfloat16
U32 = jnp.uint32

X0_SLOT = WS * NT * C
DW_OFF = 3 * X0_SLOT
X0_ROWS = DW_OFF + 2 * C


def _dot(a, b):
    return jnp.dot(a, b, preferred_element_type=F32)


def _dot_nt(a, b):
    return lax.dot_general(a, b, (((1,), (1,)), ((), ())), preferred_element_type=F32)


def _cat(xs):
    return jnp.concatenate(xs, axis=0)


def _blocks(v):
    return [v[i:i + 8] for i in range(0, v.shape[0], 8)]


def _allred(x, op):
    for sh in (4, 2, 1):
        x = op(x, pltpu.roll(x, sh, 0))
    return x


def _env(name, default):
    return type(default)(os.environ.get(name, default))


def _kernel(x_hbm, dw_ref, wqkv_ref, wo_ref, o_hbm, *scratch, H, W):
    step = functools.partial(_step, x_hbm, dw_ref, wqkv_ref, wo_ref, o_hbm, *scratch, H=H, W=W)
    nstrip = H // WS

    def loop(lo, hi, mode):
        def body(k, carry):
            step(k_=k, mode=mode)
            return carry
        lax.fori_loop(lo, hi, body, 0)

    if "ONLY" not in os.environ:
        loop(0, 1, "first")
    loop(1 + _env("SKIP", 0), nstrip + 1, "main")
    if "ONLY" not in os.environ:
        loop(nstrip + 1, nstrip + 2, "last")


def _step(x_hbm, dw_ref, wqkv_ref, wo_ref, o_hbm,
          x_ref, o_ref, sems, x0_ref, ob_ref, dws_ref, ws_ref, wos_ref, qkv_ref, t_ref, stg_ref, ms_ref,
          top_ref, *, H, W, k_, mode):
    nstrip, nwin = H // WS, W // WS

    def x_copy(k):
        return pltpu.make_async_copy(x_hbm.at[pl.ds(jnp.minimum(k * WS, H - WS - 1), WS + 1)],
                                     x_ref.at[pl.ds(0, WS + 1)], sems.at[0])

    def o_copy(k):
        return pltpu.make_async_copy(o_ref, o_hbm.at[pl.ds(k * WS, WS)], sems.at[1])

    def when(cond, modes):
        if mode in modes:
            return pl.when(cond)
        return lambda f: None

    xoff = jnp.where(k_ >= nstrip - 1, 1, 0)
    dyn0 = jnp.minimum(k_, 0)

    def rows_at(base, off, n):
        if isinstance(base, int):
            return pl.ds(base + off, n)
        return pl.ds(pl.multiple_of(base + off, 8), n)

    mk = {}

    def new_masks(blk):
        lane = lax.broadcasted_iota(jnp.int32, (8, LANES), 1)
        mk.clear()
        mk["never"] = lane < dyn0
        if blk == "x":
            mk["up"] = lax.broadcasted_iota(jnp.int32, (8, LANES), 0) < 4
            return
        key_ok = lax.broadcasted_iota(jnp.int32, (8, LANES), 0) < WS
        mk.update(
            lo=lane < DH, hi0=(lane >= DH) & ((lane < 64) | (lane >= 96)), hi1=(lane >= DH) & (lane < 96),
            v=lane < 96, key=key_ok, keep_a=key_ok & (lane < SLOTS), keep_b=key_ok & (lane >= SLOTS),
            left64=lane < 64)

    k3 = k_ - 3 * ((k_ * 171) >> 9)
    nxt = k3 * X0_SLOT
    prv = jnp.where((k3 == 2) | (k_ < 2), 0, nxt + X0_SLOT)

    def conv_group(c0):
        st = {}

        def row(i):
            if i == 0 and i not in st:
                st[i] = top_ref[pl.ds(c0, 8), :]
            if i not in st:
                v = x_ref[xoff + (i - 1), pl.ds(c0, 8), :].astype(F32)
                st[i] = jnp.concatenate([v, jnp.zeros((8, WP - W), F32)], axis=1)
                if i == WS and i - 2 in st:
                    top_ref[pl.ds(c0, 8), :] = st[i]
            return st[i]

        def bc(v):
            return jnp.concatenate([v] * NT, axis=1)

        def taps(r):
            st["tw", r] = [bc(x0_ref[rows_at(c0, DW_OFF + k * C, 8), :]) for k in range(2)]

        def piece(r):
            if "w" not in st:
                st["w"] = [bc(dws_ref[k, pl.ds(c0, 8), :]) for k in range(9)]
            wts = list(st["w"])
            if ("tw", r) in st:
                wts[6], wts[8] = st["tw", r]
            row(r)
            abc = [row(r + 1) * wts[3 + j] + row(r) * wts[j] + row(r + 2) * wts[6 + j] for j in range(3)]
            x0 = pltpu.roll(abc[0], 1, 1) + abc[1] + pltpu.roll(abc[2], WP - 1, 1)
            for t in range(NT):
                x0_ref[rows_at(nxt, (r * NT + t) * C + c0, 8), :] = x0[:, t * LANES:(t + 1) * LANES]

        return taps, piece

    @when(k_ == 0, ("first",))
    def _():
        x_copy(0).start()
        for k in range(9):
            w = dw_ref[k // 3].astype(F32)[k % 3:k % 3 + 1, :]
            w = jnp.broadcast_to(w, (LANES, C)).T
            dws_ref[k] = w + 1.0 if k == 4 else w
            if k in (6, 8):
                x0_ref[pl.ds(DW_OFF + (k - 6) // 2 * C, C), :] = w
        w = wqkv_ref[...].astype(F32)
        wq = w[:, 0:C] * ((DH ** -0.5) * math.log2(math.e))
        wk, wv = w[:, C:2 * C], w[:, 2 * C:3 * C]
        tiles = [(wq[:, 0:64], wv[:, 64:96], wq[:, 64:96]),
                 (wq[:, 96:192], wv[:, 96:128]),
                 (wk[:, 0:64], wv[:, 128:160], wk[:, 64:96]),
                 (wk[:, 96:192], wv[:, 160:192]),
                 (wv[:, 0:128],)]
        for n, parts in enumerate(tiles):
            w = jnp.concatenate(parts, axis=1)
            for i, wi in enumerate((w[0:128], w[64:192], _cat([w[0:64], w[128:192]]))):
                if n == 4:
                    wi = wi.T
                ws_ref[i, n] = pltpu.bitcast(wi.astype(BF16), U32)
        w = wo_ref[...].astype(F32)
        wx, wy, wz = w[0:64], w[64:128], w[128:192]
        for i, parts in enumerate(((wx, wy), (wz, wy), (wx, wz))):
            wos_ref[i] = pltpu.bitcast(_cat(parts).T.astype(BF16), U32)

        top_ref[...] = jnp.zeros(top_ref.shape, F32)
        x_ref[WS + 1] = jnp.zeros(x_ref.shape[1:], x_ref.dtype)

        for r in range(WS):
            ob_ref[pl.ds(r * WP + WP - 8, 8), :] = jnp.zeros((8, LANES), F32)

    cuts = [int(c) for c in _env("CUTS", "0,7").split(",")]
    bands = list(zip(cuts, cuts[1:]))
    groups = {(b, g): conv_group(8 * g) for b in range(len(bands)) for g in range(NG)}
    WLEAD = _env("WLEAD", 4)

    def conv_items(nslow):
        plist = [((b, g), r) for b, (r0, r1) in enumerate(bands) for g in range(NG) for r in range(r0, r1)]
        items, nxt_tap = [], WLEAD
        for k, (g, r) in enumerate(plist):
            fs = []
            lead = WLEAD if k < nslow else _env("WLEAD2", 5)
            while nxt_tap <= min(k + lead, len(plist) - 1):
                g2, r2 = plist[nxt_tap]
                fs.append(functools.partial(groups[g2][0], r2))
                nxt_tap += 1
            fs.append(functools.partial(groups[g][1], r))
            items.append(fs)
        return items

    def ld_x0(j, k, gs=range(NG)):
        return [x0_ref[rows_at(nxt + dyn0 * (8 * k), j * C + 8 * g, 8), :] for g in gs]

    def add2(acc, xs):
        a = functools.reduce(jnp.add, xs[0::2])
        b = functools.reduce(jnp.add, xs[1::2])
        return a + b if acc is None else (acc + a) + b

    stats_done = set()

    def stats_steps(j):
        st = {"s": None, "q": None}
        n1, n2 = _env("SEG1", 8), _env("SEG2", 6)

        def sum_step(g0):
            st["s"] = add2(st["s"], ld_x0(j, 0, range(g0, g0 + n1)))
            if g0 + n1 == NG:
                st["s"] = _allred(st["s"], jnp.add) * (1.0 / C)
            return st["s"]

        def var_step(g0):
            d = [x - st["s"] for x in ld_x0(j, 1, range(g0, g0 + n2))]
            st["q"] = add2(st["q"], [x * x for x in d])
            return st["q"]

        def last_step():
            v = _allred(st["q"], jnp.add) * (1.0 / C) + EPS
            rs = lax.rsqrt(v) if _env("RSQ", 1) else jnp.exp2(jnp.log2(v) * -0.5)
            ms_ref[j] = _cat([st["s"], rs])
            stats_done.add(j)
            return rs

        return ([functools.partial(sum_step, g) for g in range(0, NG, n1)]
                + [functools.partial(var_step, g) for g in range(0, NG, n2)] + [last_step])

    def colsum(xs):
        xs = [a + b for a, b in zip(xs[0:8], xs[16:24])] + xs[8:16]
        return _dot(jnp.ones((8, LANES), F32), _cat(xs))

    means = {}

    def mean_dot(j):
        means[j] = colsum(ld_x0(j, 0)) * (1.0 / C)

    def var_dot(j):
        xs = [x0_ref[pl.ds(nxt + (j * C + 8 * g + 4), 8), :] for g in range(NG - 1)]
        xs.append(jnp.where(mk["up"], *ld_x0(j, 0, (0, NG - 1))))
        d = [x - means[j] for x in xs]
        v = colsum([x * x for x in d]) * (1.0 / C) + EPS
        rs = lax.rsqrt(v) if _env("RSQ", 1) else jnp.exp2(jnp.log2(v) * -0.5)
        ms_ref[j] = _cat([means[j], rs])
        stats_done.add(j)

    def normed(j, blk, k):
        assert j in stats_done or "ONLY" in os.environ and j < NSTX, j
        m, rs = ms_ref[j, 0:8, :], ms_ref[j, 8:16, :]
        return _cat([(x - m) * rs for x in ld_x0(j, k, range(8 * blk, 8 * blk + 8))])

    t_done = []

    def put_t(dst, tiles):
        tt = pltpu.bitcast(jnp.concatenate(tiles, axis=1).astype(BF16).T, U32)
        for i, (u, e) in enumerate(dst):
            t_ref[u, e] = tt[64 * i:64 * i + 64]
        t_done.append(pltpu.bitcast(tt[120:128], F32))

    def t_first(u):
        ja, jb = 2 * u, 2 * u + 1
        bx = normed(jb, 0, 0)
        put_t([(u, 0), (u, 2)], [_cat([normed(ja, 0, 0) - bx, normed(ja, 1, 0)]),
                                 _cat([bx, normed(ja, 2, 0)])])

    def t_second(r):
        put_t([(u, 1) for u in (2 * r, 2 * r + 1)],
              [_cat([normed(2 * u + 1, 1, 0), normed(2 * u + 1, 2, 0) - normed(2 * u, 2, _env("RECOMP", 1))])
               for u in (2 * r, 2 * r + 1)])

    t_items = []
    for r in range(WS):
        t_items += [functools.partial(t_first, 2 * r), functools.partial(t_first, 2 * r + 1),
                    functools.partial(t_second, r)]

    def qkv_chunk(u, n, steps=(), tiny=()):
        r, tp = divmod(u, 2)
        ops = {i: [_blocks(t_ref[u, i]), _blocks(ws_ref[i, n])] for i in range(3)}
        side = 1 if _env("ATT", "l") == "w" else 0
        for q, step in enumerate(steps):
            tok = pltpu.bitcast(step(), U32)
            q = q * 24 // len(steps)
            blks = ops[(2, 0, 1)[q % 3]][side]
            e = 7 - q // 3 if side else q // 3
            blks[e] = jnp.where(mk["never"], tok, blks[e])
        p3 = None
        for f in tiny:
            f()
        for q, i in enumerate((2, 0, 1)):
            p = _dot(*[pltpu.bitcast(_cat(x), BF16) for x in ops[i]])
            if p3 is None:
                p3 = p
            else:
                qkv_ref[n, r, pl.ds((2 * tp + i) * LANES, LANES), :] = p + p3

    vr_words = {}
    job_done = {}

    def side_dots(u, n):
        r, tp = divmod(u, 2)
        st = {}

        def one(i, parts=1):
            if parts > 1:
                lhs, rows = t_ref[u, i], 64 // parts
                p = _cat([_dot(pltpu.bitcast(lhs[q * rows:(q + 1) * rows], BF16),
                               pltpu.bitcast(ws_ref[i, n], BF16)) for q in range(parts)])
            elif n == 4:
                p = _dot_nt(pltpu.bitcast(ws_ref[i, 4, 0:32, :], BF16), pltpu.bitcast(t_ref[u, i], BF16))
            else:
                p = _dot(pltpu.bitcast(t_ref[u, i], BF16), pltpu.bitcast(ws_ref[i, n], BF16))
            st[i] = p if i == 2 else p + st[2]
            if n < 4 and i < 2:
                qkv_ref[n, r, pl.ds((2 * tp + i) * LANES, LANES), :] = st[i]
            elif i == 1:
                vr_words[u] = pltpu.pack_elementwise([st[0], st[1]], packed_dtype=BF16)

        return [(64 if n == 4 else LANES, (u, n, i), functools.partial(one, i)) for i in (2, 0, 1)]

    def vr_store(u):
        r, tp = divmod(u, 2)
        w = pltpu.bitcast(vr_words[u], F32)
        wt = pltpu.bitcast(_cat([w, w]).T, U32)
        job_done["v", u] = pltpu.bitcast(wt[120:128], F32)
        for j in range(2):
            qkv_ref[4, r, pl.ds((2 * tp + j) * LANES, LANES), :] = pltpu.unpack_elementwise(
                wt, index=j, packed_dtype=BF16, unpacked_dtype=F32)

    zero8 = jnp.zeros((8, LANES), F32)

    def gather(n, off, k=0):
        return [qkv_ref[n, r, pl.ds(off + dyn0 * k if k else off, 8), :] for r in range(WS)]

    def softmax_t(st):
        rows = _blocks(st)
        m = functools.reduce(jnp.maximum, rows)
        m = _allred(jnp.where(mk["key"], m, -jnp.inf), jnp.maximum)
        p = [jnp.exp2(x - m) for x in rows]
        return p, functools.reduce(jnp.add, p)

    def s2_pair(pi, offa):
        offb = offa + WS
        st = {}

        def vprep():
            g = [gather(n, offa) + gather(n, offb) for n in range(5)]
            u1 = [jnp.where(mk["left64"], z, jnp.where(mk["v"], x, y)) for x, y, z in zip(g[0], g[1], g[4])]
            u2 = [jnp.where(mk["v"], x, y) for x, y in zip(g[2], g[3])]
            u = jnp.concatenate([_cat(u1 + [zero8, zero8]), _cat(u2 + [zero8, zero8])], axis=1)
            vt = pltpu.bitcast(u.astype(BF16).T, U32)
            vt = _cat([vt[0:64], vt[96:128]])
            st["vt"] = [pltpu.bitcast(vt[24 * h:24 * h + 24], BF16) for h in range(NH)]

        def score(i, after=None, steps=()):
            hp, sw = divmod(i, 2)
            lo, hi = mk["lo"], mk["hi%d" % hp]
            ma, mb = (lo, hi) if sw == 0 else (hi, lo)
            gq = (0, 1, 1 + sw)[_env("GQ", 0)]
            gk = (0, 1, 1 + sw)[_env("GK", 0)]
            q = _cat([jnp.where(ma, v, 0.0) for v in gather(hp, offa, gq)]
                     + [jnp.where(mb, v, 0.0) for v in gather(hp, offb, gq)] + [zero8, zero8])
            ka, kb = gather(2 + hp, offa, gk), gather(2 + hp, offb, gk)
            k = [jnp.where(lo, x, y) for x, y in (zip(ka, kb) if sw == 0 else zip(kb, ka))]
            if after is not None:
                k[0] = jnp.where(mk["never"], t_done[after], k[0])
            for q_, step in enumerate(steps):
                e = 1 + (q_ * 6) // len(steps)
                k[e] = jnp.where(mk["never"], step(), k[e])
            k = _cat(k)
            st["p", i] = softmax_t(_dot_nt(k, q))

        def value(h):
            hp, sw = divmod(h, 2)
            (pa, sa), (pb, sb) = st["p", 2 * hp + sw], st["p", 2 * hp + 1 - sw]
            pm = _cat([jnp.where(mk["keep_a"], v, 0.0) for v in pa]
                      + [jnp.where(mk["keep_b"], v, 0.0) for v in pb] + [zero8, zero8])
            den = _allred(jnp.where(mk["keep_a"], sa, jnp.where(mk["keep_b"], sb, 0.0)), jnp.add)
            rec = pl.reciprocal(den, approx=True)
            if _env("NR", 0):
                rec = rec * (2.0 - den * rec)
            st["o", h] = [b * rec for b in _blocks(_dot(st["vt"][h], pm))]

        def finish():
            o = [b for h in range(NH) for b in st["o", h]]
            w = pltpu.pack_elementwise([_cat(o[0:16]), _cat(o[16:24] + o[16:24])], packed_dtype=BF16)
            stg_ref[pi] = pltpu.bitcast(w, F32)

        def scatter():
            wt = stg_ref[pi].T
            job_done["s", pi] = wt[104:112]
            for i, off in enumerate((offa, offb)):
                for r in range(WS):
                    base = i * SLOTS + 8 * r
                    ob_ref[pl.ds(r * WP + off, WS), :] = wt[base:base + WS]

        return vprep, score, value, finish, scatter

    npair = (nwin + 1) // 2
    pairs = [s2_pair(p, min(2 * p, nwin - 2) * WS) for p in range(npair)]

    def s3_unit(r, tp, steps=()):
        def unpack(t):
            w = pltpu.bitcast(ob_ref[pl.ds(r * WP + t * LANES, LANES), :], U32)
            return [_blocks(pltpu.unpack_elementwise(w, index=i, packed_dtype=BF16, unpacked_dtype=F32))
                    for i in range(2)]

        (la, ha), (lb, hb) = unpack(2 * tp), unpack(2 * tp + 1)
        t3 = _cat([jnp.where(mk["left64"], x, y) for x, y in zip(lb, ha)])
        t1 = _cat([x - jnp.where(mk["left64"], y, 0.0) for x, y in zip(la, lb)])
        t2 = _cat([jnp.where(mk["left64"], x - y, z) for x, y, z in zip(hb, ha, lb)])
        wo = [_blocks(wos_ref[i]) for i in range(3)]
        e0, e1 = _env("E0", 0), _env("E1", 8)
        for q, step in enumerate(steps):
            q = q * 3 * (e1 - e0) // len(steps)
            blks = wo[(2, 0, 1)[q % 3]]
            blks[e0 + q // 3] = jnp.where(mk["never"], pltpu.bitcast(step(), U32), blks[e0 + q // 3])
        wo = [pltpu.bitcast(_cat(w), BF16) for w in wo]
        p3 = _dot_nt(wo[2], t3)
        ys = [_dot_nt(wo[i], t) + p3
              + x0_ref[rows_at(prv, (r * NT + 2 * tp + i) * C, C), :] for i, t in enumerate((t1, t2))]
        n = min(2 * LANES, W - 2 * tp * LANES)
        o_ref[r, :, pl.ds(2 * tp * LANES, n)] = jnp.concatenate(ys, axis=1).astype(o_ref.dtype)[:, :n]

    s3_all = [functools.partial(s3_unit, r, tp) for tp in range(2) for r in range(WS)]

    def run(prog, extra):
        extra = sorted(extra, key=lambda e: e[0])
        j = 0
        for t0, fn in prog:
            while j < len(extra) and extra[j][0] <= t0:
                extra[j][1]()
                j += 1
            fn()
        for e in extra[j:]:
            e[1]()

    MERGE = _env("MERGE", 0)
    NX3 = _env("NX3", 0)

    NSY = _env("NSY", 0)

    NSTX = _env("NSTX", 16)

    def wave_steps(lo, hi, wave):
        steps = []
        for j0 in range(lo, hi, wave):
            for grp in zip(*[stats_steps(j) for j in range(j0, min(j0 + wave, hi))]):
                steps += grp
        return steps

    def block_x():
        NJ = _env("NJ", 28)
        NSTC = _env("NSTC", 6)
        WAVE = _env("WAVE", 4)
        VRLAG = _env("VRLAG", 200)
        chunks = [(u, n) for u in range(NU) for n in range(4)]
        MXS = _env("MXS", 0)
        steps = [] if MXS else wave_steps(0, NSTX, WAVE)
        nside = 9
        side, vstep = [], _env("VRSTEP", 1)
        for q in range(NU // 2):
            side += side_dots(2 * q, 4) + side_dots(2 * q + 1, 4)
            for _ in range(vstep):
                if nside:
                    side += side_dots(*chunks.pop())
                    nside -= 1
        for _ in range(nside):
            side += side_dots(*chunks.pop())
        c0 = len(chunks) - NSTC
        plan, t, vr_ready = [], 0, {}
        for k, (u, n) in enumerate(chunks):
            if k == c0:
                t_conv = t
            mine = steps[(k - c0) * len(steps) // NSTC:(k - c0 + 1) * len(steps) // NSTC] if k >= c0 else []
            plan.append((t, u, n, list(mine), []))
            room = LANES
            while side and (room > 0 or k == len(chunks) - 1):
                rows, key, f = side.pop(0)
                plan.append((t, f if room > 0 else functools.partial(f, 4), None, [], []))
                room -= rows
                if key[1:] == (4, 1):
                    vr_ready[key[0]] = t + LANES - room + VRLAG
            t += LANES
        ci = conv_items(4 * NJ)
        slow = _env("SLOW", 32.0)
        fast = (t_conv - 4 * NJ * slow) / max(len(ci) - 4 * NJ, 1)
        t_piece = [min(j, 4 * NJ) * slow + max(j - 4 * NJ, 0) * fast for j in range(len(ci) + 1)]
        scat, vrs = list(range(npair - NSY)), list(range(NU))
        jobs = []
        for q in range(NJ):
            if vrs and vr_ready[vrs[0]] <= t_piece[4 * q + 1]:
                jobs.append((t_piece[4 * q + 1], ("v", vrs[0])))
                ci[4 * q].insert(0, functools.partial(vr_store, vrs.pop(0)))
            elif scat:
                jobs.append((t_piece[4 * q + 1], ("s", scat[0])))
                ci[4 * q].insert(0, pairs[scat.pop(0)][4])
        extra = [(t_piece[j + 1], f) for j, fs in enumerate(ci) for f in fs]
        tail = [(("v", u), functools.partial(vr_store, u)) for u in vrs] + [(("s", p), pairs[p][4]) for p in scat]
        for q, (key, f) in enumerate(tail):
            t_q = max(t_conv + 1 + (q // 3) * 128, vr_ready[key[1]] if key[0] == "v" else 0)
            extra.append((t_q, f))
            jobs.append((t_q, key))
        if MXS:
            todo = []
            for r0, r1 in bands:
                todo += [(t_piece[r1 * NG] + _env("BLAG", 300), 0, r) for r in range(r0, r1)]
            for e in plan:
                room = 0 if e[2] is None else 1 if e[0] < t_conv else _env("ROOM2", 1)
                fin = e[1:3] == chunks[-1]
                if fin:
                    room = 1000
                while room and todo and (todo[0][0] <= e[0] or fin):
                    _, kind, r = todo.pop(0)
                    e[4].extend(functools.partial((mean_dot, var_dot)[kind], r * NT + q) for q in range(NT))
                    if kind == 0:
                        todo.append((e[0] + _env("VLAG", 250), 1, r))
                        todo.sort()
                    room -= 1
        if _env("JDL", 800):
            for t_q, key in jobs:
                later = [e for e in plan if e[2] is not None and e[0] >= t_q + _env("JDL", 800)]
                if later:
                    later[0][3].insert(0, functools.partial(job_done.get, key))
        prog = [(t0, u if n is None else functools.partial(qkv_chunk, u, n, st, tn))
                for t0, u, n, st, tn in plan]
        run(prog, extra)

    def block_y():
        LSM = _env("LSM", 170)
        LFIN = _env("LFIN", 0)
        SGRP = _env("SGRP", 4)
        VGRP = _env("VGRP", 2)
        TAILGAP = _env("TAILGAP", 500)
        load = [LANES, LANES, 0, 0] if MERGE else [0] * 4
        tm = list(load)
        t_0 = LANES + _env("LQKV", 220) if MERGE else 0
        prog, extra = [], []

        def emit(rows_list, fn, ready=0):
            prog.append((min(tm), fn))
            ends = []
            for rows in rows_list:
                m = load.index(min(load))
                load[m] += rows
                tm[m] = max(tm[m], ready) + rows
                ends.append(tm[m])
            return ends

        fillers = list(s3_all[NX3:])
        total = len(fillers) * 3 * C / 4 + npair * (SLOTS + DH)
        nsc = 4 * npair
        next_s = 0
        s_end, v_end, pend_v = {}, {}, []
        t_done.clear()
        ysteps = wave_steps(NSTX, WS * NT, _env("WAVEY", 4))
        SQ = _env("SQ", 110)
        sy0, sy1 = _env("SY0", 14), _env("SY1", 70)
        sdl = {sy0 + q * (sy1 - sy0) // max(NSY, 1): npair - NSY + q for q in range(NSY)}
        S3Q = _env("S3Q", 7)
        if S3Q:
            fillers = [functools.partial(f, ysteps[q * len(ysteps) // S3Q:(q + 1) * len(ysteps) // S3Q])
                       for q, f in enumerate(fillers)]
            ysteps = []
        d0, d1 = _env("TD0", 8), _env("TD1", 0)
        dl = {d0 + j * (nsc + d1 - d0) // len(t_items): j for j in range(len(t_items))}
        def emit_scores(n):
            nonlocal next_s
            for _ in range(n):
                p, i = divmod(next_s, 4)
                if i == 0:
                    prog.append((min(tm), pairs[p][0]))
                sj = []
                if next_s in sdl:
                    extra.append((min(tm) - _env("TLEAD", 300), pairs[sdl[next_s]][4]))
                    sj = [functools.partial(job_done.get, ("s", sdl[next_s]))]
                if next_s in dl:
                    extra.append((min(tm) - _env("TLEAD", 300), t_items[dl[next_s]]))
                s_end[p, i] = emit([SLOTS], functools.partial(
                    pairs[p][1], i, dl.get(next_s),
                    ysteps[next_s * len(ysteps) // SQ:(next_s + 1) * len(ysteps) // SQ] + sj))[0]
                if i % 2 == 1:
                    pend_v.append((max(s_end[p, i], s_end[p, i - 1]) + LSM, p, i // 2))
                next_s += 1

        def emit_values(n):
            for rdy, pv, hp in pend_v[:n]:
                for h in (2 * hp, 2 * hp + 1):
                    v_end[pv, h] = emit([DH], functools.partial(pairs[pv][2], h), rdy)[0]
                if hp == 1:
                    extra.append((max(v_end[pv, h] for h in range(NH)) + LFIN, pairs[pv][3]))
            del pend_v[:n]

        if _env("PLAN", 1) == 2:
            nfill, sk = len(fillers), _env("SK", 2)
            f0, f1 = _env("F0", 0.0), _env("F1", 1.0)
            blk = [int(f0 + q * (npair - f1 - f0) / (nfill - 1) + 0.5) for q in range(nfill)]
            emit_scores(4 * sk)
            for p in range(npair):
                ahead = sk - (1 if _env("TIGHT", 0) and (p in blk or p + 1 in blk) else 0)
                while next_s < min(4 * (p + ahead + 1), nsc):
                    emit_scores(4)
                if p in blk:
                    emit([C] * 3, fillers.pop(0))
                emit_values(2)
        while fillers or next_s < nsc or pend_v:
            now = tm[load.index(min(load))]
            s_ok = next_s < nsc and now >= t_0 + (total - TAILGAP - t_0) * next_s / (nsc - 4)
            v_ok = len(pend_v) >= VGRP // 2 and all(now >= x[0] for x in pend_v[:VGRP // 2])
            if not fillers and not s_ok and not v_ok:
                if pend_v and (next_s >= nsc or len(pend_v) >= 4):
                    v_ok = True
                else:
                    s_ok = True
            if v_ok:
                emit_values(VGRP // 2)
            elif s_ok:
                emit_scores(SGRP)
            else:
                emit([C] * 3, fillers.pop(0))
        if _env("VERB", 0):
            print("Y planned", tm, load)
        extra += [(max(tm) - 600, t_items[j]) for q, j in dl.items() if q >= nsc]
        run(prog, extra)

    only = _env("ONLY", "01")
    NODMA = _env("NODMA", 0)

    @when(k_ < (1 if NODMA & 1 else nstrip), ("first", "main"))
    def _():
        x_copy(k_).wait()

    new_masks("x")
    if "0" in only:
        when(k_ <= nstrip, ("main",))(block_x)

    @when(k_ == 0, ("first",))
    def _():
        def body(g, carry):
            for j in range(FG):
                piece = conv_group(pl.multiple_of((g * FG + j) * 8, 8))[1]
                for r in range(WS):
                    piece(r)
            return carry
        FG = _env("FG", 8)
        lax.fori_loop(0, NG // FG, body, 0)

    @when(k_ < (0 if NODMA & 1 else nstrip - 1), ("first", "main"))
    def _():
        x_copy(k_ + 1).start()

    @when(k_ >= (1000 if NODMA & 2 else 3), ("main", "last"))
    def _():
        o_copy(k_ - 3).wait()

    if "1" in only:
        new_masks("y")
        when((k_ <= nstrip) & (k_ >= 1), ("main",))(block_y)

    @when(k_ == 0, ("first",))
    def _():
        for j in range(WS * NT):
            for f in stats_steps(j):
                f()
        for f in t_items:
            f()

    @when(k_ == nstrip + 1, ("last",))
    def _():
        new_masks("y")
        for p in range(npair):
            pairs[p][4]()
        for f in s3_all:
            f()

    if only != "01":
        @when(dyn0 < 0, ("main",))
        def _():
            i = pl.multiple_of(k_ * 8, 8)
            o_ref[0, 0:16, 0:128] = _cat([
                qkv_ref[k3, k3, pl.ds(i, 8), :] + ms_ref[k3, 0:8, :] + stg_ref[k3, pl.ds(i, 8), :],
                pltpu.bitcast(t_ref[k3, k3, pl.ds(i, 8), :], F32) + ob_ref[pl.ds(i, 8), :]]).astype(BF16)
            for rf in (qkv_ref.at[k3, k3], stg_ref.at[k3], ob_ref):
                rf[pl.ds(i, 8), :] = zero8
            t_ref[k3, k3, pl.ds(i, 8), :] = pltpu.bitcast(zero8, U32)

    @when(k_ >= (nstrip + 1 if NODMA & 2 else 2), ("main", "last"))
    def _():
        o_copy(k_ - 2).start()

    @when(k_ == nstrip + 1, ("last",))
    def _():
        o_copy(k_ - 2).wait()


@jax.jit
def pallas_standalone__window_attn_davit__vision_kernel(
    x: jax.Array,
    dw_pe: jax.Array,
    w_qkv: jax.Array,
    w_o: jax.Array,
):
    B, H, W, Cx = x.shape
    assert B == 1 and Cx == C and H % WS == 0 and W % WS == 0 and WP - LANES < W < WP
    xt = jnp.transpose(x[0], (0, 2, 1))

    assert H // WS + 2 <= 256
    vmem = pl.BlockSpec(memory_space=pltpu.VMEM)
    yt = pl.pallas_call(
        functools.partial(_kernel, H=H, W=W),
        in_specs=[pl.BlockSpec(memory_space=pl.ANY), vmem, vmem, vmem],
        out_specs=pl.BlockSpec(memory_space=pl.ANY),
        out_shape=jax.ShapeDtypeStruct((H, C, W), x.dtype),
        scratch_shapes=[
            pltpu.VMEM((WS + 2, C, W), x.dtype),
            pltpu.VMEM((WS, C, W), x.dtype),
            pltpu.SemaphoreType.DMA((2,)),
            pltpu.VMEM((X0_ROWS, LANES), F32),
            pltpu.VMEM((WS * WP, LANES), F32),
            pltpu.VMEM((9, C, LANES), F32),
            pltpu.VMEM((3, 5, LANES // 2, LANES), U32),
            pltpu.VMEM((3, C // 2, LANES), U32),
            pltpu.VMEM((5, WS, WP, LANES), F32),
            pltpu.VMEM((NU, 3, LANES // 2, LANES), U32),
            pltpu.VMEM((37, LANES, LANES), F32),
            pltpu.VMEM((WS * NT, 16, LANES), F32),
            pltpu.VMEM((C, WP), F32),
        ],
        compiler_params=pltpu.CompilerParams(
            vmem_limit_bytes=64 * 1024 * 1024,
            disable_bounds_checks=bool(_env("NOBC", 1)),
        ),
        name="davit_window_attn",
    )(xt, dw_pe, w_qkv, w_o)
    return jnp.transpose(yt, (0, 2, 1))[None]
```

```python
import functools
import math
import os

import jax
import jax.numpy as jnp
from jax import lax
import jax.experimental.pallas as pl
import jax.experimental.pallas.tpu as pltpu

WS = 7
NH = 4
C = 192
DH = C // NH
NG = C // 8
LANES = 128
WP = 512
NT = WP // LANES
NU = WS * NT // 2
SLOTS = 8 * WS
EPS = 1e-5
F32 = jnp.float32
BF16 = jnp.bfloat16
U32 = jnp.uint32

X0_SLOT = WS * NT * C
DW_OFF = 3 * X0_SLOT
X0_ROWS = DW_OFF + 2 * C


def _dot(a, b):
    return jnp.dot(a, b, preferred_element_type=F32)


def _dot_nt(a, b):
    return lax.dot_general(a, b, (((1,), (1,)), ((), ())), preferred_element_type=F32)


def _cat(xs):
    return jnp.concatenate(xs, axis=0)


def _blocks(v):
    return [v[i:i + 8] for i in range(0, v.shape[0], 8)]


def _allred(x, op):
    for sh in (4, 2, 1):
        x = op(x, pltpu.roll(x, sh, 0))
    return x


def _env(name, default):
    return type(default)(os.environ.get(name, default))


def _kernel(x_hbm, dw_ref, wqkv_ref, wo_ref, o_hbm, *scratch, H, W):
    step = functools.partial(_step, x_hbm, dw_ref, wqkv_ref, wo_ref, o_hbm, *scratch, H=H, W=W)
    nstrip = H // WS

    def loop(lo, hi, mode):
        def body(k, carry):
            step(k_=k, mode=mode)
            return carry
        lax.fori_loop(lo, hi, body, 0)

    if "ONLY" not in os.environ:
        loop(0, 1, "first")
    loop(1 + _env("SKIP", 0), nstrip + 1, "main")
    if "ONLY" not in os.environ:
        loop(nstrip + 1, nstrip + 2, "last")


def _step(x_hbm, dw_ref, wqkv_ref, wo_ref, o_hbm,
          x_ref, o_ref, sems, x0_ref, ob_ref, dws_ref, ws_ref, wos_ref, qkv_ref, t_ref, stg_ref, ms_ref,
          top_ref, *, H, W, k_, mode):
    nstrip, nwin = H // WS, W // WS

    def x_copy(k):
        return pltpu.make_async_copy(x_hbm.at[pl.ds(jnp.minimum(k * WS, H - WS - 1), WS + 1)],
                                     x_ref.at[pl.ds(0, WS + 1)], sems.at[0])

    def o_copy(k):
        return pltpu.make_async_copy(o_ref, o_hbm.at[pl.ds(k * WS, WS)], sems.at[1])

    def when(cond, modes):
        if mode in modes:
            return pl.when(cond)
        return lambda f: None

    xoff = jnp.where(k_ >= nstrip - 1, 1, 0)
    dyn0 = jnp.minimum(k_, 0)

    def rows_at(base, off, n):
        if isinstance(base, int):
            return pl.ds(base + off, n)
        return pl.ds(pl.multiple_of(base + off, 8), n)

    mk = {}

    def new_masks(blk):
        lane = lax.broadcasted_iota(jnp.int32, (8, LANES), 1)
        mk.clear()
        mk["never"] = lane < dyn0
        if blk == "x":
            mk["up"] = lax.broadcasted_iota(jnp.int32, (8, LANES), 0) < 4
            return
        key_ok = lax.broadcasted_iota(jnp.int32, (8, LANES), 0) < WS
        mk.update(
            lo=lane < DH, hi0=(lane >= DH) & ((lane < 64) | (lane >= 96)), hi1=(lane >= DH) & (lane < 96),
            v=lane < 96, key=key_ok, keep_a=key_ok & (lane < SLOTS), keep_b=key_ok & (lane >= SLOTS),
            left64=lane < 64)

    k3 = k_ - 3 * ((k_ * 171) >> 9)
    nxt = k3 * X0_SLOT
    prv = jnp.where((k3 == 2) | (k_ < 2), 0, nxt + X0_SLOT)

    def conv_group(c0):
        st = {}

        def row(i):
            if i == 0 and i not in st:
                st[i] = top_ref[pl.ds(c0, 8), :]
            if i not in st:
                v = x_ref[xoff + (i - 1), pl.ds(c0, 8), :].astype(F32)
                st[i] = jnp.concatenate([v, jnp.zeros((8, WP - W), F32)], axis=1)
                if i == WS and i - 2 in st:
                    top_ref[pl.ds(c0, 8), :] = st[i]
            return st[i]

        def bc(v):
            return jnp.concatenate([v] * NT, axis=1)

        def taps(r):
            st["tw", r] = [bc(x0_ref[rows_at(c0, DW_OFF + k * C, 8), :]) for k in range(2)]

        def piece(r):
            if "w" not in st:
                st["w"] = [bc(dws_ref[k, pl.ds(c0, 8), :]) for k in range(9)]
            wts = list(st["w"])
            if ("tw", r) in st:
                wts[6], wts[8] = st["tw", r]
            row(r)
            abc = [row(r + 1) * wts[3 + j] + row(r) * wts[j] + row(r + 2) * wts[6 + j] for j in range(3)]
            x0 = pltpu.roll(abc[0], 1, 1) + abc[1] + pltpu.roll(abc[2], WP - 1, 1)
            for t in range(NT):
                x0_ref[rows_at(nxt, (r * NT + t) * C + c0, 8), :] = x0[:, t * LANES:(t + 1) * LANES]

        return taps, piece

    @when(k_ == 0, ("first",))
    def _():
        x_copy(0).start()
        for k in range(9):
            w = dw_ref[k // 3].astype(F32)[k % 3:k % 3 + 1, :]
            w = jnp.broadcast_to(w, (LANES, C)).T
            dws_ref[k] = w + 1.0 if k == 4 else w
            if k in (6, 8):
                x0_ref[pl.ds(DW_OFF + (k - 6) // 2 * C, C), :] = w
        w = wqkv_ref[...].astype(F32)
        wq = w[:, 0:C] * ((DH ** -0.5) * math.log2(math.e))
        wk, wv = w[:, C:2 * C], w[:, 2 * C:3 * C]
        tiles = [(wq[:, 0:64], wv[:, 64:96], wq[:, 64:96]),
                 (wq[:, 96:192], wv[:, 96:128]),
                 (wk[:, 0:64], wv[:, 128:160], wk[:, 64:96]),
                 (wk[:, 96:192], wv[:, 160:192]),
                 (wv[:, 0:128],)]
        for n, parts in enumerate(tiles):
            w = jnp.concatenate(parts, axis=1)
            for i, wi in enumerate((w[0:128], w[64:192], _cat([w[0:64], w[128:192]]))):
                if n == 4:
                    wi = wi.T
                ws_ref[i, n] = pltpu.bitcast(wi.astype(BF16), U32)
        w = wo_ref[...].astype(F32)
        wx, wy, wz = w[0:64], w[64:128], w[128:192]
        for i, parts in enumerate(((wx, wy), (wz, wy), (wx, wz))):
            wos_ref[i] = pltpu.bitcast(_cat(parts).T.astype(BF16), U32)

        top_ref[...] = jnp.zeros(top_ref.shape, F32)
        x_ref[WS + 1] = jnp.zeros(x_ref.shape[1:], x_ref.dtype)

        for r in range(WS):
            ob_ref[pl.ds(r * WP + WP - 8, 8), :] = jnp.zeros((8, LANES), F32)

    cuts = [int(c) for c in _env("CUTS", "0,7").split(",")]
    bands = list(zip(cuts, cuts[1:]))
    groups = {(b, g): conv_group(8 * g) for b in range(len(bands)) for g in range(NG)}
    WLEAD = _env("WLEAD", 4)

    def conv_items(nslow):
        plist = [((b, g), r) for b, (r0, r1) in enumerate(bands) for g in range(NG) for r in range(r0, r1)]
        items, nxt_tap = [], WLEAD
        for k, (g, r) in enumerate(plist):
            fs = []
            lead = WLEAD if k < nslow else _env("WLEAD2", 5)
            while nxt_tap <= min(k + lead, len(plist) - 1):
                g2, r2 = plist[nxt_tap]
                fs.append(functools.partial(groups[g2][0], r2))
                nxt_tap += 1
            fs.append(functools.partial(groups[g][1], r))
            items.append(fs)
        return items

    def ld_x0(j, k, gs=range(NG)):
        return [x0_ref[rows_at(nxt + dyn0 * (8 * k), j * C + 8 * g, 8), :] for g in gs]

    def add2(acc, xs):
        a = functools.reduce(jnp.add, xs[0::2])
        b = functools.reduce(jnp.add, xs[1::2])
        return a + b if acc is None else (acc + a) + b

    stats_done = set()

    def stats_steps(j):
        st = {"s": None, "q": None}
        n1, n2 = _env("SEG1", 8), _env("SEG2", 6)

        def sum_step(g0):
            st["s"] = add2(st["s"], ld_x0(j, 0, range(g0, g0 + n1)))
            if g0 + n1 == NG:
                st["s"] = _allred(st["s"], jnp.add) * (1.0 / C)
            return st["s"]

        def var_step(g0):
            d = [x - st["s"] for x in ld_x0(j, 1, range(g0, g0 + n2))]
            st["q"] = add2(st["q"], [x * x for x in d])
            return st["q"]

        def last_step():
            v = _allred(st["q"], jnp.add) * (1.0 / C) + EPS
            rs = lax.rsqrt(v) if _env("RSQ", 1) else jnp.exp2(jnp.log2(v) * -0.5)
            ms_ref[j] = _cat([st["s"], rs])
            stats_done.add(j)
            return rs

        return ([functools.partial(sum_step, g) for g in range(0, NG, n1)]
                + [functools.partial(var_step, g) for g in range(0, NG, n2)] + [last_step])

    def colsum(xs):
        xs = [a + b for a, b in zip(xs[0:8], xs[16:24])] + xs[8:16]
        return _dot(jnp.ones((8, LANES), F32), _cat(xs))

    means = {}

    def mean_dot(j):
        means[j] = colsum(ld_x0(j, 0)) * (1.0 / C)

    def var_dot(j):
        xs = [x0_ref[pl.ds(nxt + (j * C + 8 * g + 4), 8), :] for g in range(NG - 1)]
        xs.append(jnp.where(mk["up"], *ld_x0(j, 0, (0, NG - 1))))
        d = [x - means[j] for x in xs]
        v = colsum([x * x for x in d]) * (1.0 / C) + EPS
        rs = lax.rsqrt(v) if _env("RSQ", 1) else jnp.exp2(jnp.log2(v) * -0.5)
        ms_ref[j] = _cat([means[j], rs])
        stats_done.add(j)

    def normed(j, blk, k):
        assert j in stats_done or "ONLY" in os.environ and j < NSTX, j
        m, rs = ms_ref[j, 0:8, :], ms_ref[j, 8:16, :]
        return _cat([(x - m) * rs for x in ld_x0(j, k, range(8 * blk, 8 * blk + 8))])

    t_done = []

    def put_t(dst, tiles):
        tt = pltpu.bitcast(jnp.concatenate(tiles, axis=1).astype(BF16).T, U32)
        for i, (u, e) in enumerate(dst):
            t_ref[u, e] = tt[64 * i:64 * i + 64]
        t_done.append(pltpu.bitcast(tt[120:128], F32))

    def t_first(u):
        ja, jb = 2 * u, 2 * u + 1
        bx = normed(jb, 0, 0)
        put_t([(u, 0), (u, 2)], [_cat([normed(ja, 0, 0) - bx, normed(ja, 1, 0)]),
                                 _cat([bx, normed(ja, 2, 0)])])

    def t_second(r):
        put_t([(u, 1) for u in (2 * r, 2 * r + 1)],
              [_cat([normed(2 * u + 1, 1, 0), normed(2 * u + 1, 2, 0) - normed(2 * u, 2, _env("RECOMP", 1))])
               for u in (2 * r, 2 * r + 1)])

    t_items = []
    for r in range(WS):
        t_items += [functools.partial(t_first, 2 * r), functools.partial(t_first, 2 * r + 1),
                    functools.partial(t_second, r)]

    def qkv_chunk(us, n, steps=(), tiny=()):
        lhs = {i: [b for u in us for b in _blocks(t_ref[u, i])] for i in range(3)}
        for q, step in enumerate(steps):
            tok = pltpu.bitcast(step(), U32)
            q = q * 24 * len(us) // len(steps)
            blks = lhs[(2, 0, 1)[q % 3]]
            blks[q // 3] = jnp.where(mk["never"], tok, blks[q // 3])
        p3 = None
        for i in (2, 0, 1):
            p = _dot(pltpu.bitcast(_cat(lhs[i]), BF16), pltpu.bitcast(ws_ref[i, n], BF16))
            if p3 is None:
                p3 = p
            else:
                p = p + p3
                for e, u in enumerate(us):
                    r, tp = divmod(u, 2)
                    qkv_ref[n, r, pl.ds((2 * tp + i) * LANES, LANES), :] = p[e * LANES:(e + 1) * LANES]

    vr_words = {}
    job_done = {}

    def side_dots(u, n):
        r, tp = divmod(u, 2)
        st = {}

        def one(i, parts=1):
            if parts > 1:
                lhs, rows = t_ref[u, i], 64 // parts
                p = _cat([_dot(pltpu.bitcast(lhs[q * rows:(q + 1) * rows], BF16),
                               pltpu.bitcast(ws_ref[i, n], BF16)) for q in range(parts)])
            elif n == 4:
                p = _dot_nt(pltpu.bitcast(ws_ref[i, 4, 0:32, :], BF16), pltpu.bitcast(t_ref[u, i], BF16))
            else:
                p = _dot(pltpu.bitcast(t_ref[u, i], BF16), pltpu.bitcast(ws_ref[i, n], BF16))
            st[i] = p if i == 2 else p + st[2]
            if n < 4 and i < 2:
                qkv_ref[n, r, pl.ds((2 * tp + i) * LANES, LANES), :] = st[i]
            elif i == 1:
                vr_words[u] = pltpu.pack_elementwise([st[0], st[1]], packed_dtype=BF16)

        return [(64 if n == 4 else LANES, (u, n, i), functools.partial(one, i)) for i in (2, 0, 1)]

    def vr_store(u):
        r, tp = divmod(u, 2)
        w = pltpu.bitcast(vr_words[u], F32)
        wt = pltpu.bitcast(_cat([w, w]).T, U32)
        job_done["v", u] = pltpu.bitcast(wt[120:128], F32)
        for j in range(2):
            qkv_ref[4, r, pl.ds((2 * tp + j) * LANES, LANES), :] = pltpu.unpack_elementwise(
                wt, index=j, packed_dtype=BF16, unpacked_dtype=F32)

    zero8 = jnp.zeros((8, LANES), F32)

    def gather(n, off, k=0):
        return [qkv_ref[n, r, pl.ds(off + dyn0 * k if k else off, 8), :] for r in range(WS)]

    def softmax_t(st):
        rows = _blocks(st)
        m = functools.reduce(jnp.maximum, rows)
        m = _allred(jnp.where(mk["key"], m, -jnp.inf), jnp.maximum)
        p = [jnp.exp2(x - m) for x in rows]
        return p, functools.reduce(jnp.add, p)

    def s2_pair(pi, offa):
        offb = offa + WS
        st = {}

        def vprep():
            g = [gather(n, offa) + gather(n, offb) for n in range(5)]
            u1 = [jnp.where(mk["left64"], z, jnp.where(mk["v"], x, y)) for x, y, z in zip(g[0], g[1], g[4])]
            u2 = [jnp.where(mk["v"], x, y) for x, y in zip(g[2], g[3])]
            u = jnp.concatenate([_cat(u1 + [zero8, zero8]), _cat(u2 + [zero8, zero8])], axis=1)
            vt = pltpu.bitcast(u.astype(BF16).T, U32)
            vt = _cat([vt[0:64], vt[96:128]])
            st["vt"] = [pltpu.bitcast(vt[24 * h:24 * h + 24], BF16) for h in range(NH)]

        def score(i, after=None, steps=()):
            hp, sw = divmod(i, 2)
            lo, hi = mk["lo"], mk["hi%d" % hp]
            ma, mb = (lo, hi) if sw == 0 else (hi, lo)
            gq = (0, 1, 1 + sw)[_env("GQ", 0)]
            gk = (0, 1, 1 + sw)[_env("GK", 0)]
            q = _cat([jnp.where(ma, v, 0.0) for v in gather(hp, offa, gq)]
                     + [jnp.where(mb, v, 0.0) for v in gather(hp, offb, gq)] + [zero8, zero8])
            ka, kb = gather(2 + hp, offa, gk), gather(2 + hp, offb, gk)
            k = [jnp.where(lo, x, y) for x, y in (zip(ka, kb) if sw == 0 else zip(kb, ka))]
            if after is not None:
                k[0] = jnp.where(mk["never"], t_done[after], k[0])
            for q_, step in enumerate(steps):
                e = 1 + (q_ * 6) // len(steps)
                k[e] = jnp.where(mk["never"], step(), k[e])
            k = _cat(k)
            st["p", i] = softmax_t(_dot_nt(k, q))

        def value(h):
            hp, sw = divmod(h, 2)
            (pa, sa), (pb, sb) = st["p", 2 * hp + sw], st["p", 2 * hp + 1 - sw]
            pm = _cat([jnp.where(mk["keep_a"], v, 0.0) for v in pa]
                      + [jnp.where(mk["keep_b"], v, 0.0) for v in pb] + [zero8, zero8])
            den = _allred(jnp.where(mk["keep_a"], sa, jnp.where(mk["keep_b"], sb, 0.0)), jnp.add)
            rec = pl.reciprocal(den, approx=True)
            if _env("NR", 0):
                rec = rec * (2.0 - den * rec)
            st["o", h] = [b * rec for b in _blocks(_dot(st["vt"][h], pm))]

        def finish():
            o = [b for h in range(NH) for b in st["o", h]]
            w = pltpu.pack_elementwise([_cat(o[0:16]), _cat(o[16:24] + o[16:24])], packed_dtype=BF16)
            stg_ref[pi] = pltpu.bitcast(w, F32)

        def scatter():
            wt = stg_ref[pi].T
            job_done["s", pi] = wt[104:112]
            for i, off in enumerate((offa, offb)):
                for r in range(WS):
                    base = i * SLOTS + 8 * r
                    ob_ref[pl.ds(r * WP + off, WS), :] = wt[base:base + WS]

        return vprep, score, value, finish, scatter

    npair = (nwin + 1) // 2
    pairs = [s2_pair(p, min(2 * p, nwin - 2) * WS) for p in range(npair)]

    def s3_unit(r, tp, steps=()):
        def unpack(t):
            w = pltpu.bitcast(ob_ref[pl.ds(r * WP + t * LANES, LANES), :], U32)
            return [_blocks(pltpu.unpack_elementwise(w, index=i, packed_dtype=BF16, unpacked_dtype=F32))
                    for i in range(2)]

        (la, ha), (lb, hb) = unpack(2 * tp), unpack(2 * tp + 1)
        t3 = _cat([jnp.where(mk["left64"], x, y) for x, y in zip(lb, ha)])
        t1 = _cat([x - jnp.where(mk["left64"], y, 0.0) for x, y in zip(la, lb)])
        t2 = _cat([jnp.where(mk["left64"], x - y, z) for x, y, z in zip(hb, ha, lb)])
        wo = [_blocks(wos_ref[i]) for i in range(3)]
        e0, e1 = _env("E0", 0), _env("E1", 8)
        for q, step in enumerate(steps):
            q = q * 3 * (e1 - e0) // len(steps)
            blks = wo[(2, 0, 1)[q % 3]]
            blks[e0 + q // 3] = jnp.where(mk["never"], pltpu.bitcast(step(), U32), blks[e0 + q // 3])
        wo = [pltpu.bitcast(_cat(w), BF16) for w in wo]
        p3 = _dot_nt(wo[2], t3)
        ys = [_dot_nt(wo[i], t) + p3
              + x0_ref[rows_at(prv, (r * NT + 2 * tp + i) * C, C), :] for i, t in enumerate((t1, t2))]
        n = min(2 * LANES, W - 2 * tp * LANES)
        o_ref[r, :, pl.ds(2 * tp * LANES, n)] = jnp.concatenate(ys, axis=1).astype(o_ref.dtype)[:, :n]

    s3_all = [functools.partial(s3_unit, r, tp) for tp in range(2) for r in range(WS)]

    def run(prog, extra):
        extra = sorted(extra, key=lambda e: e[0])
        j = 0
        for t0, fn in prog:
            while j < len(extra) and extra[j][0] <= t0:
                extra[j][1]()
                j += 1
            fn()
        for e in extra[j:]:
            e[1]()

    MERGE = _env("MERGE", 0)
    NX3 = _env("NX3", 0)

    NSY = _env("NSY", 0)

    NSTX = _env("NSTX", 16)

    def wave_steps(lo, hi, wave):
        steps = []
        for j0 in range(lo, hi, wave):
            for grp in zip(*[stats_steps(j) for j in range(j0, min(j0 + wave, hi))]):
                steps += grp
        return steps

    def block_x():
        NJ = _env("NJ", 28)
        NSTC = _env("NSTC", 6)
        WAVE = _env("WAVE", 4)
        VRLAG = _env("VRLAG", 200)
        chunks = [(u, n) for u in range(NU) for n in range(4)]
        MXS = _env("MXS", 0)
        steps = [] if MXS else wave_steps(0, NSTX, WAVE)
        nside = 9
        side, vstep = [], _env("VRSTEP", 1)
        for q in range(NU // 2):
            side += side_dots(2 * q, 4) + side_dots(2 * q + 1, 4)
            for _ in range(vstep):
                if nside:
                    side += side_dots(*chunks.pop())
                    nside -= 1
        for _ in range(nside):
            side += side_dots(*chunks.pop())
        mu = _env("MU", 2)
        merged = []
        for u, n in chunks:
            prev = [c for c in merged if c[1] == n and c[0][0] // mu == u // mu]
            if prev:
                prev[0][0].append(u)
            else:
                merged.append(([u], n))
        starts = [LANES * sum(len(c[0]) for c in merged[:k]) for k in range(len(merged))]
        t_conv = max(x for x in starts if x <= (len(chunks) - NSTC) * LANES)
        span = len(chunks) * LANES - t_conv
        plan, t, vr_ready = [], 0, {}
        for k, (us, n) in enumerate(merged):
            dur = LANES * len(us)
            lo, hi = (max(x - t_conv, 0) * len(steps) // span for x in (t, t + dur))
            plan.append((t, tuple(us), n, list(steps[lo:hi]), []))
            room = dur
            while side and (room > 0 or k == len(merged) - 1):
                rows, key, f = side.pop(0)
                plan.append((t, f if room > 0 else functools.partial(f, 4), None, [], []))
                room -= rows
                if key[1:] == (4, 1):
                    vr_ready[key[0]] = t + dur - room + VRLAG
            t += dur
        ci = conv_items(4 * NJ)
        slow = _env("SLOW", 32.0)
        fast = (t_conv - 4 * NJ * slow) / max(len(ci) - 4 * NJ, 1)
        t_piece = [min(j, 4 * NJ) * slow + max(j - 4 * NJ, 0) * fast for j in range(len(ci) + 1)]
        scat, vrs = list(range(npair - NSY)), list(range(NU))
        jobs = []
        for q in range(NJ):
            if vrs and vr_ready[vrs[0]] <= t_piece[4 * q + 1]:
                jobs.append((t_piece[4 * q + 1], ("v", vrs[0])))
                ci[4 * q].insert(0, functools.partial(vr_store, vrs.pop(0)))
            elif scat:
                jobs.append((t_piece[4 * q + 1], ("s", scat[0])))
                ci[4 * q].insert(0, pairs[scat.pop(0)][4])
        extra = [(t_piece[j + 1], f) for j, fs in enumerate(ci) for f in fs]
        tail = [(("v", u), functools.partial(vr_store, u)) for u in vrs] + [(("s", p), pairs[p][4]) for p in scat]
        for q, (key, f) in enumerate(tail):
            t_q = max(t_conv + 1 + (q // 3) * 128, vr_ready[key[1]] if key[0] == "v" else 0)
            extra.append((t_q, f))
            jobs.append((t_q, key))
        if _env("JDL", 800):
            for t_q, key in jobs:
                later = [e for e in plan if e[2] is not None and e[0] >= t_q + _env("JDL", 800)]
                if later:
                    later[0][3].insert(0, functools.partial(job_done.get, key))
        prog = [(t0, u if n is None else functools.partial(qkv_chunk, u, n, st, tn))
                for t0, u, n, st, tn in plan]
        run(prog, extra)

    def block_y():
        LSM = _env("LSM", 170)
        LFIN = _env("LFIN", 0)
        SGRP = _env("SGRP", 4)
        VGRP = _env("VGRP", 2)
        TAILGAP = _env("TAILGAP", 500)
        load = [LANES, LANES, 0, 0] if MERGE else [0] * 4
        tm = list(load)
        t_0 = LANES + _env("LQKV", 220) if MERGE else 0
        prog, extra = [], []

        def emit(rows_list, fn, ready=0):
            prog.append((min(tm), fn))
            ends = []
            for rows in rows_list:
                m = load.index(min(load))
                load[m] += rows
                tm[m] = max(tm[m], ready) + rows
                ends.append(tm[m])
            return ends

        fillers = list(s3_all[NX3:])
        total = len(fillers) * 3 * C / 4 + npair * (SLOTS + DH)
        nsc = 4 * npair
        next_s = 0
        s_end, v_end, pend_v = {}, {}, []
        t_done.clear()
        ysteps = wave_steps(NSTX, WS * NT, _env("WAVEY", 4))
        SQ = _env("SQ", 110)
        sy0, sy1 = _env("SY0", 14), _env("SY1", 70)
        sdl = {sy0 + q * (sy1 - sy0) // max(NSY, 1): npair - NSY + q for q in range(NSY)}
        S3Q = _env("S3Q", 7)
        if S3Q:
            fillers = [functools.partial(f, ysteps[q * len(ysteps) // S3Q:(q + 1) * len(ysteps) // S3Q])
                       for q, f in enumerate(fillers)]
            ysteps = []
        d0, d1 = _env("TD0", 8), _env("TD1", 0)
        dl = {d0 + j * (nsc + d1 - d0) // len(t_items): j for j in range(len(t_items))}
        def emit_scores(n):
            nonlocal next_s
            for _ in range(n):
                p, i = divmod(next_s, 4)
                if i == 0:
                    prog.append((min(tm), pairs[p][0]))
                sj = []
                if next_s in sdl:
                    extra.append((min(tm) - _env("TLEAD", 300), pairs[sdl[next_s]][4]))
                    sj = [functools.partial(job_done.get, ("s", sdl[next_s]))]
                if next_s in dl:
                    extra.append((min(tm) - _env("TLEAD", 300), t_items[dl[next_s]]))
                s_end[p, i] = emit([SLOTS], functools.partial(
                    pairs[p][1], i, dl.get(next_s),
                    ysteps[next_s * len(ysteps) // SQ:(next_s + 1) * len(ysteps) // SQ] + sj))[0]
                if i % 2 == 1:
                    pend_v.append((max(s_end[p, i], s_end[p, i - 1]) + LSM, p, i // 2))
                next_s += 1

        def emit_values(n):
            for rdy, pv, hp in pend_v[:n]:
                for h in (2 * hp, 2 * hp + 1):
                    v_end[pv, h] = emit([DH], functools.partial(pairs[pv][2], h), rdy)[0]
                if hp == 1:
                    extra.append((max(v_end[pv, h] for h in range(NH)) + LFIN, pairs[pv][3]))
            del pend_v[:n]

        if _env("PLAN", 1) == 2:
            nfill, sk = len(fillers), _env("SK", 2)
            f0, f1 = _env("F0", 0.0), _env("F1", 1.0)
            blk = [int(f0 + q * (npair - f1 - f0) / (nfill - 1) + 0.5) for q in range(nfill)]
            emit_scores(4 * sk)
            for p in range(npair):
                ahead = sk - (1 if _env("TIGHT", 0) and (p in blk or p + 1 in blk) else 0)
                while next_s < min(4 * (p + ahead + 1), nsc):
                    emit_scores(4)
                if p in blk:
                    emit([C] * 3, fillers.pop(0))
                emit_values(2)
        while fillers or next_s < nsc or pend_v:
            now = tm[load.index(min(load))]
            s_ok = next_s < nsc and now >= t_0 + (total - TAILGAP - t_0) * next_s / (nsc - 4)
            v_ok = len(pend_v) >= VGRP // 2 and all(now >= x[0] for x in pend_v[:VGRP // 2])
            if not fillers and not s_ok and not v_ok:
                if pend_v and (next_s >= nsc or len(pend_v) >= 4):
                    v_ok = True
                else:
                    s_ok = True
            if v_ok:
                emit_values(VGRP // 2)
            elif s_ok:
                emit_scores(SGRP)
            else:
                emit([C] * 3, fillers.pop(0))
        if _env("VERB", 0):
            print("Y planned", tm, load)
        extra += [(max(tm) - 600, t_items[j]) for q, j in dl.items() if q >= nsc]
        run(prog, extra)

    only = _env("ONLY", "01")
    NODMA = _env("NODMA", 0)

    @when(k_ < (1 if NODMA & 1 else nstrip), ("first", "main"))
    def _():
        x_copy(k_).wait()

    new_masks("x")
    if "0" in only:
        when(k_ <= nstrip, ("main",))(block_x)

    @when(k_ == 0, ("first",))
    def _():
        def body(g, carry):
            for j in range(FG):
                piece = conv_group(pl.multiple_of((g * FG + j) * 8, 8))[1]
                for r in range(WS):
                    piece(r)
            return carry
        FG = _env("FG", 8)
        lax.fori_loop(0, NG // FG, body, 0)

    @when(k_ < (0 if NODMA & 1 else nstrip - 1), ("first", "main"))
    def _():
        x_copy(k_ + 1).start()

    @when(k_ >= (1000 if NODMA & 2 else 3), ("main", "last"))
    def _():
        o_copy(k_ - 3).wait()

    if "1" in only:
        new_masks("y")
        when((k_ <= nstrip) & (k_ >= 1), ("main",))(block_y)

    @when(k_ == 0, ("first",))
    def _():
        for j in range(WS * NT):
            for f in stats_steps(j):
                f()
        for f in t_items:
            f()

    @when(k_ == nstrip + 1, ("last",))
    def _():
        new_masks("y")
        for p in range(npair):
            pairs[p][4]()
        for f in s3_all:
            f()

    if only != "01":
        @when(dyn0 < 0, ("main",))
        def _():
            i = pl.multiple_of(k_ * 8, 8)
            o_ref[0, 0:16, 0:128] = _cat([
                qkv_ref[k3, k3, pl.ds(i, 8), :] + ms_ref[k3, 0:8, :] + stg_ref[k3, pl.ds(i, 8), :],
                pltpu.bitcast(t_ref[k3, k3, pl.ds(i, 8), :], F32) + ob_ref[pl.ds(i, 8), :]]).astype(BF16)
            for rf in (qkv_ref.at[k3, k3], stg_ref.at[k3], ob_ref):
                rf[pl.ds(i, 8), :] = zero8
            t_ref[k3, k3, pl.ds(i, 8), :] = pltpu.bitcast(zero8, U32)

    @when(k_ >= (nstrip + 1 if NODMA & 2 else 2), ("main", "last"))
    def _():
        o_copy(k_ - 2).start()

    @when(k_ == nstrip + 1, ("last",))
    def _():
        o_copy(k_ - 2).wait()


@jax.jit
def pallas_standalone__window_attn_davit__vision_kernel(
    x: jax.Array,
    dw_pe: jax.Array,
    w_qkv: jax.Array,
    w_o: jax.Array,
):
    B, H, W, Cx = x.shape
    assert B == 1 and Cx == C and H % WS == 0 and W % WS == 0 and WP - LANES < W < WP
    xt = jnp.transpose(x[0], (0, 2, 1))

    assert H // WS + 2 <= 256
    vmem = pl.BlockSpec(memory_space=pltpu.VMEM)
    yt = pl.pallas_call(
        functools.partial(_kernel, H=H, W=W),
        in_specs=[pl.BlockSpec(memory_space=pl.ANY), vmem, vmem, vmem],
        out_specs=pl.BlockSpec(memory_space=pl.ANY),
        out_shape=jax.ShapeDtypeStruct((H, C, W), x.dtype),
        scratch_shapes=[
            pltpu.VMEM((WS + 2, C, W), x.dtype),
            pltpu.VMEM((WS, C, W), x.dtype),
            pltpu.SemaphoreType.DMA((2,)),
            pltpu.VMEM((X0_ROWS, LANES), F32),
            pltpu.VMEM((WS * WP, LANES), F32),
            pltpu.VMEM((9, C, LANES), F32),
            pltpu.VMEM((3, 5, LANES // 2, LANES), U32),
            pltpu.VMEM((3, C // 2, LANES), U32),
            pltpu.VMEM((5, WS, WP, LANES), F32),
            pltpu.VMEM((NU, 3, LANES // 2, LANES), U32),
            pltpu.VMEM((37, LANES, LANES), F32),
            pltpu.VMEM((WS * NT, 16, LANES), F32),
            pltpu.VMEM((C, WP), F32),
        ],
        compiler_params=pltpu.CompilerParams(
            vmem_limit_bytes=64 * 1024 * 1024,
            disable_bounds_checks=bool(_env("NOBC", 1)),
        ),
        name="davit_window_attn",
    )(xt, dw_pe, w_qkv, w_o)
    return jnp.transpose(yt, (0, 2, 1))[None]
```

```python
import functools
import math
import os

import jax
import jax.numpy as jnp
from jax import lax
import jax.experimental.pallas as pl
import jax.experimental.pallas.tpu as pltpu

WS = 7
NH = 4
C = 192
DH = C // NH
NG = C // 8
LANES = 128
WP = 512
NT = WP // LANES
NU = WS * NT // 2
SLOTS = 8 * WS
EPS = 1e-5
F32 = jnp.float32
BF16 = jnp.bfloat16
U32 = jnp.uint32

X0_SLOT = WS * NT * C
DW_OFF = 3 * X0_SLOT
X0_ROWS = DW_OFF + 2 * C


def _dot(a, b):
    return jnp.dot(a, b, preferred_element_type=F32)


def _dot_nt(a, b):
    return lax.dot_general(a, b, (((1,), (1,)), ((), ())), preferred_element_type=F32)


def _cat(xs):
    return jnp.concatenate(xs, axis=0)


def _blocks(v):
    return [v[i:i + 8] for i in range(0, v.shape[0], 8)]


def _allred(x, op):
    for sh in (4, 2, 1):
        x = op(x, pltpu.roll(x, sh, 0))
    return x


def _env(name, default):
    return type(default)(os.environ.get(name, default))


def _kernel(x_hbm, dw_ref, wqkv_ref, wo_ref, o_hbm, *scratch, H, W):
    step = functools.partial(_step, x_hbm, dw_ref, wqkv_ref, wo_ref, o_hbm, *scratch, H=H, W=W)
    nstrip = H // WS

    def loop(lo, hi, mode):
        def body(k, carry):
            step(k_=k, mode=mode)
            return carry
        lax.fori_loop(lo, hi, body, 0)

    if "ONLY" not in os.environ:
        loop(0, 1, "first")
    loop(1 + _env("SKIP", 0), nstrip + 1, "main")
    if "ONLY" not in os.environ:
        loop(nstrip + 1, nstrip + 2, "last")


def _step(x_hbm, dw_ref, wqkv_ref, wo_ref, o_hbm,
          x_ref, o_ref, sems, x0_ref, ob_ref, dws_ref, ws_ref, wos_ref, qkv_ref, t_ref, stg_ref, ms_ref,
          top_ref, *, H, W, k_, mode):
    nstrip, nwin = H // WS, W // WS

    def x_copy(k):
        return pltpu.make_async_copy(x_hbm.at[pl.ds(jnp.minimum(k * WS, H - WS - 1), WS + 1)],
                                     x_ref.at[pl.ds(0, WS + 1)], sems.at[0])

    def o_copy(k):
        return pltpu.make_async_copy(o_ref, o_hbm.at[pl.ds(k * WS, WS)], sems.at[1])

    def when(cond, modes):
        if mode in modes:
            return pl.when(cond)
        return lambda f: None

    xoff = jnp.where(k_ >= nstrip - 1, 1, 0)
    dyn0 = jnp.minimum(k_, 0)

    def rows_at(base, off, n):
        if isinstance(base, int):
            return pl.ds(base + off, n)
        return pl.ds(pl.multiple_of(base + off, 8), n)

    mk = {}

    def new_masks(blk):
        lane = lax.broadcasted_iota(jnp.int32, (8, LANES), 1)
        mk.clear()
        mk["never"] = lane < dyn0
        if blk == "x":
            mk["up"] = lax.broadcasted_iota(jnp.int32, (8, LANES), 0) < 4
            return
        key_ok = lax.broadcasted_iota(jnp.int32, (8, LANES), 0) < WS
        mk.update(
            lo=lane < DH, hi0=(lane >= DH) & ((lane < 64) | (lane >= 96)), hi1=(lane >= DH) & (lane < 96),
            v=lane < 96, key=key_ok, keep_a=key_ok & (lane < SLOTS), keep_b=key_ok & (lane >= SLOTS),
            left64=lane < 64)

    k3 = k_ - 3 * ((k_ * 171) >> 9)
    nxt = k3 * X0_SLOT
    prv = jnp.where((k3 == 2) | (k_ < 2), 0, nxt + X0_SLOT)

    def conv_group(c0):
        st = {}

        def row(i):
            if i == 0 and i not in st:
                st[i] = top_ref[pl.ds(c0, 8), :]
            if i not in st:
                v = x_ref[xoff + (i - 1), pl.ds(c0, 8), :].astype(F32)
                st[i] = jnp.concatenate([v, jnp.zeros((8, WP - W), F32)], axis=1)
                if i == WS and i - 2 in st:
                    top_ref[pl.ds(c0, 8), :] = st[i]
            return st[i]

        def bc(v):
            return jnp.concatenate([v] * NT, axis=1)

        def taps(r):
            st["tw", r] = [bc(x0_ref[rows_at(c0, DW_OFF + k * C, 8), :]) for k in range(2)]

        def piece(r):
            if "w" not in st:
                st["w"] = [bc(dws_ref[k, pl.ds(c0, 8), :]) for k in range(9)]
            wts = list(st["w"])
            if ("tw", r) in st:
                wts[6], wts[8] = st["tw", r]
            row(r)
            abc = [row(r + 1) * wts[3 + j] + row(r) * wts[j] + row(r + 2) * wts[6 + j] for j in range(3)]
            x0 = pltpu.roll(abc[0], 1, 1) + abc[1] + pltpu.roll(abc[2], WP - 1, 1)
            for t in range(NT):
                x0_ref[rows_at(nxt, (r * NT + t) * C + c0, 8), :] = x0[:, t * LANES:(t + 1) * LANES]

        return taps, piece

    @when(k_ == 0, ("first",))
    def _():
        x_copy(0).start()
        for k in range(9):
            w = dw_ref[k // 3].astype(F32)[k % 3:k % 3 + 1, :]
            w = jnp.broadcast_to(w, (LANES, C)).T
            dws_ref[k] = w + 1.0 if k == 4 else w
            if k in (6, 8):
                x0_ref[pl.ds(DW_OFF + (k - 6) // 2 * C, C), :] = w
        w = wqkv_ref[...].astype(F32)
        wq = w[:, 0:C] * ((DH ** -0.5) * math.log2(math.e))
        wk, wv = w[:, C:2 * C], w[:, 2 * C:3 * C]
        tiles = [(wq[:, 0:64], wv[:, 64:96], wq[:, 64:96]),
                 (wq[:, 96:192], wv[:, 96:128]),
                 (wk[:, 0:64], wv[:, 128:160], wk[:, 64:96]),
                 (wk[:, 96:192], wv[:, 160:192]),
                 (wv[:, 0:128],)]
        for n, parts in enumerate(tiles):
            w = jnp.concatenate(parts, axis=1)
            for i, wi in enumerate((w[0:128], w[64:192], _cat([w[0:64], w[128:192]]))):
                if n == 4:
                    wi = wi.T
                ws_ref[i, n] = pltpu.bitcast(wi.astype(BF16), U32)
        w = wo_ref[...].astype(F32)
        wx, wy, wz = w[0:64], w[64:128], w[128:192]
        for i, parts in enumerate(((wx, wy), (wz, wy), (wx, wy + wz))):
            wos_ref[i] = pltpu.bitcast(_cat(parts).T.astype(BF16), U32)

        top_ref[...] = jnp.zeros(top_ref.shape, F32)
        x_ref[WS + 1] = jnp.zeros(x_ref.shape[1:], x_ref.dtype)

        for p in range(stg_ref.shape[0]):
            stg_ref[p] = jnp.zeros(stg_ref.shape[1:], F32)
        for r in range(WS):
            ob_ref[pl.ds(r * WP + WP - 8, 8), :] = jnp.zeros((8, LANES), F32)

    cuts = [int(c) for c in _env("CUTS", "0,7").split(",")]
    bands = list(zip(cuts, cuts[1:]))
    groups = {(b, g): conv_group(8 * g) for b in range(len(bands)) for g in range(NG)}
    WLEAD = _env("WLEAD", 4)

    def conv_items(nslow):
        plist = [((b, g), r) for b, (r0, r1) in enumerate(bands) for g in range(NG) for r in range(r0, r1)]
        items, nxt_tap = [], WLEAD
        for k, (g, r) in enumerate(plist):
            fs = []
            lead = WLEAD if k < nslow else _env("WLEAD2", 5)
            while nxt_tap <= min(k + lead, len(plist) - 1):
                g2, r2 = plist[nxt_tap]
                fs.append(functools.partial(groups[g2][0], r2))
                nxt_tap += 1
            fs.append(functools.partial(groups[g][1], r))
            items.append(fs)
        return items

    def ld_x0(j, k, gs=range(NG)):
        return [x0_ref[rows_at(nxt + dyn0 * (8 * k), j * C + 8 * g, 8), :] for g in gs]

    def add2(acc, xs):
        a = functools.reduce(jnp.add, xs[0::2])
        b = functools.reduce(jnp.add, xs[1::2])
        return a + b if acc is None else (acc + a) + b

    stats_done = set()

    def stats_steps(j):
        st = {"s": None, "q": None}
        n1, n2 = _env("SEG1", 8), _env("SEG2", 6)

        def sum_step(g0):
            st["s"] = add2(st["s"], ld_x0(j, 0, range(g0, g0 + n1)))
            if g0 + n1 == NG:
                st["s"] = _allred(st["s"], jnp.add) * (1.0 / C)
            return st["s"]

        def var_step(g0):
            d = [x - st["s"] for x in ld_x0(j, 1, range(g0, g0 + n2))]
            st["q"] = add2(st["q"], [x * x for x in d])
            return st["q"]

        def last_step():
            v = _allred(st["q"], jnp.add) * (1.0 / C) + EPS
            rs = lax.rsqrt(v) if _env("RSQ", 1) else jnp.exp2(jnp.log2(v) * -0.5)
            ms_ref[j] = _cat([st["s"], rs])
            stats_done.add(j)
            return rs

        return ([functools.partial(sum_step, g) for g in range(0, NG, n1)]
                + [functools.partial(var_step, g) for g in range(0, NG, n2)] + [last_step])

    def colsum(xs):
        xs = [a + b for a, b in zip(xs[0:8], xs[16:24])] + xs[8:16]
        return _dot(jnp.ones((8, LANES), F32), _cat(xs))

    means = {}

    def mean_dot(j):
        means[j] = colsum(ld_x0(j, 0)) * (1.0 / C)

    def var_dot(j):
        xs = [x0_ref[pl.ds(nxt + (j * C + 8 * g + 4), 8), :] for g in range(NG - 1)]
        xs.append(jnp.where(mk["up"], *ld_x0(j, 0, (0, NG - 1))))
        d = [x - means[j] for x in xs]
        v = colsum([x * x for x in d]) * (1.0 / C) + EPS
        rs = lax.rsqrt(v) if _env("RSQ", 1) else jnp.exp2(jnp.log2(v) * -0.5)
        ms_ref[j] = _cat([means[j], rs])
        stats_done.add(j)

    def normed(j, blk, k):
        assert j in stats_done or "ONLY" in os.environ and j < NSTX, j
        m, rs = ms_ref[j, 0:8, :], ms_ref[j, 8:16, :]
        return _cat([(x - m) * rs for x in ld_x0(j, k, range(8 * blk, 8 * blk + 8))])

    t_done = []

    def put_t(dst, tiles):
        tt = pltpu.bitcast(jnp.concatenate(tiles, axis=1).astype(BF16).T, U32)
        for i, (u, e) in enumerate(dst):
            t_ref[u, e] = tt[64 * i:64 * i + 64]
        t_done.append(pltpu.bitcast(tt[120:128], F32))

    def t_first(u):
        ja, jb = 2 * u, 2 * u + 1
        bx = normed(jb, 0, 0)
        put_t([(u, 0), (u, 2)], [_cat([normed(ja, 0, 0) - bx, normed(ja, 1, 0)]),
                                 _cat([bx, normed(ja, 2, 0)])])

    def t_second(r):
        put_t([(u, 1) for u in (2 * r, 2 * r + 1)],
              [_cat([normed(2 * u + 1, 1, 0), normed(2 * u + 1, 2, 0) - normed(2 * u, 2, _env("RECOMP", 1))])
               for u in (2 * r, 2 * r + 1)])

    t_items = []
    for r in range(WS):
        t_items += [functools.partial(t_first, 2 * r), functools.partial(t_first, 2 * r + 1),
                    functools.partial(t_second, r)]

    def qkv_chunk(us, n, steps=(), tiny=()):
        lhs = {i: [b for u in us for b in _blocks(t_ref[u, i])] for i in range(3)}
        for q, step in enumerate(steps):
            tok = pltpu.bitcast(step(), U32)
            q = q * 24 * len(us) // len(steps)
            blks = lhs[(2, 0, 1)[q % 3]]
            blks[q // 3] = jnp.where(mk["never"], tok, blks[q // 3])
        p3 = None
        for i in (2, 0, 1):
            p = _dot(pltpu.bitcast(_cat(lhs[i]), BF16), pltpu.bitcast(ws_ref[i, n], BF16))
            if p3 is None:
                p3 = p
            else:
                p = p + p3
                for e, u in enumerate(us):
                    r, tp = divmod(u, 2)
                    qkv_ref[n, r, pl.ds((2 * tp + i) * LANES, LANES), :] = p[e * LANES:(e + 1) * LANES]

    vr_words = {}
    job_done = {}

    def side_dots(u, n):
        r, tp = divmod(u, 2)
        st = {}

        def one(i, parts=1):
            if parts > 1:
                lhs, rows = t_ref[u, i], 64 // parts
                p = _cat([_dot(pltpu.bitcast(lhs[q * rows:(q + 1) * rows], BF16),
                               pltpu.bitcast(ws_ref[i, n], BF16)) for q in range(parts)])
            elif n == 4:
                p = _dot_nt(pltpu.bitcast(ws_ref[i, 4, 0:32, :], BF16), pltpu.bitcast(t_ref[u, i], BF16))
            else:
                p = _dot(pltpu.bitcast(t_ref[u, i], BF16), pltpu.bitcast(ws_ref[i, n], BF16))
            st[i] = p if i == 2 else p + st[2]
            if n < 4 and i < 2:
                qkv_ref[n, r, pl.ds((2 * tp + i) * LANES, LANES), :] = st[i]
            elif i == 1:
                vr_words[u] = pltpu.pack_elementwise([st[0], st[1]], packed_dtype=BF16)

        return [(64 if n == 4 else LANES, (u, n, i), functools.partial(one, i)) for i in (2, 0, 1)]

    def vr_store(u):
        r, tp = divmod(u, 2)
        w = pltpu.bitcast(vr_words[u], F32)
        wt = pltpu.bitcast(_cat([w, w]).T, U32)
        job_done["v", u] = pltpu.bitcast(wt[120:128], F32)
        for j in range(2):
            qkv_ref[4, r, pl.ds((2 * tp + j) * LANES, LANES), :] = pltpu.unpack_elementwise(
                wt, index=j, packed_dtype=BF16, unpacked_dtype=F32)

    zero8 = jnp.zeros((8, LANES), F32)

    def gather(n, off, k=0):
        return [qkv_ref[n, r, pl.ds(off + dyn0 * k if k else off, 8), :] for r in range(WS)]

    def softmax_t(st):
        rows = _blocks(st)
        m = functools.reduce(jnp.maximum, rows)
        m = _allred(jnp.where(mk["key"], m, -jnp.inf), jnp.maximum)
        p = [jnp.exp2(x - m) for x in rows]
        return p, functools.reduce(jnp.add, p)

    def s2_pair(pi, offa):
        offb = offa + WS
        st = {}

        def vprep():
            g = [gather(n, offa) + gather(n, offb) for n in range(5)]
            u1 = [jnp.where(mk["left64"], z, jnp.where(mk["v"], x, y)) for x, y, z in zip(g[0], g[1], g[4])]
            u2 = [jnp.where(mk["v"], x, y) for x, y in zip(g[2], g[3])]
            u = jnp.concatenate([_cat(u1 + [zero8, zero8]), _cat(u2 + [zero8, zero8])], axis=1)
            vt = pltpu.bitcast(u.astype(BF16).T, U32)
            vt = _cat([vt[0:64], vt[96:128]])
            st["vt"] = [pltpu.bitcast(vt[24 * h:24 * h + 24], BF16) for h in range(NH)]

        def score(i, after=None, steps=()):
            hp, sw = divmod(i, 2)
            lo, hi = mk["lo"], mk["hi%d" % hp]
            ma, mb = (lo, hi) if sw == 0 else (hi, lo)
            gq = (0, 1, 1 + sw)[_env("GQ", 0)]
            gk = (0, 1, 1 + sw)[_env("GK", 0)]
            q = _cat([jnp.where(ma, v, 0.0) for v in gather(hp, offa, gq)]
                     + [jnp.where(mb, v, 0.0) for v in gather(hp, offb, gq)] + [zero8, zero8])
            ka, kb = gather(2 + hp, offa, gk), gather(2 + hp, offb, gk)
            k = [jnp.where(lo, x, y) for x, y in (zip(ka, kb) if sw == 0 else zip(kb, ka))]
            if after is not None:
                k[0] = jnp.where(mk["never"], t_done[after], k[0])
            for q_, step in enumerate(steps):
                e = 1 + (q_ * 6) // len(steps)
                k[e] = jnp.where(mk["never"], step(), k[e])
            k = _cat(k)
            st["p", i] = softmax_t(_dot_nt(k, q))

        def value(h):
            hp, sw = divmod(h, 2)
            (pa, sa), (pb, sb) = st["p", 2 * hp + sw], st["p", 2 * hp + 1 - sw]
            pm = _cat([jnp.where(mk["keep_a"], v, 0.0) for v in pa]
                      + [jnp.where(mk["keep_b"], v, 0.0) for v in pb] + [zero8, zero8])
            den = _allred(jnp.where(mk["keep_a"], sa, jnp.where(mk["keep_b"], sb, 0.0)), jnp.add)
            rec = pl.reciprocal(den, approx=True)
            if _env("NR", 0):
                rec = rec * (2.0 - den * rec)
            st["o", h] = [b * rec for b in _blocks(_dot(st["vt"][h], pm))]

        def finish():
            o = [b for h in range(NH) for b in st["o", h]]
            w = pltpu.pack_elementwise([_cat(o[0:16]), _cat(o[16:24] + o[16:24])], packed_dtype=BF16)
            stg_ref[pi] = pltpu.bitcast(w, F32)

        def scatter():
            wt = stg_ref[pi].T
            job_done["s", pi] = wt[104:112]
            for i, off in enumerate((offa, offb)):
                for r in range(WS):
                    base = i * SLOTS + 8 * r
                    ob_ref[pl.ds(r * WP + off, WS), :] = wt[base:base + WS]

        return vprep, score, value, finish, scatter

    npair = (nwin + 1) // 2
    pairs = [s2_pair(p, min(2 * p, nwin - 2) * WS) for p in range(npair)]

    def s3_unit(r, tp, steps=()):
        def unpack(t):
            w = pltpu.bitcast(ob_ref[pl.ds(r * WP + t * LANES, LANES), :], U32)
            return [_blocks(pltpu.unpack_elementwise(w, index=i, packed_dtype=BF16, unpacked_dtype=F32))
                    for i in range(2)]

        (la, ha), (lb, hb) = unpack(2 * tp), unpack(2 * tp + 1)
        t3 = [jnp.where(mk["left64"], x, y) for x, y in zip(lb, ha)]
        t1 = _cat([x - y for x, y in zip(la, t3)])
        t2 = _cat([jnp.where(mk["left64"], x, z) - y for x, y, z in zip(hb, ha, lb)])
        t3 = _cat(t3)
        wo = [_blocks(wos_ref[i]) for i in range(3)]
        e0, e1 = _env("E0", 0), _env("E1", 8)
        for q, step in enumerate(steps):
            q = q * 3 * (e1 - e0) // len(steps)
            blks = wo[(2, 0, 1)[q % 3]]
            blks[e0 + q // 3] = jnp.where(mk["never"], pltpu.bitcast(step(), U32), blks[e0 + q // 3])
        wo = [pltpu.bitcast(_cat(w), BF16) for w in wo]
        p3 = _dot_nt(wo[2], t3)
        ys = [_dot_nt(wo[i], t) + p3
              + x0_ref[rows_at(prv, (r * NT + 2 * tp + i) * C, C), :] for i, t in enumerate((t1, t2))]
        n = min(2 * LANES, W - 2 * tp * LANES)
        o_ref[r, :, pl.ds(2 * tp * LANES, n)] = jnp.concatenate(ys, axis=1).astype(o_ref.dtype)[:, :n]

    s3_all = [functools.partial(s3_unit, r, tp) for tp in range(2) for r in range(WS)]

    def run(prog, extra):
        extra = sorted(extra, key=lambda e: e[0])
        j = 0
        for t0, fn in prog:
            while j < len(extra) and extra[j][0] <= t0:
                extra[j][1]()
                j += 1
            fn()
        for e in extra[j:]:
            e[1]()

    MERGE = _env("MERGE", 0)
    NX3 = _env("NX3", 0)

    NSY = _env("NSY", 0)

    NSTX = _env("NSTX", 16)

    def wave_steps(lo, hi, wave):
        steps = []
        for j0 in range(lo, hi, wave):
            for grp in zip(*[stats_steps(j) for j in range(j0, min(j0 + wave, hi))]):
                steps += grp
        return steps

    def block_x():
        NJ = _env("NJ", 28)
        NSTC = _env("NSTC", 6)
        WAVE = _env("WAVE", 4)
        VRLAG = _env("VRLAG", 200)
        chunks = [(u, n) for u in range(NU) for n in range(4)]
        MXS = _env("MXS", 0)
        steps = [] if MXS else wave_steps(0, NSTX, WAVE)
        nside = 9
        side, vstep = [], _env("VRSTEP", 1)
        for q in range(NU // 2):
            side += side_dots(2 * q, 4) + side_dots(2 * q + 1, 4)
            for _ in range(vstep):
                if nside:
                    side += side_dots(*chunks.pop())
                    nside -= 1
        for _ in range(nside):
            side += side_dots(*chunks.pop())
        mu = _env("MU", 2)
        merged = []
        for u, n in chunks:
            prev = [c for c in merged if c[1] == n and c[0][0] // mu == u // mu]
            if prev:
                prev[0][0].append(u)
            else:
                merged.append(([u], n))
        starts = [LANES * sum(len(c[0]) for c in merged[:k]) for k in range(len(merged))]
        t_conv = max(x for x in starts if x <= (len(chunks) - NSTC) * LANES)
        span = len(chunks) * LANES - t_conv
        plan, t, vr_ready = [], 0, {}
        for k, (us, n) in enumerate(merged):
            dur = LANES * len(us)
            lo, hi = (max(x - t_conv, 0) * len(steps) // span for x in (t, t + dur))
            plan.append((t, tuple(us), n, list(steps[lo:hi]), []))
            room = dur
            while side and (room > 0 or k == len(merged) - 1):
                rows, key, f = side.pop(0)
                plan.append((t, f if room > 0 else functools.partial(f, 4), None, [], []))
                room -= rows
                if key[1:] == (4, 1):
                    vr_ready[key[0]] = t + dur - room + VRLAG
            t += dur
        ci = conv_items(4 * NJ)
        slow = _env("SLOW", 32.0)
        fast = (t_conv - 4 * NJ * slow) / max(len(ci) - 4 * NJ, 1)
        t_piece = [min(j, 4 * NJ) * slow + max(j - 4 * NJ, 0) * fast for j in range(len(ci) + 1)]
        scat, vrs = list(range(npair - NSY)), list(range(NU))
        jobs = []
        for q in range(NJ):
            if vrs and vr_ready[vrs[0]] <= t_piece[4 * q + 1]:
                jobs.append((t_piece[4 * q + 1], ("v", vrs[0])))
                ci[4 * q].insert(0, functools.partial(vr_store, vrs.pop(0)))
            elif scat:
                jobs.append((t_piece[4 * q + 1], ("s", scat[0])))
                ci[4 * q].insert(0, pairs[scat.pop(0)][4])
        extra = [(t_piece[j + 1], f) for j, fs in enumerate(ci) for f in fs]
        tail = [(("v", u), functools.partial(vr_store, u)) for u in vrs] + [(("s", p), pairs[p][4]) for p in scat]
        for q, (key, f) in enumerate(tail):
            t_q = max(t_conv + 1 + (q // 3) * 128, vr_ready[key[1]] if key[0] == "v" else 0)
            extra.append((t_q, f))
            jobs.append((t_q, key))
        if _env("JDL", 800):
            for t_q, key in jobs:
                later = [e for e in plan if e[2] is not None and e[0] >= t_q + _env("JDL", 800)]
                if later:
                    later[0][3].insert(0, functools.partial(job_done.get, key))
        prog = [(t0, u if n is None else functools.partial(qkv_chunk, u, n, st, tn))
                for t0, u, n, st, tn in plan]
        run(prog, extra)

    def block_y():
        LSM = _env("LSM", 170)
        LFIN = _env("LFIN", 0)
        SGRP = _env("SGRP", 4)
        VGRP = _env("VGRP", 2)
        TAILGAP = _env("TAILGAP", 500)
        load = [LANES, LANES, 0, 0] if MERGE else [0] * 4
        tm = list(load)
        t_0 = LANES + _env("LQKV", 220) if MERGE else 0
        prog, extra, trace = [], [], []

        def emit(rows_list, fn, ready=0):
            prog.append((min(tm), fn))
            trace.append({SLOTS: "s", DH: "v", C: "F"}[rows_list[0]])
            ends = []
            for rows in rows_list:
                m = load.index(min(load))
                load[m] += rows
                tm[m] = max(tm[m], ready) + rows
                ends.append(tm[m])
            return ends

        fillers = list(s3_all[NX3:])
        total = len(fillers) * 3 * C / 4 + npair * (SLOTS + DH)
        nsc = 4 * npair
        next_s = 0
        s_end, v_end, pend_v = {}, {}, []
        t_done.clear()
        ysteps = wave_steps(NSTX, WS * NT, _env("WAVEY", 4))
        SQ = _env("SQ", 110)
        sy0, sy1 = _env("SY0", 14), _env("SY1", 70)
        sdl = {sy0 + q * (sy1 - sy0) // max(NSY, 1): npair - NSY + q for q in range(NSY)}
        S3Q = _env("S3Q", 7)
        if S3Q:
            fillers = [functools.partial(f, ysteps[q * len(ysteps) // S3Q:(q + 1) * len(ysteps) // S3Q])
                       for q, f in enumerate(fillers)]
            ysteps = []
        d0, d1 = _env("TD0", 8), _env("TD1", 0)
        dl = {d0 + j * (nsc + d1 - d0) // len(t_items): j for j in range(len(t_items))}
        def emit_scores(n):
            nonlocal next_s
            for _ in range(n):
                p, i = divmod(next_s, 4)
                if i == 0:
                    prog.append((min(tm), pairs[p][0]))
                sj = []
                if next_s in sdl:
                    extra.append((min(tm) - _env("TLEAD", 300), pairs[sdl[next_s]][4]))
                    sj = [functools.partial(job_done.get, ("s", sdl[next_s]))]
                if next_s in dl:
                    extra.append((min(tm) - _env("TLEAD", 300), t_items[dl[next_s]]))
                s_end[p, i] = emit([SLOTS], functools.partial(
                    pairs[p][1], i, dl.get(next_s),
                    ysteps[next_s * len(ysteps) // SQ:(next_s + 1) * len(ysteps) // SQ] + sj))[0]
                if i % 2 == 1:
                    pend_v.append((max(s_end[p, i], s_end[p, i - 1]) + LSM, p, i // 2))
                next_s += 1

        def emit_values(n):
            for rdy, pv, hp in pend_v[:n]:
                for h in (2 * hp, 2 * hp + 1):
                    v_end[pv, h] = emit([DH], functools.partial(pairs[pv][2], h), rdy)[0]
                if hp == 1:
                    extra.append((max(v_end[pv, h] for h in range(NH)) + LFIN, pairs[pv][3]))
            del pend_v[:n]

        if _env("PAT", ""):
            head, body = _env("PAT", "").split(".")
            for ch in head + body * 40:
                if ch == "S" and next_s < nsc:
                    emit_scores(4)
                elif ch == "s" and next_s < nsc:
                    emit_scores(2)
                elif ch == "V" and pend_v:
                    emit_values(2)
                elif ch == "v" and pend_v:
                    emit_values(1)
                elif ch == "F" and fillers:
                    emit([C] * 3, fillers.pop(0))
        if _env("PLAN", 1) == 2:
            nfill, sk = len(fillers), _env("SK", 2)
            f0, f1 = _env("F0", 0.0), _env("F1", 1.0)
            blk = [int(f0 + q * (npair - f1 - f0) / (nfill - 1) + 0.5) for q in range(nfill)]
            emit_scores(4 * sk)
            for p in range(npair):
                ahead = sk - (1 if _env("TIGHT", 0) and (p in blk or p + 1 in blk) else 0)
                while next_s < min(4 * (p + ahead + 1), nsc):
                    emit_scores(4)
                if p in blk:
                    emit([C] * 3, fillers.pop(0))
                emit_values(2)
        while fillers or next_s < nsc or pend_v:
            now = tm[load.index(min(load))]
            s_ok = next_s < nsc and now >= t_0 + (total - TAILGAP - t_0) * next_s / (nsc - 4)
            v_ok = len(pend_v) >= VGRP // 2 and all(now >= x[0] for x in pend_v[:VGRP // 2])
            if not fillers and not s_ok and not v_ok:
                if pend_v and (next_s >= nsc or len(pend_v) >= 4):
                    v_ok = True
                else:
                    s_ok = True
            if v_ok:
                emit_values(VGRP // 2)
            elif s_ok:
                emit_scores(SGRP)
            else:
                emit([C] * 3, fillers.pop(0))
        if _env("VERB", 0):
            print("Y planned bundles", tm, load, "".join(trace))
        extra += [(max(tm) - 600, t_items[j]) for q, j in dl.items() if q >= nsc]
        run(prog, extra)

    only = _env("ONLY", "01")
    NODMA = _env("NODMA", 0)

    @when(k_ < (1 if NODMA & 1 else nstrip), ("first", "main"))
    def _():
        x_copy(k_).wait()

    new_masks("x")
    if "0" in only:
        when(k_ <= nstrip, ("main",))(block_x)

    @when(k_ == 0, ("first",))
    def _():
        def body(g, carry):
            for j in range(FG):
                piece = conv_group(pl.multiple_of((g * FG + j) * 8, 8))[1]
                for r in range(WS):
                    piece(r)
            return carry
        FG = _env("FG", 8)
        lax.fori_loop(0, NG // FG, body, 0)

    @when(k_ < (0 if NODMA & 1 else nstrip - 1), ("first", "main"))
    def _():
        x_copy(k_ + 1).start()

    @when(k_ >= (1000 if NODMA & 2 else 3), ("main", "last"))
    def _():
        o_copy(k_ - 3).wait()

    if "1" in only:
        new_masks("y")
        when((k_ <= nstrip) & (k_ >= 1), ("main",))(block_y)

    @when(k_ == 0, ("first",))
    def _():
        for j in range(WS * NT):
            for f in stats_steps(j):
                f()
        for f in t_items:
            f()

    @when(k_ == nstrip + 1, ("last",))
    def _():
        new_masks("y")
        for p in range(npair):
            pairs[p][4]()
        for f in s3_all:
            f()

    if only != "01":
        @when(dyn0 < 0, ("main",))
        def _():
            i = pl.multiple_of(k_ * 8, 8)
            o_ref[0, 0:16, 0:128] = _cat([
                qkv_ref[k3, k3, pl.ds(i, 8), :] + ms_ref[k3, 0:8, :] + stg_ref[k3, pl.ds(i, 8), :],
                pltpu.bitcast(t_ref[k3, k3, pl.ds(i, 8), :], F32) + ob_ref[pl.ds(i, 8), :]]).astype(BF16)
            for rf in (qkv_ref.at[k3, k3], stg_ref.at[k3], ob_ref):
                rf[pl.ds(i, 8), :] = zero8
            t_ref[k3, k3, pl.ds(i, 8), :] = pltpu.bitcast(zero8, U32)

    @when(k_ >= (nstrip + 1 if NODMA & 2 else 2), ("main", "last"))
    def _():
        o_copy(k_ - 2).start()

    @when(k_ == nstrip + 1, ("last",))
    def _():
        o_copy(k_ - 2).wait()


@jax.jit
def pallas_standalone__window_attn_davit__vision_kernel(
    x: jax.Array,
    dw_pe: jax.Array,
    w_qkv: jax.Array,
    w_o: jax.Array,
):
    B, H, W, Cx = x.shape
    assert B == 1 and Cx == C and H % WS == 0 and W % WS == 0 and WP - LANES < W < WP
    xt = jnp.transpose(x[0], (0, 2, 1))

    assert H // WS + 2 <= 256
    vmem = pl.BlockSpec(memory_space=pltpu.VMEM)
    yt = pl.pallas_call(
        functools.partial(_kernel, H=H, W=W),
        in_specs=[pl.BlockSpec(memory_space=pl.ANY), vmem, vmem, vmem],
        out_specs=pl.BlockSpec(memory_space=pl.ANY),
        out_shape=jax.ShapeDtypeStruct((H, C, W), x.dtype),
        scratch_shapes=[
            pltpu.VMEM((WS + 2, C, W), x.dtype),
            pltpu.VMEM((WS, C, W), x.dtype),
            pltpu.SemaphoreType.DMA((2,)),
            pltpu.VMEM((X0_ROWS, LANES), F32),
            pltpu.VMEM((WS * WP, LANES), F32),
            pltpu.VMEM((9, C, LANES), F32),
            pltpu.VMEM((3, 5, LANES // 2, LANES), U32),
            pltpu.VMEM((3, C // 2, LANES), U32),
            pltpu.VMEM((5, WS, WP, LANES), F32),
            pltpu.VMEM((NU, 3, LANES // 2, LANES), U32),
            pltpu.VMEM((37, LANES, LANES), F32),
            pltpu.VMEM((WS * NT, 16, LANES), F32),
            pltpu.VMEM((C, WP), F32),
        ],
        compiler_params=pltpu.CompilerParams(
            vmem_limit_bytes=64 * 1024 * 1024,
            disable_bounds_checks=bool(_env("NOBC", 1)),
        ),
        name="davit_window_attn",
    )(xt, dw_pe, w_qkv, w_o)
    return jnp.transpose(yt, (0, 2, 1))[None]
```

```python
import functools
import math
import os

import jax
import jax.numpy as jnp
from jax import lax
import jax.experimental.pallas as pl
import jax.experimental.pallas.tpu as pltpu

WS = 7
NH = 4
C = 192
DH = C // NH
NG = C // 8
LANES = 128
WP = 512
NT = WP // LANES
NU = WS * NT // 2
SLOTS = 8 * WS
EPS = 1e-5
F32 = jnp.float32
BF16 = jnp.bfloat16
U32 = jnp.uint32

X0_SLOT = WS * NT * C
DW_OFF = 3 * X0_SLOT
X0_ROWS = DW_OFF + 2 * C


def _dot(a, b):
    return jnp.dot(a, b, preferred_element_type=F32)


def _dot_nt(a, b):
    return lax.dot_general(a, b, (((1,), (1,)), ((), ())), preferred_element_type=F32)


def _cat(xs):
    return jnp.concatenate(xs, axis=0)


def _blocks(v):
    return [v[i:i + 8] for i in range(0, v.shape[0], 8)]


def _allred(x, op):
    for sh in (4, 2, 1):
        x = op(x, pltpu.roll(x, sh, 0))
    return x


def _env(name, default):
    return type(default)(os.environ.get(name, default))


def _kernel(x_hbm, dw_ref, wqkv_ref, wo_ref, o_hbm, *scratch, H, W):
    step = functools.partial(_step, x_hbm, dw_ref, wqkv_ref, wo_ref, o_hbm, *scratch, H=H, W=W)
    nstrip = H // WS

    def loop(lo, hi, mode):
        def body(k, carry):
            step(k_=k, mode=mode)
            return carry
        lax.fori_loop(lo, hi, body, 0)

    if "ONLY" not in os.environ:
        loop(0, 1, "first")
    loop(1 + _env("SKIP", 0), nstrip + 1, "main")
    if "ONLY" not in os.environ:
        loop(nstrip + 1, nstrip + 2, "last")


def _step(x_hbm, dw_ref, wqkv_ref, wo_ref, o_hbm,
          x_ref, o_ref, sems, x0_ref, ob_ref, dws_ref, ws_ref, wos_ref, qkv_ref, t_ref, stg_ref, ms_ref,
          top_ref, *, H, W, k_, mode):
    nstrip, nwin = H // WS, W // WS

    def x_copy(k):
        return pltpu.make_async_copy(x_hbm.at[pl.ds(jnp.minimum(k * WS, H - WS - 1), WS + 1)],
                                     x_ref.at[pl.ds(0, WS + 1)], sems.at[0])

    def o_copy(k):
        return pltpu.make_async_copy(o_ref, o_hbm.at[pl.ds(k * WS, WS)], sems.at[1])

    def when(cond, modes):
        if mode in modes:
            return pl.when(cond)
        return lambda f: None

    xoff = jnp.where(k_ >= nstrip - 1, 1, 0)
    dyn0 = jnp.minimum(k_, 0)

    def rows_at(base, off, n):
        if isinstance(base, int):
            return pl.ds(base + off, n)
        return pl.ds(pl.multiple_of(base + off, 8), n)

    mk = {}

    def new_masks(blk):
        lane = lax.broadcasted_iota(jnp.int32, (8, LANES), 1)
        mk.clear()
        mk["never"] = lane < dyn0
        if blk == "x":
            mk["up"] = lax.broadcasted_iota(jnp.int32, (8, LANES), 0) < 4
            return
        key_ok = lax.broadcasted_iota(jnp.int32, (8, LANES), 0) < WS
        mk.update(
            lo=lane < DH, hi0=(lane >= DH) & ((lane < 64) | (lane >= 96)), hi1=(lane >= DH) & (lane < 96),
            v=lane < 96, key=key_ok, keep_a=key_ok & (lane < SLOTS), keep_b=key_ok & (lane >= SLOTS),
            left64=lane < 64)

    k3 = k_ - 3 * ((k_ * 171) >> 9)
    nxt = k3 * X0_SLOT
    prv = jnp.where((k3 == 2) | (k_ < 2), 0, nxt + X0_SLOT)

    def conv_group(c0):
        st = {}

        def row(i):
            if i == 0 and i not in st:
                st[i] = top_ref[pl.ds(c0, 8), :]
            if i not in st:
                v = x_ref[xoff + (i - 1), pl.ds(c0, 8), :].astype(F32)
                st[i] = jnp.concatenate([v, jnp.zeros((8, WP - W), F32)], axis=1)
                if i == WS and i - 2 in st:
                    top_ref[pl.ds(c0, 8), :] = st[i]
            return st[i]

        def bc(v):
            return jnp.concatenate([v] * NT, axis=1)

        def taps(r):
            st["tw", r] = [bc(x0_ref[rows_at(c0, DW_OFF + k * C, 8), :]) for k in range(2)]

        def piece(r):
            if "w" not in st:
                st["w"] = [bc(dws_ref[k, pl.ds(c0, 8), :]) for k in range(9)]
            wts = list(st["w"])
            if ("tw", r) in st:
                wts[6], wts[8] = st["tw", r]
            row(r)
            abc = [row(r + 1) * wts[3 + j] + row(r) * wts[j] + row(r + 2) * wts[6 + j] for j in range(3)]
            x0 = pltpu.roll(abc[0], 1, 1) + abc[1] + pltpu.roll(abc[2], WP - 1, 1)
            for t in range(NT):
                x0_ref[rows_at(nxt, (r * NT + t) * C + c0, 8), :] = x0[:, t * LANES:(t + 1) * LANES]

        return taps, piece

    @when(k_ == 0, ("first",))
    def _():
        x_copy(0).start()
        for k in range(9):
            w = dw_ref[k // 3].astype(F32)[k % 3:k % 3 + 1, :]
            w = jnp.broadcast_to(w, (LANES, C)).T
            dws_ref[k] = w + 1.0 if k == 4 else w
            if k in (6, 8):
                x0_ref[pl.ds(DW_OFF + (k - 6) // 2 * C, C), :] = w
        w = wqkv_ref[...].astype(F32)
        wq = w[:, 0:C] * ((DH ** -0.5) * math.log2(math.e))
        wk, wv = w[:, C:2 * C], w[:, 2 * C:3 * C]
        tiles = [(wq[:, 0:64], wv[:, 64:96], wq[:, 64:96]),
                 (wq[:, 96:192], wv[:, 96:128]),
                 (wk[:, 0:64], wv[:, 128:160], wk[:, 64:96]),
                 (wk[:, 96:192], wv[:, 160:192]),
                 (wv[:, 0:128],)]
        for n, parts in enumerate(tiles):
            w = jnp.concatenate(parts, axis=1)
            for i, wi in enumerate((w[0:128], w[64:192], _cat([w[0:64], w[128:192]]))):
                if n == 4:
                    wi = wi.T
                ws_ref[i, n] = pltpu.bitcast(wi.astype(BF16), U32)
        w = wo_ref[...].astype(F32)
        wx, wy, wz = w[0:64], w[64:128], w[128:192]
        for i, parts in enumerate(((wx, wy), (wz, wy), (wx, wy + wz))):
            wos_ref[i] = pltpu.bitcast(_cat(parts).T.astype(BF16), U32)

        top_ref[...] = jnp.zeros(top_ref.shape, F32)
        x_ref[WS + 1] = jnp.zeros(x_ref.shape[1:], x_ref.dtype)

        for p in range(stg_ref.shape[0]):
            stg_ref[p] = jnp.zeros(stg_ref.shape[1:], F32)
        for r in range(WS):
            ob_ref[pl.ds(r * WP + WP - 8, 8), :] = jnp.zeros((8, LANES), F32)

    cuts = [int(c) for c in _env("CUTS", "0,7").split(",")]
    bands = list(zip(cuts, cuts[1:]))
    groups = {(b, g): conv_group(8 * g) for b in range(len(bands)) for g in range(NG)}
    WLEAD = _env("WLEAD", 4)

    def conv_items(nslow):
        plist = [((b, g), r) for b, (r0, r1) in enumerate(bands) for g in range(NG) for r in range(r0, r1)]
        items, nxt_tap = [], WLEAD
        for k, (g, r) in enumerate(plist):
            fs = []
            lead = WLEAD if k < nslow else _env("WLEAD2", 5)
            while nxt_tap <= min(k + lead, len(plist) - 1):
                g2, r2 = plist[nxt_tap]
                fs.append(functools.partial(groups[g2][0], r2))
                nxt_tap += 1
            fs.append(functools.partial(groups[g][1], r))
            items.append(fs)
        return items

    def ld_x0(j, k, gs=range(NG)):
        return [x0_ref[rows_at(nxt + dyn0 * (8 * k), j * C + 8 * g, 8), :] for g in gs]

    def add2(acc, xs):
        a = functools.reduce(jnp.add, xs[0::2])
        b = functools.reduce(jnp.add, xs[1::2])
        return a + b if acc is None else (acc + a) + b

    stats_done = set()

    def stats_steps(j):
        st = {"s": None, "q": None}
        n1, n2 = _env("SEG1", 8), _env("SEG2", 6)

        def sum_step(g0):
            st["s"] = add2(st["s"], ld_x0(j, 0, range(g0, g0 + n1)))
            if g0 + n1 == NG:
                st["s"] = _allred(st["s"], jnp.add) * (1.0 / C)
            return st["s"]

        def var_step(g0):
            d = [x - st["s"] for x in ld_x0(j, 1, range(g0, g0 + n2))]
            st["q"] = add2(st["q"], [x * x for x in d])
            return st["q"]

        def last_step():
            v = _allred(st["q"], jnp.add) * (1.0 / C) + EPS
            rs = lax.rsqrt(v) if _env("RSQ", 1) else jnp.exp2(jnp.log2(v) * -0.5)
            ms_ref[j] = _cat([st["s"], rs])
            stats_done.add(j)
            return rs

        return ([functools.partial(sum_step, g) for g in range(0, NG, n1)]
                + [functools.partial(var_step, g) for g in range(0, NG, n2)] + [last_step])

    def colsum(xs):
        xs = [a + b for a, b in zip(xs[0:8], xs[16:24])] + xs[8:16]
        return _dot(jnp.ones((8, LANES), F32), _cat(xs))

    means = {}

    def mean_dot(j):
        means[j] = colsum(ld_x0(j, 0)) * (1.0 / C)

    def var_dot(j):
        xs = [x0_ref[pl.ds(nxt + (j * C + 8 * g + 4), 8), :] for g in range(NG - 1)]
        xs.append(jnp.where(mk["up"], *ld_x0(j, 0, (0, NG - 1))))
        d = [x - means[j] for x in xs]
        v = colsum([x * x for x in d]) * (1.0 / C) + EPS
        rs = lax.rsqrt(v) if _env("RSQ", 1) else jnp.exp2(jnp.log2(v) * -0.5)
        ms_ref[j] = _cat([means[j], rs])
        stats_done.add(j)

    def normed(j, blk, k):
        assert j in stats_done or "ONLY" in os.environ and j < NSTX, j
        m, rs = ms_ref[j, 0:8, :], ms_ref[j, 8:16, :]
        return _cat([(x - m) * rs for x in ld_x0(j, k, range(8 * blk, 8 * blk + 8))])

    t_done = {}

    def put_t(dst, tiles):
        tt = pltpu.bitcast(jnp.concatenate(tiles, axis=1).astype(BF16).T, U32)
        for i, (u, e) in enumerate(dst):
            t_ref[u, e] = tt[64 * i:64 * i + 64]
        t_done[len(t_done)] = pltpu.bitcast(tt[120:128], F32)

    def t_first(u):
        ja, jb = 2 * u, 2 * u + 1
        bx = normed(jb, 0, 0)
        put_t([(u, 0), (u, 2)], [_cat([normed(ja, 0, 0) - bx, normed(ja, 1, 0)]),
                                 _cat([bx, normed(ja, 2, 0)])])

    def t_second(r):
        put_t([(u, 1) for u in (2 * r, 2 * r + 1)],
              [_cat([normed(2 * u + 1, 1, 0), normed(2 * u + 1, 2, 0) - normed(2 * u, 2, _env("RECOMP", 1))])
               for u in (2 * r, 2 * r + 1)])

    t_items = []
    for r in range(WS):
        t_items += [functools.partial(t_first, 2 * r), functools.partial(t_first, 2 * r + 1),
                    functools.partial(t_second, r)]

    def qkv_chunk(us, n, steps=(), tiny=()):
        lhs = {i: [b for u in us for b in _blocks(t_ref[u, i])] for i in range(3)}
        for q, step in enumerate(steps):
            tok = pltpu.bitcast(step(), U32)
            q = q * 24 * len(us) // len(steps)
            blks = lhs[(2, 0, 1)[q % 3]]
            blks[q // 3] = jnp.where(mk["never"], tok, blks[q // 3])
        p3 = None
        for i in (2, 0, 1):
            p = _dot(pltpu.bitcast(_cat(lhs[i]), BF16), pltpu.bitcast(ws_ref[i, n], BF16))
            if p3 is None:
                p3 = p
            else:
                p = p + p3
                for e, u in enumerate(us):
                    r, tp = divmod(u, 2)
                    qkv_ref[n, r, pl.ds((2 * tp + i) * LANES, LANES), :] = p[e * LANES:(e + 1) * LANES]

    vr_words = {}
    job_done = {}

    def side_dots(u, n):
        r, tp = divmod(u, 2)
        st = {}

        def one(i, parts=1):
            if parts > 1:
                lhs, rows = t_ref[u, i], 64 // parts
                p = _cat([_dot(pltpu.bitcast(lhs[q * rows:(q + 1) * rows], BF16),
                               pltpu.bitcast(ws_ref[i, n], BF16)) for q in range(parts)])
            elif n == 4:
                p = _dot_nt(pltpu.bitcast(ws_ref[i, 4, 0:32, :], BF16), pltpu.bitcast(t_ref[u, i], BF16))
            else:
                p = _dot(pltpu.bitcast(t_ref[u, i], BF16), pltpu.bitcast(ws_ref[i, n], BF16))
            st[i] = p if i == 2 else p + st[2]
            if n < 4 and i < 2:
                qkv_ref[n, r, pl.ds((2 * tp + i) * LANES, LANES), :] = st[i]
            elif i == 1:
                vr_words[u] = pltpu.pack_elementwise([st[0], st[1]], packed_dtype=BF16)

        return [(64 if n == 4 else LANES, (u, n, i), functools.partial(one, i)) for i in (2, 0, 1)]

    def vr_store(u):
        r, tp = divmod(u, 2)
        w = pltpu.bitcast(vr_words[u], F32)
        wt = pltpu.bitcast(_cat([w, w]).T, U32)
        job_done["v", u] = pltpu.bitcast(wt[120:128], F32)
        for j in range(2):
            qkv_ref[4, r, pl.ds((2 * tp + j) * LANES, LANES), :] = pltpu.unpack_elementwise(
                wt, index=j, packed_dtype=BF16, unpacked_dtype=F32)

    zero8 = jnp.zeros((8, LANES), F32)

    def gather(n, off, k=0):
        return [qkv_ref[n, r, pl.ds(off + dyn0 * k if k else off, 8), :] for r in range(WS)]

    def softmax_t(st):
        rows = _blocks(st)
        m = functools.reduce(jnp.maximum, rows)
        m = _allred(jnp.where(mk["key"], m, -jnp.inf), jnp.maximum)
        p = [jnp.exp2(x - m) for x in rows]
        return p, functools.reduce(jnp.add, p)

    def s2_pair(pi, offa):
        offb = offa + WS
        st = {}

        def vprep():
            g = [gather(n, offa) + gather(n, offb) for n in range(5)]
            u1 = [jnp.where(mk["left64"], z, jnp.where(mk["v"], x, y)) for x, y, z in zip(g[0], g[1], g[4])]
            u2 = [jnp.where(mk["v"], x, y) for x, y in zip(g[2], g[3])]
            u = jnp.concatenate([_cat(u1 + [zero8, zero8]), _cat(u2 + [zero8, zero8])], axis=1)
            vt = pltpu.bitcast(u.astype(BF16).T, U32)
            vt = _cat([vt[0:64], vt[96:128]])
            st["vt"] = [pltpu.bitcast(vt[24 * h:24 * h + 24], BF16) for h in range(NH)]

        def score(i, ties=()):
            hp, sw = divmod(i, 2)
            lo, hi = mk["lo"], mk["hi%d" % hp]
            ma, mb = (lo, hi) if sw == 0 else (hi, lo)
            gq = (0, 1, 1 + sw)[_env("GQ", 0)]
            gk = (0, 1, 1 + sw)[_env("GK", 0)]
            q = _cat([jnp.where(ma, v, 0.0) for v in gather(hp, offa, gq)]
                     + [jnp.where(mb, v, 0.0) for v in gather(hp, offb, gq)] + [zero8, zero8])
            ka, kb = gather(2 + hp, offa, gk), gather(2 + hp, offb, gk)
            k = [jnp.where(lo, x, y) for x, y in (zip(ka, kb) if sw == 0 else zip(kb, ka))]
            for _, job in ties:
                k[0] = jnp.where(mk["never"], job(), k[0])
            k = _cat(k)
            st["p", i] = softmax_t(_dot_nt(k, q))

        def value(h):
            hp, sw = divmod(h, 2)
            (pa, sa), (pb, sb) = st["p", 2 * hp + sw], st["p", 2 * hp + 1 - sw]
            pm = _cat([jnp.where(mk["keep_a"], v, 0.0) for v in pa]
                      + [jnp.where(mk["keep_b"], v, 0.0) for v in pb] + [zero8, zero8])
            den = _allred(jnp.where(mk["keep_a"], sa, jnp.where(mk["keep_b"], sb, 0.0)), jnp.add)
            rec = pl.reciprocal(den, approx=True)
            if _env("NR", 0):
                rec = rec * (2.0 - den * rec)
            st["o", h] = [b * rec for b in _blocks(_dot(st["vt"][h], pm))]

        def finish():
            o = [b for h in range(NH) for b in st["o", h]]
            w = pltpu.pack_elementwise([_cat(o[0:16]), _cat(o[16:24] + o[16:24])], packed_dtype=BF16)
            stg_ref[pi] = pltpu.bitcast(w, F32)

        def scatter():
            wt = stg_ref[pi].T
            job_done["s", pi] = wt[104:112]
            for i, off in enumerate((offa, offb)):
                for r in range(WS):
                    base = i * SLOTS + 8 * r
                    ob_ref[pl.ds(r * WP + off, WS), :] = wt[base:base + WS]

        return vprep, score, value, finish, scatter

    npair = (nwin + 1) // 2
    pairs = [s2_pair(p, min(2 * p, nwin - 2) * WS) for p in range(npair)]

    def s3_unit(r, tp, ties=()):
        def unpack(t):
            w = pltpu.bitcast(ob_ref[pl.ds(r * WP + t * LANES, LANES), :], U32)
            return [_blocks(pltpu.unpack_elementwise(w, index=i, packed_dtype=BF16, unpacked_dtype=F32))
                    for i in range(2)]

        (la, ha), (lb, hb) = unpack(2 * tp), unpack(2 * tp + 1)
        t3 = [jnp.where(mk["left64"], x, y) for x, y in zip(lb, ha)]
        t1 = _cat([x - y for x, y in zip(la, t3)])
        t2 = _cat([jnp.where(mk["left64"], x, z) - y for x, y, z in zip(hb, ha, lb)])
        t3 = _cat(t3)
        wo = [_blocks(wos_ref[i]) for i in range(3)]
        for q, (e, job) in enumerate(ties):
            blks = wo[(2, 0, 1)[q % 3]]
            blks[e] = jnp.where(mk["never"], pltpu.bitcast(job(), U32), blks[e])
        wo = [pltpu.bitcast(_cat(w), BF16) for w in wo]
        p3 = _dot_nt(wo[2], t3)
        ys = [_dot_nt(wo[i], t) + p3
              + x0_ref[rows_at(prv, (r * NT + 2 * tp + i) * C, C), :] for i, t in enumerate((t1, t2))]
        n = min(2 * LANES, W - 2 * tp * LANES)
        o_ref[r, :, pl.ds(2 * tp * LANES, n)] = jnp.concatenate(ys, axis=1).astype(o_ref.dtype)[:, :n]

    s3_all = [functools.partial(s3_unit, r, tp) for tp in range(2) for r in range(WS)]

    def run(prog, extra):
        extra = sorted(extra, key=lambda e: e[0])
        j = 0
        for t0, fn in prog:
            while j < len(extra) and extra[j][0] <= t0:
                extra[j][1]()
                j += 1
            fn()
        for e in extra[j:]:
            e[1]()

    MERGE = _env("MERGE", 0)
    NX3 = _env("NX3", 0)

    NSY = 0

    NSTX = _env("NSTX", 20)

    def wave_steps(lo, hi, wave):
        steps = []
        for j0 in range(lo, hi, wave):
            for grp in zip(*[stats_steps(j) for j in range(j0, min(j0 + wave, hi))]):
                steps += grp
        return steps

    def block_x():
        NJ = _env("NJ", 28)
        NSTC = _env("NSTC", 6)
        WAVE = _env("WAVE", 4)
        VRLAG = _env("VRLAG", 200)
        chunks = [(u, n) for u in range(NU) for n in range(4)]
        MXS = _env("MXS", 0)
        steps = [] if MXS else wave_steps(0, NSTX, WAVE)
        loose = steps[len(steps) - _env("LOOSE", 0):]
        steps = steps[:len(steps) - len(loose)]
        nside = 9
        side, vstep = [], _env("VRSTEP", 1)
        for q in range(NU // 2):
            side += side_dots(2 * q, 4) + side_dots(2 * q + 1, 4)
            for _ in range(vstep):
                if nside:
                    side += side_dots(*chunks.pop())
                    nside -= 1
        for _ in range(nside):
            side += side_dots(*chunks.pop())
        mu = _env("MU", 2)
        merged = []
        for u, n in chunks:
            prev = [c for c in merged if c[1] == n and c[0][0] // mu == u // mu]
            if prev:
                prev[0][0].append(u)
            else:
                merged.append(([u], n))
        starts = [LANES * sum(len(c[0]) for c in merged[:k]) for k in range(len(merged))]
        t_conv = max(x for x in starts if x <= (len(chunks) - NSTC) * LANES)
        span = len(chunks) * LANES - t_conv
        plan, t, vr_ready = [], 0, {}
        for k, (us, n) in enumerate(merged):
            dur = LANES * len(us)
            lo, hi = (max(x - t_conv, 0) * len(steps) // span for x in (t, t + dur))
            plan.append((t, tuple(us), n, list(steps[lo:hi]), []))
            room = dur
            while side and (room > 0 or k == len(merged) - 1):
                rows, key, f = side.pop(0)
                plan.append((t, f if room > 0 else functools.partial(f, 4), None, [], []))
                room -= rows
                if key[1:] == (4, 1):
                    vr_ready[key[0]] = t + dur - room + VRLAG
            t += dur
        ci = conv_items(4 * NJ)
        slow = _env("SLOW", 32.0)
        fast = (t_conv - 4 * NJ * slow) / max(len(ci) - 4 * NJ, 1)
        t_piece = [min(j, 4 * NJ) * slow + max(j - 4 * NJ, 0) * fast for j in range(len(ci) + 1)]
        scat, vrs = list(range(npair - NSY)), list(range(NU))
        jobs = []
        for q in range(NJ):
            if vrs and vr_ready[vrs[0]] <= t_piece[4 * q + 1]:
                jobs.append((t_piece[4 * q + 1], ("v", vrs[0])))
                ci[4 * q].insert(0, functools.partial(vr_store, vrs.pop(0)))
            elif scat:
                jobs.append((t_piece[4 * q + 1], ("s", scat[0])))
                ci[4 * q].insert(0, pairs[scat.pop(0)][4])
        extra = [(t_piece[j + 1], f) for j, fs in enumerate(ci) for f in fs]
        tail = [(("v", u), functools.partial(vr_store, u)) for u in vrs] + [(("s", p), pairs[p][4]) for p in scat]
        for q, (key, f) in enumerate(tail):
            t_q = max(t_conv + 1 + (q // 3) * 128, vr_ready[key[1]] if key[0] == "v" else 0)
            extra.append((t_q, f))
            jobs.append((t_q, key))
        if _env("JDL", 800):
            for t_q, key in jobs:
                later = [e for e in plan if e[2] is not None and e[0] >= t_q + _env("JDL", 800)]
                if later:
                    later[0][3].insert(0, functools.partial(job_done.get, key))
        prog = [(t0, u if n is None else functools.partial(qkv_chunk, u, n, st, tn))
                for t0, u, n, st, tn in plan]
        run(prog, extra + [(t, f) for f in loose])

    def block_y():
        pattern = _env("PAT", "SFFVFFFF" + "SSSSFVVVV" * 8 + "SSSSVVVV").rstrip(".")
        load = [0] * 4
        items, ns, nv, nf = [], 0, 0, 0
        for ch in pattern:
            if ch in "Ss":
                todo = [("s", ns + i, [SLOTS]) for i in range(4 if ch == "S" else 2)]
                ns += len(todo)
            elif ch in "Vv":
                todo = [("v", nv + i, [DH]) for i in range(4 if ch == "V" else 2)]
                nv += len(todo)
            else:
                todo = [("f", nf, [C] * 3)]
                nf += 1
            for kind, idx, rows in todo:
                items.append((min(load), kind, idx, []))
                for x in rows:
                    load[load.index(min(load))] += x
        assert (ns, nv, nf) == (4 * npair, 4 * npair, NU)
        spots = sorted([(it[0], it, 0) for it in items if it[1] == "s"]
                       + [(it[0] + 16 * e, it, e) for it in items if it[1] == "f" for e in range(12)],
                       key=lambda x: x[0])
        ysteps = wave_steps(NSTX, WS * NT, _env("WAVEY", 4))
        fspots = [x for x in spots if x[1][1] == "f" and x[1][2] < _env("S3Q", 6)
                  and _env("E0", 1) <= x[2] < _env("E1", 8)]
        fspots.sort(key=lambda x: (x[1][2], x[2]))
        for q, step in enumerate(ysteps):
            _, it, e = fspots[q * len(fspots) // len(ysteps)]
            it[3].append((e, step))
        t_done.clear()
        extra = []
        tpos = [int(x) for x in _env("TPOS", "8,9").split(",")]
        late = [x for x in spots if x[1][1] == "s" and x[1][2] >= 4 and (x[1][2] - 4) % 16 in tpos]
        late.sort(key=lambda x: x[1][2])
        n1 = max(_env("NT1", 3), len(t_items) - len(late))
        ta0, ta1 = _env("TA0", 500), _env("TA1", 900)
        late = late[_env("TSKIP", 0):]
        for j, f in enumerate(t_items):
            if j < n1:
                t_s, it, e = [x for x in spots if x[0] >= ta0 + j * (ta1 - ta0) / n1][0]
            else:
                t_s, it, e = late[(j - n1) * len(late) // (len(t_items) - n1)]
            it[3].append((e, functools.partial(t_done.__getitem__, j)))
            extra.append((min(t_s - _env("TLEAD", 300), it[0]), f))
        prog = []
        for t0, kind, idx, ties in items:
            p, i = divmod(idx, 4)
            if kind == "s":
                if i == 0:
                    prog.append((t0, pairs[p][0]))
                prog.append((t0, functools.partial(pairs[p][1], i, ties)))
            elif kind == "v":
                prog.append((t0, functools.partial(pairs[p][2], i)))
                if i == 3:
                    extra.append((t0 + DH + _env("LFIN", 0), pairs[p][3]))
            else:
                prog.append((t0, functools.partial(s3_all[idx], ties)))
        run(prog, extra)

    only = _env("ONLY", "01")
    NODMA = _env("NODMA", 0)

    @when(k_ < (1 if NODMA & 1 else nstrip), ("first", "main"))
    def _():
        x_copy(k_).wait()

    new_masks("x")
    if "0" in only:
        when(k_ <= nstrip, ("main",))(block_x)

    @when(k_ == 0, ("first",))
    def _():
        def body(g, carry):
            for j in range(FG):
                piece = conv_group(pl.multiple_of((g * FG + j) * 8, 8))[1]
                for r in range(WS):
                    piece(r)
            return carry
        FG = _env("FG", 8)
        lax.fori_loop(0, NG // FG, body, 0)

    @when(k_ < (0 if NODMA & 1 else nstrip - 1), ("first", "main"))
    def _():
        x_copy(k_ + 1).start()

    @when(k_ >= (1000 if NODMA & 2 else 3), ("main", "last"))
    def _():
        o_copy(k_ - 3).wait()

    if "1" in only:
        new_masks("y")
        when((k_ <= nstrip) & (k_ >= 1), ("main",))(block_y)

    @when(k_ == 0, ("first",))
    def _():
        for j in range(WS * NT):
            for f in stats_steps(j):
                f()
        for f in t_items:
            f()

    @when(k_ == nstrip + 1, ("last",))
    def _():
        new_masks("y")
        for p in range(npair):
            pairs[p][4]()
        for f in s3_all:
            f()

    if only != "01":
        @when(dyn0 < 0, ("main",))
        def _():
            i = pl.multiple_of(k_ * 8, 8)
            o_ref[0, 0:16, 0:128] = _cat([
                qkv_ref[k3, k3, pl.ds(i, 8), :] + ms_ref[k3, 0:8, :] + stg_ref[k3, pl.ds(i, 8), :],
                pltpu.bitcast(t_ref[k3, k3, pl.ds(i, 8), :], F32) + ob_ref[pl.ds(i, 8), :]]).astype(BF16)
            for rf in (qkv_ref.at[k3, k3], stg_ref.at[k3], ob_ref):
                rf[pl.ds(i, 8), :] = zero8
            t_ref[k3, k3, pl.ds(i, 8), :] = pltpu.bitcast(zero8, U32)

    @when(k_ >= (nstrip + 1 if NODMA & 2 else 2), ("main", "last"))
    def _():
        o_copy(k_ - 2).start()

    @when(k_ == nstrip + 1, ("last",))
    def _():
        o_copy(k_ - 2).wait()


@jax.jit
def pallas_standalone__window_attn_davit__vision_kernel(
    x: jax.Array,
    dw_pe: jax.Array,
    w_qkv: jax.Array,
    w_o: jax.Array,
):
    B, H, W, Cx = x.shape
    assert B == 1 and Cx == C and H % WS == 0 and W % WS == 0 and WP - LANES < W < WP
    xt = jnp.transpose(x[0], (0, 2, 1))

    assert H // WS + 2 <= 256
    vmem = pl.BlockSpec(memory_space=pltpu.VMEM)
    yt = pl.pallas_call(
        functools.partial(_kernel, H=H, W=W),
        in_specs=[pl.BlockSpec(memory_space=pl.ANY), vmem, vmem, vmem],
        out_specs=pl.BlockSpec(memory_space=pl.ANY),
        out_shape=jax.ShapeDtypeStruct((H, C, W), x.dtype),
        scratch_shapes=[
            pltpu.VMEM((WS + 2, C, W), x.dtype),
            pltpu.VMEM((WS, C, W), x.dtype),
            pltpu.SemaphoreType.DMA((2,)),
            pltpu.VMEM((X0_ROWS, LANES), F32),
            pltpu.VMEM((WS * WP, LANES), F32),
            pltpu.VMEM((9, C, LANES), F32),
            pltpu.VMEM((3, 5, LANES // 2, LANES), U32),
            pltpu.VMEM((3, C // 2, LANES), U32),
            pltpu.VMEM((5, WS, WP, LANES), F32),
            pltpu.VMEM((NU, 3, LANES // 2, LANES), U32),
            pltpu.VMEM((37, LANES, LANES), F32),
            pltpu.VMEM((WS * NT, 16, LANES), F32),
            pltpu.VMEM((C, WP), F32),
        ],
        compiler_params=pltpu.CompilerParams(
            vmem_limit_bytes=64 * 1024 * 1024,
            disable_bounds_checks=bool(_env("NOBC", 1)),
        ),
        name="davit_window_attn",
    )(xt, dw_pe, w_qkv, w_o)
    return jnp.transpose(yt, (0, 2, 1))[None]
```

```python
import functools
import math
import os

import jax
import jax.numpy as jnp
from jax import lax
import jax.experimental.pallas as pl
import jax.experimental.pallas.tpu as pltpu

WS = 7
NH = 4
C = 192
DH = C // NH
NG = C // 8
LANES = 128
WP = 512
NT = WP // LANES
NU = WS * NT // 2
SLOTS = 8 * WS
EPS = 1e-5
F32 = jnp.float32
BF16 = jnp.bfloat16
U32 = jnp.uint32

X0_SLOT = WS * NT * C
DW_OFF = 3 * X0_SLOT
X0_ROWS = DW_OFF + 2 * C


def _dot(a, b):
    return jnp.dot(a, b, preferred_element_type=F32)


def _dot_nt(a, b):
    return lax.dot_general(a, b, (((1,), (1,)), ((), ())), preferred_element_type=F32)


def _cat(xs):
    return jnp.concatenate(xs, axis=0)


def _blocks(v):
    return [v[i:i + 8] for i in range(0, v.shape[0], 8)]


def _allred(x, op):
    for sh in (4, 2, 1):
        x = op(x, pltpu.roll(x, sh, 0))
    return x


def _env(name, default):
    return type(default)(os.environ.get(name, default))


def _kernel(x_hbm, dw_ref, wqkv_ref, wo_ref, o_hbm, *scratch, H, W):
    step = functools.partial(_step, x_hbm, dw_ref, wqkv_ref, wo_ref, o_hbm, *scratch, H=H, W=W)
    nstrip = H // WS

    def loop(lo, hi, mode):
        def body(k, carry):
            step(k_=k, mode=mode)
            return carry
        lax.fori_loop(lo, hi, body, 0)

    if "ONLY" not in os.environ:
        loop(0, 1, "first")
    loop(1 + _env("SKIP", 0), nstrip + 1, "main")
    if "ONLY" not in os.environ:
        loop(nstrip + 1, nstrip + 2, "last")


def _step(x_hbm, dw_ref, wqkv_ref, wo_ref, o_hbm,
          x_ref, o_ref, sems, x0_ref, ob_ref, dws_ref, ws_ref, wos_ref, qkv_ref, t_ref, stg_ref, ms_ref,
          top_ref, *, H, W, k_, mode):
    nstrip, nwin = H // WS, W // WS

    def x_copy(k):
        return pltpu.make_async_copy(x_hbm.at[pl.ds(jnp.minimum(k * WS, H - WS - 1), WS + 1)],
                                     x_ref.at[pl.ds((k & 1) * (WS + 2), WS + 1)], sems.at[0])

    def o_copy(k):
        return pltpu.make_async_copy(o_ref.at[pl.ds((k & 1) * WS, WS)], o_hbm.at[pl.ds(k * WS, WS)],
                                     sems.at[1])

    def when(cond, modes):
        if mode in modes:
            return pl.when(cond)
        return lambda f: None

    xoff = (k_ & 1) * (WS + 2) + jnp.where(k_ >= nstrip - 1, 1, 0)
    ooff = (k_ & 1) * WS
    dyn0 = jnp.minimum(k_, 0)

    def rows_at(base, off, n):
        if isinstance(base, int):
            return pl.ds(base + off, n)
        return pl.ds(pl.multiple_of(base + off, 8), n)

    mk = {}

    def new_masks(blk):
        lane = lax.broadcasted_iota(jnp.int32, (8, LANES), 1)
        mk.clear()
        mk["never"] = lane < dyn0
        if blk == "x":
            mk["up"] = lax.broadcasted_iota(jnp.int32, (8, LANES), 0) < 4
            return
        key_ok = lax.broadcasted_iota(jnp.int32, (8, LANES), 0) < WS
        mk.update(
            lo=lane < DH, hi0=(lane >= DH) & ((lane < 64) | (lane >= 96)), hi1=(lane >= DH) & (lane < 96),
            v=lane < 96, key=key_ok, keep_a=key_ok & (lane < SLOTS), keep_b=key_ok & (lane >= SLOTS),
            left64=lane < 64)

    k3 = k_ - 3 * ((k_ * 171) >> 9)
    nxt = k3 * X0_SLOT
    prv = jnp.where((k3 == 2) | (k_ < 2), 0, nxt + X0_SLOT)

    def conv_group(c0):
        st = {}

        def row(i):
            if i == 0 and i not in st:
                st[i] = top_ref[pl.ds(c0, 8), :]
            if i not in st:
                v = x_ref[xoff + (i - 1), pl.ds(c0, 8), :].astype(F32)
                st[i] = jnp.concatenate([v, jnp.zeros((8, WP - W), F32)], axis=1)
                if i == WS and i - 2 in st:
                    top_ref[pl.ds(c0, 8), :] = st[i]
            return st[i]

        def bc(v):
            return jnp.concatenate([v] * NT, axis=1)

        def taps(r):
            st["tw", r] = [bc(x0_ref[rows_at(c0, DW_OFF + k * C, 8), :]) for k in range(2)]

        def piece(r):
            if "w" not in st:
                st["w"] = [bc(dws_ref[k, pl.ds(c0, 8), :]) for k in range(9)]
            wts = list(st["w"])
            if ("tw", r) in st:
                wts[6], wts[8] = st["tw", r]
            row(r)
            abc = [row(r + 1) * wts[3 + j] + row(r) * wts[j] + row(r + 2) * wts[6 + j] for j in range(3)]
            x0 = pltpu.roll(abc[0], 1, 1) + abc[1] + pltpu.roll(abc[2], WP - 1, 1)
            for t in range(NT):
                x0_ref[rows_at(nxt, (r * NT + t) * C + c0, 8), :] = x0[:, t * LANES:(t + 1) * LANES]

        return taps, piece

    @when(k_ == 0, ("first",))
    def _():
        x_copy(0).start()
        for k in range(9):
            w = dw_ref[k // 3].astype(F32)[k % 3:k % 3 + 1, :]
            w = jnp.broadcast_to(w, (LANES, C)).T
            dws_ref[k] = w + 1.0 if k == 4 else w
            if k in (6, 8):
                x0_ref[pl.ds(DW_OFF + (k - 6) // 2 * C, C), :] = w
        w = wqkv_ref[...].astype(F32)
        wq = w[:, 0:C] * ((DH ** -0.5) * math.log2(math.e))
        wk, wv = w[:, C:2 * C], w[:, 2 * C:3 * C]
        tiles = [(wq[:, 0:64], wv[:, 64:96], wq[:, 64:96]),
                 (wq[:, 96:192], wv[:, 96:128]),
                 (wk[:, 0:64], wv[:, 128:160], wk[:, 64:96]),
                 (wk[:, 96:192], wv[:, 160:192]),
                 (wv[:, 0:128],)]
        for n, parts in enumerate(tiles):
            w = jnp.concatenate(parts, axis=1)
            for i, wi in enumerate((w[0:128], w[64:192], _cat([w[0:64], w[128:192]]))):
                if n == 4:
                    wi = wi.T
                ws_ref[i, n] = pltpu.bitcast(wi.astype(BF16), U32)
        w = wo_ref[...].astype(F32)
        wx, wy, wz = w[0:64], w[64:128], w[128:192]
        for i, parts in enumerate(((wx, wy), (wz, wy), (wx, wy + wz))):
            wos_ref[i] = pltpu.bitcast(_cat(parts).T.astype(BF16), U32)

        top_ref[...] = jnp.zeros(top_ref.shape, F32)
        for i in (WS + 1, 2 * WS + 3):
            x_ref[i] = jnp.zeros(x_ref.shape[1:], x_ref.dtype)

        for p in range(stg_ref.shape[0]):
            stg_ref[p] = jnp.zeros(stg_ref.shape[1:], F32)
        for r in range(WS):
            ob_ref[pl.ds(r * WP + WP - 8, 8), :] = jnp.zeros((8, LANES), F32)

    cuts = [int(c) for c in _env("CUTS", "0,7").split(",")]
    bands = list(zip(cuts, cuts[1:]))
    groups = {(b, g): conv_group(8 * g) for b in range(len(bands)) for g in range(NG)}
    WLEAD = _env("WLEAD", 4)

    def conv_items(nslow):
        plist = [((b, g), r) for b, (r0, r1) in enumerate(bands) for g in range(NG) for r in range(r0, r1)]
        items, nxt_tap = [], WLEAD
        for k, (g, r) in enumerate(plist):
            fs = []
            lead = WLEAD if k < nslow else _env("WLEAD2", 5)
            while nxt_tap <= min(k + lead, len(plist) - 1):
                g2, r2 = plist[nxt_tap]
                fs.append(functools.partial(groups[g2][0], r2))
                nxt_tap += 1
            fs.append(functools.partial(groups[g][1], r))
            items.append(fs)
        return items

    def ld_x0(j, k, gs=range(NG)):
        return [x0_ref[rows_at(nxt + dyn0 * (8 * k), j * C + 8 * g, 8), :] for g in gs]

    def add2(acc, xs):
        a = functools.reduce(jnp.add, xs[0::2])
        b = functools.reduce(jnp.add, xs[1::2])
        return a + b if acc is None else (acc + a) + b

    stats_done = set()

    def stats_steps(j):
        st = {"s": None, "q": None}
        n1, n2 = _env("SEG1", 8), _env("SEG2", 6)

        def sum_step(g0):
            st["s"] = add2(st["s"], ld_x0(j, 0, range(g0, g0 + n1)))
            if g0 + n1 == NG:
                st["s"] = _allred(st["s"], jnp.add) * (1.0 / C)
            return st["s"]

        def var_step(g0):
            d = [x - st["s"] for x in ld_x0(j, 1, range(g0, g0 + n2))]
            st["q"] = add2(st["q"], [x * x for x in d])
            return st["q"]

        def last_step():
            v = _allred(st["q"], jnp.add) * (1.0 / C) + EPS
            rs = lax.rsqrt(v) if _env("RSQ", 1) else jnp.exp2(jnp.log2(v) * -0.5)
            ms_ref[j] = _cat([st["s"], rs])
            stats_done.add(j)
            return rs

        return ([functools.partial(sum_step, g) for g in range(0, NG, n1)]
                + [functools.partial(var_step, g) for g in range(0, NG, n2)] + [last_step])

    def colsum(xs):
        xs = [a + b for a, b in zip(xs[0:8], xs[16:24])] + xs[8:16]
        return _dot(jnp.ones((8, LANES), F32), _cat(xs))

    means = {}

    def mean_dot(j):
        means[j] = colsum(ld_x0(j, 0)) * (1.0 / C)

    def var_dot(j):
        xs = [x0_ref[pl.ds(nxt + (j * C + 8 * g + 4), 8), :] for g in range(NG - 1)]
        xs.append(jnp.where(mk["up"], *ld_x0(j, 0, (0, NG - 1))))
        d = [x - means[j] for x in xs]
        v = colsum([x * x for x in d]) * (1.0 / C) + EPS
        rs = lax.rsqrt(v) if _env("RSQ", 1) else jnp.exp2(jnp.log2(v) * -0.5)
        ms_ref[j] = _cat([means[j], rs])
        stats_done.add(j)

    def normed(j, blk, k):
        assert j in stats_done or "ONLY" in os.environ and j < NSTX, j
        m, rs = ms_ref[j, 0:8, :], ms_ref[j, 8:16, :]
        return _cat([(x - m) * rs for x in ld_x0(j, k, range(8 * blk, 8 * blk + 8))])

    t_done = {}

    def put_t(dst, tiles):
        tt = pltpu.bitcast(jnp.concatenate(tiles, axis=1).astype(BF16).T, U32)
        for i, (u, e) in enumerate(dst):
            t_ref[u, e] = tt[64 * i:64 * i + 64]
        t_done[len(t_done)] = pltpu.bitcast(tt[120:128], F32)

    def t_first(u):
        ja, jb = 2 * u, 2 * u + 1
        bx = normed(jb, 0, 0)
        put_t([(u, 0), (u, 2)], [_cat([normed(ja, 0, 0) - bx, normed(ja, 1, 0)]),
                                 _cat([bx, normed(ja, 2, 0)])])

    def t_second(r):
        put_t([(u, 1) for u in (2 * r, 2 * r + 1)],
              [_cat([normed(2 * u + 1, 1, 0), normed(2 * u + 1, 2, 0) - normed(2 * u, 2, _env("RECOMP", 1))])
               for u in (2 * r, 2 * r + 1)])

    t_items = []
    for r in range(WS):
        t_items += [functools.partial(t_first, 2 * r), functools.partial(t_first, 2 * r + 1),
                    functools.partial(t_second, r)]

    def qkv_chunk(us, n, steps=(), tiny=()):
        lhs = {i: [b for u in us for b in _blocks(t_ref[u, i])] for i in range(3)}
        for q, step in enumerate(steps):
            tok = pltpu.bitcast(step(), U32)
            q = q * 24 * len(us) // len(steps)
            blks = lhs[(2, 0, 1)[q % 3]]
            blks[q // 3] = jnp.where(mk["never"], tok, blks[q // 3])
        p3 = None
        for i in (2, 0, 1):
            p = _dot(pltpu.bitcast(_cat(lhs[i]), BF16), pltpu.bitcast(ws_ref[i, n], BF16))
            if p3 is None:
                p3 = p
            else:
                p = p + p3
                for e, u in enumerate(us):
                    r, tp = divmod(u, 2)
                    qkv_ref[n, r, pl.ds((2 * tp + i) * LANES, LANES), :] = p[e * LANES:(e + 1) * LANES]

    vr_words = {}
    job_done = {}

    def side_dots(u, n):
        r, tp = divmod(u, 2)
        st = {}

        def one(i, parts=1):
            if parts > 1:
                lhs, rows = t_ref[u, i], 64 // parts
                p = _cat([_dot(pltpu.bitcast(lhs[q * rows:(q + 1) * rows], BF16),
                               pltpu.bitcast(ws_ref[i, n], BF16)) for q in range(parts)])
            elif n == 4:
                p = _dot_nt(pltpu.bitcast(ws_ref[i, 4, 0:32, :], BF16), pltpu.bitcast(t_ref[u, i], BF16))
            else:
                p = _dot(pltpu.bitcast(t_ref[u, i], BF16), pltpu.bitcast(ws_ref[i, n], BF16))
            st[i] = p if i == 2 else p + st[2]
            if n < 4 and i < 2:
                qkv_ref[n, r, pl.ds((2 * tp + i) * LANES, LANES), :] = st[i]
            elif i == 1:
                vr_words[u] = pltpu.pack_elementwise([st[0], st[1]], packed_dtype=BF16)

        return [(64 if n == 4 else LANES, (u, n, i), functools.partial(one, i)) for i in (2, 0, 1)]

    def vr_store(u):
        r, tp = divmod(u, 2)
        w = pltpu.bitcast(vr_words[u], F32)
        wt = pltpu.bitcast(_cat([w, w]).T, U32)
        job_done["v", u] = pltpu.bitcast(wt[120:128], F32)
        for j in range(2):
            qkv_ref[4, r, pl.ds((2 * tp + j) * LANES, LANES), :] = pltpu.unpack_elementwise(
                wt, index=j, packed_dtype=BF16, unpacked_dtype=F32)

    zero8 = jnp.zeros((8, LANES), F32)

    def gather(n, off, k=0):
        return [qkv_ref[n, r, pl.ds(off + dyn0 * k if k else off, 8), :] for r in range(WS)]

    def softmax_t(st):
        rows = _blocks(st)
        m = functools.reduce(jnp.maximum, rows)
        m = _allred(jnp.where(mk["key"], m, -jnp.inf), jnp.maximum)
        p = [jnp.exp2(x - m) for x in rows]
        return p, functools.reduce(jnp.add, p)

    def s2_pair(pi, offa):
        offb = offa + WS
        st = {}

        def vprep():
            g = [gather(n, offa) + gather(n, offb) for n in range(5)]
            u1 = [jnp.where(mk["left64"], z, jnp.where(mk["v"], x, y)) for x, y, z in zip(g[0], g[1], g[4])]
            u2 = [jnp.where(mk["v"], x, y) for x, y in zip(g[2], g[3])]
            u = jnp.concatenate([_cat(u1 + [zero8, zero8]), _cat(u2 + [zero8, zero8])], axis=1)
            vt = pltpu.bitcast(u.astype(BF16).T, U32)
            vt = _cat([vt[0:64], vt[96:128]])
            st["vt"] = [pltpu.bitcast(vt[24 * h:24 * h + 24], BF16) for h in range(NH)]

        def score(i, ties=()):
            hp, sw = divmod(i, 2)
            lo, hi = mk["lo"], mk["hi%d" % hp]
            ma, mb = (lo, hi) if sw == 0 else (hi, lo)
            gq = (0, 1, 1 + sw)[_env("GQ", 0)]
            gk = (0, 1, 1 + sw)[_env("GK", 0)]
            q = _cat([jnp.where(ma, v, 0.0) for v in gather(hp, offa, gq)]
                     + [jnp.where(mb, v, 0.0) for v in gather(hp, offb, gq)] + [zero8, zero8])
            ka, kb = gather(2 + hp, offa, gk), gather(2 + hp, offb, gk)
            k = [jnp.where(lo, x, y) for x, y in (zip(ka, kb) if sw == 0 else zip(kb, ka))]
            for _, job in ties:
                k[0] = jnp.where(mk["never"], job(), k[0])
            k = _cat(k)
            st["p", i] = softmax_t(_dot_nt(k, q))

        def value(h):
            hp, sw = divmod(h, 2)
            (pa, sa), (pb, sb) = st["p", 2 * hp + sw], st["p", 2 * hp + 1 - sw]
            pm = _cat([jnp.where(mk["keep_a"], v, 0.0) for v in pa]
                      + [jnp.where(mk["keep_b"], v, 0.0) for v in pb] + [zero8, zero8])
            den = _allred(jnp.where(mk["keep_a"], sa, jnp.where(mk["keep_b"], sb, 0.0)), jnp.add)
            rec = pl.reciprocal(den, approx=True)
            if _env("NR", 0):
                rec = rec * (2.0 - den * rec)
            st["o", h] = [b * rec for b in _blocks(_dot(st["vt"][h], pm))]

        def finish():
            o = [b for h in range(NH) for b in st["o", h]]
            w = pltpu.pack_elementwise([_cat(o[0:16]), _cat(o[16:24] + o[16:24])], packed_dtype=BF16)
            stg_ref[pi] = pltpu.bitcast(w, F32)

        def scatter():
            wt = stg_ref[pi].T
            job_done["s", pi] = wt[104:112]
            for i, off in enumerate((offa, offb)):
                for r in range(WS):
                    base = i * SLOTS + 8 * r
                    ob_ref[pl.ds(r * WP + off, WS), :] = wt[base:base + WS]

        return vprep, score, value, finish, scatter

    npair = (nwin + 1) // 2
    pairs = [s2_pair(p, min(2 * p, nwin - 2) * WS) for p in range(npair)]

    def s3_unit(r, tp, ties=()):
        def unpack(t):
            w = pltpu.bitcast(ob_ref[pl.ds(r * WP + t * LANES, LANES), :], U32)
            return [_blocks(pltpu.unpack_elementwise(w, index=i, packed_dtype=BF16, unpacked_dtype=F32))
                    for i in range(2)]

        (la, ha), (lb, hb) = unpack(2 * tp), unpack(2 * tp + 1)
        t3 = [jnp.where(mk["left64"], x, y) for x, y in zip(lb, ha)]
        t1 = _cat([x - y for x, y in zip(la, t3)])
        t2 = _cat([jnp.where(mk["left64"], x, z) - y for x, y, z in zip(hb, ha, lb)])
        t3 = _cat(t3)
        wo = [_blocks(wos_ref[i]) for i in range(3)]
        for q, (e, job) in enumerate(ties):
            blks = wo[(2, 0, 1)[q % 3]]
            blks[e] = jnp.where(mk["never"], pltpu.bitcast(job(), U32), blks[e])
        wo = [pltpu.bitcast(_cat(w), BF16) for w in wo]
        p3 = _dot_nt(wo[2], t3)
        ys = [_dot_nt(wo[i], t) + p3
              + x0_ref[rows_at(prv, (r * NT + 2 * tp + i) * C, C), :] for i, t in enumerate((t1, t2))]
        n = min(2 * LANES, W - 2 * tp * LANES)
        o_ref[ooff + r, :, pl.ds(2 * tp * LANES, n)] = jnp.concatenate(ys, axis=1).astype(o_ref.dtype)[:, :n]

    s3_all = [functools.partial(s3_unit, r, tp) for tp in range(2) for r in range(WS)]

    def run(prog, extra):
        extra = sorted(extra, key=lambda e: e[0])
        j = 0
        for t0, fn in prog:
            while j < len(extra) and extra[j][0] <= t0:
                extra[j][1]()
                j += 1
            fn()
        for e in extra[j:]:
            e[1]()

    MERGE = _env("MERGE", 0)
    NX3 = _env("NX3", 0)

    NSY = 0

    NSTX = _env("NSTX", 20)

    def wave_steps(lo, hi, wave):
        steps = []
        for j0 in range(lo, hi, wave):
            for grp in zip(*[stats_steps(j) for j in range(j0, min(j0 + wave, hi))]):
                steps += grp
        return steps

    def block_x():
        NJ = _env("NJ", 28)
        NSTC = _env("NSTC", 6)
        WAVE = _env("WAVE", 4)
        VRLAG = _env("VRLAG", 200)
        chunks = [(u, n) for u in range(NU) for n in range(4)]
        MXS = _env("MXS", 0)
        steps = [] if MXS else wave_steps(0, NSTX, WAVE)
        loose = steps[len(steps) - _env("LOOSE", 0):]
        steps = steps[:len(steps) - len(loose)]
        nside = 9
        side, vstep = [], _env("VRSTEP", 1)
        for q in range(NU // 2):
            side += side_dots(2 * q, 4) + side_dots(2 * q + 1, 4)
            for _ in range(vstep):
                if nside:
                    side += side_dots(*chunks.pop())
                    nside -= 1
        for _ in range(nside):
            side += side_dots(*chunks.pop())
        mu = _env("MU", 2)
        merged = []
        for u, n in chunks:
            prev = [c for c in merged if c[1] == n and c[0][0] // mu == u // mu]
            if prev:
                prev[0][0].append(u)
            else:
                merged.append(([u], n))
        starts = [LANES * sum(len(c[0]) for c in merged[:k]) for k in range(len(merged))]
        t_conv = max(x for x in starts if x <= (len(chunks) - NSTC) * LANES)
        span = len(chunks) * LANES - t_conv
        plan, t, vr_ready = [], 0, {}
        for k, (us, n) in enumerate(merged):
            dur = LANES * len(us)
            lo, hi = (max(x - t_conv, 0) * len(steps) // span for x in (t, t + dur))
            plan.append((t, tuple(us), n, list(steps[lo:hi]), []))
            room = dur
            while side and (room > 0 or k == len(merged) - 1):
                rows, key, f = side.pop(0)
                plan.append((t, f if room > 0 else functools.partial(f, 4), None, [], []))
                room -= rows
                if key[1:] == (4, 1):
                    vr_ready[key[0]] = t + dur - room + VRLAG
            t += dur
        ci = conv_items(4 * NJ)
        slow = _env("SLOW", 32.0)
        fast = (t_conv - 4 * NJ * slow) / max(len(ci) - 4 * NJ, 1)
        t_piece = [min(j, 4 * NJ) * slow + max(j - 4 * NJ, 0) * fast for j in range(len(ci) + 1)]
        scat, vrs = list(range(npair - NSY)), list(range(NU))
        jobs = []
        for q in range(NJ):
            if vrs and vr_ready[vrs[0]] <= t_piece[4 * q + 1]:
                jobs.append((t_piece[4 * q + 1], ("v", vrs[0])))
                ci[4 * q].insert(0, functools.partial(vr_store, vrs.pop(0)))
            elif scat:
                jobs.append((t_piece[4 * q + 1], ("s", scat[0])))
                ci[4 * q].insert(0, pairs[scat.pop(0)][4])
        extra = [(t_piece[j + 1], f) for j, fs in enumerate(ci) for f in fs]
        tail = [(("v", u), functools.partial(vr_store, u)) for u in vrs] + [(("s", p), pairs[p][4]) for p in scat]
        for q, (key, f) in enumerate(tail):
            t_q = max(t_conv + 1 + (q // 3) * 128, vr_ready[key[1]] if key[0] == "v" else 0)
            extra.append((t_q, f))
            jobs.append((t_q, key))
        if _env("JDL", 800):
            for t_q, key in jobs:
                later = [e for e in plan if e[2] is not None and e[0] >= t_q + _env("JDL", 800)]
                if later:
                    later[0][3].insert(0, functools.partial(job_done.get, key))
        prog = [(t0, u if n is None else functools.partial(qkv_chunk, u, n, st, tn))
                for t0, u, n, st, tn in plan]
        run(prog, extra + [(t, f) for f in loose])

    def block_y():
        pattern = _env("PAT", "SFFVFFFF" + "SSSSFVVVV" * 8 + "SSSSVVVV").rstrip(".")
        load = [0] * 4
        items, ns, nv, nf = [], 0, 0, 0
        for ch in pattern:
            if ch in "Ss":
                todo = [("s", ns + i, [SLOTS]) for i in range(4 if ch == "S" else 2)]
                ns += len(todo)
            elif ch in "Vv":
                todo = [("v", nv + i, [DH]) for i in range(4 if ch == "V" else 2)]
                nv += len(todo)
            else:
                todo = [("f", nf, [C] * 3)]
                nf += 1
            for kind, idx, rows in todo:
                items.append((min(load), kind, idx, []))
                for x in rows:
                    load[load.index(min(load))] += x
        assert (ns, nv, nf) == (4 * npair, 4 * npair, NU)
        spots = sorted([(it[0], it, 0) for it in items if it[1] == "s"]
                       + [(it[0] + 16 * e, it, e) for it in items if it[1] == "f" for e in range(12)],
                       key=lambda x: x[0])
        ysteps = wave_steps(NSTX, WS * NT, _env("WAVEY", 4))
        fspots = [x for x in spots if x[1][1] == "f" and x[1][2] < _env("S3Q", 6)
                  and _env("E0", 1) <= x[2] < _env("E1", 8)]
        fspots.sort(key=lambda x: (x[1][2], x[2]))
        for q, step in enumerate(ysteps):
            _, it, e = fspots[q * len(fspots) // len(ysteps)]
            it[3].append((e, step))
        t_done.clear()
        extra = []
        tpos = [int(x) for x in _env("TPOS", "8,9").split(",")]
        late = [x for x in spots if x[1][1] == "s" and x[1][2] >= 4 and (x[1][2] - 4) % 16 in tpos]
        late.sort(key=lambda x: x[1][2])
        n1 = max(_env("NT1", 3), len(t_items) - len(late))
        ta0, ta1 = _env("TA0", 500), _env("TA1", 900)
        late = late[_env("TSKIP", 0):]
        for j, f in enumerate(t_items):
            if j < n1:
                t_s, it, e = [x for x in spots if x[0] >= ta0 + j * (ta1 - ta0) / n1][0]
            else:
                t_s, it, e = late[(j - n1) * len(late) // (len(t_items) - n1)]
            it[3].append((e, functools.partial(t_done.__getitem__, j)))
            extra.append((min(t_s - _env("TLEAD", 300), it[0]), f))
        prog = []
        for t0, kind, idx, ties in items:
            p, i = divmod(idx, 4)
            if kind == "s":
                if i == 0:
                    prog.append((t0, pairs[p][0]))
                prog.append((t0, functools.partial(pairs[p][1], i, ties)))
            elif kind == "v":
                prog.append((t0, functools.partial(pairs[p][2], i)))
                if i == 3:
                    extra.append((t0 + DH + _env("LFIN", 0), pairs[p][3]))
            else:
                prog.append((t0, functools.partial(s3_all[idx], ties)))
        run(prog, extra)

    only = _env("ONLY", "01")

    @when(k_ < nstrip, ("first", "main"))
    def _():
        x_copy(k_).wait()

    @when(k_ < nstrip - 1, ("first", "main"))
    def _():
        x_copy(k_ + 1).start()

    new_masks("x")
    if "0" in only:
        when(k_ <= nstrip, ("main",))(block_x)

    @when(k_ == 0, ("first",))
    def _():
        def body(g, carry):
            for j in range(FG):
                piece = conv_group(pl.multiple_of((g * FG + j) * 8, 8))[1]
                for r in range(WS):
                    piece(r)
            return carry
        FG = _env("FG", 8)
        lax.fori_loop(0, NG // FG, body, 0)

    @when(k_ >= 4, ("main", "last"))
    def _():
        o_copy(k_ - 4).wait()

    @when(k_ >= 3, ("main", "last"))
    def _():
        o_copy(k_ - 3).start()

    if "1" in only:
        new_masks("y")
        when((k_ <= nstrip) & (k_ >= 1), ("main",))(block_y)

    @when(k_ == 0, ("first",))
    def _():
        for j in range(WS * NT):
            for f in stats_steps(j):
                f()
        for f in t_items:
            f()

    @when(k_ == nstrip + 1, ("last",))
    def _():
        new_masks("y")
        for p in range(npair):
            pairs[p][4]()
        for f in s3_all:
            f()

    if only != "01":
        @when(dyn0 < 0, ("main",))
        def _():
            i = pl.multiple_of(k_ * 8, 8)
            o_ref[0, 0:16, 0:128] = _cat([
                qkv_ref[k3, k3, pl.ds(i, 8), :] + ms_ref[k3, 0:8, :] + stg_ref[k3, pl.ds(i, 8), :],
                pltpu.bitcast(t_ref[k3, k3, pl.ds(i, 8), :], F32) + ob_ref[pl.ds(i, 8), :]]).astype(BF16)
            for rf in (qkv_ref.at[k3, k3], stg_ref.at[k3], ob_ref):
                rf[pl.ds(i, 8), :] = zero8
            t_ref[k3, k3, pl.ds(i, 8), :] = pltpu.bitcast(zero8, U32)

    @when(k_ == nstrip + 1, ("last",))
    def _():
        o_copy(k_ - 3).wait()
        o_copy(k_ - 2).start()
        o_copy(k_ - 2).wait()


@jax.jit
def pallas_standalone__window_attn_davit__vision_kernel(
    x: jax.Array,
    dw_pe: jax.Array,
    w_qkv: jax.Array,
    w_o: jax.Array,
):
    B, H, W, Cx = x.shape
    assert B == 1 and Cx == C and H % WS == 0 and W % WS == 0 and WP - LANES < W < WP
    xt = jnp.transpose(x[0], (0, 2, 1))

    assert H // WS + 2 <= 256
    vmem = pl.BlockSpec(memory_space=pltpu.VMEM)
    yt = pl.pallas_call(
        functools.partial(_kernel, H=H, W=W),
        in_specs=[pl.BlockSpec(memory_space=pl.ANY), vmem, vmem, vmem],
        out_specs=pl.BlockSpec(memory_space=pl.ANY),
        out_shape=jax.ShapeDtypeStruct((H, C, W), x.dtype),
        scratch_shapes=[
            pltpu.VMEM((2 * (WS + 2), C, W), x.dtype),
            pltpu.VMEM((2 * WS, C, W), x.dtype),
            pltpu.SemaphoreType.DMA((2,)),
            pltpu.VMEM((X0_ROWS, LANES), F32),
            pltpu.VMEM((WS * WP, LANES), F32),
            pltpu.VMEM((9, C, LANES), F32),
            pltpu.VMEM((3, 5, LANES // 2, LANES), U32),
            pltpu.VMEM((3, C // 2, LANES), U32),
            pltpu.VMEM((5, WS, WP, LANES), F32),
            pltpu.VMEM((NU, 3, LANES // 2, LANES), U32),
            pltpu.VMEM((37, LANES, LANES), F32),
            pltpu.VMEM((WS * NT, 16, LANES), F32),
            pltpu.VMEM((C, WP), F32),
        ],
        compiler_params=pltpu.CompilerParams(
            vmem_limit_bytes=64 * 1024 * 1024,
            disable_bounds_checks=bool(_env("NOBC", 1)),
        ),
        name="davit_window_attn",
    )(xt, dw_pe, w_qkv, w_o)
    return jnp.transpose(yt, (0, 2, 1))[None]
```

```python
import functools
import math
import os

import jax
import jax.numpy as jnp
from jax import lax
import jax.experimental.pallas as pl
import jax.experimental.pallas.tpu as pltpu

WS = 7
NH = 4
C = 192
DH = C // NH
NG = C // 8
LANES = 128
WP = 512
NT = WP // LANES
NU = WS * NT // 2
SLOTS = 8 * WS
EPS = 1e-5
F32 = jnp.float32
BF16 = jnp.bfloat16
U32 = jnp.uint32

X0_SLOT = WS * NT * C
DW_OFF = 3 * X0_SLOT
X0_ROWS = DW_OFF + 2 * C


def _dot(a, b):
    return jnp.dot(a, b, preferred_element_type=F32)


def _dot_nt(a, b):
    return lax.dot_general(a, b, (((1,), (1,)), ((), ())), preferred_element_type=F32)


def _cat(xs):
    return jnp.concatenate(xs, axis=0)


def _blocks(v):
    return [v[i:i + 8] for i in range(0, v.shape[0], 8)]


def _allred(x, op):
    for sh in (4, 2, 1):
        x = op(x, pltpu.roll(x, sh, 0))
    return x


def _env(name, default):
    return type(default)(os.environ.get(name, default))


def _kernel(x_hbm, dw_ref, wqkv_ref, wo_ref, o_hbm, *scratch, H, W):
    step = functools.partial(_step, x_hbm, dw_ref, wqkv_ref, wo_ref, o_hbm, *scratch, H=H, W=W)
    nstrip = H // WS

    def loop(lo, hi, mode):
        def body(k, carry):
            step(k_=k, mode=mode)
            return carry
        lax.fori_loop(lo, hi, body, 0)

    if "ONLY" not in os.environ:
        loop(0, 1, "first")
    loop(1 + _env("SKIP", 0), nstrip + 1, "main")
    if "ONLY" not in os.environ:
        loop(nstrip + 1, nstrip + 2, "last")


def _step(x_hbm, dw_ref, wqkv_ref, wo_ref, o_hbm,
          x_ref, o_ref, sems, x0_ref, ob_ref, dws_ref, ws_ref, wos_ref, qkv_ref, t_ref, stg_ref, ms_ref,
          top_ref, *, H, W, k_, mode):
    nstrip, nwin = H // WS, W // WS

    def x_copy(k):
        return pltpu.make_async_copy(x_hbm.at[pl.ds(jnp.minimum(k * WS, H - WS - 1), WS + 1)],
                                     x_ref.at[pl.ds((k & 1) * (WS + 2), WS + 1)], sems.at[0])

    def o_copy(k):
        return pltpu.make_async_copy(o_ref.at[pl.ds((k & 1) * WS, WS)], o_hbm.at[pl.ds(k * WS, WS)],
                                     sems.at[1])

    FG = 8

    def x0_copy(g):
        cs = pl.ds(pl.multiple_of(g * (8 * FG), 8 * FG), 8 * FG)
        return pltpu.make_async_copy(x_hbm.at[pl.ds(0, WS + 1), cs], x_ref.at[pl.ds(0, WS + 1), cs],
                                     sems.at[2 + g])

    def row_copy(r):
        return pltpu.make_async_copy(o_ref.at[ooff + r], o_hbm.at[H - WS + r], sems.at[2])

    def when(cond, modes):
        if mode in modes:
            return pl.when(cond)
        return lambda f: None

    xoff = (k_ & 1) * (WS + 2) + jnp.where(k_ >= nstrip - 1, 1, 0)
    ooff = (k_ & 1) * WS
    dyn0 = jnp.minimum(k_, 0)

    def rows_at(base, off, n):
        if isinstance(base, int):
            return pl.ds(base + off, n)
        return pl.ds(pl.multiple_of(base + off, 8), n)

    mk = {}

    def new_masks(blk):
        lane = lax.broadcasted_iota(jnp.int32, (8, LANES), 1)
        mk.clear()
        mk["never"] = lane < dyn0
        if blk == "x":
            mk["up"] = lax.broadcasted_iota(jnp.int32, (8, LANES), 0) < 4
            return
        key_ok = lax.broadcasted_iota(jnp.int32, (8, LANES), 0) < WS
        mk.update(
            lo=lane < DH, hi0=(lane >= DH) & ((lane < 64) | (lane >= 96)), hi1=(lane >= DH) & (lane < 96),
            v=lane < 96, key=key_ok, keep_a=key_ok & (lane < SLOTS), keep_b=key_ok & (lane >= SLOTS),
            left64=lane < 64)

    k3 = k_ - 3 * ((k_ * 171) >> 9)
    nxt = k3 * X0_SLOT
    prv = jnp.where((k3 == 2) | (k_ < 2), 0, nxt + X0_SLOT)

    def conv_group(c0):
        st = {}

        def row(i):
            if i == 0 and i not in st:
                st[i] = top_ref[pl.ds(c0, 8), :]
            if i not in st:
                v = x_ref[xoff + (i - 1), pl.ds(c0, 8), :].astype(F32)
                st[i] = jnp.concatenate([v, jnp.zeros((8, WP - W), F32)], axis=1)
                if i == WS and i - 2 in st:
                    top_ref[pl.ds(c0, 8), :] = st[i]
            return st[i]

        def bc(v):
            return jnp.concatenate([v] * NT, axis=1)

        def taps(r):
            st["tw", r] = [bc(x0_ref[rows_at(c0, DW_OFF + k * C, 8), :]) for k in range(2)]

        def piece(r):
            if "w" not in st:
                st["w"] = [bc(dws_ref[k, pl.ds(c0, 8), :]) for k in range(9)]
            wts = list(st["w"])
            if ("tw", r) in st:
                wts[6], wts[8] = st["tw", r]
            row(r)
            abc = [row(r + 1) * wts[3 + j] + row(r) * wts[j] + row(r + 2) * wts[6 + j] for j in range(3)]
            x0 = pltpu.roll(abc[0], 1, 1) + abc[1] + pltpu.roll(abc[2], WP - 1, 1)
            for t in range(NT):
                x0_ref[rows_at(nxt, (r * NT + t) * C + c0, 8), :] = x0[:, t * LANES:(t + 1) * LANES]

        return taps, piece

    @when(k_ == 0, ("first",))
    def _():
        for g in range(NG // FG):
            x0_copy(g).start()
        for k in range(9):
            w = dw_ref[k // 3].astype(F32)[k % 3:k % 3 + 1, :]
            w = jnp.broadcast_to(w, (LANES, C)).T
            dws_ref[k] = w + 1.0 if k == 4 else w
            if k in (6, 8):
                x0_ref[pl.ds(DW_OFF + (k - 6) // 2 * C, C), :] = w
        w = wqkv_ref[...].astype(F32)
        wq = w[:, 0:C] * ((DH ** -0.5) * math.log2(math.e))
        wk, wv = w[:, C:2 * C], w[:, 2 * C:3 * C]
        tiles = [(wq[:, 0:64], wv[:, 64:96], wq[:, 64:96]),
                 (wq[:, 96:192], wv[:, 96:128]),
                 (wk[:, 0:64], wv[:, 128:160], wk[:, 64:96]),
                 (wk[:, 96:192], wv[:, 160:192]),
                 (wv[:, 0:128],)]
        for n, parts in enumerate(tiles):
            w = jnp.concatenate(parts, axis=1)
            for i, wi in enumerate((w[0:128], w[64:192], _cat([w[0:64], w[128:192]]))):
                if n == 4:
                    wi = wi.T
                ws_ref[i, n] = pltpu.bitcast(wi.astype(BF16), U32)
        w = wo_ref[...].astype(F32)
        wx, wy, wz = w[0:64], w[64:128], w[128:192]
        for i, parts in enumerate(((wx, wy), (wz, wy), (wx, wy + wz))):
            wos_ref[i] = pltpu.bitcast(_cat(parts).T.astype(BF16), U32)

        top_ref[...] = jnp.zeros(top_ref.shape, F32)
        for i in (WS + 1, 2 * WS + 3):
            x_ref[i] = jnp.zeros(x_ref.shape[1:], x_ref.dtype)

        for p in range(stg_ref.shape[0]):
            stg_ref[p] = jnp.zeros(stg_ref.shape[1:], F32)
        for r in range(WS):
            ob_ref[pl.ds(r * WP + WP - 8, 8), :] = jnp.zeros((8, LANES), F32)

    cuts = [int(c) for c in _env("CUTS", "0,7").split(",")]
    bands = list(zip(cuts, cuts[1:]))
    groups = {(b, g): conv_group(8 * g) for b in range(len(bands)) for g in range(NG)}
    WLEAD = _env("WLEAD", 4)

    def conv_items(nslow):
        plist = [((b, g), r) for b, (r0, r1) in enumerate(bands) for g in range(NG) for r in range(r0, r1)]
        items, nxt_tap = [], WLEAD
        for k, (g, r) in enumerate(plist):
            fs = []
            lead = WLEAD if k < nslow else _env("WLEAD2", 5)
            while nxt_tap <= min(k + lead, len(plist) - 1):
                g2, r2 = plist[nxt_tap]
                fs.append(functools.partial(groups[g2][0], r2))
                nxt_tap += 1
            fs.append(functools.partial(groups[g][1], r))
            items.append(fs)
        return items

    def ld_x0(j, k, gs=range(NG)):
        return [x0_ref[rows_at(nxt + dyn0 * (8 * k), j * C + 8 * g, 8), :] for g in gs]

    def add2(acc, xs):
        a = functools.reduce(jnp.add, xs[0::2])
        b = functools.reduce(jnp.add, xs[1::2])
        return a + b if acc is None else (acc + a) + b

    stats_done = set()

    def stats_steps(j):
        st = {"s": None, "q": None}
        n1, n2 = _env("SEG1", 8), _env("SEG2", 6)

        def sum_step(g0):
            st["s"] = add2(st["s"], ld_x0(j, 0, range(g0, g0 + n1)))
            if g0 + n1 == NG:
                st["s"] = _allred(st["s"], jnp.add) * (1.0 / C)
            return st["s"]

        def var_step(g0):
            d = [x - st["s"] for x in ld_x0(j, 1, range(g0, g0 + n2))]
            st["q"] = add2(st["q"], [x * x for x in d])
            return st["q"]

        def last_step():
            v = _allred(st["q"], jnp.add) * (1.0 / C) + EPS
            rs = lax.rsqrt(v) if _env("RSQ", 1) else jnp.exp2(jnp.log2(v) * -0.5)
            ms_ref[j] = _cat([st["s"], rs])
            stats_done.add(j)
            return rs

        return ([functools.partial(sum_step, g) for g in range(0, NG, n1)]
                + [functools.partial(var_step, g) for g in range(0, NG, n2)] + [last_step])

    def colsum(xs):
        xs = [a + b for a, b in zip(xs[0:8], xs[16:24])] + xs[8:16]
        return _dot(jnp.ones((8, LANES), F32), _cat(xs))

    means = {}

    def mean_dot(j):
        means[j] = colsum(ld_x0(j, 0)) * (1.0 / C)

    def var_dot(j):
        xs = [x0_ref[pl.ds(nxt + (j * C + 8 * g + 4), 8), :] for g in range(NG - 1)]
        xs.append(jnp.where(mk["up"], *ld_x0(j, 0, (0, NG - 1))))
        d = [x - means[j] for x in xs]
        v = colsum([x * x for x in d]) * (1.0 / C) + EPS
        rs = lax.rsqrt(v) if _env("RSQ", 1) else jnp.exp2(jnp.log2(v) * -0.5)
        ms_ref[j] = _cat([means[j], rs])
        stats_done.add(j)

    def normed(j, blk, k):
        assert j in stats_done or "ONLY" in os.environ and j < NSTX, j
        m, rs = ms_ref[j, 0:8, :], ms_ref[j, 8:16, :]
        return _cat([(x - m) * rs for x in ld_x0(j, k, range(8 * blk, 8 * blk + 8))])

    t_done = {}

    def put_t(dst, tiles):
        tt = pltpu.bitcast(jnp.concatenate(tiles, axis=1).astype(BF16).T, U32)
        for i, (u, e) in enumerate(dst):
            t_ref[u, e] = tt[64 * i:64 * i + 64]
        t_done[len(t_done)] = pltpu.bitcast(tt[120:128], F32)

    def t_first(u):
        ja, jb = 2 * u, 2 * u + 1
        bx = normed(jb, 0, 0)
        put_t([(u, 0), (u, 2)], [_cat([normed(ja, 0, 0) - bx, normed(ja, 1, 0)]),
                                 _cat([bx, normed(ja, 2, 0)])])

    def t_second(r):
        put_t([(u, 1) for u in (2 * r, 2 * r + 1)],
              [_cat([normed(2 * u + 1, 1, 0), normed(2 * u + 1, 2, 0) - normed(2 * u, 2, _env("RECOMP", 1))])
               for u in (2 * r, 2 * r + 1)])

    t_items = []
    for r in range(WS):
        t_items += [functools.partial(t_first, 2 * r), functools.partial(t_first, 2 * r + 1),
                    functools.partial(t_second, r)]

    def qkv_chunk(us, n, steps=(), tiny=()):
        lhs = {i: [b for u in us for b in _blocks(t_ref[u, i])] for i in range(3)}
        for q, step in enumerate(steps):
            tok = pltpu.bitcast(step(), U32)
            q = q * 24 * len(us) // len(steps)
            blks = lhs[(2, 0, 1)[q % 3]]
            blks[q // 3] = jnp.where(mk["never"], tok, blks[q // 3])
        p3 = None
        for i in (2, 0, 1):
            p = _dot(pltpu.bitcast(_cat(lhs[i]), BF16), pltpu.bitcast(ws_ref[i, n], BF16))
            if p3 is None:
                p3 = p
            else:
                p = p + p3
                for e, u in enumerate(us):
                    r, tp = divmod(u, 2)
                    qkv_ref[n, r, pl.ds((2 * tp + i) * LANES, LANES), :] = p[e * LANES:(e + 1) * LANES]

    vr_words = {}
    job_done = {}

    def side_dots(u, n):
        r, tp = divmod(u, 2)
        st = {}

        def one(i, parts=1):
            if parts > 1:
                lhs, rows = t_ref[u, i], 64 // parts
                p = _cat([_dot(pltpu.bitcast(lhs[q * rows:(q + 1) * rows], BF16),
                               pltpu.bitcast(ws_ref[i, n], BF16)) for q in range(parts)])
            elif n == 4:
                p = _dot_nt(pltpu.bitcast(ws_ref[i, 4, 0:32, :], BF16), pltpu.bitcast(t_ref[u, i], BF16))
            else:
                p = _dot(pltpu.bitcast(t_ref[u, i], BF16), pltpu.bitcast(ws_ref[i, n], BF16))
            st[i] = p if i == 2 else p + st[2]
            if n < 4 and i < 2:
                qkv_ref[n, r, pl.ds((2 * tp + i) * LANES, LANES), :] = st[i]
            elif i == 1:
                vr_words[u] = pltpu.pack_elementwise([st[0], st[1]], packed_dtype=BF16)

        return [(64 if n == 4 else LANES, (u, n, i), functools.partial(one, i)) for i in (2, 0, 1)]

    def vr_store(u):
        r, tp = divmod(u, 2)
        w = pltpu.bitcast(vr_words[u], F32)
        wt = pltpu.bitcast(_cat([w, w]).T, U32)
        job_done["v", u] = pltpu.bitcast(wt[120:128], F32)
        for j in range(2):
            qkv_ref[4, r, pl.ds((2 * tp + j) * LANES, LANES), :] = pltpu.unpack_elementwise(
                wt, index=j, packed_dtype=BF16, unpacked_dtype=F32)

    zero8 = jnp.zeros((8, LANES), F32)

    def gather(n, off, k=0):
        return [qkv_ref[n, r, pl.ds(off + dyn0 * k if k else off, 8), :] for r in range(WS)]

    def softmax_t(st):
        rows = _blocks(st)
        m = functools.reduce(jnp.maximum, rows)
        m = _allred(jnp.where(mk["key"], m, -jnp.inf), jnp.maximum)
        p = [jnp.exp2(x - m) for x in rows]
        return p, functools.reduce(jnp.add, p)

    def s2_pair(pi, offa):
        offb = offa + WS
        st = {}

        def vprep():
            g = [gather(n, offa) + gather(n, offb) for n in range(5)]
            u1 = [jnp.where(mk["left64"], z, jnp.where(mk["v"], x, y)) for x, y, z in zip(g[0], g[1], g[4])]
            u2 = [jnp.where(mk["v"], x, y) for x, y in zip(g[2], g[3])]
            u = jnp.concatenate([_cat(u1 + [zero8, zero8]), _cat(u2 + [zero8, zero8])], axis=1)
            vt = pltpu.bitcast(u.astype(BF16).T, U32)
            vt = _cat([vt[0:64], vt[96:128]])
            st["vt"] = [pltpu.bitcast(vt[24 * h:24 * h + 24], BF16) for h in range(NH)]

        def score(i, ties=()):
            hp, sw = divmod(i, 2)
            lo, hi = mk["lo"], mk["hi%d" % hp]
            ma, mb = (lo, hi) if sw == 0 else (hi, lo)
            gq = (0, 1, 1 + sw)[_env("GQ", 0)]
            gk = (0, 1, 1 + sw)[_env("GK", 0)]
            q = _cat([jnp.where(ma, v, 0.0) for v in gather(hp, offa, gq)]
                     + [jnp.where(mb, v, 0.0) for v in gather(hp, offb, gq)] + [zero8, zero8])
            ka, kb = gather(2 + hp, offa, gk), gather(2 + hp, offb, gk)
            k = [jnp.where(lo, x, y) for x, y in (zip(ka, kb) if sw == 0 else zip(kb, ka))]
            for _, job in ties:
                k[0] = jnp.where(mk["never"], job(), k[0])
            k = _cat(k)
            st["p", i] = softmax_t(_dot_nt(k, q))

        def value(h):
            hp, sw = divmod(h, 2)
            (pa, sa), (pb, sb) = st["p", 2 * hp + sw], st["p", 2 * hp + 1 - sw]
            pm = _cat([jnp.where(mk["keep_a"], v, 0.0) for v in pa]
                      + [jnp.where(mk["keep_b"], v, 0.0) for v in pb] + [zero8, zero8])
            den = _allred(jnp.where(mk["keep_a"], sa, jnp.where(mk["keep_b"], sb, 0.0)), jnp.add)
            rec = pl.reciprocal(den, approx=True)
            if _env("NR", 0):
                rec = rec * (2.0 - den * rec)
            st["o", h] = [b * rec for b in _blocks(_dot(st["vt"][h], pm))]

        def finish():
            o = [b for h in range(NH) for b in st["o", h]]
            w = pltpu.pack_elementwise([_cat(o[0:16]), _cat(o[16:24] + o[16:24])], packed_dtype=BF16)
            stg_ref[pi] = pltpu.bitcast(w, F32)

        def scatter():
            wt = stg_ref[pi].T
            job_done["s", pi] = wt[104:112]
            for i, off in enumerate((offa, offb)):
                for r in range(WS):
                    base = i * SLOTS + 8 * r
                    ob_ref[pl.ds(r * WP + off, WS), :] = wt[base:base + WS]

        return vprep, score, value, finish, scatter

    npair = (nwin + 1) // 2
    pairs = [s2_pair(p, min(2 * p, nwin - 2) * WS) for p in range(npair)]

    def s3_unit(r, tp, ties=()):
        def unpack(t):
            w = pltpu.bitcast(ob_ref[pl.ds(r * WP + t * LANES, LANES), :], U32)
            return [_blocks(pltpu.unpack_elementwise(w, index=i, packed_dtype=BF16, unpacked_dtype=F32))
                    for i in range(2)]

        (la, ha), (lb, hb) = unpack(2 * tp), unpack(2 * tp + 1)
        t3 = [jnp.where(mk["left64"], x, y) for x, y in zip(lb, ha)]
        t1 = _cat([x - y for x, y in zip(la, t3)])
        t2 = _cat([jnp.where(mk["left64"], x, z) - y for x, y, z in zip(hb, ha, lb)])
        t3 = _cat(t3)
        wo = [_blocks(wos_ref[i]) for i in range(3)]
        for q, (e, job) in enumerate(ties):
            blks = wo[(2, 0, 1)[q % 3]]
            blks[e] = jnp.where(mk["never"], pltpu.bitcast(job(), U32), blks[e])
        wo = [pltpu.bitcast(_cat(w), BF16) for w in wo]
        p3 = _dot_nt(wo[2], t3)
        ys = [_dot_nt(wo[i], t) + p3
              + x0_ref[rows_at(prv, (r * NT + 2 * tp + i) * C, C), :] for i, t in enumerate((t1, t2))]
        n = min(2 * LANES, W - 2 * tp * LANES)
        o_ref[ooff + r, :, pl.ds(2 * tp * LANES, n)] = jnp.concatenate(ys, axis=1).astype(o_ref.dtype)[:, :n]

    s3_all = [functools.partial(s3_unit, r, tp) for tp in range(2) for r in range(WS)]

    def run(prog, extra):
        extra = sorted(extra, key=lambda e: e[0])
        j = 0
        for t0, fn in prog:
            while j < len(extra) and extra[j][0] <= t0:
                extra[j][1]()
                j += 1
            fn()
        for e in extra[j:]:
            e[1]()

    MERGE = _env("MERGE", 0)
    NX3 = _env("NX3", 0)

    NSY = 0

    NSTX = _env("NSTX", 20)

    def wave_steps(lo, hi, wave):
        steps = []
        for j0 in range(lo, hi, wave):
            for grp in zip(*[stats_steps(j) for j in range(j0, min(j0 + wave, hi))]):
                steps += grp
        return steps

    def block_x():
        NJ = _env("NJ", 28)
        NSTC = _env("NSTC", 6)
        WAVE = _env("WAVE", 4)
        VRLAG = _env("VRLAG", 200)
        chunks = [(u, n) for u in range(NU) for n in range(4)]
        MXS = _env("MXS", 0)
        steps = [] if MXS else wave_steps(0, NSTX, WAVE)
        loose = steps[len(steps) - _env("LOOSE", 0):]
        steps = steps[:len(steps) - len(loose)]
        nside = 9
        side, vstep = [], _env("VRSTEP", 1)
        for q in range(NU // 2):
            side += side_dots(2 * q, 4) + side_dots(2 * q + 1, 4)
            for _ in range(vstep):
                if nside:
                    side += side_dots(*chunks.pop())
                    nside -= 1
        for _ in range(nside):
            side += side_dots(*chunks.pop())
        mu = _env("MU", 2)
        merged = []
        for u, n in chunks:
            prev = [c for c in merged if c[1] == n and c[0][0] // mu == u // mu]
            if prev:
                prev[0][0].append(u)
            else:
                merged.append(([u], n))
        starts = [LANES * sum(len(c[0]) for c in merged[:k]) for k in range(len(merged))]
        t_conv = max(x for x in starts if x <= (len(chunks) - NSTC) * LANES)
        span = len(chunks) * LANES - t_conv
        plan, t, vr_ready = [], 0, {}
        for k, (us, n) in enumerate(merged):
            dur = LANES * len(us)
            lo, hi = (max(x - t_conv, 0) * len(steps) // span for x in (t, t + dur))
            plan.append((t, tuple(us), n, list(steps[lo:hi]), []))
            room = dur
            while side and (room > 0 or k == len(merged) - 1):
                rows, key, f = side.pop(0)
                plan.append((t, f if room > 0 else functools.partial(f, 4), None, [], []))
                room -= rows
                if key[1:] == (4, 1):
                    vr_ready[key[0]] = t + dur - room + VRLAG
            t += dur
        ci = conv_items(4 * NJ)
        slow = _env("SLOW", 32.0)
        fast = (t_conv - 4 * NJ * slow) / max(len(ci) - 4 * NJ, 1)
        t_piece = [min(j, 4 * NJ) * slow + max(j - 4 * NJ, 0) * fast for j in range(len(ci) + 1)]
        scat, vrs = list(range(npair - NSY)), list(range(NU))
        jobs = []
        for q in range(NJ):
            if vrs and vr_ready[vrs[0]] <= t_piece[4 * q + 1]:
                jobs.append((t_piece[4 * q + 1], ("v", vrs[0])))
                ci[4 * q].insert(0, functools.partial(vr_store, vrs.pop(0)))
            elif scat:
                jobs.append((t_piece[4 * q + 1], ("s", scat[0])))
                ci[4 * q].insert(0, pairs[scat.pop(0)][4])
        extra = [(t_piece[j + 1], f) for j, fs in enumerate(ci) for f in fs]
        tail = [(("v", u), functools.partial(vr_store, u)) for u in vrs] + [(("s", p), pairs[p][4]) for p in scat]
        for q, (key, f) in enumerate(tail):
            t_q = max(t_conv + 1 + (q // 3) * 128, vr_ready[key[1]] if key[0] == "v" else 0)
            extra.append((t_q, f))
            jobs.append((t_q, key))
        if _env("JDL", 800):
            for t_q, key in jobs:
                later = [e for e in plan if e[2] is not None and e[0] >= t_q + _env("JDL", 800)]
                if later:
                    later[0][3].insert(0, functools.partial(job_done.get, key))
        prog = [(t0, u if n is None else functools.partial(qkv_chunk, u, n, st, tn))
                for t0, u, n, st, tn in plan]
        run(prog, extra + [(t, f) for f in loose])

    def block_y():
        pattern = _env("PAT", "SFFVFFFF" + "SSSSFVVVV" * 8 + "SSSSVVVV").rstrip(".")
        load = [0] * 4
        items, ns, nv, nf = [], 0, 0, 0
        for ch in pattern:
            if ch in "Ss":
                todo = [("s", ns + i, [SLOTS]) for i in range(4 if ch == "S" else 2)]
                ns += len(todo)
            elif ch in "Vv":
                todo = [("v", nv + i, [DH]) for i in range(4 if ch == "V" else 2)]
                nv += len(todo)
            else:
                todo = [("f", nf, [C] * 3)]
                nf += 1
            for kind, idx, rows in todo:
                items.append((min(load), kind, idx, []))
                for x in rows:
                    load[load.index(min(load))] += x
        assert (ns, nv, nf) == (4 * npair, 4 * npair, NU)
        spots = sorted([(it[0], it, 0) for it in items if it[1] == "s"]
                       + [(it[0] + 16 * e, it, e) for it in items if it[1] == "f" for e in range(12)],
                       key=lambda x: x[0])
        ysteps = wave_steps(NSTX, WS * NT, _env("WAVEY", 4))
        fspots = [x for x in spots if x[1][1] == "f" and x[1][2] < _env("S3Q", 6)
                  and _env("E0", 1) <= x[2] < _env("E1", 8)]
        fspots.sort(key=lambda x: (x[1][2], x[2]))
        for q, step in enumerate(ysteps):
            _, it, e = fspots[q * len(fspots) // len(ysteps)]
            it[3].append((e, step))
        t_done.clear()
        extra = []
        tpos = [int(x) for x in _env("TPOS", "8,9").split(",")]
        late = [x for x in spots if x[1][1] == "s" and x[1][2] >= 4 and (x[1][2] - 4) % 16 in tpos]
        late.sort(key=lambda x: x[1][2])
        n1 = max(_env("NT1", 3), len(t_items) - len(late))
        ta0, ta1 = _env("TA0", 500), _env("TA1", 900)
        late = late[_env("TSKIP", 0):]
        for j, f in enumerate(t_items):
            if j < n1:
                t_s, it, e = [x for x in spots if x[0] >= ta0 + j * (ta1 - ta0) / n1][0]
            else:
                t_s, it, e = late[(j - n1) * len(late) // (len(t_items) - n1)]
            it[3].append((e, functools.partial(t_done.__getitem__, j)))
            extra.append((min(t_s - _env("TLEAD", 300), it[0]), f))
        prog = []
        for t0, kind, idx, ties in items:
            p, i = divmod(idx, 4)
            if kind == "s":
                if i == 0:
                    prog.append((t0, pairs[p][0]))
                prog.append((t0, functools.partial(pairs[p][1], i, ties)))
            elif kind == "v":
                prog.append((t0, functools.partial(pairs[p][2], i)))
                if i == 3:
                    extra.append((t0 + DH + _env("LFIN", 0), pairs[p][3]))
            else:
                prog.append((t0, functools.partial(s3_all[idx], ties)))
        run(prog, extra)

    only = _env("ONLY", "01")

    @when(k_ < nstrip, ("main",))
    def _():
        x_copy(k_).wait()

    @when(k_ < nstrip - 1, ("first", "main"))
    def _():
        x_copy(k_ + 1).start()

    new_masks("x")
    if "0" in only:
        when(k_ <= nstrip, ("main",))(block_x)

    @when(k_ == 0, ("first",))
    def _():
        def body(g, carry):
            x0_copy(g).wait()
            for j in range(FG):
                piece = conv_group(pl.multiple_of((g * FG + j) * 8, 8))[1]
                for r in range(WS):
                    piece(r)
            return carry
        lax.fori_loop(0, NG // FG, body, 0)

    @when(k_ >= 4, ("main", "last"))
    def _():
        o_copy(k_ - 4).wait()

    @when(k_ >= 3, ("main", "last"))
    def _():
        o_copy(k_ - 3).start()

    if "1" in only:
        new_masks("y")
        when((k_ <= nstrip) & (k_ >= 1), ("main",))(block_y)

    @when(k_ == 0, ("first",))
    def _():
        for j in range(WS * NT):
            for f in stats_steps(j):
                f()
        for f in t_items:
            f()

    @when(k_ == nstrip + 1, ("last",))
    def _():
        new_masks("y")
        for p in range(npair):
            pairs[p][4]()
        for q, f in enumerate(s3_all):
            f()
            if q >= WS:
                row_copy(q - WS).start()

    if only != "01":
        @when(dyn0 < 0, ("main",))
        def _():
            i = pl.multiple_of(k_ * 8, 8)
            o_ref[0, 0:16, 0:128] = _cat([
                qkv_ref[k3, k3, pl.ds(i, 8), :] + ms_ref[k3, 0:8, :] + stg_ref[k3, pl.ds(i, 8), :],
                pltpu.bitcast(t_ref[k3, k3, pl.ds(i, 8), :], F32) + ob_ref[pl.ds(i, 8), :]]).astype(BF16)
            for rf in (qkv_ref.at[k3, k3], stg_ref.at[k3], ob_ref):
                rf[pl.ds(i, 8), :] = zero8
            t_ref[k3, k3, pl.ds(i, 8), :] = pltpu.bitcast(zero8, U32)

    @when(k_ == nstrip + 1, ("last",))
    def _():
        o_copy(k_ - 3).wait()
        for r in range(WS):
            row_copy(r).wait()


@jax.jit
def pallas_standalone__window_attn_davit__vision_kernel(
    x: jax.Array,
    dw_pe: jax.Array,
    w_qkv: jax.Array,
    w_o: jax.Array,
):
    B, H, W, Cx = x.shape
    assert B == 1 and Cx == C and H % WS == 0 and W % WS == 0 and WP - LANES < W < WP
    xt = jnp.transpose(x[0], (0, 2, 1))

    assert H // WS + 2 <= 256
    vmem = pl.BlockSpec(memory_space=pltpu.VMEM)
    yt = pl.pallas_call(
        functools.partial(_kernel, H=H, W=W),
        in_specs=[pl.BlockSpec(memory_space=pl.ANY), vmem, vmem, vmem],
        out_specs=pl.BlockSpec(memory_space=pl.ANY),
        out_shape=jax.ShapeDtypeStruct((H, C, W), x.dtype),
        scratch_shapes=[
            pltpu.VMEM((2 * (WS + 2), C, W), x.dtype),
            pltpu.VMEM((2 * WS, C, W), x.dtype),
            pltpu.SemaphoreType.DMA((5,)),
            pltpu.VMEM((X0_ROWS, LANES), F32),
            pltpu.VMEM((WS * WP, LANES), F32),
            pltpu.VMEM((9, C, LANES), F32),
            pltpu.VMEM((3, 5, LANES // 2, LANES), U32),
            pltpu.VMEM((3, C // 2, LANES), U32),
            pltpu.VMEM((5, WS, WP, LANES), F32),
            pltpu.VMEM((NU, 3, LANES // 2, LANES), U32),
            pltpu.VMEM((37, LANES, LANES), F32),
            pltpu.VMEM((WS * NT, 16, LANES), F32),
            pltpu.VMEM((C, WP), F32),
        ],
        compiler_params=pltpu.CompilerParams(
            vmem_limit_bytes=64 * 1024 * 1024,
            disable_bounds_checks=bool(_env("NOBC", 1)),
        ),
        name="davit_window_attn",
    )(xt, dw_pe, w_qkv, w_o)
    return jnp.transpose(yt, (0, 2, 1))[None]
```

```python
import functools
import math
import os

import jax
import jax.numpy as jnp
from jax import lax
import jax.experimental.pallas as pl
import jax.experimental.pallas.tpu as pltpu

WS = 7
NH = 4
C = 192
DH = C // NH
NG = C // 8
LANES = 128
WP = 512
NT = WP // LANES
NU = WS * NT // 2
SLOTS = 8 * WS
EPS = 1e-5
F32 = jnp.float32
BF16 = jnp.bfloat16
U32 = jnp.uint32

X0_SLOT = WS * NT * C
DW_OFF = 3 * X0_SLOT
X0_ROWS = DW_OFF + 2 * C


def _dot(a, b):
    return jnp.dot(a, b, preferred_element_type=F32)


def _dot_nt(a, b):
    return lax.dot_general(a, b, (((1,), (1,)), ((), ())), preferred_element_type=F32)


def _cat(xs):
    return jnp.concatenate(xs, axis=0)


def _blocks(v):
    return [v[i:i + 8] for i in range(0, v.shape[0], 8)]


def _allred(x, op):
    for sh in (4, 2, 1):
        x = op(x, pltpu.roll(x, sh, 0))
    return x


def _env(name, default):
    return type(default)(os.environ.get(name, default))


def _kernel(x_hbm, dw_ref, wqkv_ref, wo_ref, o_hbm, *scratch, H, W):
    step = functools.partial(_step, x_hbm, dw_ref, wqkv_ref, wo_ref, o_hbm, *scratch, H=H, W=W)
    nstrip = H // WS

    def loop(lo, hi, mode):
        def body(k, carry):
            step(k_=k, mode=mode)
            return carry
        lax.fori_loop(lo, hi, body, 0)

    if "ONLY" not in os.environ:
        loop(0, 1, "first")
    loop(1 + _env("SKIP", 0), nstrip + 1, "main")
    if "ONLY" not in os.environ:
        loop(nstrip + 1, nstrip + 2, "last")


def _step(x_hbm, dw_ref, wqkv_ref, wo_ref, o_hbm,
          x_ref, o_ref, sems, x0_ref, ob_ref, dws_ref, ws_ref, wos_ref, qkv_ref, t_ref, stg_ref, ms_ref,
          top_ref, *, H, W, k_, mode):
    nstrip, nwin = H // WS, W // WS

    def x_copy(k):
        return pltpu.make_async_copy(x_hbm.at[pl.ds(jnp.minimum(k * WS, H - WS - 1), WS + 1)],
                                     x_ref.at[pl.ds((k & 1) * (WS + 2), WS + 1)], sems.at[0])

    def o_copy(k):
        return pltpu.make_async_copy(o_ref.at[pl.ds((k & 1) * WS, WS)], o_hbm.at[pl.ds(k * WS, WS)],
                                     sems.at[1])

    FG = 8

    def x0_copy(g):
        cs = pl.ds(pl.multiple_of(g * (8 * FG), 8 * FG), 8 * FG)
        return pltpu.make_async_copy(x_hbm.at[pl.ds(0, WS + 1), cs], x_ref.at[pl.ds(0, WS + 1), cs],
                                     sems.at[2 + g])

    def row_copy(r):
        return pltpu.make_async_copy(o_ref.at[ooff + r], o_hbm.at[H - WS + r], sems.at[2])

    def when(cond, modes):
        if mode in modes:
            return pl.when(cond)
        return lambda f: None

    xoff = (k_ & 1) * (WS + 2) + jnp.where(k_ >= nstrip - 1, 1, 0)
    ooff = (k_ & 1) * WS
    dyn0 = jnp.minimum(k_, 0)

    def rows_at(base, off, n):
        if isinstance(base, int):
            return pl.ds(base + off, n)
        return pl.ds(pl.multiple_of(base + off, 8), n)

    mk = {}

    def new_masks(blk):
        lane = lax.broadcasted_iota(jnp.int32, (8, LANES), 1)
        mk.clear()
        mk["never"] = lane < dyn0
        if blk == "x":
            mk["up"] = lax.broadcasted_iota(jnp.int32, (8, LANES), 0) < 4
            return
        key_ok = lax.broadcasted_iota(jnp.int32, (8, LANES), 0) < WS
        mk.update(
            lo=lane < DH, hi0=(lane >= DH) & ((lane < 64) | (lane >= 96)), hi1=(lane >= DH) & (lane < 96),
            v=lane < 96, key=key_ok, keep_a=key_ok & (lane < SLOTS), keep_b=key_ok & (lane >= SLOTS),
            left64=lane < 64)

    k3 = k_ - 3 * ((k_ * 171) >> 9)
    nxt = k3 * X0_SLOT
    prv = jnp.where((k3 == 2) | (k_ < 2), 0, nxt + X0_SLOT)

    def conv_group(c0):
        st = {}

        def row(i):
            if i == 0 and i not in st:
                st[i] = top_ref[pl.ds(c0, 8), :]
            if i not in st:
                v = x_ref[xoff + (i - 1), pl.ds(c0, 8), :].astype(F32)
                st[i] = jnp.concatenate([v, jnp.zeros((8, WP - W), F32)], axis=1)
                if i == WS and i - 2 in st:
                    top_ref[pl.ds(c0, 8), :] = st[i]
            return st[i]

        def bc(v):
            return jnp.concatenate([v] * NT, axis=1)

        def taps(r):
            st["tw", r] = [bc(x0_ref[rows_at(c0, DW_OFF + k * C, 8), :]) for k in range(2)]

        def piece(r):
            if "w" not in st:
                st["w"] = [bc(dws_ref[k, pl.ds(c0, 8), :]) for k in range(9)]
            wts = list(st["w"])
            if ("tw", r) in st:
                wts[6], wts[8] = st["tw", r]
            row(r)
            abc = [row(r + 1) * wts[3 + j] + row(r) * wts[j] + row(r + 2) * wts[6 + j] for j in range(3)]
            x0 = pltpu.roll(abc[0], 1, 1) + abc[1] + pltpu.roll(abc[2], WP - 1, 1)
            for t in range(NT):
                x0_ref[rows_at(nxt, (r * NT + t) * C + c0, 8), :] = x0[:, t * LANES:(t + 1) * LANES]

        return taps, piece

    @when(k_ == 0, ("first",))
    def _():
        for g in range(NG // FG):
            x0_copy(g).start()
        for k in range(9):
            w = dw_ref[k // 3].astype(F32)[k % 3:k % 3 + 1, :]
            w = jnp.broadcast_to(w, (LANES, C)).T
            dws_ref[k] = w + 1.0 if k == 4 else w
            if k in (6, 8):
                x0_ref[pl.ds(DW_OFF + (k - 6) // 2 * C, C), :] = w
        w = wqkv_ref[...].astype(F32)
        wq = w[:, 0:C] * ((DH ** -0.5) * math.log2(math.e))
        wk, wv = w[:, C:2 * C], w[:, 2 * C:3 * C]
        tiles = [(wq[:, 0:64], wv[:, 64:96], wq[:, 64:96]),
                 (wq[:, 96:192], wv[:, 96:128]),
                 (wk[:, 0:64], wv[:, 128:160], wk[:, 64:96]),
                 (wk[:, 96:192], wv[:, 160:192]),
                 (wv[:, 0:128],)]
        for n, parts in enumerate(tiles):
            w = jnp.concatenate(parts, axis=1)
            for i, wi in enumerate((w[0:128], w[64:192], _cat([w[0:64], w[128:192]]))):
                if n == 4:
                    wi = wi.T
                ws_ref[i, n] = pltpu.bitcast(wi.astype(BF16), U32)
        w = wo_ref[...].astype(F32)
        wx, wy, wz = w[0:64], w[64:128], w[128:192]
        for i, parts in enumerate(((wx, wy), (wz, wy), (wx, wy + wz))):
            wos_ref[i] = pltpu.bitcast(_cat(parts).T.astype(BF16), U32)

        top_ref[...] = jnp.zeros(top_ref.shape, F32)
        for i in (WS + 1, 2 * WS + 3):
            x_ref[i] = jnp.zeros(x_ref.shape[1:], x_ref.dtype)

        for p in range(stg_ref.shape[0]):
            stg_ref[p] = jnp.zeros(stg_ref.shape[1:], F32)
        for r in range(WS):
            ob_ref[pl.ds(r * WP + WP - 8, 8), :] = jnp.zeros((8, LANES), F32)

    cuts = [int(c) for c in _env("CUTS", "0,7").split(",")]
    bands = list(zip(cuts, cuts[1:]))
    groups = {(b, g): conv_group(8 * g) for b in range(len(bands)) for g in range(NG)}
    WLEAD = _env("WLEAD", 4)

    def conv_items(nslow):
        plist = [((b, g), r) for b, (r0, r1) in enumerate(bands) for g in range(NG) for r in range(r0, r1)]
        items, nxt_tap = [], WLEAD
        for k, (g, r) in enumerate(plist):
            fs = []
            lead = WLEAD if k < nslow else _env("WLEAD2", 5)
            while nxt_tap <= min(k + lead, len(plist) - 1):
                g2, r2 = plist[nxt_tap]
                fs.append(functools.partial(groups[g2][0], r2))
                nxt_tap += 1
            fs.append(functools.partial(groups[g][1], r))
            items.append(fs)
        return items

    def ld_x0(j, k, gs=range(NG)):
        return [x0_ref[rows_at(nxt + dyn0 * (8 * k), j * C + 8 * g, 8), :] for g in gs]

    def add2(acc, xs):
        a = functools.reduce(jnp.add, xs[0::2])
        b = functools.reduce(jnp.add, xs[1::2])
        return a + b if acc is None else (acc + a) + b

    stats_done = set()

    def stats_steps(j):
        st = {"s": None, "q": None}
        n1, n2 = _env("SEG1", 12), _env("SEG2", 6)

        def sum_step(g0):
            st["s"] = add2(st["s"], ld_x0(j, 0, range(g0, g0 + n1)))
            if g0 + n1 == NG:
                st["s"] = _allred(st["s"], jnp.add) * (1.0 / C)
            return st["s"]

        def var_step(g0):
            d = [x - st["s"] for x in ld_x0(j, 1, range(g0, g0 + n2))]
            st["q"] = add2(st["q"], [x * x for x in d])
            return st["q"]

        def last_step():
            v = _allred(st["q"], jnp.add) * (1.0 / C) + EPS
            rs = lax.rsqrt(v) if _env("RSQ", 1) else jnp.exp2(jnp.log2(v) * -0.5)
            ms_ref[j] = _cat([st["s"], rs])
            stats_done.add(j)
            return rs

        return ([functools.partial(sum_step, g) for g in range(0, NG, n1)]
                + [functools.partial(var_step, g) for g in range(0, NG, n2)] + [last_step])

    def colsum(xs):
        xs = [a + b for a, b in zip(xs[0:8], xs[16:24])] + xs[8:16]
        return _dot(jnp.ones((8, LANES), F32), _cat(xs))

    means = {}

    def mean_dot(j):
        means[j] = colsum(ld_x0(j, 0)) * (1.0 / C)

    def var_dot(j):
        xs = [x0_ref[pl.ds(nxt + (j * C + 8 * g + 4), 8), :] for g in range(NG - 1)]
        xs.append(jnp.where(mk["up"], *ld_x0(j, 0, (0, NG - 1))))
        d = [x - means[j] for x in xs]
        v = colsum([x * x for x in d]) * (1.0 / C) + EPS
        rs = lax.rsqrt(v) if _env("RSQ", 1) else jnp.exp2(jnp.log2(v) * -0.5)
        ms_ref[j] = _cat([means[j], rs])
        stats_done.add(j)

    def normed(j, blk, k):
        assert j in stats_done or "ONLY" in os.environ and j < NSTX, j
        m, rs = ms_ref[j, 0:8, :], ms_ref[j, 8:16, :]
        return _cat([(x - m) * rs for x in ld_x0(j, k, range(8 * blk, 8 * blk + 8))])

    t_done = {}

    def put_t(dst, tiles):
        tt = pltpu.bitcast(jnp.concatenate(tiles, axis=1).astype(BF16).T, U32)
        for i, (u, e) in enumerate(dst):
            t_ref[u, e] = tt[64 * i:64 * i + 64]
        t_done[len(t_done)] = pltpu.bitcast(tt[120:128], F32)

    def t_first(u):
        ja, jb = 2 * u, 2 * u + 1
        bx = normed(jb, 0, 0)
        put_t([(u, 0), (u, 2)], [_cat([normed(ja, 0, 0) - bx, normed(ja, 1, 0)]),
                                 _cat([bx, normed(ja, 2, 0)])])

    def t_second(r):
        put_t([(u, 1) for u in (2 * r, 2 * r + 1)],
              [_cat([normed(2 * u + 1, 1, 0), normed(2 * u + 1, 2, 0) - normed(2 * u, 2, _env("RECOMP", 0))])
               for u in (2 * r, 2 * r + 1)])

    t_items = []
    for r in range(WS):
        t_items += [functools.partial(t_first, 2 * r), functools.partial(t_first, 2 * r + 1),
                    functools.partial(t_second, r)]

    def qkv_chunk(us, n, steps=(), tiny=()):
        lhs = {i: [b for u in us for b in _blocks(t_ref[u, i])] for i in range(3)}
        for q, step in enumerate(steps):
            tok = pltpu.bitcast(step(), U32)
            q = q * 24 * len(us) // len(steps)
            blks = lhs[(2, 0, 1)[q % 3]]
            blks[q // 3] = jnp.where(mk["never"], tok, blks[q // 3])
        p3 = None
        for i in (2, 0, 1):
            p = _dot(pltpu.bitcast(_cat(lhs[i]), BF16), pltpu.bitcast(ws_ref[i, n], BF16))
            if p3 is None:
                p3 = p
            else:
                p = p + p3
                for e, u in enumerate(us):
                    r, tp = divmod(u, 2)
                    qkv_ref[n, r, pl.ds((2 * tp + i) * LANES, LANES), :] = p[e * LANES:(e + 1) * LANES]

    vr_words = {}
    job_done = {}

    def side_dots(u, n):
        r, tp = divmod(u, 2)
        st = {}

        def one(i, parts=1):
            if parts > 1:
                lhs, rows = t_ref[u, i], 64 // parts
                p = _cat([_dot(pltpu.bitcast(lhs[q * rows:(q + 1) * rows], BF16),
                               pltpu.bitcast(ws_ref[i, n], BF16)) for q in range(parts)])
            elif n == 4:
                p = _dot_nt(pltpu.bitcast(ws_ref[i, 4, 0:32, :], BF16), pltpu.bitcast(t_ref[u, i], BF16))
            else:
                p = _dot(pltpu.bitcast(t_ref[u, i], BF16), pltpu.bitcast(ws_ref[i, n], BF16))
            st[i] = p if i == 2 else p + st[2]
            if n < 4 and i < 2:
                qkv_ref[n, r, pl.ds((2 * tp + i) * LANES, LANES), :] = st[i]
            elif i == 1:
                vr_words[u] = pltpu.pack_elementwise([st[0], st[1]], packed_dtype=BF16)

        return [(64 if n == 4 else LANES, (u, n, i), functools.partial(one, i)) for i in (2, 0, 1)]

    def vr_store(u):
        r, tp = divmod(u, 2)
        w = pltpu.bitcast(vr_words[u], F32)
        wt = pltpu.bitcast(_cat([w, w]).T, U32)
        job_done["v", u] = pltpu.bitcast(wt[120:128], F32)
        for j in range(2):
            qkv_ref[4, r, pl.ds((2 * tp + j) * LANES, LANES), :] = pltpu.unpack_elementwise(
                wt, index=j, packed_dtype=BF16, unpacked_dtype=F32)

    zero8 = jnp.zeros((8, LANES), F32)

    def gather(n, off, k=0):
        return [qkv_ref[n, r, pl.ds(off + dyn0 * k if k else off, 8), :] for r in range(WS)]

    def softmax_t(st):
        rows = _blocks(st)
        m = functools.reduce(jnp.maximum, rows)
        m = _allred(jnp.where(mk["key"], m, -jnp.inf), jnp.maximum)
        p = [jnp.exp2(x - m) for x in rows]
        return p, functools.reduce(jnp.add, p)

    def s2_pair(pi, offa):
        offb = offa + WS
        st = {}

        def vprep():
            g = [gather(n, offa) + gather(n, offb) for n in range(5)]
            u1 = [jnp.where(mk["left64"], z, jnp.where(mk["v"], x, y)) for x, y, z in zip(g[0], g[1], g[4])]
            u2 = [jnp.where(mk["v"], x, y) for x, y in zip(g[2], g[3])]
            u = jnp.concatenate([_cat(u1 + [zero8, zero8]), _cat(u2 + [zero8, zero8])], axis=1)
            vt = pltpu.bitcast(u.astype(BF16).T, U32)
            vt = _cat([vt[0:64], vt[96:128]])
            st["vt"] = [pltpu.bitcast(vt[24 * h:24 * h + 24], BF16) for h in range(NH)]

        def score(i, ties=()):
            hp, sw = divmod(i, 2)
            lo, hi = mk["lo"], mk["hi%d" % hp]
            ma, mb = (lo, hi) if sw == 0 else (hi, lo)
            gq = (0, 1, 1 + sw)[_env("GQ", 0)]
            gk = (0, 1, 1 + sw)[_env("GK", 0)]
            q = _cat([jnp.where(ma, v, 0.0) for v in gather(hp, offa, gq)]
                     + [jnp.where(mb, v, 0.0) for v in gather(hp, offb, gq)] + [zero8, zero8])
            ka, kb = gather(2 + hp, offa, gk), gather(2 + hp, offb, gk)
            k = [jnp.where(lo, x, y) for x, y in (zip(ka, kb) if sw == 0 else zip(kb, ka))]
            for _, job in ties:
                k[0] = jnp.where(mk["never"], job(), k[0])
            k = _cat(k)
            st["p", i] = softmax_t(_dot_nt(k, q))

        def value(h):
            hp, sw = divmod(h, 2)
            (pa, sa), (pb, sb) = st["p", 2 * hp + sw], st["p", 2 * hp + 1 - sw]
            pm = _cat([jnp.where(mk["keep_a"], v, 0.0) for v in pa]
                      + [jnp.where(mk["keep_b"], v, 0.0) for v in pb] + [zero8, zero8])
            den = _allred(jnp.where(mk["keep_a"], sa, jnp.where(mk["keep_b"], sb, 0.0)), jnp.add)
            rec = pl.reciprocal(den, approx=True)
            if _env("NR", 0):
                rec = rec * (2.0 - den * rec)
            st["o", h] = [b * rec for b in _blocks(_dot(st["vt"][h], pm))]

        def finish():
            o = [b for h in range(NH) for b in st["o", h]]
            w = pltpu.pack_elementwise([_cat(o[0:16]), _cat(o[16:24] + o[16:24])], packed_dtype=BF16)
            stg_ref[pi] = pltpu.bitcast(w, F32)

        def scatter():
            wt = stg_ref[pi].T
            job_done["s", pi] = wt[104:112]
            for i, off in enumerate((offa, offb)):
                for r in range(WS):
                    base = i * SLOTS + 8 * r
                    ob_ref[pl.ds(r * WP + off, WS), :] = wt[base:base + WS]

        return vprep, score, value, finish, scatter

    npair = (nwin + 1) // 2
    pairs = [s2_pair(p, min(2 * p, nwin - 2) * WS) for p in range(npair)]

    def s3_unit(r, tp, ties=()):
        def unpack(t):
            w = pltpu.bitcast(ob_ref[pl.ds(r * WP + t * LANES, LANES), :], U32)
            return [_blocks(pltpu.unpack_elementwise(w, index=i, packed_dtype=BF16, unpacked_dtype=F32))
                    for i in range(2)]

        (la, ha), (lb, hb) = unpack(2 * tp), unpack(2 * tp + 1)
        t3 = [jnp.where(mk["left64"], x, y) for x, y in zip(lb, ha)]
        t1 = _cat([x - y for x, y in zip(la, t3)])
        t2 = _cat([jnp.where(mk["left64"], x, z) - y for x, y, z in zip(hb, ha, lb)])
        t3 = _cat(t3)
        wo = [_blocks(wos_ref[i]) for i in range(3)]
        for q, (e, job) in enumerate(ties):
            blks = wo[(2, 0, 1)[q % 3]]
            blks[e] = jnp.where(mk["never"], pltpu.bitcast(job(), U32), blks[e])
        wo = [pltpu.bitcast(_cat(w), BF16) for w in wo]
        p3 = _dot_nt(wo[2], t3)
        ys = [_dot_nt(wo[i], t) + p3
              + x0_ref[rows_at(prv, (r * NT + 2 * tp + i) * C, C), :] for i, t in enumerate((t1, t2))]
        n = min(2 * LANES, W - 2 * tp * LANES)
        o_ref[ooff + r, :, pl.ds(2 * tp * LANES, n)] = jnp.concatenate(ys, axis=1).astype(o_ref.dtype)[:, :n]

    s3_all = [functools.partial(s3_unit, r, tp) for tp in range(2) for r in range(WS)]

    def run(prog, extra):
        extra = sorted(extra, key=lambda e: e[0])
        j = 0
        for t0, fn in prog:
            while j < len(extra) and extra[j][0] <= t0:
                extra[j][1]()
                j += 1
            fn()
        for e in extra[j:]:
            e[1]()

    MERGE = _env("MERGE", 0)
    NX3 = _env("NX3", 0)

    NSY = 0

    NSTX = _env("NSTX", 24)

    def wave_steps(lo, hi, wave):
        steps = []
        for j0 in range(lo, hi, wave):
            for grp in zip(*[stats_steps(j) for j in range(j0, min(j0 + wave, hi))]):
                steps += grp
        return steps

    def block_x():
        NJ = _env("NJ", 28)
        NSTC = _env("NSTC", 7)
        WAVE = _env("WAVE", 4)
        VRLAG = _env("VRLAG", 150)
        chunks = [(u, n) for u in range(NU) for n in range(4)]
        MXS = _env("MXS", 0)
        steps = [] if MXS else wave_steps(0, NSTX, WAVE)
        loose = steps[len(steps) - _env("LOOSE", 0):]
        steps = steps[:len(steps) - len(loose)]
        nside = 9
        side, vstep = [], _env("VRSTEP", 0)
        for _ in range(_env("SIDE0", 1)):
            side += side_dots(*chunks.pop())
            nside -= 1
        for q in range(NU // 2):
            side += side_dots(2 * q, 4) + side_dots(2 * q + 1, 4)
            for _ in range(vstep):
                if nside:
                    side += side_dots(*chunks.pop())
                    nside -= 1
        for _ in range(nside):
            side += side_dots(*chunks.pop())
        mu = _env("MU", 2)
        merged = []
        for u, n in chunks:
            prev = [c for c in merged if c[1] == n and c[0][0] // mu == u // mu]
            if prev:
                prev[0][0].append(u)
            else:
                merged.append(([u], n))
        starts = [LANES * sum(len(c[0]) for c in merged[:k]) for k in range(len(merged))]
        t_conv = max(x for x in starts if x <= (len(chunks) - NSTC) * LANES)
        span = len(chunks) * LANES - t_conv
        plan, t, vr_ready = [], 0, {}
        for k, (us, n) in enumerate(merged):
            dur = LANES * len(us)
            lo, hi = (max(x - t_conv, 0) * len(steps) // span for x in (t, t + dur))
            plan.append((t, tuple(us), n, list(steps[lo:hi]), []))
            room = dur
            while side and (room > 0 or k == len(merged) - 1):
                rows, key, f = side.pop(0)
                plan.append((t, f if room > 0 else functools.partial(f, 4), None, [], []))
                room -= rows
                if key[1:] == (4, 1):
                    vr_ready[key[0]] = t + dur - room + VRLAG
            t += dur
        ci = conv_items(4 * NJ)
        slow = _env("SLOW", 32.0)
        fast = (t_conv - 4 * NJ * slow) / max(len(ci) - 4 * NJ, 1)
        t_piece = [min(j, 4 * NJ) * slow + max(j - 4 * NJ, 0) * fast for j in range(len(ci) + 1)]
        scat, vrs = list(range(npair - NSY)), list(range(NU))
        jobs = []
        for q in range(NJ):
            if vrs and vr_ready[vrs[0]] <= t_piece[4 * q + 1]:
                jobs.append((t_piece[4 * q + 1], ("v", vrs[0])))
                ci[4 * q].insert(0, functools.partial(vr_store, vrs.pop(0)))
            elif scat:
                jobs.append((t_piece[4 * q + 1], ("s", scat[0])))
                ci[4 * q].insert(0, pairs[scat.pop(0)][4])
        extra = [(t_piece[j + 1], f) for j, fs in enumerate(ci) for f in fs]
        tail = [(("v", u), functools.partial(vr_store, u)) for u in vrs] + [(("s", p), pairs[p][4]) for p in scat]
        for q, (key, f) in enumerate(tail):
            t_q = max(t_conv + 1 + (q // 3) * 128, vr_ready[key[1]] if key[0] == "v" else 0)
            extra.append((t_q, f))
            jobs.append((t_q, key))
        if _env("JDL", 800):
            for t_q, key in jobs:
                later = [e for e in plan if e[2] is not None and e[0] >= t_q + _env("JDL", 800)]
                if later:
                    later[0][3].insert(0, functools.partial(job_done.get, key))
        prog = [(t0, u if n is None else functools.partial(qkv_chunk, u, n, st, tn))
                for t0, u, n, st, tn in plan]
        run(prog, extra + [(t, f) for f in loose])

    def block_y():
        pattern = _env("PAT", "SFFVFFFF" + "SSSSFVVVV" * 8 + "SSSSVVVV").rstrip(".")
        load = [0] * 4
        items, ns, nv, nf = [], 0, 0, 0
        for ch in pattern:
            if ch in "Ss":
                todo = [("s", ns + i, [SLOTS]) for i in range(4 if ch == "S" else 2)]
                ns += len(todo)
            elif ch in "Vv":
                todo = [("v", nv + i, [DH]) for i in range(4 if ch == "V" else 2)]
                nv += len(todo)
            else:
                todo = [("f", nf, [C] * 3)]
                nf += 1
            for kind, idx, rows in todo:
                items.append((min(load), kind, idx, []))
                for x in rows:
                    load[load.index(min(load))] += x
        assert (ns, nv, nf) == (4 * npair, 4 * npair, NU)
        spots = sorted([(it[0], it, 0) for it in items if it[1] == "s"]
                       + [(it[0] + 16 * e, it, e) for it in items if it[1] == "f" for e in range(12)],
                       key=lambda x: x[0])
        ysteps = wave_steps(NSTX, WS * NT, _env("WAVEY", 4))
        fspots = [x for x in spots if x[1][1] == "f" and x[1][2] < _env("S3Q", 3)
                  and _env("E0", 1) <= x[2] < _env("E1", 12)]
        fspots.sort(key=lambda x: (x[1][2], x[2]))
        for q, step in enumerate(ysteps):
            _, it, e = fspots[q * len(fspots) // len(ysteps)]
            it[3].append((e, step))
        t_done.clear()
        extra = []
        tpos = [int(x) for x in _env("TPOS", "4,8").split(",")]
        late = [x for x in spots if x[1][1] == "s" and x[1][2] >= 4 and (x[1][2] - 4) % 16 in tpos]
        late.sort(key=lambda x: x[1][2])
        n1 = max(_env("NT1", 3), len(t_items) - len(late))
        ta0, ta1 = _env("TA0", 500), _env("TA1", 900)
        late = late[_env("TSKIP", 0):]
        for j, f in enumerate(t_items):
            if j < n1:
                t_s, it, e = [x for x in spots if x[0] >= ta0 + j * (ta1 - ta0) / n1][0]
            else:
                t_s, it, e = late[(j - n1) * len(late) // (len(t_items) - n1)]
            it[3].append((e, functools.partial(t_done.__getitem__, j)))
            extra.append((min(t_s - _env("TLEAD", 450), it[0]), f))
        prog = []
        for t0, kind, idx, ties in items:
            p, i = divmod(idx, 4)
            if kind == "s":
                if i == 0:
                    prog.append((t0, pairs[p][0]))
                prog.append((t0, functools.partial(pairs[p][1], i, ties)))
            elif kind == "v":
                prog.append((t0, functools.partial(pairs[p][2], i)))
                if i == 3:
                    extra.append((t0 + DH + _env("LFIN", 50), pairs[p][3]))
            else:
                prog.append((t0, functools.partial(s3_all[idx], ties)))
        run(prog, extra)

    only = _env("ONLY", "01")

    @when(k_ < nstrip, ("main",))
    def _():
        x_copy(k_).wait()

    @when(k_ < nstrip - 1, ("first", "main"))
    def _():
        x_copy(k_ + 1).start()

    new_masks("x")
    if "0" in only:
        when(k_ <= nstrip, ("main",))(block_x)

    @when(k_ == 0, ("first",))
    def _():
        def body(g, carry):
            x0_copy(g).wait()
            for j in range(FG):
                piece = conv_group(pl.multiple_of((g * FG + j) * 8, 8))[1]
                for r in range(WS):
                    piece(r)
            return carry
        lax.fori_loop(0, NG // FG, body, 0)

    @when(k_ >= 4, ("main", "last"))
    def _():
        o_copy(k_ - 4).wait()

    @when(k_ >= 3, ("main", "last"))
    def _():
        o_copy(k_ - 3).start()

    if "1" in only:
        new_masks("y")
        when((k_ <= nstrip) & (k_ >= 1), ("main",))(block_y)

    @when(k_ == 0, ("first",))
    def _():
        for j in range(WS * NT):
            for f in stats_steps(j):
                f()
        for f in t_items:
            f()

    @when(k_ == nstrip + 1, ("last",))
    def _():
        new_masks("y")
        for p in range(npair):
            pairs[p][4]()
        for q, f in enumerate(s3_all):
            f()
            if q >= WS:
                row_copy(q - WS).start()

    if only != "01":
        @when(dyn0 < 0, ("main",))
        def _():
            i = pl.multiple_of(k_ * 8, 8)
            o_ref[0, 0:16, 0:128] = _cat([
                qkv_ref[k3, k3, pl.ds(i, 8), :] + ms_ref[k3, 0:8, :] + stg_ref[k3, pl.ds(i, 8), :],
                pltpu.bitcast(t_ref[k3, k3, pl.ds(i, 8), :], F32) + ob_ref[pl.ds(i, 8), :]]).astype(BF16)
            for rf in (qkv_ref.at[k3, k3], stg_ref.at[k3], ob_ref):
                rf[pl.ds(i, 8), :] = zero8
            t_ref[k3, k3, pl.ds(i, 8), :] = pltpu.bitcast(zero8, U32)

    @when(k_ == nstrip + 1, ("last",))
    def _():
        o_copy(k_ - 3).wait()
        for r in range(WS):
            row_copy(r).wait()


@jax.jit
def pallas_standalone__window_attn_davit__vision_kernel(
    x: jax.Array,
    dw_pe: jax.Array,
    w_qkv: jax.Array,
    w_o: jax.Array,
):
    B, H, W, Cx = x.shape
    assert B == 1 and Cx == C and H % WS == 0 and W % WS == 0 and WP - LANES < W < WP
    xt = jnp.transpose(x[0], (0, 2, 1))

    assert H // WS + 2 <= 256
    vmem = pl.BlockSpec(memory_space=pltpu.VMEM)
    yt = pl.pallas_call(
        functools.partial(_kernel, H=H, W=W),
        in_specs=[pl.BlockSpec(memory_space=pl.ANY), vmem, vmem, vmem],
        out_specs=pl.BlockSpec(memory_space=pl.ANY),
        out_shape=jax.ShapeDtypeStruct((H, C, W), x.dtype),
        scratch_shapes=[
            pltpu.VMEM((2 * (WS + 2), C, W), x.dtype),
            pltpu.VMEM((2 * WS, C, W), x.dtype),
            pltpu.SemaphoreType.DMA((5,)),
            pltpu.VMEM((X0_ROWS, LANES), F32),
            pltpu.VMEM((WS * WP, LANES), F32),
            pltpu.VMEM((9, C, LANES), F32),
            pltpu.VMEM((3, 5, LANES // 2, LANES), U32),
            pltpu.VMEM((3, C // 2, LANES), U32),
            pltpu.VMEM((5, WS, WP, LANES), F32),
            pltpu.VMEM((NU, 3, LANES // 2, LANES), U32),
            pltpu.VMEM((37, LANES, LANES), F32),
            pltpu.VMEM((WS * NT, 16, LANES), F32),
            pltpu.VMEM((C, WP), F32),
        ],
        compiler_params=pltpu.CompilerParams(
            vmem_limit_bytes=64 * 1024 * 1024,
            disable_bounds_checks=bool(_env("NOBC", 1)),
        ),
        name="davit_window_attn",
    )(xt, dw_pe, w_qkv, w_o)
    return jnp.transpose(yt, (0, 2, 1))[None]
```

```python
import functools
import math
import os

import jax
import jax.numpy as jnp
from jax import lax
import jax.experimental.pallas as pl
import jax.experimental.pallas.tpu as pltpu

WS = 7
NH = 4
C = 192
DH = C // NH
NG = C // 8
LANES = 128
WP = 512
NT = WP // LANES
NU = WS * NT // 2
SLOTS = 8 * WS
EPS = 1e-5
F32 = jnp.float32
BF16 = jnp.bfloat16
U32 = jnp.uint32

X0_SLOT = WS * NT * C
DW_OFF = 3 * X0_SLOT
X0_ROWS = DW_OFF + 2 * C


def _dot(a, b):
    return jnp.dot(a, b, preferred_element_type=F32)


def _dot_nt(a, b):
    return lax.dot_general(a, b, (((1,), (1,)), ((), ())), preferred_element_type=F32)


def _cat(xs):
    return jnp.concatenate(xs, axis=0)


def _blocks(v):
    return [v[i:i + 8] for i in range(0, v.shape[0], 8)]


def _allred(x, op):
    for sh in (4, 2, 1):
        x = op(x, pltpu.roll(x, sh, 0))
    return x


def _env(name, default):
    return type(default)(os.environ.get(name, default))


def _kernel(x_hbm, dw_ref, wqkv_ref, wo_ref, o_hbm, *scratch, H, W):
    step = functools.partial(_step, x_hbm, dw_ref, wqkv_ref, wo_ref, o_hbm, *scratch, H=H, W=W)
    nstrip = H // WS

    def loop(lo, hi, mode):
        def body(k, carry):
            step(k_=k, mode=mode)
            return carry
        lax.fori_loop(lo, hi, body, 0)

    if "ONLY" not in os.environ:
        loop(0, 1, "first")
    loop(1 + _env("SKIP", 0), nstrip + 1, "main")
    if "ONLY" not in os.environ:
        loop(nstrip + 1, nstrip + 2, "last")


def _step(x_hbm, dw_ref, wqkv_ref, wo_ref, o_hbm,
          x_ref, o_ref, sems, x0_ref, ob_ref, dws_ref, ws_ref, wos_ref, qkv_ref, t_ref, stg_ref, ms_ref,
          top_ref, *, H, W, k_, mode):
    nstrip, nwin = H // WS, W // WS

    def x_copy(k):
        return pltpu.make_async_copy(x_hbm.at[pl.ds(jnp.minimum(k * WS, H - WS - 1), WS + 1)],
                                     x_ref.at[pl.ds((k & 1) * (WS + 2), WS + 1)], sems.at[0])

    def o_copy(k):
        return pltpu.make_async_copy(o_ref.at[pl.ds((k & 1) * WS, WS)], o_hbm.at[pl.ds(k * WS, WS)],
                                     sems.at[1])

    FG = 8

    def x0_copy(g):
        cs = pl.ds(pl.multiple_of(g * (8 * FG), 8 * FG), 8 * FG)
        return pltpu.make_async_copy(x_hbm.at[pl.ds(0, WS + 1), cs], x_ref.at[pl.ds(0, WS + 1), cs],
                                     sems.at[2 + g])

    def row_copy(r):
        return pltpu.make_async_copy(o_ref.at[sc["ooff"] + r], o_hbm.at[H - WS + r], sems.at[2])

    def when(cond, modes):
        if mode in modes:
            return pl.when(cond)
        return lambda f: None

    sc = {}

    def new_scalars():
        k3 = k_ - 3 * ((k_ * 171) >> 9)
        sc["nxt"] = k3 * X0_SLOT
        sc["prv"] = jnp.where((k3 == 2) | (k_ < 2), 0, sc["nxt"] + X0_SLOT)
        sc["xoff"] = (k_ & 1) * (WS + 2) + jnp.where(k_ >= nstrip - 1, 1, 0)
        sc["ooff"] = (k_ & 1) * WS

    dyn0 = jnp.minimum(k_, 0)

    def rows_at(base, off, n):
        if isinstance(base, int):
            return pl.ds(base + off, n)
        return pl.ds(pl.multiple_of(base + off, 8), n)

    mk = {}

    def new_masks(blk):
        lane = lax.broadcasted_iota(jnp.int32, (8, LANES), 1)
        mk.clear()
        mk["never"] = lane < dyn0
        if blk == "x":
            mk["up"] = lax.broadcasted_iota(jnp.int32, (8, LANES), 0) < 4
            return
        key_ok = lax.broadcasted_iota(jnp.int32, (8, LANES), 0) < WS
        mk.update(
            lo=lane < DH, hi0=(lane >= DH) & ((lane < 64) | (lane >= 96)), hi1=(lane >= DH) & (lane < 96),
            v=lane < 96, key=key_ok, keep_a=key_ok & (lane < SLOTS), keep_b=key_ok & (lane >= SLOTS),
            left64=lane < 64)

    def conv_group(c0):
        st = {}

        def row(i):
            if i == 0 and i not in st:
                st[i] = top_ref[pl.ds(c0, 8), :]
            if i not in st:
                v = x_ref[sc["xoff"] + (i - 1), pl.ds(c0, 8), :].astype(F32)
                st[i] = jnp.concatenate([v, jnp.zeros((8, WP - W), F32)], axis=1)
                if i == WS and i - 2 in st:
                    top_ref[pl.ds(c0, 8), :] = st[i]
            return st[i]

        def bc(v):
            return jnp.concatenate([v] * NT, axis=1)

        def taps(r):
            st["tw", r] = [bc(x0_ref[rows_at(c0, DW_OFF + k * C, 8), :]) for k in range(2)]

        def piece(r):
            if "w" not in st:
                st["w"] = [bc(dws_ref[k, pl.ds(c0, 8), :]) for k in range(9)]
            wts = list(st["w"])
            if ("tw", r) in st:
                wts[6], wts[8] = st["tw", r]
            row(r)
            abc = [row(r + 1) * wts[3 + j] + row(r) * wts[j] + row(r + 2) * wts[6 + j] for j in range(3)]
            x0 = pltpu.roll(abc[0], 1, 1) + abc[1] + pltpu.roll(abc[2], WP - 1, 1)
            for t in range(NT):
                x0_ref[rows_at(sc["nxt"], (r * NT + t) * C + c0, 8), :] = x0[:, t * LANES:(t + 1) * LANES]

        return taps, piece

    @when(k_ == 0, ("first",))
    def _():
        for g in range(NG // FG):
            x0_copy(g).start()
        for k in range(9):
            w = dw_ref[k // 3].astype(F32)[k % 3:k % 3 + 1, :]
            w = jnp.broadcast_to(w, (LANES, C)).T
            dws_ref[k] = w + 1.0 if k == 4 else w
            if k in (6, 8):
                x0_ref[pl.ds(DW_OFF + (k - 6) // 2 * C, C), :] = w
        w = wqkv_ref[...].astype(F32)
        wq = w[:, 0:C] * ((DH ** -0.5) * math.log2(math.e))
        wk, wv = w[:, C:2 * C], w[:, 2 * C:3 * C]
        tiles = [(wq[:, 0:64], wv[:, 64:96], wq[:, 64:96]),
                 (wq[:, 96:192], wv[:, 96:128]),
                 (wk[:, 0:64], wv[:, 128:160], wk[:, 64:96]),
                 (wk[:, 96:192], wv[:, 160:192]),
                 (wv[:, 0:128],)]
        for n, parts in enumerate(tiles):
            w = jnp.concatenate(parts, axis=1)
            for i, wi in enumerate((w[0:128], w[64:192], _cat([w[0:64], w[128:192]]))):
                if n == 4:
                    wi = wi.T
                ws_ref[i, n] = pltpu.bitcast(wi.astype(BF16), U32)
        w = wo_ref[...].astype(F32)
        wx, wy, wz = w[0:64], w[64:128], w[128:192]
        for i, parts in enumerate(((wx, wy), (wz, wy), (wx, wy + wz))):
            wos_ref[i] = pltpu.bitcast(_cat(parts).T.astype(BF16), U32)

        top_ref[...] = jnp.zeros(top_ref.shape, F32)
        for i in (WS + 1, 2 * WS + 3):
            x_ref[i] = jnp.zeros(x_ref.shape[1:], x_ref.dtype)

        for p in range(stg_ref.shape[0]):
            stg_ref[p] = jnp.zeros(stg_ref.shape[1:], F32)
        for r in range(WS):
            ob_ref[pl.ds(r * WP + WP - 8, 8), :] = jnp.zeros((8, LANES), F32)

    cuts = [int(c) for c in _env("CUTS", "0,7").split(",")]
    bands = list(zip(cuts, cuts[1:]))
    groups = {(b, g): conv_group(8 * g) for b in range(len(bands)) for g in range(NG)}
    WLEAD = _env("WLEAD", 4)

    def conv_items(nslow):
        plist = [((b, g), r) for b, (r0, r1) in enumerate(bands) for g in range(NG) for r in range(r0, r1)]
        items, nxt_tap = [], WLEAD
        for k, (g, r) in enumerate(plist):
            fs = []
            lead = WLEAD if k < nslow else _env("WLEAD2", 5)
            while nxt_tap <= min(k + lead, len(plist) - 1):
                g2, r2 = plist[nxt_tap]
                fs.append(functools.partial(groups[g2][0], r2))
                nxt_tap += 1
            fs.append(functools.partial(groups[g][1], r))
            items.append(fs)
        return items

    def ld_x0(j, k, gs=range(NG)):
        return [x0_ref[rows_at(sc["nxt"] + dyn0 * (8 * k), j * C + 8 * g, 8), :] for g in gs]

    def add2(acc, xs):
        a = functools.reduce(jnp.add, xs[0::2])
        b = functools.reduce(jnp.add, xs[1::2])
        return a + b if acc is None else (acc + a) + b

    stats_done = set()

    def stats_steps(j):
        st = {"s": None, "q": None}
        n1, n2 = _env("SEG1", 12), _env("SEG2", 6)

        def sum_step(g0):
            st["s"] = add2(st["s"], ld_x0(j, 0, range(g0, g0 + n1)))
            if g0 + n1 == NG:
                st["s"] = _allred(st["s"], jnp.add) * (1.0 / C)
            return st["s"]

        def var_step(g0):
            d = [x - st["s"] for x in ld_x0(j, 1, range(g0, g0 + n2))]
            st["q"] = add2(st["q"], [x * x for x in d])
            return st["q"]

        def last_step():
            v = _allred(st["q"], jnp.add) * (1.0 / C) + EPS
            rs = lax.rsqrt(v) if _env("RSQ", 1) else jnp.exp2(jnp.log2(v) * -0.5)
            ms_ref[j] = _cat([st["s"], rs])
            stats_done.add(j)
            return rs

        return ([functools.partial(sum_step, g) for g in range(0, NG, n1)]
                + [functools.partial(var_step, g) for g in range(0, NG, n2)] + [last_step])

    def colsum(xs):
        xs = [a + b for a, b in zip(xs[0:8], xs[16:24])] + xs[8:16]
        return _dot(jnp.ones((8, LANES), F32), _cat(xs))

    means = {}

    def mean_dot(j):
        means[j] = colsum(ld_x0(j, 0)) * (1.0 / C)

    def var_dot(j):
        xs = [x0_ref[pl.ds(sc["nxt"] + (j * C + 8 * g + 4), 8), :] for g in range(NG - 1)]
        xs.append(jnp.where(mk["up"], *ld_x0(j, 0, (0, NG - 1))))
        d = [x - means[j] for x in xs]
        v = colsum([x * x for x in d]) * (1.0 / C) + EPS
        rs = lax.rsqrt(v) if _env("RSQ", 1) else jnp.exp2(jnp.log2(v) * -0.5)
        ms_ref[j] = _cat([means[j], rs])
        stats_done.add(j)

    def normed(j, blk, k):
        assert j in stats_done or "ONLY" in os.environ and j < NSTX, j
        m, rs = ms_ref[j, 0:8, :], ms_ref[j, 8:16, :]
        return _cat([(x - m) * rs for x in ld_x0(j, k, range(8 * blk, 8 * blk + 8))])

    t_done = {}

    def put_t(dst, tiles):
        tt = pltpu.bitcast(jnp.concatenate(tiles, axis=1).astype(BF16).T, U32)
        for i, (u, e) in enumerate(dst):
            t_ref[u, e] = tt[64 * i:64 * i + 64]
        t_done[len(t_done)] = pltpu.bitcast(tt[120:128], F32)

    def t_first(u):
        ja, jb = 2 * u, 2 * u + 1
        bx = normed(jb, 0, 0)
        put_t([(u, 0), (u, 2)], [_cat([normed(ja, 0, 0) - bx, normed(ja, 1, 0)]),
                                 _cat([bx, normed(ja, 2, 0)])])

    def t_second(r):
        put_t([(u, 1) for u in (2 * r, 2 * r + 1)],
              [_cat([normed(2 * u + 1, 1, 0), normed(2 * u + 1, 2, 0) - normed(2 * u, 2, _env("RECOMP", 0))])
               for u in (2 * r, 2 * r + 1)])

    t_items = []
    for r in range(WS):
        t_items += [functools.partial(t_first, 2 * r), functools.partial(t_first, 2 * r + 1),
                    functools.partial(t_second, r)]

    def qkv_chunk(us, n, steps=(), tiny=()):
        lhs = {i: [b for u in us for b in _blocks(t_ref[u, i])] for i in range(3)}
        for q, step in enumerate(steps):
            tok = pltpu.bitcast(step(), U32)
            q = q * 24 * len(us) // len(steps)
            blks = lhs[(2, 0, 1)[q % 3]]
            blks[q // 3] = jnp.where(mk["never"], tok, blks[q // 3])
        p3 = None
        for i in (2, 0, 1):
            p = _dot(pltpu.bitcast(_cat(lhs[i]), BF16), pltpu.bitcast(ws_ref[i, n], BF16))
            if p3 is None:
                p3 = p
            else:
                p = p + p3
                for e, u in enumerate(us):
                    r, tp = divmod(u, 2)
                    qkv_ref[n, r, pl.ds((2 * tp + i) * LANES, LANES), :] = p[e * LANES:(e + 1) * LANES]

    vr_words = {}
    job_done = {}

    def side_dots(u, n):
        r, tp = divmod(u, 2)
        st = {}

        def one(i, parts=1):
            if parts > 1:
                lhs, rows = t_ref[u, i], 64 // parts
                p = _cat([_dot(pltpu.bitcast(lhs[q * rows:(q + 1) * rows], BF16),
                               pltpu.bitcast(ws_ref[i, n], BF16)) for q in range(parts)])
            elif n == 4:
                p = _dot_nt(pltpu.bitcast(ws_ref[i, 4, 0:32, :], BF16), pltpu.bitcast(t_ref[u, i], BF16))
            else:
                p = _dot(pltpu.bitcast(t_ref[u, i], BF16), pltpu.bitcast(ws_ref[i, n], BF16))
            st[i] = p if i == 2 else p + st[2]
            if n < 4 and i < 2:
                qkv_ref[n, r, pl.ds((2 * tp + i) * LANES, LANES), :] = st[i]
            elif i == 1:
                vr_words[u] = pltpu.pack_elementwise([st[0], st[1]], packed_dtype=BF16)

        return [(64 if n == 4 else LANES, (u, n, i), functools.partial(one, i)) for i in (2, 0, 1)]

    def vr_store(u):
        r, tp = divmod(u, 2)
        w = pltpu.bitcast(vr_words[u], F32)
        wt = pltpu.bitcast(_cat([w, w]).T, U32)
        job_done["v", u] = pltpu.bitcast(wt[120:128], F32)
        for j in range(2):
            qkv_ref[4, r, pl.ds((2 * tp + j) * LANES, LANES), :] = pltpu.unpack_elementwise(
                wt, index=j, packed_dtype=BF16, unpacked_dtype=F32)

    zero8 = jnp.zeros((8, LANES), F32)

    def gather(n, off, k=0):
        return [qkv_ref[n, r, pl.ds(off + dyn0 * k if k else off, 8), :] for r in range(WS)]

    def softmax_t(st):
        rows = _blocks(st)
        m = functools.reduce(jnp.maximum, rows)
        m = _allred(jnp.where(mk["key"], m, -jnp.inf), jnp.maximum)
        p = [jnp.exp2(x - m) for x in rows]
        return p, functools.reduce(jnp.add, p)

    def s2_pair(pi, offa):
        offb = offa + WS
        st = {}

        def vprep():
            g = [gather(n, offa) + gather(n, offb) for n in range(5)]
            u1 = [jnp.where(mk["left64"], z, jnp.where(mk["v"], x, y)) for x, y, z in zip(g[0], g[1], g[4])]
            u2 = [jnp.where(mk["v"], x, y) for x, y in zip(g[2], g[3])]
            u = jnp.concatenate([_cat(u1 + [zero8, zero8]), _cat(u2 + [zero8, zero8])], axis=1)
            vt = pltpu.bitcast(u.astype(BF16).T, U32)
            vt = _cat([vt[0:64], vt[96:128]])
            st["vt"] = [pltpu.bitcast(vt[24 * h:24 * h + 24], BF16) for h in range(NH)]

        def score(i, ties=()):
            hp, sw = divmod(i, 2)
            lo, hi = mk["lo"], mk["hi%d" % hp]
            ma, mb = (lo, hi) if sw == 0 else (hi, lo)
            gq = (0, 1, 1 + sw)[_env("GQ", 0)]
            gk = (0, 1, 1 + sw)[_env("GK", 0)]
            q = _cat([jnp.where(ma, v, 0.0) for v in gather(hp, offa, gq)]
                     + [jnp.where(mb, v, 0.0) for v in gather(hp, offb, gq)] + [zero8, zero8])
            ka, kb = gather(2 + hp, offa, gk), gather(2 + hp, offb, gk)
            k = [jnp.where(lo, x, y) for x, y in (zip(ka, kb) if sw == 0 else zip(kb, ka))]
            for _, job in ties:
                k[0] = jnp.where(mk["never"], job(), k[0])
            k = _cat(k)
            st["p", i] = softmax_t(_dot_nt(k, q))

        def value(h):
            hp, sw = divmod(h, 2)
            (pa, sa), (pb, sb) = st["p", 2 * hp + sw], st["p", 2 * hp + 1 - sw]
            pm = _cat([jnp.where(mk["keep_a"], v, 0.0) for v in pa]
                      + [jnp.where(mk["keep_b"], v, 0.0) for v in pb] + [zero8, zero8])
            den = _allred(jnp.where(mk["keep_a"], sa, jnp.where(mk["keep_b"], sb, 0.0)), jnp.add)
            rec = pl.reciprocal(den, approx=True)
            if _env("NR", 0):
                rec = rec * (2.0 - den * rec)
            st["o", h] = [b * rec for b in _blocks(_dot(st["vt"][h], pm))]

        def finish():
            o = [b for h in range(NH) for b in st["o", h]]
            w = pltpu.pack_elementwise([_cat(o[0:16]), _cat(o[16:24] + o[16:24])], packed_dtype=BF16)
            stg_ref[pi] = pltpu.bitcast(w, F32)

        def scatter():
            wt = stg_ref[pi].T
            job_done["s", pi] = wt[104:112]
            for i, off in enumerate((offa, offb)):
                for r in range(WS):
                    base = i * SLOTS + 8 * r
                    ob_ref[pl.ds(r * WP + off, WS), :] = wt[base:base + WS]

        return vprep, score, value, finish, scatter

    npair = (nwin + 1) // 2
    pairs = [s2_pair(p, min(2 * p, nwin - 2) * WS) for p in range(npair)]

    def s3_unit(r, tp, ties=()):
        def unpack(t):
            w = pltpu.bitcast(ob_ref[pl.ds(r * WP + t * LANES, LANES), :], U32)
            return [_blocks(pltpu.unpack_elementwise(w, index=i, packed_dtype=BF16, unpacked_dtype=F32))
                    for i in range(2)]

        (la, ha), (lb, hb) = unpack(2 * tp), unpack(2 * tp + 1)
        t3 = [jnp.where(mk["left64"], x, y) for x, y in zip(lb, ha)]
        t1 = _cat([x - y for x, y in zip(la, t3)])
        t2 = _cat([jnp.where(mk["left64"], x, z) - y for x, y, z in zip(hb, ha, lb)])
        t3 = _cat(t3)
        wo = [_blocks(wos_ref[i]) for i in range(3)]
        for q, (e, job) in enumerate(ties):
            blks = wo[(2, 0, 1)[q % 3]]
            blks[e] = jnp.where(mk["never"], pltpu.bitcast(job(), U32), blks[e])
        wo = [pltpu.bitcast(_cat(w), BF16) for w in wo]
        p3 = _dot_nt(wo[2], t3)
        ys = [_dot_nt(wo[i], t) + p3
              + x0_ref[rows_at(sc["prv"], (r * NT + 2 * tp + i) * C, C), :] for i, t in enumerate((t1, t2))]
        n = min(2 * LANES, W - 2 * tp * LANES)
        o_ref[sc["ooff"] + r, :, pl.ds(2 * tp * LANES, n)] = jnp.concatenate(ys, axis=1).astype(o_ref.dtype)[:, :n]

    s3_all = [functools.partial(s3_unit, r, tp) for tp in range(2) for r in range(WS)]

    def run(prog, extra):
        extra = sorted(extra, key=lambda e: e[0])
        j = 0
        for t0, fn in prog:
            while j < len(extra) and extra[j][0] <= t0:
                extra[j][1]()
                j += 1
            fn()
        for e in extra[j:]:
            e[1]()

    MERGE = _env("MERGE", 0)
    NX3 = _env("NX3", 0)

    NSY = 0

    NSTX = _env("NSTX", 24)

    def wave_steps(lo, hi, wave):
        steps = []
        for j0 in range(lo, hi, wave):
            for grp in zip(*[stats_steps(j) for j in range(j0, min(j0 + wave, hi))]):
                steps += grp
        return steps

    def block_x():
        new_scalars()
        NJ = _env("NJ", 28)
        NSTC = _env("NSTC", 7)
        WAVE = _env("WAVE", 4)
        VRLAG = _env("VRLAG", 150)
        chunks = [(u, n) for u in range(NU) for n in range(4)]
        MXS = _env("MXS", 0)
        steps = [] if MXS else wave_steps(0, NSTX, WAVE)
        loose = steps[len(steps) - _env("LOOSE", 0):]
        steps = steps[:len(steps) - len(loose)]
        nside = 9
        side, vstep = [], _env("VRSTEP", 0)
        for _ in range(_env("SIDE0", 1)):
            side += side_dots(*chunks.pop())
            nside -= 1
        for q in range(NU // 2):
            side += side_dots(2 * q, 4) + side_dots(2 * q + 1, 4)
            for _ in range(vstep):
                if nside:
                    side += side_dots(*chunks.pop())
                    nside -= 1
        for _ in range(nside):
            side += side_dots(*chunks.pop())
        mu = _env("MU", 2)
        merged = []
        for u, n in chunks:
            prev = [c for c in merged if c[1] == n and c[0][0] // mu == u // mu]
            if prev:
                prev[0][0].append(u)
            else:
                merged.append(([u], n))
        starts = [LANES * sum(len(c[0]) for c in merged[:k]) for k in range(len(merged))]
        t_conv = max(x for x in starts if x <= (len(chunks) - NSTC) * LANES)
        span = len(chunks) * LANES - t_conv
        plan, t, vr_ready = [], 0, {}
        for k, (us, n) in enumerate(merged):
            dur = LANES * len(us)
            lo, hi = (max(x - t_conv, 0) * len(steps) // span for x in (t, t + dur))
            plan.append((t, tuple(us), n, list(steps[lo:hi]), []))
            room = dur
            while side and (room > 0 or k == len(merged) - 1):
                rows, key, f = side.pop(0)
                plan.append((t, f if room > 0 else functools.partial(f, 4), None, [], []))
                room -= rows
                if key[1:] == (4, 1):
                    vr_ready[key[0]] = t + dur - room + VRLAG
            t += dur
        ci = conv_items(4 * NJ)
        slow = _env("SLOW", 32.0)
        fast = (t_conv - 4 * NJ * slow) / max(len(ci) - 4 * NJ, 1)
        t_piece = [min(j, 4 * NJ) * slow + max(j - 4 * NJ, 0) * fast for j in range(len(ci) + 1)]
        scat, vrs = list(range(npair - NSY)), list(range(NU))
        jobs = []
        for q in range(NJ):
            if vrs and vr_ready[vrs[0]] <= t_piece[4 * q + 1]:
                jobs.append((t_piece[4 * q + 1], ("v", vrs[0])))
                ci[4 * q].insert(0, functools.partial(vr_store, vrs.pop(0)))
            elif scat:
                jobs.append((t_piece[4 * q + 1], ("s", scat[0])))
                ci[4 * q].insert(0, pairs[scat.pop(0)][4])
        extra = [(t_piece[j + 1], f) for j, fs in enumerate(ci) for f in fs]
        tail = [(("v", u), functools.partial(vr_store, u)) for u in vrs] + [(("s", p), pairs[p][4]) for p in scat]
        for q, (key, f) in enumerate(tail):
            t_q = max(t_conv + 1 + (q // 3) * 128, vr_ready[key[1]] if key[0] == "v" else 0)
            extra.append((t_q, f))
            jobs.append((t_q, key))
        if _env("JDL", 800):
            for t_q, key in jobs:
                later = [e for e in plan if e[2] is not None and e[0] >= t_q + _env("JDL", 800)]
                if later:
                    later[0][3].insert(0, functools.partial(job_done.get, key))
        prog = [(t0, u if n is None else functools.partial(qkv_chunk, u, n, st, tn))
                for t0, u, n, st, tn in plan]
        run(prog, extra + [(t, f) for f in loose])

    def block_y():
        new_scalars()
        pattern = _env("PAT", "SFFVFFFF" + "SSSSFVVVV" * 8 + "SSSSVVVV").rstrip(".")
        load = [0] * 4
        items, ns, nv, nf = [], 0, 0, 0
        for ch in pattern:
            if ch in "Ss":
                todo = [("s", ns + i, [SLOTS]) for i in range(4 if ch == "S" else 2)]
                ns += len(todo)
            elif ch in "Vv":
                todo = [("v", nv + i, [DH]) for i in range(4 if ch == "V" else 2)]
                nv += len(todo)
            else:
                todo = [("f", nf, [C] * 3)]
                nf += 1
            for kind, idx, rows in todo:
                items.append((min(load), kind, idx, []))
                for x in rows:
                    load[load.index(min(load))] += x
        assert (ns, nv, nf) == (4 * npair, 4 * npair, NU)
        spots = sorted([(it[0], it, 0) for it in items if it[1] == "s"]
                       + [(it[0] + 16 * e, it, e) for it in items if it[1] == "f" for e in range(12)],
                       key=lambda x: x[0])
        ysteps = wave_steps(NSTX, WS * NT, _env("WAVEY", 4))
        fspots = [x for x in spots if x[1][1] == "f" and x[1][2] < _env("S3Q", 3)
                  and _env("E0", 1) <= x[2] < _env("E1", 12)]
        fspots.sort(key=lambda x: (x[1][2], x[2]))
        for q, step in enumerate(ysteps):
            _, it, e = fspots[q * len(fspots) // len(ysteps)]
            it[3].append((e, step))
        t_done.clear()
        extra = []
        tpos = [int(x) for x in _env("TPOS", "4,8").split(",")]
        late = [x for x in spots if x[1][1] == "s" and x[1][2] >= _env("TOFS", 4) and (x[1][2] - _env("TOFS", 4)) % _env("TRUN", 16) in tpos]
        late.sort(key=lambda x: x[1][2])
        n1 = max(_env("NT1", 3), len(t_items) - len(late))
        ta0, ta1 = _env("TA0", 500), _env("TA1", 900)
        late = late[_env("TSKIP", 0):]
        for j, f in enumerate(t_items):
            if j < n1:
                t_s, it, e = [x for x in spots if x[0] >= ta0 + j * (ta1 - ta0) / n1][0]
            else:
                t_s, it, e = late[(j - n1) * len(late) // (len(t_items) - n1)]
            it[3].append((e, functools.partial(t_done.__getitem__, j)))
            extra.append((min(t_s - _env("TLEAD", 450), it[0]), f))
        prog = []
        for t0, kind, idx, ties in items:
            p, i = divmod(idx, 4)
            if kind == "s":
                if i == 0:
                    prog.append((t0, pairs[p][0]))
                prog.append((t0, functools.partial(pairs[p][1], i, ties)))
            elif kind == "v":
                prog.append((t0, functools.partial(pairs[p][2], i)))
                if i == 3:
                    extra.append((t0 + DH + _env("LFIN", 50), pairs[p][3]))
            else:
                prog.append((t0, functools.partial(s3_all[idx], ties)))
        run(prog, extra)

    only = _env("ONLY", "01")
    if mode != "main":
        new_scalars()

    @when(k_ < nstrip, ("main",))
    def _():
        x_copy(k_).wait()

    @when(k_ < nstrip - 1, ("first", "main"))
    def _():
        x_copy(k_ + 1).start()

    new_masks("x")
    if "0" in only:
        when(k_ <= nstrip, ("main",))(block_x)

    @when(k_ == 0, ("first",))
    def _():
        def body(g, carry):
            x0_copy(g).wait()
            for j in range(FG):
                piece = conv_group(pl.multiple_of((g * FG + j) * 8, 8))[1]
                for r in range(WS):
                    piece(r)
            return carry
        lax.fori_loop(0, NG // FG, body, 0)

    @when(k_ >= 4, ("main", "last"))
    def _():
        o_copy(k_ - 4).wait()

    @when(k_ >= 3, ("main", "last"))
    def _():
        o_copy(k_ - 3).start()

    if "1" in only:
        new_masks("y")
        when((k_ <= nstrip) & (k_ >= 1), ("main",))(block_y)

    @when(k_ == 0, ("first",))
    def _():
        for j in range(WS * NT):
            for f in stats_steps(j):
                f()
        for f in t_items:
            f()

    @when(k_ == nstrip + 1, ("last",))
    def _():
        new_masks("y")
        for p in range(npair):
            pairs[p][4]()
        for q, f in enumerate(s3_all):
            f()
            if q >= WS:
                row_copy(q - WS).start()

    if only != "01":
        @when(dyn0 < 0, ("main",))
        def _():
            i = pl.multiple_of(k_ * 8, 8)
            k3 = k_ & 1
            o_ref[0, 0:16, 0:128] = _cat([
                qkv_ref[k3, k3, pl.ds(i, 8), :] + ms_ref[k3, 0:8, :] + stg_ref[k3, pl.ds(i, 8), :],
                pltpu.bitcast(t_ref[k3, k3, pl.ds(i, 8), :], F32) + ob_ref[pl.ds(i, 8), :]]).astype(BF16)
            for rf in (qkv_ref.at[k3, k3], stg_ref.at[k3], ob_ref):
                rf[pl.ds(i, 8), :] = zero8
            t_ref[k3, k3, pl.ds(i, 8), :] = pltpu.bitcast(zero8, U32)

    @when(k_ == nstrip + 1, ("last",))
    def _():
        o_copy(k_ - 3).wait()
        for r in range(WS):
            row_copy(r).wait()


@jax.jit
def pallas_standalone__window_attn_davit__vision_kernel(
    x: jax.Array,
    dw_pe: jax.Array,
    w_qkv: jax.Array,
    w_o: jax.Array,
):
    B, H, W, Cx = x.shape
    assert B == 1 and Cx == C and H % WS == 0 and W % WS == 0 and WP - LANES < W < WP
    xt = jnp.transpose(x[0], (0, 2, 1))

    assert H // WS + 2 <= 256
    vmem = pl.BlockSpec(memory_space=pltpu.VMEM)
    yt = pl.pallas_call(
        functools.partial(_kernel, H=H, W=W),
        in_specs=[pl.BlockSpec(memory_space=pl.ANY), vmem, vmem, vmem],
        out_specs=pl.BlockSpec(memory_space=pl.ANY),
        out_shape=jax.ShapeDtypeStruct((H, C, W), x.dtype),
        scratch_shapes=[
            pltpu.VMEM((2 * (WS + 2), C, W), x.dtype),
            pltpu.VMEM((2 * WS, C, W), x.dtype),
            pltpu.SemaphoreType.DMA((5,)),
            pltpu.VMEM((X0_ROWS, LANES), F32),
            pltpu.VMEM((WS * WP, LANES), F32),
            pltpu.VMEM((9, C, LANES), F32),
            pltpu.VMEM((3, 5, LANES // 2, LANES), U32),
            pltpu.VMEM((3, C // 2, LANES), U32),
            pltpu.VMEM((5, WS, WP, LANES), F32),
            pltpu.VMEM((NU, 3, LANES // 2, LANES), U32),
            pltpu.VMEM((37, LANES, LANES), F32),
            pltpu.VMEM((WS * NT, 16, LANES), F32),
            pltpu.VMEM((C, WP), F32),
        ],
        compiler_params=pltpu.CompilerParams(
            vmem_limit_bytes=64 * 1024 * 1024,
            disable_bounds_checks=bool(_env("NOBC", 1)),
        ),
        name="davit_window_attn",
    )(xt, dw_pe, w_qkv, w_o)
    return jnp.transpose(yt, (0, 2, 1))[None]
```

```python
import functools
import math
import os

import jax
import jax.numpy as jnp
from jax import lax
import jax.experimental.pallas as pl
import jax.experimental.pallas.tpu as pltpu

WS = 7
NH = 4
C = 192
DH = C // NH
NG = C // 8
LANES = 128
WP = 512
NT = WP // LANES
NU = WS * NT // 2
SLOTS = 8 * WS
EPS = 1e-5
F32 = jnp.float32
BF16 = jnp.bfloat16
U32 = jnp.uint32

X0_SLOT = WS * NT * C
DW_OFF = 3 * X0_SLOT
X0_ROWS = DW_OFF + 2 * C


def _dot(a, b):
    return jnp.dot(a, b, preferred_element_type=F32)


def _dot_nt(a, b):
    return lax.dot_general(a, b, (((1,), (1,)), ((), ())), preferred_element_type=F32)


def _cat(xs):
    return jnp.concatenate(xs, axis=0)


def _blocks(v):
    return [v[i:i + 8] for i in range(0, v.shape[0], 8)]


def _allred(x, op):
    for sh in (4, 2, 1):
        x = op(x, pltpu.roll(x, sh, 0))
    return x


def _env(name, default):
    return type(default)(os.environ.get(name, default))


def _kernel(x_hbm, dw_ref, wqkv_ref, wo_ref, o_hbm, *scratch, H, W):
    step = functools.partial(_step, x_hbm, dw_ref, wqkv_ref, wo_ref, o_hbm, *scratch, H=H, W=W)
    nstrip = H // WS

    def loop(lo, hi, mode):
        def body(k, carry):
            step(k_=k, mode=mode)
            return carry
        lax.fori_loop(lo, hi, body, 0)

    if "ONLY" not in os.environ:
        loop(0, 1, "first")
    loop(1 + _env("SKIP", 0), nstrip + 1, "main")
    if "ONLY" not in os.environ:
        loop(nstrip + 1, nstrip + 2, "last")


def _step(x_hbm, dw_ref, wqkv_ref, wo_ref, o_hbm,
          x_ref, o_ref, sems, x0_ref, ob_ref, dws_ref, ws_ref, wos_ref, qkv_ref, t_ref, stg_ref, ms_ref,
          top_ref, *, H, W, k_, mode):
    nstrip, nwin = H // WS, W // WS

    def x_copy(k):
        return pltpu.make_async_copy(x_hbm.at[pl.ds(jnp.minimum(k * WS, H - WS - 1), WS + 1)],
                                     x_ref.at[pl.ds((k & 1) * (WS + 2), WS + 1)], sems.at[0])

    def o_copy(k):
        return pltpu.make_async_copy(o_ref.at[pl.ds((k & 1) * WS, WS)], o_hbm.at[pl.ds(k * WS, WS)],
                                     sems.at[1])

    FG = 8

    def x0_copy(g):
        cs = pl.ds(pl.multiple_of(g * (8 * FG), 8 * FG), 8 * FG)
        return pltpu.make_async_copy(x_hbm.at[pl.ds(0, WS + 1), cs], x_ref.at[pl.ds(0, WS + 1), cs],
                                     sems.at[2 + g])

    def row_copy(r):
        return pltpu.make_async_copy(o_ref.at[sc["ooff"] + r], o_hbm.at[H - WS + r], sems.at[2])

    def when(cond, modes):
        if mode in modes:
            return pl.when(cond)
        return lambda f: None

    sc = {}

    def new_scalars():
        k3 = k_ - 3 * ((k_ * 171) >> 9)
        sc["nxt"] = k3 * X0_SLOT
        sc["prv"] = jnp.where((k3 == 2) | (k_ < 2), 0, sc["nxt"] + X0_SLOT)
        sc["xoff"] = (k_ & 1) * (WS + 2) + jnp.where(k_ >= nstrip - 1, 1, 0)
        sc["ooff"] = (k_ & 1) * WS

    dyn0 = jnp.minimum(k_, 0)

    def rows_at(base, off, n):
        if isinstance(base, int):
            return pl.ds(base + off, n)
        return pl.ds(pl.multiple_of(base + off, 8), n)

    mk = {}

    def new_masks(blk):
        lane = lax.broadcasted_iota(jnp.int32, (8, LANES), 1)
        mk.clear()
        mk["never"] = lane < dyn0
        if blk == "x":
            mk["up"] = lax.broadcasted_iota(jnp.int32, (8, LANES), 0) < 4
            return
        key_ok = lax.broadcasted_iota(jnp.int32, (8, LANES), 0) < WS
        mk.update(
            lo=lane < DH, hi0=(lane >= DH) & ((lane < 64) | (lane >= 96)), hi1=(lane >= DH) & (lane < 96),
            v=lane < 96, key=key_ok, keep_a=key_ok & (lane < SLOTS), keep_b=key_ok & (lane >= SLOTS),
            left64=lane < 64)

    def conv_group(c0):
        st = {}

        def row(i):
            if i == 0 and i not in st:
                st[i] = top_ref[pl.ds(c0, 8), :]
            if i not in st:
                v = x_ref[sc["xoff"] + (i - 1), pl.ds(c0, 8), :].astype(F32)
                st[i] = jnp.concatenate([v, jnp.zeros((8, WP - W), F32)], axis=1)
                if i == WS and i - 2 in st:
                    top_ref[pl.ds(c0, 8), :] = st[i]
            return st[i]

        def bc(v):
            return jnp.concatenate([v] * NT, axis=1)

        def taps(r):
            st["tw", r] = [bc(x0_ref[rows_at(c0, DW_OFF + k * C, 8), :]) for k in range(2)]

        def piece(r):
            if "w" not in st:
                st["w"] = [bc(dws_ref[k, pl.ds(c0, 8), :]) for k in range(9)]
            wts = list(st["w"])
            if ("tw", r) in st:
                wts[6], wts[8] = st["tw", r]
            row(r)
            abc = [row(r + 1) * wts[3 + j] + row(r) * wts[j] + row(r + 2) * wts[6 + j] for j in range(3)]
            x0 = pltpu.roll(abc[0], 1, 1) + abc[1] + pltpu.roll(abc[2], WP - 1, 1)
            for t in range(NT):
                x0_ref[rows_at(sc["nxt"], (r * NT + t) * C + c0, 8), :] = x0[:, t * LANES:(t + 1) * LANES]

        return taps, piece

    @when(k_ == 0, ("first",))
    def _():
        for g in range(NG // FG):
            x0_copy(g).start()
        for k in range(9):
            w = dw_ref[k // 3].astype(F32)[k % 3:k % 3 + 1, :]
            w = jnp.broadcast_to(w, (LANES, C)).T
            dws_ref[k] = w + 1.0 if k == 4 else w
            if k in (6, 8):
                x0_ref[pl.ds(DW_OFF + (k - 6) // 2 * C, C), :] = w
        w = wqkv_ref[...].astype(F32)
        wq = w[:, 0:C] * ((DH ** -0.5) * math.log2(math.e))
        wk, wv = w[:, C:2 * C], w[:, 2 * C:3 * C]
        tiles = [(wq[:, 0:64], wv[:, 64:96], wq[:, 64:96]),
                 (wq[:, 96:192], wv[:, 96:128]),
                 (wk[:, 0:64], wv[:, 128:160], wk[:, 64:96]),
                 (wk[:, 96:192], wv[:, 160:192]),
                 (wv[:, 0:128],)]
        for n, parts in enumerate(tiles):
            w = jnp.concatenate(parts, axis=1)
            for i, wi in enumerate((w[0:128], w[64:192], _cat([w[0:64], w[128:192]]))):
                if n == 4:
                    wi = wi.T
                ws_ref[i, n] = pltpu.bitcast(wi.astype(BF16), U32)
        w = wo_ref[...].astype(F32)
        wx, wy, wz = w[0:64], w[64:128], w[128:192]
        for i, parts in enumerate(((wx, wy), (wz, wy), (wx, wy + wz))):
            wos_ref[i] = pltpu.bitcast(_cat(parts).T.astype(BF16), U32)

        top_ref[...] = jnp.zeros(top_ref.shape, F32)
        for i in (WS + 1, 2 * WS + 3):
            x_ref[i] = jnp.zeros(x_ref.shape[1:], x_ref.dtype)

        for p in range(stg_ref.shape[0]):
            stg_ref[p] = jnp.zeros(stg_ref.shape[1:], F32)
        for r in range(WS):
            ob_ref[pl.ds(r * WP + WP - 8, 8), :] = jnp.zeros((8, LANES), F32)

    cuts = [int(c) for c in _env("CUTS", "0,7").split(",")]
    bands = list(zip(cuts, cuts[1:]))
    groups = {(b, g): conv_group(8 * g) for b in range(len(bands)) for g in range(NG)}
    WLEAD = _env("WLEAD", 4)

    def conv_items(nslow):
        plist = [((b, g), r) for b, (r0, r1) in enumerate(bands) for g in range(NG) for r in range(r0, r1)]
        items, nxt_tap = [], WLEAD
        for k, (g, r) in enumerate(plist):
            fs = []
            lead = WLEAD if k < nslow else _env("WLEAD2", 5)
            while nxt_tap <= min(k + lead, len(plist) - 1):
                g2, r2 = plist[nxt_tap]
                fs.append(functools.partial(groups[g2][0], r2))
                nxt_tap += 1
            fs.append(functools.partial(groups[g][1], r))
            items.append(fs)
        return items

    def ld_x0(j, k, gs=range(NG)):
        return [x0_ref[rows_at(sc["nxt"] + dyn0 * (8 * k), j * C + 8 * g, 8), :] for g in gs]

    def add2(acc, xs):
        a = functools.reduce(jnp.add, xs[0::2])
        b = functools.reduce(jnp.add, xs[1::2])
        return a + b if acc is None else (acc + a) + b

    stats_done = set()

    def stats_steps(j):
        st = {"s": None, "q": None}
        n1, n2 = _env("SEG1", 12), _env("SEG2", 6)

        def sum_step(g0):
            st["s"] = add2(st["s"], ld_x0(j, 0, range(g0, g0 + n1)))
            if g0 + n1 == NG:
                st["s"] = _allred(st["s"], jnp.add) * (1.0 / C)
            return st["s"]

        def var_step(g0):
            d = [x - st["s"] for x in ld_x0(j, 1, range(g0, g0 + n2))]
            st["q"] = add2(st["q"], [x * x for x in d])
            return st["q"]

        def last_step():
            v = _allred(st["q"], jnp.add) * (1.0 / C) + EPS
            rs = lax.rsqrt(v) if _env("RSQ", 1) else jnp.exp2(jnp.log2(v) * -0.5)
            ms_ref[j] = _cat([st["s"], rs])
            stats_done.add(j)
            return rs

        return ([functools.partial(sum_step, g) for g in range(0, NG, n1)]
                + [functools.partial(var_step, g) for g in range(0, NG, n2)] + [last_step])

    def colsum(xs):
        xs = [a + b for a, b in zip(xs[0:8], xs[16:24])] + xs[8:16]
        return _dot(jnp.ones((8, LANES), F32), _cat(xs))

    means = {}

    def mean_dot(j):
        means[j] = colsum(ld_x0(j, 0)) * (1.0 / C)

    def var_dot(j):
        xs = [x0_ref[pl.ds(sc["nxt"] + (j * C + 8 * g + 4), 8), :] for g in range(NG - 1)]
        xs.append(jnp.where(mk["up"], *ld_x0(j, 0, (0, NG - 1))))
        d = [x - means[j] for x in xs]
        v = colsum([x * x for x in d]) * (1.0 / C) + EPS
        rs = lax.rsqrt(v) if _env("RSQ", 1) else jnp.exp2(jnp.log2(v) * -0.5)
        ms_ref[j] = _cat([means[j], rs])
        stats_done.add(j)

    def normed(j, blk, k):
        assert j in stats_done or "ONLY" in os.environ and j < NSTX, j
        m, rs = ms_ref[j, 0:8, :], ms_ref[j, 8:16, :]
        return _cat([(x - m) * rs for x in ld_x0(j, k, range(8 * blk, 8 * blk + 8))])

    t_done = {}

    def put_t(dst, tiles):
        tt = pltpu.bitcast(jnp.concatenate(tiles, axis=1).astype(BF16).T, U32)
        for i, (u, e) in enumerate(dst):
            t_ref[u, e] = tt[64 * i:64 * i + 64]
        t_done[len(t_done)] = pltpu.bitcast(tt[120:128], F32)

    def t_first(u):
        ja, jb = 2 * u, 2 * u + 1
        bx = normed(jb, 0, 0)
        put_t([(u, 0), (u, 2)], [_cat([normed(ja, 0, 0) - bx, normed(ja, 1, 0)]),
                                 _cat([bx, normed(ja, 2, 0)])])

    def t_second(r):
        put_t([(u, 1) for u in (2 * r, 2 * r + 1)],
              [_cat([normed(2 * u + 1, 1, 0), normed(2 * u + 1, 2, 0) - normed(2 * u, 2, _env("RECOMP", 0))])
               for u in (2 * r, 2 * r + 1)])

    t_items = []
    for r in range(WS):
        t_items += [functools.partial(t_first, 2 * r), functools.partial(t_first, 2 * r + 1),
                    functools.partial(t_second, r)]

    def qkv_chunk(us, n, steps=(), tiny=()):
        lhs = {i: [b for u in us for b in _blocks(t_ref[u, i])] for i in range(3)}
        for q, step in enumerate(steps):
            tok = pltpu.bitcast(step(), U32)
            q = q * 24 * len(us) // len(steps)
            blks = lhs[(2, 0, 1)[q % 3]]
            blks[q // 3] = jnp.where(mk["never"], tok, blks[q // 3])
        p3 = None
        for i in (2, 0, 1):
            p = _dot(pltpu.bitcast(_cat(lhs[i]), BF16), pltpu.bitcast(ws_ref[i, n], BF16))
            if p3 is None:
                p3 = p
            else:
                p = p + p3
                for e, u in enumerate(us):
                    r, tp = divmod(u, 2)
                    qkv_ref[n, r, pl.ds((2 * tp + i) * LANES, LANES), :] = p[e * LANES:(e + 1) * LANES]

    vr_words = {}
    job_done = {}

    def side_dots(u, n):
        r, tp = divmod(u, 2)
        st = {}

        def one(i, parts=1):
            if parts > 1:
                lhs, rows = t_ref[u, i], 64 // parts
                p = _cat([_dot(pltpu.bitcast(lhs[q * rows:(q + 1) * rows], BF16),
                               pltpu.bitcast(ws_ref[i, n], BF16)) for q in range(parts)])
            elif n == 4:
                p = _dot_nt(pltpu.bitcast(ws_ref[i, 4, 0:32, :], BF16), pltpu.bitcast(t_ref[u, i], BF16))
            else:
                p = _dot(pltpu.bitcast(t_ref[u, i], BF16), pltpu.bitcast(ws_ref[i, n], BF16))
            st[i] = p if i == 2 else p + st[2]
            if n < 4 and i < 2:
                qkv_ref[n, r, pl.ds((2 * tp + i) * LANES, LANES), :] = st[i]
            elif i == 1:
                vr_words[u] = pltpu.pack_elementwise([st[0], st[1]], packed_dtype=BF16)

        return [(64 if n == 4 else LANES, (u, n, i), functools.partial(one, i)) for i in (2, 0, 1)]

    def vr_store(u):
        r, tp = divmod(u, 2)
        w = pltpu.bitcast(vr_words[u], F32)
        wt = pltpu.bitcast(_cat([w, w]).T, U32)
        job_done["v", u] = pltpu.bitcast(wt[120:128], F32)
        for j in range(2):
            qkv_ref[4, r, pl.ds((2 * tp + j) * LANES, LANES), :] = pltpu.unpack_elementwise(
                wt, index=j, packed_dtype=BF16, unpacked_dtype=F32)

    zero8 = jnp.zeros((8, LANES), F32)

    def gather(n, off, k=0):
        return [qkv_ref[n, r, pl.ds(off + dyn0 * k if k else off, 8), :] for r in range(WS)]

    def softmax_t(st):
        rows = _blocks(st)
        m = functools.reduce(jnp.maximum, rows)
        m = _allred(jnp.where(mk["key"], m, -jnp.inf), jnp.maximum)
        p = [jnp.exp2(x - m) for x in rows]
        return p, functools.reduce(jnp.add, p)

    def s2_pair(pi, offa):
        offb = offa + WS
        st = {}

        def vprep():
            g = [gather(n, offa) + gather(n, offb) for n in range(5)]
            u1 = [jnp.where(mk["left64"], z, jnp.where(mk["v"], x, y)) for x, y, z in zip(g[0], g[1], g[4])]
            u2 = [jnp.where(mk["v"], x, y) for x, y in zip(g[2], g[3])]
            u = jnp.concatenate([_cat(u1 + [zero8, zero8]), _cat(u2 + [zero8, zero8])], axis=1)
            vt = pltpu.bitcast(u.astype(BF16).T, U32)
            vt = _cat([vt[0:64], vt[96:128]])
            st["vt"] = [pltpu.bitcast(vt[24 * h:24 * h + 24], BF16) for h in range(NH)]

        def score(i, ties=()):
            hp, sw = divmod(i, 2)
            lo, hi = mk["lo"], mk["hi%d" % hp]
            ma, mb = (lo, hi) if sw == 0 else (hi, lo)
            gq = (0, 1, 1 + sw)[_env("GQ", 0)]
            gk = (0, 1, 1 + sw)[_env("GK", 0)]
            q = _cat([jnp.where(ma, v, 0.0) for v in gather(hp, offa, gq)]
                     + [jnp.where(mb, v, 0.0) for v in gather(hp, offb, gq)] + [zero8, zero8])
            ka, kb = gather(2 + hp, offa, gk), gather(2 + hp, offb, gk)
            k = [jnp.where(lo, x, y) for x, y in (zip(ka, kb) if sw == 0 else zip(kb, ka))]
            for _, job in ties:
                k[0] = jnp.where(mk["never"], job(), k[0])
            k = _cat(k)
            st["p", i] = softmax_t(_dot_nt(k, q))

        def value(h):
            hp, sw = divmod(h, 2)
            (pa, sa), (pb, sb) = st["p", 2 * hp + sw], st["p", 2 * hp + 1 - sw]
            pm = _cat([jnp.where(mk["keep_a"], v, 0.0) for v in pa]
                      + [jnp.where(mk["keep_b"], v, 0.0) for v in pb] + [zero8, zero8])
            den = _allred(jnp.where(mk["keep_a"], sa, jnp.where(mk["keep_b"], sb, 0.0)), jnp.add)
            rec = pl.reciprocal(den, approx=True)
            if _env("NR", 0):
                rec = rec * (2.0 - den * rec)
            st["o", h] = [b * rec for b in _blocks(_dot(st["vt"][h], pm))]

        def finish():
            o = [b for h in range(NH) for b in st["o", h]]
            w = pltpu.pack_elementwise([_cat(o[0:16]), _cat(o[16:24] + o[16:24])], packed_dtype=BF16)
            stg_ref[pi] = pltpu.bitcast(w, F32)

        def scatter():
            wt = stg_ref[pi].T
            job_done["s", pi] = wt[104:112]
            for i, off in enumerate((offa, offb)):
                for r in range(WS):
                    base = i * SLOTS + 8 * r
                    ob_ref[pl.ds(r * WP + off, WS), :] = wt[base:base + WS]

        return vprep, score, value, finish, scatter

    npair = (nwin + 1) // 2
    pairs = [s2_pair(p, min(2 * p, nwin - 2) * WS) for p in range(npair)]

    def s3_unit(r, tp, ties=()):
        def unpack(t):
            w = pltpu.bitcast(ob_ref[pl.ds(r * WP + t * LANES, LANES), :], U32)
            return [_blocks(pltpu.unpack_elementwise(w, index=i, packed_dtype=BF16, unpacked_dtype=F32))
                    for i in range(2)]

        (la, ha), (lb, hb) = unpack(2 * tp), unpack(2 * tp + 1)
        t3 = [jnp.where(mk["left64"], x, y) for x, y in zip(lb, ha)]
        t1 = _cat([x - y for x, y in zip(la, t3)])
        t2 = _cat([jnp.where(mk["left64"], x, z) - y for x, y, z in zip(hb, ha, lb)])
        t3 = _cat(t3)
        wo = [_blocks(wos_ref[i]) for i in range(3)]
        for q, (e, job) in enumerate(ties):
            blks = wo[(2, 0, 1)[q % 3]]
            blks[e] = jnp.where(mk["never"], pltpu.bitcast(job(), U32), blks[e])
        wo = [pltpu.bitcast(_cat(w), BF16) for w in wo]
        p3 = _dot_nt(wo[2], t3)
        ys = [_dot_nt(wo[i], t) + p3
              + x0_ref[rows_at(sc["prv"], (r * NT + 2 * tp + i) * C, C), :] for i, t in enumerate((t1, t2))]
        n = min(2 * LANES, W - 2 * tp * LANES)
        o_ref[sc["ooff"] + r, :, pl.ds(2 * tp * LANES, n)] = jnp.concatenate(ys, axis=1).astype(o_ref.dtype)[:, :n]

    s3_all = [functools.partial(s3_unit, r, tp) for tp in range(2) for r in range(WS)]

    def run(prog, extra):
        extra = sorted(extra, key=lambda e: e[0])
        j = 0
        for t0, fn in prog:
            while j < len(extra) and extra[j][0] <= t0:
                extra[j][1]()
                j += 1
            fn()
        for e in extra[j:]:
            e[1]()

    MERGE = _env("MERGE", 0)
    NX3 = _env("NX3", 0)

    NSY = 0

    NSTX = _env("NSTX", 24)

    def wave_steps(lo, hi, wave):
        steps = []
        for j0 in range(lo, hi, wave):
            for grp in zip(*[stats_steps(j) for j in range(j0, min(j0 + wave, hi))]):
                steps += grp
        return steps

    def block_x():
        new_scalars()
        NJ = _env("NJ", 28)
        NSTC = _env("NSTC", 7)
        WAVE = _env("WAVE", 4)
        VRLAG = _env("VRLAG", 150)
        chunks = [(u, n) for u in range(NU) for n in range(4)]
        MXS = _env("MXS", 0)
        steps = [] if MXS else wave_steps(0, NSTX, WAVE)
        loose = steps[len(steps) - _env("LOOSE", 0):]
        steps = steps[:len(steps) - len(loose)]
        nside = 9
        side, vstep = [], _env("VRSTEP", 0)
        for _ in range(_env("SIDE0", 1)):
            side += side_dots(*chunks.pop())
            nside -= 1
        for q in range(NU // 2):
            side += side_dots(2 * q, 4) + side_dots(2 * q + 1, 4)
            for _ in range(vstep):
                if nside:
                    side += side_dots(*chunks.pop())
                    nside -= 1
        for _ in range(nside):
            side += side_dots(*chunks.pop())
        mu = _env("MU", 2)
        merged = []
        for u, n in chunks:
            prev = [c for c in merged if c[1] == n and c[0][0] // mu == u // mu]
            if prev:
                prev[0][0].append(u)
            else:
                merged.append(([u], n))
        starts = [LANES * sum(len(c[0]) for c in merged[:k]) for k in range(len(merged))]
        t_conv = max(x for x in starts if x <= (len(chunks) - NSTC) * LANES)
        span = len(chunks) * LANES - t_conv
        plan, t, vr_ready = [], 0, {}
        for k, (us, n) in enumerate(merged):
            dur = LANES * len(us)
            lo, hi = (max(x - t_conv, 0) * len(steps) // span for x in (t, t + dur))
            plan.append((t, tuple(us), n, list(steps[lo:hi]), []))
            room = dur
            while side and (room > 0 or k == len(merged) - 1):
                rows, key, f = side.pop(0)
                plan.append((t, f if room > 0 else functools.partial(f, 4), None, [], []))
                room -= rows
                if key[1:] == (4, 1):
                    vr_ready[key[0]] = t + dur - room + VRLAG
            t += dur
        ci = conv_items(4 * NJ)
        slow = _env("SLOW", 32.0)
        fast = (t_conv - 4 * NJ * slow) / max(len(ci) - 4 * NJ, 1)
        t_piece = [min(j, 4 * NJ) * slow + max(j - 4 * NJ, 0) * fast for j in range(len(ci) + 1)]
        scat, vrs = list(range(npair - NSY)), list(range(NU))
        jobs = []
        for q in range(NJ):
            if vrs and vr_ready[vrs[0]] <= t_piece[4 * q + 1]:
                jobs.append((t_piece[4 * q + 1], ("v", vrs[0])))
                ci[4 * q].insert(0, functools.partial(vr_store, vrs.pop(0)))
            elif scat:
                jobs.append((t_piece[4 * q + 1], ("s", scat[0])))
                ci[4 * q].insert(0, pairs[scat.pop(0)][4])
        extra = [(t_piece[j + 1], f) for j, fs in enumerate(ci) for f in fs]
        tail = [(("v", u), functools.partial(vr_store, u)) for u in vrs] + [(("s", p), pairs[p][4]) for p in scat]
        for q, (key, f) in enumerate(tail):
            t_q = max(t_conv + 1 + (q // 3) * 128, vr_ready[key[1]] if key[0] == "v" else 0)
            extra.append((t_q, f))
            jobs.append((t_q, key))
        if _env("JDL", 800):
            for t_q, key in jobs:
                later = [e for e in plan if e[2] is not None and e[0] >= t_q + _env("JDL", 800)]
                if later:
                    later[0][3].insert(0, functools.partial(job_done.get, key))
        prog = [(t0, u if n is None else functools.partial(qkv_chunk, u, n, st, tn))
                for t0, u, n, st, tn in plan]
        run(prog, extra + [(t, f) for f in loose])

    def block_y():
        new_scalars()
        pattern = _env("PAT", "SFFVFFFF" + "SSSSFVVVV" * 8 + "SSSSVVVV").rstrip(".")
        load = [0] * 4
        items, ns, nv, nf = [], 0, 0, 0
        for ch in pattern:
            if ch in "Ss":
                todo = [("s", ns + i, [SLOTS]) for i in range(4 if ch == "S" else 2)]
                ns += len(todo)
            elif ch in "Vv":
                todo = [("v", nv + i, [DH]) for i in range(4 if ch == "V" else 2)]
                nv += len(todo)
            else:
                todo = [("f", nf, [C] * 3)]
                nf += 1
            for kind, idx, rows in todo:
                items.append((min(load), kind, idx, []))
                for x in rows:
                    load[load.index(min(load))] += x
        assert (ns, nv, nf) == (4 * npair, 4 * npair, NU)
        spots = sorted([(it[0], it, 0) for it in items if it[1] == "s"]
                       + [(it[0] + 16 * e, it, e) for it in items if it[1] == "f" for e in range(12)],
                       key=lambda x: x[0])
        ysteps = wave_steps(NSTX, WS * NT, _env("WAVEY", 4))
        fspots = [x for x in spots if x[1][1] == "f" and x[1][2] < _env("S3Q", 6)
                  and _env("E0", 2) <= x[2] < _env("E1", 12)]
        fspots.sort(key=lambda x: (x[1][2], x[2]))
        for q, step in enumerate(ysteps):
            _, it, e = fspots[q * len(fspots) // len(ysteps)]
            it[3].append((e, step))
        t_done.clear()
        extra = []
        tpos = [int(x) for x in _env("TPOS", "4,8").split(",")]
        late = [x for x in spots if x[1][1] == "s" and x[1][2] >= _env("TOFS", 4) and (x[1][2] - _env("TOFS", 4)) % _env("TRUN", 16) in tpos]
        late.sort(key=lambda x: x[1][2])
        n1 = max(_env("NT1", 0), len(t_items) - len(late))
        ta0, ta1 = _env("TA0", 500), _env("TA1", 850)
        late = late[_env("TSKIP", 0):]
        for j, f in enumerate(t_items):
            if j < n1:
                t_s, it, e = [x for x in spots if x[0] >= ta0 + j * (ta1 - ta0) / n1][0]
            else:
                t_s, it, e = late[(j - n1) * len(late) // (len(t_items) - n1)]
            it[3].append((e, functools.partial(t_done.__getitem__, j)))
            extra.append((min(t_s - _env("TLEAD", 450), it[0]), f))
        prog = []
        for t0, kind, idx, ties in items:
            p, i = divmod(idx, 4)
            if kind == "s":
                if i == 0:
                    prog.append((t0, pairs[p][0]))
                prog.append((t0, functools.partial(pairs[p][1], i, ties)))
            elif kind == "v":
                prog.append((t0, functools.partial(pairs[p][2], i)))
                if i == 3:
                    extra.append((t0 + DH + _env("LFIN", 0), pairs[p][3]))
            else:
                prog.append((t0, functools.partial(s3_all[idx], ties)))
        run(prog, extra)

    only = _env("ONLY", "01")
    if mode != "main":
        new_scalars()

    @when(k_ < nstrip, ("main",))
    def _():
        x_copy(k_).wait()

    @when(k_ < nstrip - 1, ("first", "main"))
    def _():
        x_copy(k_ + 1).start()

    new_masks("x")
    if "0" in only:
        when(k_ <= nstrip, ("main",))(block_x)

    @when(k_ == 0, ("first",))
    def _():
        def body(g, carry):
            x0_copy(g).wait()
            for j in range(FG):
                piece = conv_group(pl.multiple_of((g * FG + j) * 8, 8))[1]
                for r in range(WS):
                    piece(r)
            return carry
        lax.fori_loop(0, NG // FG, body, 0)

    @when(k_ >= 4, ("main", "last"))
    def _():
        o_copy(k_ - 4).wait()

    @when(k_ >= 3, ("main", "last"))
    def _():
        o_copy(k_ - 3).start()

    if "1" in only:
        new_masks("y")
        when((k_ <= nstrip) & (k_ >= 1), ("main",))(block_y)

    @when(k_ == 0, ("first",))
    def _():
        for j in range(WS * NT):
            for f in stats_steps(j):
                f()
        for f in t_items:
            f()

    @when(k_ == nstrip + 1, ("last",))
    def _():
        new_masks("y")
        for p in range(npair):
            pairs[p][4]()
        for q, f in enumerate(s3_all):
            f()
            if q >= WS:
                row_copy(q - WS).start()

    if only != "01":
        @when(dyn0 < 0, ("main",))
        def _():
            i = pl.multiple_of(k_ * 8, 8)
            k3 = k_ & 1
            o_ref[0, 0:16, 0:128] = _cat([
                qkv_ref[k3, k3, pl.ds(i, 8), :] + ms_ref[k3, 0:8, :] + stg_ref[k3, pl.ds(i, 8), :],
                pltpu.bitcast(t_ref[k3, k3, pl.ds(i, 8), :], F32) + ob_ref[pl.ds(i, 8), :]]).astype(BF16)
            for rf in (qkv_ref.at[k3, k3], stg_ref.at[k3], ob_ref):
                rf[pl.ds(i, 8), :] = zero8
            t_ref[k3, k3, pl.ds(i, 8), :] = pltpu.bitcast(zero8, U32)

    @when(k_ == nstrip + 1, ("last",))
    def _():
        o_copy(k_ - 3).wait()
        for r in range(WS):
            row_copy(r).wait()


@jax.jit
def pallas_standalone__window_attn_davit__vision_kernel(
    x: jax.Array,
    dw_pe: jax.Array,
    w_qkv: jax.Array,
    w_o: jax.Array,
):
    B, H, W, Cx = x.shape
    assert B == 1 and Cx == C and H % WS == 0 and W % WS == 0 and WP - LANES < W < WP
    xt = jnp.transpose(x[0], (0, 2, 1))

    assert H // WS + 2 <= 256
    vmem = pl.BlockSpec(memory_space=pltpu.VMEM)
    yt = pl.pallas_call(
        functools.partial(_kernel, H=H, W=W),
        in_specs=[pl.BlockSpec(memory_space=pl.ANY), vmem, vmem, vmem],
        out_specs=pl.BlockSpec(memory_space=pl.ANY),
        out_shape=jax.ShapeDtypeStruct((H, C, W), x.dtype),
        scratch_shapes=[
            pltpu.VMEM((2 * (WS + 2), C, W), x.dtype),
            pltpu.VMEM((2 * WS, C, W), x.dtype),
            pltpu.SemaphoreType.DMA((5,)),
            pltpu.VMEM((X0_ROWS, LANES), F32),
            pltpu.VMEM((WS * WP, LANES), F32),
            pltpu.VMEM((9, C, LANES), F32),
            pltpu.VMEM((3, 5, LANES // 2, LANES), U32),
            pltpu.VMEM((3, C // 2, LANES), U32),
            pltpu.VMEM((5, WS, WP, LANES), F32),
            pltpu.VMEM((NU, 3, LANES // 2, LANES), U32),
            pltpu.VMEM((37, LANES, LANES), F32),
            pltpu.VMEM((WS * NT, 16, LANES), F32),
            pltpu.VMEM((C, WP), F32),
        ],
        compiler_params=pltpu.CompilerParams(
            vmem_limit_bytes=64 * 1024 * 1024,
            disable_bounds_checks=bool(_env("NOBC", 1)),
        ),
        name="davit_window_attn",
    )(xt, dw_pe, w_qkv, w_o)
    return jnp.transpose(yt, (0, 2, 1))[None]
```

```python
import functools
import math

import jax
import jax.numpy as jnp
from jax import lax
import jax.experimental.pallas as pl
import jax.experimental.pallas.tpu as pltpu

WS = 7
NH = 4
C = 192
DH = C // NH
NG = C // 8
LANES = 128
WP = 512
NT = WP // LANES
NU = WS * NT // 2
SLOTS = 8 * WS
EPS = 1e-5
F32 = jnp.float32
BF16 = jnp.bfloat16
U32 = jnp.uint32

X0_SLOT = WS * NT * C
DW_OFF = 3 * X0_SLOT
X0_ROWS = DW_OFF + 2 * C

FG = 8
NSTX = 24


def _dot(a, b):
    return jnp.dot(a, b, preferred_element_type=F32)


def _dot_nt(a, b):
    return lax.dot_general(a, b, (((1,), (1,)), ((), ())), preferred_element_type=F32)


def _cat(xs):
    return jnp.concatenate(xs, axis=0)


def _blocks(v):
    return [v[i:i + 8] for i in range(0, v.shape[0], 8)]


def _allred(x, op):
    for sh in (4, 2, 1):
        x = op(x, pltpu.roll(x, sh, 0))
    return x


def _run(prog, extra):
    extra = sorted(extra, key=lambda e: e[0])
    j = 0
    for t0, fn in prog:
        while j < len(extra) and extra[j][0] <= t0:
            extra[j][1]()
            j += 1
        fn()
    for e in extra[j:]:
        e[1]()


def _kernel(*refs, H, W):
    nstrip = H // WS
    for lo, hi, mode in ((0, 1, "first"), (1, nstrip + 1, "main"), (nstrip + 1, nstrip + 2, "last")):
        def body(k, carry, mode=mode):
            _step(*refs, H=H, W=W, k_=k, mode=mode)
            return carry
        lax.fori_loop(lo, hi, body, 0)


def _step(x_hbm, dw_ref, wqkv_ref, wo_ref, o_hbm,
          x_ref, o_ref, sems, x0_ref, ob_ref, dws_ref, ws_ref, wos_ref, qkv_ref, t_ref, stg_ref, ms_ref,
          top_ref, *, H, W, k_, mode):
    nstrip, nwin = H // WS, W // WS
    npair = (nwin + 1) // 2

    def x_copy(k):
        return pltpu.make_async_copy(x_hbm.at[pl.ds(jnp.minimum(k * WS, H - WS - 1), WS + 1)],
                                     x_ref.at[pl.ds((k & 1) * (WS + 2), WS + 1)], sems.at[0])

    def o_copy(k):
        return pltpu.make_async_copy(o_ref.at[pl.ds((k & 1) * WS, WS)], o_hbm.at[pl.ds(k * WS, WS)],
                                     sems.at[1])

    def x0_copy(g):
        cs = pl.ds(pl.multiple_of(g * (8 * FG), 8 * FG), 8 * FG)
        return pltpu.make_async_copy(x_hbm.at[pl.ds(0, WS + 1), cs], x_ref.at[pl.ds(0, WS + 1), cs],
                                     sems.at[2 + g])

    def row_copy(r):
        return pltpu.make_async_copy(o_ref.at[sc["ooff"] + r], o_hbm.at[H - WS + r], sems.at[2])

    def when(cond, modes):
        return pl.when(cond) if mode in modes else (lambda f: None)

    sc = {}

    def new_scalars():
        k3 = k_ - 3 * ((k_ * 171) >> 9)
        sc["nxt"] = k3 * X0_SLOT
        sc["prv"] = jnp.where((k3 == 2) | (k_ < 2), 0, sc["nxt"] + X0_SLOT)
        sc["xoff"] = (k_ & 1) * (WS + 2) + jnp.where(k_ >= nstrip - 1, 1, 0)
        sc["ooff"] = (k_ & 1) * WS

    dyn0 = jnp.minimum(k_, 0)

    def rows_at(base, off, n):
        if isinstance(base, int):
            return pl.ds(base + off, n)
        return pl.ds(pl.multiple_of(base + off, 8), n)

    mk = {}

    def new_masks(blk):
        lane = lax.broadcasted_iota(jnp.int32, (8, LANES), 1)
        mk.clear()
        mk["never"] = lane < dyn0
        if blk == "y":
            key_ok = lax.broadcasted_iota(jnp.int32, (8, LANES), 0) < WS
            mk.update(
                lo=lane < DH, hi0=(lane >= DH) & ((lane < 64) | (lane >= 96)),
                hi1=(lane >= DH) & (lane < 96), v=lane < 96, key=key_ok,
                keep_a=key_ok & (lane < SLOTS), keep_b=key_ok & (lane >= SLOTS), left64=lane < 64)

    conv_done = []

    def conv_group(c0):
        st = {}

        def row(i):
            if i == 0 and i not in st:
                st[i] = top_ref[pl.ds(c0, 8), :]
            if i not in st:
                v = x_ref[sc["xoff"] + (i - 1), pl.ds(c0, 8), :].astype(F32)
                st[i] = jnp.concatenate([v, jnp.zeros((8, WP - W), F32)], axis=1)
                if i == WS:
                    top_ref[pl.ds(c0, 8), :] = st[i]
            return st[i]

        def bc(v):
            return jnp.concatenate([v] * NT, axis=1)

        def taps(r):
            st["tw", r] = [bc(x0_ref[rows_at(c0, DW_OFF + k * C, 8), :]) for k in range(2)]

        def piece(r):
            if "w" not in st:
                st["w"] = [bc(dws_ref[k, pl.ds(c0, 8), :]) for k in range(9)]
            wts = list(st["w"])
            if ("tw", r) in st:
                wts[6], wts[8] = st["tw", r]
            row(r)
            abc = [row(r + 1) * wts[3 + j] + row(r) * wts[j] + row(r + 2) * wts[6 + j] for j in range(3)]
            x0 = pltpu.roll(abc[0], 1, 1) + abc[1] + pltpu.roll(abc[2], WP - 1, 1)
            for t in range(NT):
                x0_ref[rows_at(sc["nxt"], (r * NT + t) * C + c0, 8), :] = x0[:, t * LANES:(t + 1) * LANES]
            conv_done.append(r)

        return taps, piece

    def conv_items(nslow):
        groups = [conv_group(8 * g) for g in range(NG)]
        plist = [(g, r) for g in range(NG) for r in range(WS)]
        items, tap = [], 4
        for k, (g, r) in enumerate(plist):
            fs = []
            while tap <= min(k + (4 if k < nslow else 5), len(plist) - 1):
                fs.append(functools.partial(groups[plist[tap][0]][0], plist[tap][1]))
                tap += 1
            fs.append(functools.partial(groups[g][1], r))
            items.append(fs)
        return items

    @when(k_ == 0, ("first",))
    def _():
        for g in range(NG // FG):
            x0_copy(g).start()
        for k in range(9):
            w = dw_ref[k // 3].astype(F32)[k % 3:k % 3 + 1, :]
            w = jnp.broadcast_to(w, (LANES, C)).T
            dws_ref[k] = w + 1.0 if k == 4 else w
            if k in (6, 8):
                x0_ref[pl.ds(DW_OFF + (k - 6) // 2 * C, C), :] = w
        w = wqkv_ref[...].astype(F32)
        wq = w[:, 0:C] * ((DH ** -0.5) * math.log2(math.e))
        wk, wv = w[:, C:2 * C], w[:, 2 * C:3 * C]
        tiles = [(wq[:, 0:64], wv[:, 64:96], wq[:, 64:96]),
                 (wq[:, 96:192], wv[:, 96:128]),
                 (wk[:, 0:64], wv[:, 128:160], wk[:, 64:96]),
                 (wk[:, 96:192], wv[:, 160:192]),
                 (wv[:, 0:128],)]
        for n, parts in enumerate(tiles):
            w = jnp.concatenate(parts, axis=1)
            for i, wi in enumerate((w[0:128], w[64:192], _cat([w[0:64], w[128:192]]))):
                if n == 4:
                    wi = wi.T
                ws_ref[i, n] = pltpu.bitcast(wi.astype(BF16), U32)
        w = wo_ref[...].astype(F32)
        wx, wy, wz = w[0:64], w[64:128], w[128:192]
        for i, parts in enumerate(((wx, wy), (wz, wy), (wx, wy + wz))):
            wos_ref[i] = pltpu.bitcast(_cat(parts).T.astype(BF16), U32)

        top_ref[...] = jnp.zeros(top_ref.shape, F32)
        for i in (WS + 1, 2 * WS + 3):
            x_ref[i] = jnp.zeros(x_ref.shape[1:], x_ref.dtype)
        for p in range(npair):
            stg_ref[p] = jnp.zeros(stg_ref.shape[1:], F32)
        for r in range(WS):
            ob_ref[pl.ds(r * WP + WP - 8, 8), :] = jnp.zeros((8, LANES), F32)

    def ld_x0(j, k, gs):
        return [x0_ref[rows_at(sc["nxt"] + dyn0 * (8 * k), j * C + 8 * g, 8), :] for g in gs]

    def add2(acc, xs):
        a = functools.reduce(jnp.add, xs[0::2])
        b = functools.reduce(jnp.add, xs[1::2])
        return a + b if acc is None else (acc + a) + b

    stats_done = set()

    def stats_steps(j):
        st = {"s": None, "q": None}

        def sum_step(g0):
            assert mode != "main" or len(conv_done) == NG * WS
            st["s"] = add2(st["s"], ld_x0(j, 0, range(g0, g0 + 12)))
            if g0 + 12 == NG:
                st["s"] = _allred(st["s"], jnp.add) * (1.0 / C)
            return st["s"]

        def var_step(g0):
            d = [x - st["s"] for x in ld_x0(j, 1, range(g0, g0 + 6))]
            st["q"] = add2(st["q"], [x * x for x in d])
            return st["q"]

        def last_step():
            rs = lax.rsqrt(_allred(st["q"], jnp.add) * (1.0 / C) + EPS)
            ms_ref[j] = _cat([st["s"], rs])
            stats_done.add(j)
            return rs

        return ([functools.partial(sum_step, g) for g in range(0, NG, 12)]
                + [functools.partial(var_step, g) for g in range(0, NG, 6)] + [last_step])

    def wave_steps(lo, hi):
        steps = []
        for j0 in range(lo, hi, 4):
            for grp in zip(*[stats_steps(j) for j in range(j0, j0 + 4)]):
                steps += grp
        return steps

    def normed(j, blk):
        assert j in stats_done
        m, rs = ms_ref[j, 0:8, :], ms_ref[j, 8:16, :]
        return _cat([(x - m) * rs for x in ld_x0(j, 0, range(8 * blk, 8 * blk + 8))])

    t_done = {}

    def put_t(dst, tiles):
        tt = pltpu.bitcast(jnp.concatenate(tiles, axis=1).astype(BF16).T, U32)
        for i, (u, e) in enumerate(dst):
            t_ref[u, e] = tt[64 * i:64 * i + 64]
        t_done[len(t_done)] = pltpu.bitcast(tt[120:128], F32)

    def t_first(u):
        ja, jb = 2 * u, 2 * u + 1
        bx = normed(jb, 0)
        put_t([(u, 0), (u, 2)], [_cat([normed(ja, 0) - bx, normed(ja, 1)]), _cat([bx, normed(ja, 2)])])

    def t_second(r):
        put_t([(u, 1) for u in (2 * r, 2 * r + 1)],
              [_cat([normed(2 * u + 1, 1), normed(2 * u + 1, 2) - normed(2 * u, 2)])
               for u in (2 * r, 2 * r + 1)])

    t_items = []
    for r in range(WS):
        t_items += [functools.partial(t_first, 2 * r), functools.partial(t_first, 2 * r + 1),
                    functools.partial(t_second, r)]

    def qkv_chunk(us, n, steps):
        lhs = {i: [b for u in us for b in _blocks(t_ref[u, i])] for i in range(3)}
        for q, step in enumerate(steps):
            tok = pltpu.bitcast(step(), U32)
            q = q * 24 * len(us) // len(steps)
            blks = lhs[(2, 0, 1)[q % 3]]
            blks[q // 3] = jnp.where(mk["never"], tok, blks[q // 3])
        p3 = None
        for i in (2, 0, 1):
            p = _dot(pltpu.bitcast(_cat(lhs[i]), BF16), pltpu.bitcast(ws_ref[i, n], BF16))
            if p3 is None:
                p3 = p
            else:
                p = p + p3
                for e, u in enumerate(us):
                    r, tp = divmod(u, 2)
                    qkv_ref[n, r, pl.ds((2 * tp + i) * LANES, LANES), :] = p[e * LANES:(e + 1) * LANES]

    vr_words = {}
    job_done = {}

    def side_dots(u, n):
        r, tp = divmod(u, 2)
        st = {}

        def one(i, parts=1):
            if parts > 1:
                lhs, rows = t_ref[u, i], 64 // parts
                p = _cat([_dot(pltpu.bitcast(lhs[q * rows:(q + 1) * rows], BF16),
                               pltpu.bitcast(ws_ref[i, n], BF16)) for q in range(parts)])
            elif n == 4:
                p = _dot_nt(pltpu.bitcast(ws_ref[i, 4, 0:32, :], BF16), pltpu.bitcast(t_ref[u, i], BF16))
            else:
                p = _dot(pltpu.bitcast(t_ref[u, i], BF16), pltpu.bitcast(ws_ref[i, n], BF16))
            st[i] = p if i == 2 else p + st[2]
            if n < 4 and i < 2:
                qkv_ref[n, r, pl.ds((2 * tp + i) * LANES, LANES), :] = st[i]
            elif i == 1:
                vr_words[u] = pltpu.pack_elementwise([st[0], st[1]], packed_dtype=BF16)

        return [(64 if n == 4 else LANES, (u, n, i), functools.partial(one, i)) for i in (2, 0, 1)]

    def vr_store(u):
        r, tp = divmod(u, 2)
        w = pltpu.bitcast(vr_words[u], F32)
        wt = pltpu.bitcast(_cat([w, w]).T, U32)
        job_done["v", u] = pltpu.bitcast(wt[120:128], F32)
        for j in range(2):
            qkv_ref[4, r, pl.ds((2 * tp + j) * LANES, LANES), :] = pltpu.unpack_elementwise(
                wt, index=j, packed_dtype=BF16, unpacked_dtype=F32)

    zero8 = jnp.zeros((8, LANES), F32)

    def gather(n, off):
        return [qkv_ref[n, r, pl.ds(off, 8), :] for r in range(WS)]

    def softmax_t(st):
        rows = _blocks(st)
        m = functools.reduce(jnp.maximum, rows)
        m = _allred(jnp.where(mk["key"], m, -jnp.inf), jnp.maximum)
        p = [jnp.exp2(x - m) for x in rows]
        return p, functools.reduce(jnp.add, p)

    def s2_pair(pi, offa):
        offb = offa + WS
        st = {}

        def vprep():
            g = [gather(n, offa) + gather(n, offb) for n in range(5)]
            u1 = [jnp.where(mk["left64"], z, jnp.where(mk["v"], x, y)) for x, y, z in zip(g[0], g[1], g[4])]
            u2 = [jnp.where(mk["v"], x, y) for x, y in zip(g[2], g[3])]
            u = jnp.concatenate([_cat(u1 + [zero8, zero8]), _cat(u2 + [zero8, zero8])], axis=1)
            vt = pltpu.bitcast(u.astype(BF16).T, U32)
            vt = _cat([vt[0:64], vt[96:128]])
            st["vt"] = [pltpu.bitcast(vt[24 * h:24 * h + 24], BF16) for h in range(NH)]

        def score(i, ties):
            hp, sw = divmod(i, 2)
            lo, hi = mk["lo"], mk["hi%d" % hp]
            ma, mb = (lo, hi) if sw == 0 else (hi, lo)
            q = _cat([jnp.where(ma, v, 0.0) for v in gather(hp, offa)]
                     + [jnp.where(mb, v, 0.0) for v in gather(hp, offb)] + [zero8, zero8])
            ka, kb = gather(2 + hp, offa), gather(2 + hp, offb)
            k = [jnp.where(lo, x, y) for x, y in (zip(ka, kb) if sw == 0 else zip(kb, ka))]
            for _, job in ties:
                k[0] = jnp.where(mk["never"], job(), k[0])
            st["p", i] = softmax_t(_dot_nt(_cat(k), q))

        def value(h):
            hp, sw = divmod(h, 2)
            (pa, sa), (pb, sb) = st["p", 2 * hp + sw], st["p", 2 * hp + 1 - sw]
            pm = _cat([jnp.where(mk["keep_a"], v, 0.0) for v in pa]
                      + [jnp.where(mk["keep_b"], v, 0.0) for v in pb] + [zero8, zero8])
            den = _allred(jnp.where(mk["keep_a"], sa, jnp.where(mk["keep_b"], sb, 0.0)), jnp.add)
            rec = pl.reciprocal(den, approx=True)
            st["o", h] = [b * rec for b in _blocks(_dot(st["vt"][h], pm))]

        def finish():
            o = [b for h in range(NH) for b in st["o", h]]
            w = pltpu.pack_elementwise([_cat(o[0:16]), _cat(o[16:24] + o[16:24])], packed_dtype=BF16)
            stg_ref[pi] = pltpu.bitcast(w, F32)

        def scatter():
            wt = stg_ref[pi].T
            job_done["s", pi] = wt[104:112]
            for i, off in enumerate((offa, offb)):
                for r in range(WS):
                    base = i * SLOTS + 8 * r
                    ob_ref[pl.ds(r * WP + off, WS), :] = wt[base:base + WS]

        return vprep, score, value, finish, scatter

    pairs = [s2_pair(p, min(2 * p, nwin - 2) * WS) for p in range(npair)]

    def s3_unit(r, tp, ties=()):
        def unpack(t):
            w = pltpu.bitcast(ob_ref[pl.ds(r * WP + t * LANES, LANES), :], U32)
            return [_blocks(pltpu.unpack_elementwise(w, index=i, packed_dtype=BF16, unpacked_dtype=F32))
                    for i in range(2)]

        (la, ha), (lb, hb) = unpack(2 * tp), unpack(2 * tp + 1)
        t3 = [jnp.where(mk["left64"], x, y) for x, y in zip(lb, ha)]
        t1 = _cat([x - y for x, y in zip(la, t3)])
        t2 = _cat([jnp.where(mk["left64"], x, z) - y for x, y, z in zip(hb, ha, lb)])
        t3 = _cat(t3)
        wo = [_blocks(wos_ref[i]) for i in range(3)]
        for q, (e, job) in enumerate(ties):
            blks = wo[(2, 0, 1)[q % 3]]
            blks[e] = jnp.where(mk["never"], pltpu.bitcast(job(), U32), blks[e])
        wo = [pltpu.bitcast(_cat(w), BF16) for w in wo]
        p3 = _dot_nt(wo[2], t3)
        ys = [_dot_nt(wo[i], t) + p3
              + x0_ref[rows_at(sc["prv"], (r * NT + 2 * tp + i) * C, C), :] for i, t in enumerate((t1, t2))]
        n = min(2 * LANES, W - 2 * tp * LANES)
        o_ref[sc["ooff"] + r, :, pl.ds(2 * tp * LANES, n)] = (
            jnp.concatenate(ys, axis=1).astype(o_ref.dtype)[:, :n])

    s3_all = [functools.partial(s3_unit, r, tp) for tp in range(2) for r in range(WS)]

    def block_x():
        new_scalars()
        njob = 28
        steps = wave_steps(0, NSTX)
        chunks = [(u, n) for u in range(NU) for n in range(4)]
        side = side_dots(*chunks.pop())
        for u in range(NU):
            side += side_dots(u, 4)
        for _ in range(8):
            side += side_dots(*chunks.pop())
        merged = []
        for u, n in chunks:
            prev = [c for c in merged if c[1] == n and c[0][0] // 2 == u // 2]
            if prev:
                prev[0][0].append(u)
            else:
                merged.append(([u], n))
        t_conv = (len(chunks) - 7) * LANES
        span = len(chunks) * LANES - t_conv
        plan, t, vr_ready = [], 0, {}
        for k, (us, n) in enumerate(merged):
            dur = LANES * len(us)
            assert not t < t_conv < t + dur
            lo, hi = (max(x - t_conv, 0) * len(steps) // span for x in (t, t + dur))
            plan.append((t, tuple(us), n, list(steps[lo:hi])))
            room = dur
            while side and (room > 0 or k == len(merged) - 1):
                rows, key, f = side.pop(0)
                plan.append((t, f if room > 0 else functools.partial(f, 4), None, []))
                room -= rows
                if key[1:] == (4, 1):
                    vr_ready[key[0]] = t + dur - room + 150
            t += dur
        ci = conv_items(4 * njob)
        fast = (t_conv - 4 * njob * 32.0) / (len(ci) - 4 * njob)
        t_piece = [min(min(j, 4 * njob) * 32.0 + max(j - 4 * njob, 0) * fast, t_conv)
                   for j in range(len(ci) + 1)]
        scat, vrs = list(range(npair)), list(range(NU))
        jobs = []
        for q in range(njob):
            if vrs and vr_ready[vrs[0]] <= t_piece[4 * q + 1]:
                jobs.append((t_piece[4 * q + 1], ("v", vrs[0])))
                ci[4 * q].insert(0, functools.partial(vr_store, vrs.pop(0)))
            elif scat:
                jobs.append((t_piece[4 * q + 1], ("s", scat[0])))
                ci[4 * q].insert(0, pairs[scat.pop(0)][4])
        extra = [(t_piece[j + 1], f) for j, fs in enumerate(ci) for f in fs]
        tail = ([(("v", u), functools.partial(vr_store, u)) for u in vrs]
                + [(("s", p), pairs[p][4]) for p in scat])
        for q, (key, f) in enumerate(tail):
            t_q = max(t_conv + 1 + (q // 3) * 128, vr_ready[key[1]] if key[0] == "v" else 0)
            extra.append((t_q, f))
            jobs.append((t_q, key))
        for t_q, key in jobs:
            later = [e for e in plan if e[2] is not None and e[0] >= t_q + 800]
            if later:
                later[0][3].insert(0, functools.partial(job_done.get, key))
        _run([(t0, u if n is None else functools.partial(qkv_chunk, u, n, st)) for t0, u, n, st in plan],
             extra)

    def block_y():
        new_scalars()
        pattern = "SFFVFFFF" + "SSSSFVVVV" * 8 + "SSSSVVVV"
        load = [0] * 4
        items, cnt = [], {"S": 0, "V": 0, "F": 0}
        for ch in pattern:
            for _ in range(1 if ch == "F" else 4):
                items.append((min(load), ch, cnt[ch], []))
                cnt[ch] += 1
                for x in {"S": [SLOTS], "V": [DH], "F": [C] * 3}[ch]:
                    load[load.index(min(load))] += x
        assert cnt == {"S": 4 * npair, "V": 4 * npair, "F": NU}
        spots = sorted([(it[0], it, 0) for it in items if it[1] == "S"]
                       + [(it[0] + 16 * e, it, e) for it in items if it[1] == "F" for e in range(12)],
                       key=lambda x: x[0])
        steps = wave_steps(NSTX, WS * NT)
        fspots = sorted([x for x in spots if x[1][1] == "F" and x[1][2] < 6 and x[2] >= 2],
                        key=lambda x: (x[1][2], x[2]))
        for q, step in enumerate(steps):
            _, it, e = fspots[q * len(fspots) // len(steps)]
            it[3].append((e, step))
        late = sorted([x for x in spots if x[1][1] == "S" and x[1][2] % 16 in (8, 12)],
                      key=lambda x: x[1][2])
        n1 = len(t_items) - len(late)
        extra = []
        for j, f in enumerate(t_items):
            if j < n1:
                t_s, it, e = [x for x in spots if x[0] >= 500 + j * 350 / n1][0]
            else:
                t_s, it, e = late[j - n1]
            it[3].append((e, functools.partial(t_done.get, j)))
            extra.append((min(t_s - 450, it[0]), f))
        prog = []
        for t0, ch, idx, ties in items:
            p, i = divmod(idx, 4)
            if ch == "S":
                if i == 0:
                    prog.append((t0, pairs[p][0]))
                prog.append((t0, functools.partial(pairs[p][1], i, ties)))
            elif ch == "V":
                prog.append((t0, functools.partial(pairs[p][2], i)))
                if i == 3:
                    extra.append((t0 + DH, pairs[p][3]))
            else:
                prog.append((t0, functools.partial(s3_all[idx], ties)))
        _run(prog, extra)

    if mode != "main":
        new_scalars()

    @when(k_ < nstrip, ("main",))
    def _():
        x_copy(k_).wait()

    @when(k_ < nstrip - 1, ("first", "main"))
    def _():
        x_copy(k_ + 1).start()

    new_masks("x")
    when(k_ <= nstrip, ("main",))(block_x)

    @when(k_ == 0, ("first",))
    def _():
        def body(g, carry):
            x0_copy(g).wait()
            for j in range(FG):
                piece = conv_group(pl.multiple_of((g * FG + j) * 8, 8))[1]
                for r in range(WS):
                    piece(r)
            return carry
        lax.fori_loop(0, NG // FG, body, 0)

    @when(k_ >= 4, ("main", "last"))
    def _():
        o_copy(k_ - 4).wait()

    @when(k_ >= 3, ("main", "last"))
    def _():
        o_copy(k_ - 3).start()

    new_masks("y")
    when((k_ <= nstrip) & (k_ >= 1), ("main",))(block_y)

    @when(k_ == 0, ("first",))
    def _():
        for j in range(WS * NT):
            for f in stats_steps(j):
                f()
        for f in t_items:
            f()

    @when(k_ == nstrip + 1, ("last",))
    def _():
        new_masks("y")
        for p in range(npair):
            pairs[p][4]()
        for q, f in enumerate(s3_all):
            f()
            if q >= WS:
                row_copy(q - WS).start()

    @when(k_ == nstrip + 1, ("last",))
    def _():
        o_copy(k_ - 3).wait()
        for r in range(WS):
            row_copy(r).wait()


@jax.jit
def pallas_standalone__window_attn_davit__vision_kernel(
    x: jax.Array,
    dw_pe: jax.Array,
    w_qkv: jax.Array,
    w_o: jax.Array,
):
    B, H, W, Cx = x.shape
    assert B == 1 and Cx == C and W == WP - 1 and H % WS == 0 and 3 <= H // WS <= 250
    xt = jnp.transpose(x[0], (0, 2, 1))

    vmem = pl.BlockSpec(memory_space=pltpu.VMEM)
    yt = pl.pallas_call(
        functools.partial(_kernel, H=H, W=W),
        in_specs=[pl.BlockSpec(memory_space=pl.ANY), vmem, vmem, vmem],
        out_specs=pl.BlockSpec(memory_space=pl.ANY),
        out_shape=jax.ShapeDtypeStruct((H, C, W), x.dtype),
        scratch_shapes=[
            pltpu.VMEM((2 * (WS + 2), C, W), x.dtype),
            pltpu.VMEM((2 * WS, C, W), x.dtype),
            pltpu.SemaphoreType.DMA((2 + NG // FG,)),
            pltpu.VMEM((X0_ROWS, LANES), F32),
            pltpu.VMEM((WS * WP, LANES), F32),
            pltpu.VMEM((9, C, LANES), F32),
            pltpu.VMEM((3, 5, LANES // 2, LANES), U32),
            pltpu.VMEM((3, C // 2, LANES), U32),
            pltpu.VMEM((5, WS, WP, LANES), F32),
            pltpu.VMEM((NU, 3, LANES // 2, LANES), U32),
            pltpu.VMEM(((W // WS + 1) // 2, LANES, LANES), F32),
            pltpu.VMEM((WS * NT, 16, LANES), F32),
            pltpu.VMEM((C, WP), F32),
        ],
        compiler_params=pltpu.CompilerParams(
            vmem_limit_bytes=64 * 1024 * 1024,
            disable_bounds_checks=True,
        ),
        name="davit_window_attn",
    )(xt, dw_pe, w_qkv, w_o)
    return jnp.transpose(yt, (0, 2, 1))[None]
```

```python
import functools
import math

import jax
import jax.numpy as jnp
from jax import lax
import jax.experimental.pallas as pl
import jax.experimental.pallas.tpu as pltpu

WS = 7
NH = 4
C = 192
DH = C // NH
NG = C // 8
LANES = 128
WP = 512
NT = WP // LANES
NU = WS * NT // 2
SLOTS = 8 * WS
EPS = 1e-5
F32 = jnp.float32
BF16 = jnp.bfloat16
U32 = jnp.uint32

X0_SLOT = WS * NT * C
DW_OFF = 3 * X0_SLOT
X0_ROWS = DW_OFF + 2 * C

FG = 8
NSTX = 24


def _dot(a, b):
    return jnp.dot(a, b, preferred_element_type=F32)


def _dot_nt(a, b):
    return lax.dot_general(a, b, (((1,), (1,)), ((), ())), preferred_element_type=F32)


def _cat(xs):
    return jnp.concatenate(xs, axis=0)


def _blocks(v):
    return [v[i:i + 8] for i in range(0, v.shape[0], 8)]


def _allred(x, op):
    for sh in (4, 2, 1):
        x = op(x, pltpu.roll(x, sh, 0))
    return x


def _round_bits(x):
    return pltpu.bitcast(x, U32) + jnp.uint32(0x8000)


def _hi(w):
    return w & jnp.uint32(0xFFFF0000)


def _halves(w):
    return pltpu.bitcast(w << 16, F32), pltpu.bitcast(_hi(w), F32)


def _run(prog, extra):
    extra = sorted(extra, key=lambda e: e[0])
    j = 0
    for t0, fn in prog:
        while j < len(extra) and extra[j][0] <= t0:
            extra[j][1]()
            j += 1
        fn()
    for e in extra[j:]:
        e[1]()


def _kernel(*refs, H, W):
    nstrip = H // WS
    for lo, hi, mode in ((0, 1, "first"), (1, nstrip + 1, "main"), (nstrip + 1, nstrip + 2, "last")):
        def body(k, carry, mode=mode):
            _step(*refs, H=H, W=W, k_=k, mode=mode)
            return carry
        lax.fori_loop(lo, hi, body, 0)


def _step(x_hbm, dw_ref, wqkv_ref, wo_ref, o_hbm,
          x_ref, o_ref, sems, x0_ref, ob_ref, dws_ref, ws_ref, wos_ref, qkv_ref, t_ref, stg_ref, ms_ref,
          top_ref, *, H, W, k_, mode):
    nstrip, nwin = H // WS, W // WS
    npair = (nwin + 1) // 2

    def x_copy(k):
        return pltpu.make_async_copy(x_hbm.at[pl.ds(jnp.minimum(k * WS, H - WS - 1), WS + 1)],
                                     x_ref.at[pl.ds((k & 1) * (WS + 2), WS + 1)], sems.at[0])

    def o_copy(k):
        return pltpu.make_async_copy(o_ref.at[pl.ds((k & 1) * WS, WS)], o_hbm.at[pl.ds(k * WS, WS)],
                                     sems.at[1])

    def x0_copy(g):
        cs = pl.ds(pl.multiple_of(g * (8 * FG), 8 * FG), 8 * FG)
        return pltpu.make_async_copy(x_hbm.at[pl.ds(0, WS + 1), cs], x_ref.at[pl.ds(0, WS + 1), cs],
                                     sems.at[2 + g])

    def row_copy(r):
        return pltpu.make_async_copy(o_ref.at[sc["ooff"] + r], o_hbm.at[H - WS + r], sems.at[2])

    def when(cond, modes):
        return pl.when(cond) if mode in modes else (lambda f: None)

    sc = {}

    def new_scalars():
        k3 = k_ - 3 * ((k_ * 171) >> 9)
        sc["nxt"] = k3 * X0_SLOT
        sc["prv"] = jnp.where((k3 == 2) | (k_ < 2), 0, sc["nxt"] + X0_SLOT)
        sc["xoff"] = (k_ & 1) * (WS + 2) + jnp.where(k_ >= nstrip - 1, 1, 0)
        sc["ooff"] = (k_ & 1) * WS

    dyn0 = jnp.minimum(k_, 0)

    def rows_at(base, off, n):
        if isinstance(base, int):
            return pl.ds(base + off, n)
        return pl.ds(pl.multiple_of(base + off, 8), n)

    mk = {}

    def new_masks(blk):
        lane = lax.broadcasted_iota(jnp.int32, (8, LANES), 1)
        mk.clear()
        mk["never"] = lane < dyn0
        if blk == "y":
            key_ok = lax.broadcasted_iota(jnp.int32, (8, LANES), 0) < WS
            mk.update(
                lo=lane < DH, hi0=(lane >= DH) & ((lane < 64) | (lane >= 96)),
                hi1=(lane >= DH) & (lane < 96), v=lane < 96, key=key_ok,
                keep_a=key_ok & (lane < SLOTS), keep_b=key_ok & (lane >= SLOTS), left64=lane < 64)

    conv_done = []

    def conv_group(c0):
        st = {}

        def row(i):
            if i == 0 and i not in st:
                st[i] = top_ref[pl.ds(c0, 8), :]
            if i not in st:
                v = x_ref[sc["xoff"] + (i - 1), pl.ds(c0, 8), :].astype(F32)
                st[i] = jnp.concatenate([v, jnp.zeros((8, WP - W), F32)], axis=1)
                if i == WS:
                    top_ref[pl.ds(c0, 8), :] = st[i]
            return st[i]

        def bc(v):
            return jnp.concatenate([v] * NT, axis=1)

        def taps(r):
            st["tw", r] = [bc(x0_ref[rows_at(c0, DW_OFF + k * C, 8), :]) for k in range(2)]

        def piece(r):
            if "w" not in st:
                st["w"] = [bc(dws_ref[k, pl.ds(c0, 8), :]) for k in range(9)]
            wts = list(st["w"])
            if ("tw", r) in st:
                wts[6], wts[8] = st["tw", r]
            row(r)
            abc = [row(r + 1) * wts[3 + j] + row(r) * wts[j] + row(r + 2) * wts[6 + j] for j in range(3)]
            x0 = pltpu.roll(abc[0], 1, 1) + abc[1] + pltpu.roll(abc[2], WP - 1, 1)
            for t in range(NT):
                x0_ref[rows_at(sc["nxt"], (r * NT + t) * C + c0, 8), :] = x0[:, t * LANES:(t + 1) * LANES]
            conv_done.append(r)

        return taps, piece

    def conv_items(nslow):
        groups = [conv_group(8 * g) for g in range(NG)]
        plist = [(g, r) for g in range(NG) for r in range(WS)]
        items, tap = [], 4
        for k, (g, r) in enumerate(plist):
            fs = []
            while tap <= min(k + (4 if k < nslow else 5), len(plist) - 1):
                fs.append(functools.partial(groups[plist[tap][0]][0], plist[tap][1]))
                tap += 1
            fs.append(functools.partial(groups[g][1], r))
            items.append(fs)
        return items

    @when(k_ == 0, ("first",))
    def _():
        for g in range(NG // FG):
            x0_copy(g).start()
        for k in range(9):
            w = dw_ref[k // 3].astype(F32)[k % 3:k % 3 + 1, :]
            w = jnp.broadcast_to(w, (LANES, C)).T
            dws_ref[k] = w + 1.0 if k == 4 else w
            if k in (6, 8):
                x0_ref[pl.ds(DW_OFF + (k - 6) // 2 * C, C), :] = w
        w = wqkv_ref[...].astype(F32)
        wq = w[:, 0:C] * ((DH ** -0.5) * math.log2(math.e))
        wk, wv = w[:, C:2 * C], w[:, 2 * C:3 * C]
        tiles = [(wq[:, 0:64], wv[:, 64:96], wq[:, 64:96]),
                 (wq[:, 96:192], wv[:, 96:128]),
                 (wk[:, 0:64], wv[:, 128:160], wk[:, 64:96]),
                 (wk[:, 96:192], wv[:, 160:192]),
                 (wv[:, 0:128],)]
        for n, parts in enumerate(tiles):
            w = jnp.concatenate(parts, axis=1)
            for i, wi in enumerate((w[0:128], w[64:192], _cat([w[0:64], w[128:192]]))):
                if n == 4:
                    wi = wi.T
                ws_ref[i, n] = pltpu.bitcast(wi.astype(BF16), U32)
        w = wo_ref[...].astype(F32)
        wx, wy, wz = w[0:64], w[64:128], w[128:192]
        for i, parts in enumerate(((wx, wy), (wz, wy), (wx, wy + wz))):
            wos_ref[i] = pltpu.bitcast(_cat(parts).T.astype(BF16), U32)

        top_ref[...] = jnp.zeros(top_ref.shape, F32)
        for i in (WS + 1, 2 * WS + 3):
            x_ref[i] = jnp.zeros(x_ref.shape[1:], x_ref.dtype)
        for p in range(npair):
            stg_ref[p] = jnp.zeros(stg_ref.shape[1:], F32)
        for r in range(WS):
            ob_ref[pl.ds(r * WP + WP - 8, 8), :] = jnp.zeros((8, LANES), F32)

    def ld_x0(j, k, gs):
        return [x0_ref[rows_at(sc["nxt"] + dyn0 * (8 * k), j * C + 8 * g, 8), :] for g in gs]

    def add2(acc, xs):
        a = functools.reduce(jnp.add, xs[0::2])
        b = functools.reduce(jnp.add, xs[1::2])
        return a + b if acc is None else (acc + a) + b

    stats_done = set()

    def stats_steps(j):
        st = {"s": None, "q": None}

        def sum_step(g0):
            assert mode != "main" or len(conv_done) == NG * WS
            st["s"] = add2(st["s"], ld_x0(j, 0, range(g0, g0 + 12)))
            if g0 + 12 == NG:
                st["s"] = _allred(st["s"], jnp.add) * (1.0 / C)
            return st["s"]

        def var_step(g0):
            d = [x - st["s"] for x in ld_x0(j, 1, range(g0, g0 + 6))]
            st["q"] = add2(st["q"], [x * x for x in d])
            return st["q"]

        def last_step():
            rs = lax.rsqrt(_allred(st["q"], jnp.add) * (1.0 / C) + EPS)
            ms_ref[j] = _cat([st["s"], rs])
            stats_done.add(j)
            return rs

        return ([functools.partial(sum_step, g) for g in range(0, NG, 12)]
                + [functools.partial(var_step, g) for g in range(0, NG, 6)] + [last_step])

    def wave_steps(lo, hi):
        steps = []
        for j0 in range(lo, hi, 4):
            for grp in zip(*[stats_steps(j) for j in range(j0, j0 + 4)]):
                steps += grp
        return steps

    def normed(j, blk):
        assert j in stats_done
        m, rs = ms_ref[j, 0:8, :], ms_ref[j, 8:16, :]
        return _cat([(x - m) * rs for x in ld_x0(j, 0, range(8 * blk, 8 * blk + 8))])

    t_done = {}

    def put_t(dst, tiles):
        tt = pltpu.bitcast(jnp.concatenate(tiles, axis=1).astype(BF16).T, U32)
        for i, (u, e) in enumerate(dst):
            t_ref[u, e] = tt[64 * i:64 * i + 64]
        t_done[len(t_done)] = pltpu.bitcast(tt[120:128], F32)

    def t_first(u):
        ja, jb = 2 * u, 2 * u + 1
        bx = normed(jb, 0)
        put_t([(u, 0), (u, 2)], [_cat([normed(ja, 0) - bx, normed(ja, 1)]), _cat([bx, normed(ja, 2)])])

    def t_second(r):
        put_t([(u, 1) for u in (2 * r, 2 * r + 1)],
              [_cat([normed(2 * u + 1, 1), normed(2 * u + 1, 2) - normed(2 * u, 2)])
               for u in (2 * r, 2 * r + 1)])

    t_items = []
    for r in range(WS):
        t_items += [functools.partial(t_first, 2 * r), functools.partial(t_first, 2 * r + 1),
                    functools.partial(t_second, r)]

    def qkv_chunk(us, n, steps):
        lhs = {i: [b for u in us for b in _blocks(t_ref[u, i])] for i in range(3)}
        for q, step in enumerate(steps):
            tok = pltpu.bitcast(step(), U32)
            q = q * 24 * len(us) // len(steps)
            blks = lhs[(2, 0, 1)[q % 3]]
            blks[q // 3] = jnp.where(mk["never"], tok, blks[q // 3])
        p3 = None
        for i in (2, 0, 1):
            p = _dot(pltpu.bitcast(_cat(lhs[i]), BF16), pltpu.bitcast(ws_ref[i, n], BF16))
            if p3 is None:
                p3 = p
            else:
                p = p + p3
                for e, u in enumerate(us):
                    r, tp = divmod(u, 2)
                    qkv_ref[n, r, pl.ds((2 * tp + i) * LANES, LANES), :] = p[e * LANES:(e + 1) * LANES]

    vr_words = {}
    job_done = {}

    def side_dots(u, n):
        r, tp = divmod(u, 2)
        st = {}

        def one(i, parts=1):
            if parts > 1:
                lhs, rows = t_ref[u, i], 64 // parts
                p = _cat([_dot(pltpu.bitcast(lhs[q * rows:(q + 1) * rows], BF16),
                               pltpu.bitcast(ws_ref[i, n], BF16)) for q in range(parts)])
            elif n == 4:
                p = _dot_nt(pltpu.bitcast(ws_ref[i, 4, 0:32, :], BF16), pltpu.bitcast(t_ref[u, i], BF16))
            else:
                p = _dot(pltpu.bitcast(t_ref[u, i], BF16), pltpu.bitcast(ws_ref[i, n], BF16))
            st[i] = p if i == 2 else p + st[2]
            if n < 4 and i < 2:
                qkv_ref[n, r, pl.ds((2 * tp + i) * LANES, LANES), :] = st[i]
            elif i == 1:
                vr_words[u] = (_round_bits(st[0]) >> 16) | _hi(_round_bits(st[1]))

        return [(64 if n == 4 else LANES, (u, n, i), functools.partial(one, i)) for i in (2, 0, 1)]

    def vr_store(u):
        r, tp = divmod(u, 2)
        w = pltpu.bitcast(vr_words[u], F32)
        wt = pltpu.bitcast(_cat([w, w]).T, U32)
        job_done["v", u] = pltpu.bitcast(wt[120:128], F32)
        for j in range(2):
            qkv_ref[4, r, pl.ds((2 * tp + j) * LANES, LANES), :] = _halves(wt)[j]

    zero8 = jnp.zeros((8, LANES), F32)

    def gather(n, off):
        return [qkv_ref[n, r, pl.ds(off, 8), :] for r in range(WS)]

    def softmax_t(st):
        rows = _blocks(st)
        m = functools.reduce(jnp.maximum, rows)
        m = _allred(jnp.where(mk["key"], m, -jnp.inf), jnp.maximum)
        p = [jnp.exp2(x - m) for x in rows]
        return p, functools.reduce(jnp.add, p)

    def s2_pair(pi, offa):
        offb = offa + WS
        st = {}

        def vprep():
            g = [gather(n, offa) + gather(n, offb) for n in range(5)]
            u1 = [jnp.where(mk["left64"], z, jnp.where(mk["v"], x, y)) for x, y, z in zip(g[0], g[1], g[4])]
            u2 = [jnp.where(mk["v"], x, y) for x, y in zip(g[2], g[3])]
            u = jnp.concatenate([_cat(u1 + [zero8, zero8]), _cat(u2 + [zero8, zero8])], axis=1)
            vt = pltpu.bitcast(u.astype(BF16).T, U32)
            vt = _cat([vt[0:64], vt[96:128]])
            st["vt"] = [pltpu.bitcast(vt[24 * h:24 * h + 24], BF16) for h in range(NH)]

        def score(i, ties):
            hp, sw = divmod(i, 2)
            lo, hi = mk["lo"], mk["hi%d" % hp]
            ma, mb = (lo, hi) if sw == 0 else (hi, lo)
            q = _cat([jnp.where(ma, v, 0.0) for v in gather(hp, offa)]
                     + [jnp.where(mb, v, 0.0) for v in gather(hp, offb)] + [zero8, zero8])
            ka, kb = gather(2 + hp, offa), gather(2 + hp, offb)
            k = [jnp.where(lo, x, y) for x, y in (zip(ka, kb) if sw == 0 else zip(kb, ka))]
            for _, job in ties:
                k[0] = jnp.where(mk["never"], job(), k[0])
            st["p", i] = softmax_t(_dot_nt(_cat(k), q))

        def value(h):
            hp, sw = divmod(h, 2)
            (pa, sa), (pb, sb) = st["p", 2 * hp + sw], st["p", 2 * hp + 1 - sw]
            pm = _cat([jnp.where(mk["keep_a"], v, 0.0) for v in pa]
                      + [jnp.where(mk["keep_b"], v, 0.0) for v in pb] + [zero8, zero8])
            den = _allred(jnp.where(mk["keep_a"], sa, jnp.where(mk["keep_b"], sb, 0.0)), jnp.add)
            rec = pl.reciprocal(den, approx=True)
            st["o", h] = [b * rec for b in _blocks(_dot(st["vt"][h], pm))]

        def finish():
            o = [_round_bits(b) for h in range(NH) for b in st["o", h]]
            hi = [_hi(b) for b in o[16:24]]
            w = _cat([(b >> 16) | z for b, z in zip(o[0:16], hi + hi)])
            stg_ref[pi] = pltpu.bitcast(w, F32)

        def scatter():
            wt = stg_ref[pi].T
            job_done["s", pi] = wt[104:112]
            for i, off in enumerate((offa, offb)):
                for r in range(WS):
                    base = i * SLOTS + 8 * r
                    ob_ref[pl.ds(r * WP + off, WS), :] = wt[base:base + WS]

        return vprep, score, value, finish, scatter

    pairs = [s2_pair(p, min(2 * p, nwin - 2) * WS) for p in range(npair)]

    def s3_unit(r, tp, ties=()):
        def unpack(t):
            w = pltpu.bitcast(ob_ref[pl.ds(r * WP + t * LANES, LANES), :], U32)
            return [_blocks(v) for v in _halves(w)]

        (la, ha), (lb, hb) = unpack(2 * tp), unpack(2 * tp + 1)
        t3 = [jnp.where(mk["left64"], x, y) for x, y in zip(lb, ha)]
        t1 = _cat([x - y for x, y in zip(la, t3)])
        t2 = _cat([jnp.where(mk["left64"], x, z) - y for x, y, z in zip(hb, ha, lb)])
        t3 = _cat(t3)
        wo = [_blocks(wos_ref[i]) for i in range(3)]
        for q, (e, job) in enumerate(ties):
            blks = wo[(2, 0, 1)[q % 3]]
            blks[e] = jnp.where(mk["never"], pltpu.bitcast(job(), U32), blks[e])
        wo = [pltpu.bitcast(_cat(w), BF16) for w in wo]
        p3 = _dot_nt(wo[2], t3)
        ys = [_dot_nt(wo[i], t) + p3
              + x0_ref[rows_at(sc["prv"], (r * NT + 2 * tp + i) * C, C), :] for i, t in enumerate((t1, t2))]
        n = min(2 * LANES, W - 2 * tp * LANES)
        o_ref[sc["ooff"] + r, :, pl.ds(2 * tp * LANES, n)] = (
            jnp.concatenate(ys, axis=1).astype(o_ref.dtype)[:, :n])

    s3_all = [functools.partial(s3_unit, r, tp) for tp in range(2) for r in range(WS)]

    def block_x():
        new_scalars()
        njob = 28
        steps = wave_steps(0, NSTX)
        chunks = [(u, n) for u in range(NU) for n in range(4)]
        side = side_dots(*chunks.pop())
        for u in range(NU):
            side += side_dots(u, 4)
        for _ in range(8):
            side += side_dots(*chunks.pop())
        merged = []
        for u, n in chunks:
            prev = [c for c in merged if c[1] == n and c[0][0] // 2 == u // 2]
            if prev:
                prev[0][0].append(u)
            else:
                merged.append(([u], n))
        t_conv = (len(chunks) - 7) * LANES
        span = len(chunks) * LANES - t_conv
        plan, t, vr_ready = [], 0, {}
        for k, (us, n) in enumerate(merged):
            dur = LANES * len(us)
            assert not t < t_conv < t + dur
            lo, hi = (max(x - t_conv, 0) * len(steps) // span for x in (t, t + dur))
            plan.append((t, tuple(us), n, list(steps[lo:hi])))
            room = dur
            while side and (room > 0 or k == len(merged) - 1):
                rows, key, f = side.pop(0)
                plan.append((t, f if room > 0 else functools.partial(f, 4), None, []))
                room -= rows
                if key[1:] == (4, 1):
                    vr_ready[key[0]] = t + dur - room + 150
            t += dur
        ci = conv_items(4 * njob)
        fast = (t_conv - 4 * njob * 32.0) / (len(ci) - 4 * njob)
        t_piece = [min(min(j, 4 * njob) * 32.0 + max(j - 4 * njob, 0) * fast, t_conv)
                   for j in range(len(ci) + 1)]
        scat, vrs = list(range(npair)), list(range(NU))
        jobs = []
        for q in range(njob):
            if vrs and vr_ready[vrs[0]] <= t_piece[4 * q + 1]:
                jobs.append((t_piece[4 * q + 1], ("v", vrs[0])))
                ci[4 * q].insert(0, functools.partial(vr_store, vrs.pop(0)))
            elif scat:
                jobs.append((t_piece[4 * q + 1], ("s", scat[0])))
                ci[4 * q].insert(0, pairs[scat.pop(0)][4])
        extra = [(t_piece[j + 1], f) for j, fs in enumerate(ci) for f in fs]
        tail = ([(("v", u), functools.partial(vr_store, u)) for u in vrs]
                + [(("s", p), pairs[p][4]) for p in scat])
        for q, (key, f) in enumerate(tail):
            t_q = max(t_conv + 1 + (q // 3) * 128, vr_ready[key[1]] if key[0] == "v" else 0)
            extra.append((t_q, f))
            jobs.append((t_q, key))
        for t_q, key in jobs:
            later = [e for e in plan if e[2] is not None and e[0] >= t_q + 800]
            if later:
                later[0][3].insert(0, functools.partial(job_done.get, key))
        _run([(t0, u if n is None else functools.partial(qkv_chunk, u, n, st)) for t0, u, n, st in plan],
             extra)

    def block_y():
        new_scalars()
        pattern = "SFFVFFFF" + "SSSSFVVVV" * 8 + "SSSSVVVV"
        load = [0] * 4
        items, cnt = [], {"S": 0, "V": 0, "F": 0}
        for ch in pattern:
            for _ in range(1 if ch == "F" else 4):
                items.append((min(load), ch, cnt[ch], []))
                cnt[ch] += 1
                for x in {"S": [SLOTS], "V": [DH], "F": [C] * 3}[ch]:
                    load[load.index(min(load))] += x
        assert cnt == {"S": 4 * npair, "V": 4 * npair, "F": NU}
        spots = sorted([(it[0], it, 0) for it in items if it[1] == "S"]
                       + [(it[0] + 16 * e, it, e) for it in items if it[1] == "F" for e in range(12)],
                       key=lambda x: x[0])
        steps = wave_steps(NSTX, WS * NT)
        fspots = sorted([x for x in spots if x[1][1] == "F" and x[1][2] < 6 and x[2] >= 2],
                        key=lambda x: (x[1][2], x[2]))
        for q, step in enumerate(steps):
            _, it, e = fspots[q * len(fspots) // len(steps)]
            it[3].append((e, step))
        late = sorted([x for x in spots if x[1][1] == "S" and x[1][2] % 16 in (8, 12)],
                      key=lambda x: x[1][2])
        n1 = len(t_items) - len(late)
        extra = []
        for j, f in enumerate(t_items):
            if j < n1:
                t_s, it, e = [x for x in spots if x[0] >= 500 + j * 350 / n1][0]
            else:
                t_s, it, e = late[j - n1]
            it[3].append((e, functools.partial(t_done.get, j)))
            extra.append((min(t_s - 450, it[0]), f))
        prog = []
        for t0, ch, idx, ties in items:
            p, i = divmod(idx, 4)
            if ch == "S":
                if i == 0:
                    prog.append((t0, pairs[p][0]))
                prog.append((t0, functools.partial(pairs[p][1], i, ties)))
            elif ch == "V":
                prog.append((t0, functools.partial(pairs[p][2], i)))
                if i == 3:
                    extra.append((t0 + DH, pairs[p][3]))
            else:
                prog.append((t0, functools.partial(s3_all[idx], ties)))
        _run(prog, extra)

    if mode != "main":
        new_scalars()

    @when(k_ < nstrip, ("main",))
    def _():
        x_copy(k_).wait()

    @when(k_ < nstrip - 1, ("first", "main"))
    def _():
        x_copy(k_ + 1).start()

    new_masks("x")
    when(k_ <= nstrip, ("main",))(block_x)

    @when(k_ == 0, ("first",))
    def _():
        def body(g, carry):
            x0_copy(g).wait()
            for j in range(FG):
                piece = conv_group(pl.multiple_of((g * FG + j) * 8, 8))[1]
                for r in range(WS):
                    piece(r)
            return carry
        lax.fori_loop(0, NG // FG, body, 0)

    @when(k_ >= 4, ("main", "last"))
    def _():
        o_copy(k_ - 4).wait()

    @when(k_ >= 3, ("main", "last"))
    def _():
        o_copy(k_ - 3).start()

    new_masks("y")
    when((k_ <= nstrip) & (k_ >= 1), ("main",))(block_y)

    @when(k_ == 0, ("first",))
    def _():
        for j in range(WS * NT):
            for f in stats_steps(j):
                f()
        for f in t_items:
            f()

    @when(k_ == nstrip + 1, ("last",))
    def _():
        new_masks("y")
        for p in range(npair):
            pairs[p][4]()
        for q, f in enumerate(s3_all):
            f()
            if q >= WS:
                row_copy(q - WS).start()

    @when(k_ == nstrip + 1, ("last",))
    def _():
        o_copy(k_ - 3).wait()
        for r in range(WS):
            row_copy(r).wait()


@jax.jit
def pallas_standalone__window_attn_davit__vision_kernel(
    x: jax.Array,
    dw_pe: jax.Array,
    w_qkv: jax.Array,
    w_o: jax.Array,
):
    B, H, W, Cx = x.shape
    assert B == 1 and Cx == C and W == WP - 1 and H % WS == 0 and 3 <= H // WS <= 250
    xt = jnp.transpose(x[0], (0, 2, 1))

    vmem = pl.BlockSpec(memory_space=pltpu.VMEM)
    yt = pl.pallas_call(
        functools.partial(_kernel, H=H, W=W),
        in_specs=[pl.BlockSpec(memory_space=pl.ANY), vmem, vmem, vmem],
        out_specs=pl.BlockSpec(memory_space=pl.ANY),
        out_shape=jax.ShapeDtypeStruct((H, C, W), x.dtype),
        scratch_shapes=[
            pltpu.VMEM((2 * (WS + 2), C, W), x.dtype),
            pltpu.VMEM((2 * WS, C, W), x.dtype),
            pltpu.SemaphoreType.DMA((2 + NG // FG,)),
            pltpu.VMEM((X0_ROWS, LANES), F32),
            pltpu.VMEM((WS * WP, LANES), F32),
            pltpu.VMEM((9, C, LANES), F32),
            pltpu.VMEM((3, 5, LANES // 2, LANES), U32),
            pltpu.VMEM((3, C // 2, LANES), U32),
            pltpu.VMEM((5, WS, WP + 8, LANES), F32),
            pltpu.VMEM((NU, 3, LANES // 2, LANES), U32),
            pltpu.VMEM(((W // WS + 1) // 2, LANES, LANES), F32),
            pltpu.VMEM((WS * NT, 16, LANES), F32),
            pltpu.VMEM((C, WP), F32),
        ],
        compiler_params=pltpu.CompilerParams(
            vmem_limit_bytes=64 * 1024 * 1024,
            disable_bounds_checks=True,
        ),
        name="davit_window_attn",
    )(xt, dw_pe, w_qkv, w_o)
    return jnp.transpose(yt, (0, 2, 1))[None]
```

```python
import functools
import math

import jax
import jax.numpy as jnp
from jax import lax
import jax.experimental.pallas as pl
import jax.experimental.pallas.tpu as pltpu

WS = 7
NH = 4
C = 192
DH = C // NH
NG = C // 8
LANES = 128
WP = 512
NT = WP // LANES
NU = WS * NT // 2
SLOTS = 8 * WS
EPS = 1e-5
F32 = jnp.float32
BF16 = jnp.bfloat16
U32 = jnp.uint32

X0_SLOT = WS * NT * C
DW_OFF = 3 * X0_SLOT
X0_ROWS = DW_OFF + 2 * C

FG = 8
NSTX = 24


def _dot(a, b):
    return jnp.dot(a, b, preferred_element_type=F32)


def _dot_nt(a, b):
    return lax.dot_general(a, b, (((1,), (1,)), ((), ())), preferred_element_type=F32)


def _cat(xs):
    return jnp.concatenate(xs, axis=0)


def _blocks(v):
    return [v[i:i + 8] for i in range(0, v.shape[0], 8)]


def _allred(x, op):
    for sh in (4, 2, 1):
        x = op(x, pltpu.roll(x, sh, 0))
    return x


def _round_bits(x):
    return pltpu.bitcast(x, U32) + jnp.uint32(0x8000)


def _hi(w):
    return w & jnp.uint32(0xFFFF0000)


def _halves(w):
    return pltpu.bitcast(w << 16, F32), pltpu.bitcast(_hi(w), F32)


def _run(prog, extra):
    extra = sorted(extra, key=lambda e: e[0])
    j = 0
    for t0, fn in prog:
        while j < len(extra) and extra[j][0] <= t0:
            extra[j][1]()
            j += 1
        fn()
    for e in extra[j:]:
        e[1]()


def _kernel(*refs, H, W):
    nstrip = H // WS
    for lo, hi, mode in ((0, 1, "first"), (1, nstrip + 1, "main"), (nstrip + 1, nstrip + 2, "last")):
        def body(k, carry, mode=mode):
            _step(*refs, H=H, W=W, k_=k, mode=mode)
            return carry
        lax.fori_loop(lo, hi, body, 0)


def _step(x_hbm, dw_ref, wqkv_ref, wo_ref, o_hbm,
          x_ref, o_ref, sems, x0_ref, ob_ref, dws_ref, ws_ref, wos_ref, qkv_ref, t_ref, stg_ref, ms_ref,
          top_ref, *, H, W, k_, mode):
    nstrip, nwin = H // WS, W // WS
    npair = (nwin + 1) // 2

    def x_copy(k):
        return pltpu.make_async_copy(x_hbm.at[pl.ds(jnp.minimum(k * WS, H - WS - 1), WS + 1)],
                                     x_ref.at[pl.ds((k & 1) * (WS + 2), WS + 1)], sems.at[0])

    def o_copy(k):
        return pltpu.make_async_copy(o_ref.at[pl.ds((k & 1) * WS, WS)], o_hbm.at[pl.ds(k * WS, WS)],
                                     sems.at[1])

    def x0_copy(g):
        cs = pl.ds(pl.multiple_of(g * (8 * FG), 8 * FG), 8 * FG)
        return pltpu.make_async_copy(x_hbm.at[pl.ds(0, WS + 1), cs], x_ref.at[pl.ds(0, WS + 1), cs],
                                     sems.at[2 + g])

    def row_copy(r):
        return pltpu.make_async_copy(o_ref.at[sc["ooff"] + r], o_hbm.at[H - WS + r], sems.at[2])

    def when(cond, modes):
        return pl.when(cond) if mode in modes else (lambda f: None)

    sc = {}

    def new_scalars():
        k3 = k_ - 3 * ((k_ * 171) >> 9)
        sc["nxt"] = k3 * X0_SLOT
        sc["prv"] = jnp.where((k3 == 2) | (k_ < 2), 0, sc["nxt"] + X0_SLOT)
        sc["xoff"] = (k_ & 1) * (WS + 2) + jnp.where(k_ >= nstrip - 1, 1, 0)
        sc["ooff"] = (k_ & 1) * WS

    dyn0 = jnp.minimum(k_, 0)

    def rows_at(base, off, n):
        if isinstance(base, int):
            return pl.ds(base + off, n)
        return pl.ds(pl.multiple_of(base + off, 8), n)

    mk = {}

    def new_masks(blk):
        lane = lax.broadcasted_iota(jnp.int32, (8, LANES), 1)
        mk.clear()
        mk["never"] = lane < dyn0
        if blk == "y":
            key_ok = lax.broadcasted_iota(jnp.int32, (8, LANES), 0) < WS
            mk.update(
                lo=lane < DH, hi0=(lane >= DH) & ((lane < 64) | (lane >= 96)),
                hi1=(lane >= DH) & (lane < 96), v=lane < 96, key=key_ok,
                keep_a=key_ok & (lane < SLOTS), keep_b=key_ok & (lane >= SLOTS), left64=lane < 64)

    conv_done = []

    def conv_group(c0):
        st = {}

        def row(i):
            if i == 0 and i not in st:
                st[i] = top_ref[pl.ds(c0, 8), :]
            if i not in st:
                v = x_ref[sc["xoff"] + (i - 1), pl.ds(c0, 8), :].astype(F32)
                st[i] = jnp.concatenate([v, jnp.zeros((8, WP - W), F32)], axis=1)
                if i == WS:
                    top_ref[pl.ds(c0, 8), :] = st[i]
            return st[i]

        def bc(v):
            return jnp.concatenate([v] * NT, axis=1)

        def taps(r):
            st["tw", r] = [bc(x0_ref[rows_at(c0, DW_OFF + k * C, 8), :]) for k in range(2)]

        def piece(r):
            if "w" not in st:
                st["w"] = [bc(dws_ref[k, pl.ds(c0, 8), :]) for k in range(9)]
            wts = list(st["w"])
            if ("tw", r) in st:
                wts[6], wts[8] = st["tw", r]
            row(r)
            abc = [row(r + 1) * wts[3 + j] + row(r) * wts[j] + row(r + 2) * wts[6 + j] for j in range(3)]
            x0 = pltpu.roll(abc[0], 1, 1) + abc[1] + pltpu.roll(abc[2], WP - 1, 1)
            for t in range(NT):
                x0_ref[rows_at(sc["nxt"], (r * NT + t) * C + c0, 8), :] = x0[:, t * LANES:(t + 1) * LANES]
            conv_done.append(r)

        return taps, piece

    def conv_items(nslow):
        groups = [conv_group(8 * g) for g in range(NG)]
        plist = [(g, r) for g in range(NG) for r in range(WS)]
        items, tap = [], 4
        for k, (g, r) in enumerate(plist):
            fs = []
            while tap <= min(k + (4 if k < nslow else 5), len(plist) - 1):
                fs.append(functools.partial(groups[plist[tap][0]][0], plist[tap][1]))
                tap += 1
            fs.append(functools.partial(groups[g][1], r))
            items.append(fs)
        return items

    @when(k_ == 0, ("first",))
    def _():
        for g in range(NG // FG):
            x0_copy(g).start()
        for k in range(9):
            w = dw_ref[k // 3].astype(F32)[k % 3:k % 3 + 1, :]
            w = jnp.broadcast_to(w, (LANES, C)).T
            dws_ref[k] = w + 1.0 if k == 4 else w
            if k in (6, 8):
                x0_ref[pl.ds(DW_OFF + (k - 6) // 2 * C, C), :] = w
        w = wqkv_ref[...].astype(F32)
        wq = w[:, 0:C] * ((DH ** -0.5) * math.log2(math.e))
        wk, wv = w[:, C:2 * C], w[:, 2 * C:3 * C]
        tiles = [(wq[:, 0:64], wv[:, 64:96], wq[:, 64:96]),
                 (wq[:, 96:192], wv[:, 96:128]),
                 (wk[:, 0:64], wv[:, 128:160], wk[:, 64:96]),
                 (wk[:, 96:192], wv[:, 160:192]),
                 (wv[:, 0:128],)]
        for n, parts in enumerate(tiles):
            w = jnp.concatenate(parts, axis=1)
            for i, wi in enumerate((w[0:128], w[64:192], _cat([w[0:64], w[128:192]]))):
                if n == 4:
                    wi = wi.T
                ws_ref[i, n] = pltpu.bitcast(wi.astype(BF16), U32)
        w = wo_ref[...].astype(F32)
        wx, wy, wz = w[0:64], w[64:128], w[128:192]
        for i, parts in enumerate(((wx, wy), (wz, wy), (wx, wy + wz))):
            wos_ref[i] = pltpu.bitcast(_cat(parts).T.astype(BF16), U32)

        top_ref[...] = jnp.zeros(top_ref.shape, F32)
        for i in (WS + 1, 2 * WS + 3):
            x_ref[i] = jnp.zeros(x_ref.shape[1:], x_ref.dtype)
        for p in range(npair):
            stg_ref[p] = jnp.zeros(stg_ref.shape[1:], F32)
        for r in range(WS):
            ob_ref[pl.ds(r * WP + WP - 8, 8), :] = jnp.zeros((8, LANES), F32)

    def ld_x0(j, k, gs):
        return [x0_ref[rows_at(sc["nxt"] + dyn0 * (8 * k), j * C + 8 * g, 8), :] for g in gs]

    def add2(acc, xs):
        a = functools.reduce(jnp.add, xs[0::2])
        b = functools.reduce(jnp.add, xs[1::2])
        return a + b if acc is None else (acc + a) + b

    stats_done = set()

    def stats_steps(j):
        st = {"s": None, "q": None}

        def sum_step(g0):
            assert mode != "main" or len(conv_done) == NG * WS
            st["s"] = add2(st["s"], ld_x0(j, 0, range(g0, g0 + 12)))
            if g0 + 12 == NG:
                st["s"] = _allred(st["s"], jnp.add) * (1.0 / C)
            return st["s"]

        def var_step(g0):
            d = [x - st["s"] for x in ld_x0(j, 1, range(g0, g0 + 6))]
            st["q"] = add2(st["q"], [x * x for x in d])
            return st["q"]

        def last_step():
            rs = lax.rsqrt(_allred(st["q"], jnp.add) * (1.0 / C) + EPS)
            ms_ref[j] = _cat([st["s"], rs])
            stats_done.add(j)
            return rs

        return ([functools.partial(sum_step, g) for g in range(0, NG, 12)]
                + [functools.partial(var_step, g) for g in range(0, NG, 6)] + [last_step])

    def wave_steps(lo, hi):
        steps = []
        for j0 in range(lo, hi, 4):
            for grp in zip(*[stats_steps(j) for j in range(j0, j0 + 4)]):
                steps += grp
        return steps

    def normed(j, blk, k=0):
        assert j in stats_done
        m, rs = ms_ref[j, 0:8, :], ms_ref[j, 8:16, :]
        return _cat([(x - m) * rs for x in ld_x0(j, k, range(8 * blk, 8 * blk + 8))])

    t_done = {}

    def put_t(dst, tiles):
        tt = pltpu.bitcast(jnp.concatenate(tiles, axis=1).astype(BF16).T, U32)
        for i, (u, e) in enumerate(dst):
            t_ref[u, e] = tt[64 * i:64 * i + 64]
        t_done[len(t_done)] = pltpu.bitcast(tt[120:128], F32)

    def t_first(u):
        ja, jb = 2 * u, 2 * u + 1
        bx = normed(jb, 0)
        put_t([(u, 0), (u, 2)], [_cat([normed(ja, 0) - bx, normed(ja, 1)]), _cat([bx, normed(ja, 2)])])

    def t_second(r):
        put_t([(u, 1) for u in (2 * r, 2 * r + 1)],
              [_cat([normed(2 * u + 1, 1), normed(2 * u + 1, 2) - normed(2 * u, 2, 1)])
               for u in (2 * r, 2 * r + 1)])

    t_items = []
    for r in range(WS):
        t_items += [functools.partial(t_first, 2 * r), functools.partial(t_first, 2 * r + 1),
                    functools.partial(t_second, r)]

    def qkv_chunk(us, n, steps):
        lhs = {i: [b for u in us for b in _blocks(t_ref[u, i])] for i in range(3)}
        for q, step in enumerate(steps):
            tok = pltpu.bitcast(step(), U32)
            q = q * 24 * len(us) // len(steps)
            blks = lhs[(2, 0, 1)[q % 3]]
            blks[q // 3] = jnp.where(mk["never"], tok, blks[q // 3])
        p3 = None
        for i in (2, 0, 1):
            p = _dot(pltpu.bitcast(_cat(lhs[i]), BF16), pltpu.bitcast(ws_ref[i, n], BF16))
            if p3 is None:
                p3 = p
            else:
                p = p + p3
                for e, u in enumerate(us):
                    r, tp = divmod(u, 2)
                    qkv_ref[n, r, pl.ds((2 * tp + i) * LANES, LANES), :] = p[e * LANES:(e + 1) * LANES]

    vr_words = {}
    job_done = {}

    def side_dots(u, n):
        r, tp = divmod(u, 2)
        st = {}

        def one(i, parts=1):
            if parts > 1:
                lhs, rows = t_ref[u, i], 64 // parts
                p = _cat([_dot(pltpu.bitcast(lhs[q * rows:(q + 1) * rows], BF16),
                               pltpu.bitcast(ws_ref[i, n], BF16)) for q in range(parts)])
            elif n == 4:
                p = _dot_nt(pltpu.bitcast(ws_ref[i, 4, 0:32, :], BF16), pltpu.bitcast(t_ref[u, i], BF16))
            else:
                p = _dot(pltpu.bitcast(t_ref[u, i], BF16), pltpu.bitcast(ws_ref[i, n], BF16))
            st[i] = p if i == 2 else p + st[2]
            if n < 4 and i < 2:
                qkv_ref[n, r, pl.ds((2 * tp + i) * LANES, LANES), :] = st[i]
            elif i == 1:
                vr_words[u] = (_round_bits(st[0]) >> 16) | _hi(_round_bits(st[1]))

        return [(64 if n == 4 else LANES, (u, n, i), functools.partial(one, i)) for i in (2, 0, 1)]

    def vr_store(u):
        r, tp = divmod(u, 2)
        w = pltpu.bitcast(vr_words[u], F32)
        wt = pltpu.bitcast(_cat([w, w]).T, U32)
        job_done["v", u] = pltpu.bitcast(wt[120:128], F32)
        for j in range(2):
            qkv_ref[4, r, pl.ds((2 * tp + j) * LANES, LANES), :] = _halves(wt)[j]

    zero8 = jnp.zeros((8, LANES), F32)

    def gather(n, off):
        return [qkv_ref[n, r, pl.ds(off, 8), :] for r in range(WS)]

    def softmax_t(st):
        rows = _blocks(st)
        m = functools.reduce(jnp.maximum, rows)
        m = _allred(jnp.where(mk["key"], m, -jnp.inf), jnp.maximum)
        p = [jnp.exp2(x - m) for x in rows]
        return p, functools.reduce(jnp.add, p)

    def s2_pair(pi, offa):
        offb = offa + WS
        st = {}

        def vprep():
            g = [gather(n, a) + gather(n, b) for n in range(5)
                 for a, b in [(offa + dyn0 * 3, offb + dyn0 * 3) if n in (2, 3) else (offa, offb)]]
            u1 = [jnp.where(mk["left64"], z, jnp.where(mk["v"], x, y)) for x, y, z in zip(g[0], g[1], g[4])]
            u2 = [jnp.where(mk["v"], x, y) for x, y in zip(g[2], g[3])]
            u = jnp.concatenate([_cat(u1 + [zero8, zero8]), _cat(u2 + [zero8, zero8])], axis=1)
            vt = pltpu.bitcast(u.astype(BF16).T, U32)
            vt = _cat([vt[0:64], vt[96:128]])
            st["vt"] = [pltpu.bitcast(vt[24 * h:24 * h + 24], BF16) for h in range(NH)]

        def score(i, ties):
            hp, sw = divmod(i, 2)
            lo, hi = mk["lo"], mk["hi%d" % hp]
            ma, mb = (lo, hi) if sw == 0 else (hi, lo)
            q = _cat([jnp.where(ma, v, 0.0) for v in gather(hp, offa)]
                     + [jnp.where(mb, v, 0.0) for v in gather(hp, offb)] + [zero8, zero8])
            ka, kb = gather(2 + hp, offa), gather(2 + hp, offb)
            k = [jnp.where(lo, x, y) for x, y in (zip(ka, kb) if sw == 0 else zip(kb, ka))]
            for _, job in ties:
                k[0] = jnp.where(mk["never"], job(), k[0])
            st["p", i] = softmax_t(_dot_nt(_cat(k), q))

        def value(h):
            hp, sw = divmod(h, 2)
            (pa, sa), (pb, sb) = st["p", 2 * hp + sw], st["p", 2 * hp + 1 - sw]
            pm = _cat([jnp.where(mk["keep_a"], v, 0.0) for v in pa]
                      + [jnp.where(mk["keep_b"], v, 0.0) for v in pb] + [zero8, zero8])
            den = _allred(jnp.where(mk["keep_a"], sa, jnp.where(mk["keep_b"], sb, 0.0)), jnp.add)
            rec = pl.reciprocal(den, approx=True)
            st["o", h] = [b * rec for b in _blocks(_dot(st["vt"][h], pm))]

        def finish():
            o = [_round_bits(b) for h in range(NH) for b in st["o", h]]
            hi = [_hi(b) for b in o[16:24]]
            w = _cat([(b >> 16) | z for b, z in zip(o[0:16], hi + hi)])
            stg_ref[pi] = pltpu.bitcast(w, F32)

        def scatter():
            wt = stg_ref[pi].T
            job_done["s", pi] = wt[104:112]
            for i, off in enumerate((offa, offb)):
                for r in range(WS):
                    base = i * SLOTS + 8 * r
                    ob_ref[pl.ds(r * WP + off, WS), :] = wt[base:base + WS]

        return vprep, score, value, finish, scatter

    pairs = [s2_pair(p, min(2 * p, nwin - 2) * WS) for p in range(npair)]

    def s3_unit(r, tp, ties=()):
        def unpack(t):
            w = pltpu.bitcast(ob_ref[pl.ds(r * WP + t * LANES, LANES), :], U32)
            return [_blocks(v) for v in _halves(w)]

        (la, ha), (lb, hb) = unpack(2 * tp), unpack(2 * tp + 1)
        t3 = [jnp.where(mk["left64"], x, y) for x, y in zip(lb, ha)]
        t1 = _cat([x - y for x, y in zip(la, t3)])
        t2 = _cat([jnp.where(mk["left64"], x, z) - y for x, y, z in zip(hb, ha, lb)])
        t3 = _cat(t3)
        wo = [_blocks(wos_ref[i]) for i in range(3)]
        for q, (e, job) in enumerate(ties):
            blks = wo[(2, 0, 1)[q % 3]]
            blks[e] = jnp.where(mk["never"], pltpu.bitcast(job(), U32), blks[e])
        wo = [pltpu.bitcast(_cat(w), BF16) for w in wo]
        p3 = _dot_nt(wo[2], t3)
        ys = [_dot_nt(wo[i], t) + p3
              + x0_ref[rows_at(sc["prv"], (r * NT + 2 * tp + i) * C, C), :] for i, t in enumerate((t1, t2))]
        n = min(2 * LANES, W - 2 * tp * LANES)
        o_ref[sc["ooff"] + r, :, pl.ds(2 * tp * LANES, n)] = (
            jnp.concatenate(ys, axis=1).astype(o_ref.dtype)[:, :n])

    s3_all = [functools.partial(s3_unit, r, tp) for tp in range(2) for r in range(WS)]

    def block_x():
        new_scalars()
        njob = 28
        steps = wave_steps(0, NSTX)
        chunks = [(u, n) for u in range(NU) for n in range(4)]
        side = side_dots(*chunks.pop())
        for u in range(NU):
            side += side_dots(u, 4)
        for _ in range(8):
            side += side_dots(*chunks.pop())
        merged = []
        for u, n in chunks:
            prev = [c for c in merged if c[1] == n and c[0][0] // 2 == u // 2]
            if prev:
                prev[0][0].append(u)
            else:
                merged.append(([u], n))
        t_conv = (len(chunks) - 7) * LANES
        span = len(chunks) * LANES - t_conv
        plan, t, vr_ready = [], 0, {}
        for k, (us, n) in enumerate(merged):
            dur = LANES * len(us)
            assert not t < t_conv < t + dur
            lo, hi = (max(x - t_conv, 0) * len(steps) // span for x in (t, t + dur))
            plan.append((t, tuple(us), n, list(steps[lo:hi])))
            room = dur
            while side and (room > 0 or k == len(merged) - 1):
                rows, key, f = side.pop(0)
                plan.append((t, f if room > 0 else functools.partial(f, 4), None, []))
                room -= rows
                if key[1:] == (4, 1):
                    vr_ready[key[0]] = t + dur - room + 150
            t += dur
        ci = conv_items(4 * njob)
        fast = (t_conv - 4 * njob * 32.0) / (len(ci) - 4 * njob)
        t_piece = [min(min(j, 4 * njob) * 32.0 + max(j - 4 * njob, 0) * fast, t_conv)
                   for j in range(len(ci) + 1)]
        scat, vrs = list(range(npair)), list(range(NU))
        jobs = []
        for q in range(njob):
            if vrs and vr_ready[vrs[0]] <= t_piece[4 * q + 1]:
                jobs.append((t_piece[4 * q + 1], ("v", vrs[0])))
                ci[4 * q].insert(0, functools.partial(vr_store, vrs.pop(0)))
            elif scat:
                jobs.append((t_piece[4 * q + 1], ("s", scat[0])))
                ci[4 * q].insert(0, pairs[scat.pop(0)][4])
        extra = [(t_piece[j + 1], f) for j, fs in enumerate(ci) for f in fs]
        tail = ([(("v", u), functools.partial(vr_store, u)) for u in vrs]
                + [(("s", p), pairs[p][4]) for p in scat])
        for q, (key, f) in enumerate(tail):
            t_q = max(t_conv + 1 + (q // 3) * 128, vr_ready[key[1]] if key[0] == "v" else 0)
            extra.append((t_q, f))
            jobs.append((t_q, key))
        for t_q, key in jobs:
            later = [e for e in plan if e[2] is not None and e[0] >= t_q + 800]
            if later:
                later[0][3].insert(0, functools.partial(job_done.get, key))
        _run([(t0, u if n is None else functools.partial(qkv_chunk, u, n, st)) for t0, u, n, st in plan],
             extra)

    def block_y():
        new_scalars()
        pattern = "SFFVFFFF" + "SSSSFVVVV" * 8 + "SSSSVVVV"
        load = [0] * 4
        items, cnt = [], {"S": 0, "V": 0, "F": 0}
        for ch in pattern:
            for _ in range(1 if ch == "F" else 4):
                items.append((min(load), ch, cnt[ch], []))
                cnt[ch] += 1
                for x in {"S": [SLOTS], "V": [DH], "F": [C] * 3}[ch]:
                    load[load.index(min(load))] += x
        assert cnt == {"S": 4 * npair, "V": 4 * npair, "F": NU}
        spots = sorted([(it[0], it, 0) for it in items if it[1] == "S"]
                       + [(it[0] + 16 * e, it, e) for it in items if it[1] == "F" for e in range(12)],
                       key=lambda x: x[0])
        steps = wave_steps(NSTX, WS * NT)
        fspots = sorted([x for x in spots if x[1][1] == "F" and x[1][2] < 6 and x[2] >= 2],
                        key=lambda x: (x[1][2], x[2]))
        for q, step in enumerate(steps):
            _, it, e = fspots[q * len(fspots) // len(steps)]
            it[3].append((e, step))
        late = sorted([x for x in spots if x[1][1] == "S" and x[1][2] % 16 in (13, 15)],
                      key=lambda x: x[1][2])
        n1 = len(t_items) - len(late)
        extra = []
        for j, f in enumerate(t_items):
            if j < n1:
                t_s, it, e = [x for x in spots if x[0] >= 500 + j * 350 / n1][0]
            else:
                t_s, it, e = late[j - n1]
            it[3].append((e, functools.partial(t_done.get, j)))
            extra.append((min(t_s - 450, it[0]), f))
        prog = []
        for t0, ch, idx, ties in items:
            p, i = divmod(idx, 4)
            if ch == "S":
                if i == 0:
                    prog.append((t0, pairs[p][0]))
                prog.append((t0, functools.partial(pairs[p][1], i, ties)))
            elif ch == "V":
                prog.append((t0, functools.partial(pairs[p][2], i)))
                if i == 3:
                    extra.append((t0 + DH, pairs[p][3]))
            else:
                prog.append((t0, functools.partial(s3_all[idx], ties)))
        _run(prog, extra)

    if mode != "main":
        new_scalars()

    @when(k_ < nstrip, ("main",))
    def _():
        x_copy(k_).wait()

    @when(k_ < nstrip - 1, ("first", "main"))
    def _():
        x_copy(k_ + 1).start()

    new_masks("x")
    when(k_ <= nstrip, ("main",))(block_x)

    @when(k_ == 0, ("first",))
    def _():
        def body(g, carry):
            x0_copy(g).wait()
            for j in range(FG):
                piece = conv_group(pl.multiple_of((g * FG + j) * 8, 8))[1]
                for r in range(WS):
                    piece(r)
            return carry
        lax.fori_loop(0, NG // FG, body, 0)

    @when(k_ >= 4, ("main", "last"))
    def _():
        o_copy(k_ - 4).wait()

    @when(k_ >= 3, ("main", "last"))
    def _():
        o_copy(k_ - 3).start()

    new_masks("y")
    when((k_ <= nstrip) & (k_ >= 1), ("main",))(block_y)

    @when(k_ == 0, ("first",))
    def _():
        for j in range(WS * NT):
            for f in stats_steps(j):
                f()
        for f in t_items:
            f()

    @when(k_ == nstrip + 1, ("last",))
    def _():
        new_masks("y")
        for p in range(npair):
            pairs[p][4]()
        for q, f in enumerate(s3_all):
            f()
            if q >= WS:
                row_copy(q - WS).start()

    @when(k_ == nstrip + 1, ("last",))
    def _():
        o_copy(k_ - 3).wait()
        for r in range(WS):
            row_copy(r).wait()


@jax.jit
def pallas_standalone__window_attn_davit__vision_kernel(
    x: jax.Array,
    dw_pe: jax.Array,
    w_qkv: jax.Array,
    w_o: jax.Array,
):
    B, H, W, Cx = x.shape
    assert B == 1 and Cx == C and W == WP - 1 and H % WS == 0 and 3 <= H // WS <= 250
    xt = jnp.transpose(x[0], (0, 2, 1))

    vmem = pl.BlockSpec(memory_space=pltpu.VMEM)
    yt = pl.pallas_call(
        functools.partial(_kernel, H=H, W=W),
        in_specs=[pl.BlockSpec(memory_space=pl.ANY), vmem, vmem, vmem],
        out_specs=pl.BlockSpec(memory_space=pl.ANY),
        out_shape=jax.ShapeDtypeStruct((H, C, W), x.dtype),
        scratch_shapes=[
            pltpu.VMEM((2 * (WS + 2), C, W), x.dtype),
            pltpu.VMEM((2 * WS, C, W), x.dtype),
            pltpu.SemaphoreType.DMA((2 + NG // FG,)),
            pltpu.VMEM((X0_ROWS, LANES), F32),
            pltpu.VMEM((WS * WP, LANES), F32),
            pltpu.VMEM((9, C, LANES), F32),
            pltpu.VMEM((3, 5, LANES // 2, LANES), U32),
            pltpu.VMEM((3, C // 2, LANES), U32),
            pltpu.VMEM((5, WS, WP + 8, LANES), F32),
            pltpu.VMEM((NU, 3, LANES // 2, LANES), U32),
            pltpu.VMEM(((W // WS + 1) // 2, LANES, LANES), F32),
            pltpu.VMEM((WS * NT, 16, LANES), F32),
            pltpu.VMEM((C, WP), F32),
        ],
        compiler_params=pltpu.CompilerParams(
            vmem_limit_bytes=64 * 1024 * 1024,
            disable_bounds_checks=True,
        ),
        name="davit_window_attn",
    )(xt, dw_pe, w_qkv, w_o)
    return jnp.transpose(yt, (0, 2, 1))[None]
```

```python
import functools
import math

import jax
import jax.numpy as jnp
from jax import lax
import jax.experimental.pallas as pl
import jax.experimental.pallas.tpu as pltpu

WS = 7
NH = 4
C = 192
DH = C // NH
NG = C // 8
LANES = 128
WP = 512
NT = WP // LANES
NU = WS * NT // 2
SLOTS = 8 * WS
EPS = 1e-5
F32 = jnp.float32
BF16 = jnp.bfloat16
U32 = jnp.uint32

X0_SLOT = WS * NT * C
DW_OFF = 3 * X0_SLOT
X0_ROWS = DW_OFF + 2 * C

FG = 8
NSTX = 24


def _dot(a, b):
    return jnp.dot(a, b, preferred_element_type=F32)


def _dot_nt(a, b):
    return lax.dot_general(a, b, (((1,), (1,)), ((), ())), preferred_element_type=F32)


def _cat(xs):
    return jnp.concatenate(xs, axis=0)


def _blocks(v):
    return [v[i:i + 8] for i in range(0, v.shape[0], 8)]


def _allred(x, op):
    for sh in (4, 2, 1):
        x = op(x, pltpu.roll(x, sh, 0))
    return x


def _round_bits(x):
    return pltpu.bitcast(x, U32) + jnp.uint32(0x8000)


def _hi(w):
    return w & jnp.uint32(0xFFFF0000)


def _halves(w):
    return pltpu.bitcast(w << 16, F32), pltpu.bitcast(_hi(w), F32)


def _run(prog, extra):
    extra = sorted(extra, key=lambda e: e[0])
    j = 0
    for t0, fn in prog:
        while j < len(extra) and extra[j][0] <= t0:
            extra[j][1]()
            j += 1
        fn()
    for e in extra[j:]:
        e[1]()


def _kernel(*refs, H, W):
    nstrip = H // WS
    for lo, hi, mode in ((0, 1, "first"), (1, nstrip + 1, "main"), (nstrip + 1, nstrip + 2, "last")):
        def body(k, carry, mode=mode):
            _step(*refs, H=H, W=W, k_=k, mode=mode)
            return carry
        lax.fori_loop(lo, hi, body, 0)


def _step(x_hbm, dw_ref, wqkv_ref, wo_ref, o_hbm,
          x_ref, o_ref, sems, x0_ref, ob_ref, dws_ref, ws_ref, wos_ref, qkv_ref, t_ref, stg_ref, ms_ref,
          top_ref, *, H, W, k_, mode):
    nstrip, nwin = H // WS, W // WS
    npair = (nwin + 1) // 2

    def x_copy(k):
        return pltpu.make_async_copy(x_hbm.at[pl.ds(jnp.minimum(k * WS, H - WS - 1), WS + 1)],
                                     x_ref.at[pl.ds((k & 1) * (WS + 2), WS + 1)], sems.at[0])

    def o_copy(k):
        return pltpu.make_async_copy(o_ref.at[pl.ds((k & 1) * WS, WS)], o_hbm.at[pl.ds(k * WS, WS)],
                                     sems.at[1])

    def x0_copy(g):
        cs = pl.ds(pl.multiple_of(g * (8 * FG), 8 * FG), 8 * FG)
        return pltpu.make_async_copy(x_hbm.at[pl.ds(0, WS + 1), cs], x_ref.at[pl.ds(0, WS + 1), cs],
                                     sems.at[2 + g])

    def row_copy(r):
        return pltpu.make_async_copy(o_ref.at[sc["ooff"] + r], o_hbm.at[H - WS + r], sems.at[2])

    def when(cond, modes):
        return pl.when(cond) if mode in modes else (lambda f: None)

    sc = {}

    def new_scalars():
        k3 = k_ - 3 * ((k_ * 171) >> 9)
        sc["nxt"] = k3 * X0_SLOT
        sc["prv"] = jnp.where((k3 == 2) | (k_ < 2), 0, sc["nxt"] + X0_SLOT)
        sc["xoff"] = (k_ & 1) * (WS + 2) + jnp.where(k_ >= nstrip - 1, 1, 0)
        sc["ooff"] = (k_ & 1) * WS

    dyn0 = jnp.minimum(k_, 0)

    def rows_at(base, off, n):
        if isinstance(base, int):
            return pl.ds(base + off, n)
        return pl.ds(pl.multiple_of(base + off, 8), n)

    mk = {}

    def new_masks(blk):
        lane = lax.broadcasted_iota(jnp.int32, (8, LANES), 1)
        mk.clear()
        mk["never"] = lane < dyn0
        if blk == "y":
            key_ok = lax.broadcasted_iota(jnp.int32, (8, LANES), 0) < WS
            mk.update(
                lo=lane < DH, hi0=(lane >= DH) & ((lane < 64) | (lane >= 96)),
                hi1=(lane >= DH) & (lane < 96), v=lane < 96, key=key_ok,
                keep_a=key_ok & (lane < SLOTS), keep_b=key_ok & (lane >= SLOTS), left64=lane < 64,
                left=lane < SLOTS)

    conv_done = []

    def conv_group(c0):
        st = {}

        def row(i):
            if i == 0 and i not in st:
                st[i] = top_ref[pl.ds(c0, 8), :]
            if i not in st:
                v = x_ref[sc["xoff"] + (i - 1), pl.ds(c0, 8), :].astype(F32)
                st[i] = jnp.concatenate([v, jnp.zeros((8, WP - W), F32)], axis=1)
                if i == WS:
                    top_ref[pl.ds(c0, 8), :] = st[i]
            return st[i]

        def bc(v):
            return jnp.concatenate([v] * NT, axis=1)

        def taps(r):
            st["tw", r] = [bc(x0_ref[rows_at(c0, DW_OFF + k * C, 8), :]) for k in range(2)]

        def piece(r):
            if "w" not in st:
                st["w"] = [bc(dws_ref[k, pl.ds(c0, 8), :]) for k in range(9)]
            wts = list(st["w"])
            if ("tw", r) in st:
                wts[6], wts[8] = st["tw", r]
            row(r)
            abc = [row(r + 1) * wts[3 + j] + row(r) * wts[j] + row(r + 2) * wts[6 + j] for j in range(3)]
            x0 = pltpu.roll(abc[0], 1, 1) + abc[1] + pltpu.roll(abc[2], WP - 1, 1)
            for t in range(NT):
                x0_ref[rows_at(sc["nxt"], (r * NT + t) * C + c0, 8), :] = x0[:, t * LANES:(t + 1) * LANES]
            conv_done.append(r)

        return taps, piece

    def conv_items(nslow):
        groups = [conv_group(8 * g) for g in range(NG)]
        plist = [(g, r) for g in range(NG) for r in range(WS)]
        items, tap = [], 4
        for k, (g, r) in enumerate(plist):
            fs = []
            while tap <= min(k + (4 if k < nslow else 5), len(plist) - 1):
                fs.append(functools.partial(groups[plist[tap][0]][0], plist[tap][1]))
                tap += 1
            fs.append(functools.partial(groups[g][1], r))
            items.append(fs)
        return items

    @when(k_ == 0, ("first",))
    def _():
        for g in range(NG // FG):
            x0_copy(g).start()
        for k in range(9):
            w = dw_ref[k // 3].astype(F32)[k % 3:k % 3 + 1, :]
            w = jnp.broadcast_to(w, (LANES, C)).T
            dws_ref[k] = w + 1.0 if k == 4 else w
            if k in (6, 8):
                x0_ref[pl.ds(DW_OFF + (k - 6) // 2 * C, C), :] = w
        w = wqkv_ref[...].astype(F32)
        wq = w[:, 0:C] * ((DH ** -0.5) * math.log2(math.e))
        wk, wv = w[:, C:2 * C], w[:, 2 * C:3 * C]
        tiles = [(wq[:, 0:64], wv[:, 64:96], wq[:, 64:96]),
                 (wq[:, 96:192], wv[:, 96:128]),
                 (wk[:, 0:64], wv[:, 128:160], wk[:, 64:96]),
                 (wk[:, 96:192], wv[:, 160:192]),
                 (wv[:, 0:128],)]
        for n, parts in enumerate(tiles):
            w = jnp.concatenate(parts, axis=1)
            for i, wi in enumerate((w[0:128], w[64:192], _cat([w[0:64], w[128:192]]))):
                if n == 4:
                    wi = wi.T
                ws_ref[i, n] = pltpu.bitcast(wi.astype(BF16), U32)
        w = wo_ref[...].astype(F32)
        wx, wy, wz = w[0:64], w[64:128], w[128:192]
        for i, parts in enumerate(((wx, wy), (wz, wy), (wx, wy + wz))):
            wos_ref[i] = pltpu.bitcast(_cat(parts).T.astype(BF16), U32)

        top_ref[...] = jnp.zeros(top_ref.shape, F32)
        for i in (WS + 1, 2 * WS + 3):
            x_ref[i] = jnp.zeros(x_ref.shape[1:], x_ref.dtype)
        for p in range(npair):
            stg_ref[p] = jnp.zeros(stg_ref.shape[1:], F32)
        for r in range(WS):
            ob_ref[pl.ds(r * WP + WP - 8, 8), :] = jnp.zeros((8, LANES), F32)

    def ld_x0(j, k, gs):
        return [x0_ref[rows_at(sc["nxt"] + dyn0 * (8 * k), j * C + 8 * g, 8), :] for g in gs]

    def add2(acc, xs):
        a = functools.reduce(jnp.add, xs[0::2])
        b = functools.reduce(jnp.add, xs[1::2])
        return a + b if acc is None else (acc + a) + b

    stats_done = set()

    def stats_steps(j):
        st = {"s": None, "q": None}

        def sum_step(g0):
            assert mode != "main" or len(conv_done) == NG * WS
            st["s"] = add2(st["s"], ld_x0(j, 0, range(g0, g0 + 12)))
            if g0 + 12 == NG:
                st["s"] = _allred(st["s"], jnp.add) * (1.0 / C)
            return st["s"]

        def var_step(g0):
            d = [x - st["s"] for x in ld_x0(j, 1, range(g0, g0 + 6))]
            st["q"] = add2(st["q"], [x * x for x in d])
            return st["q"]

        def last_step():
            rs = lax.rsqrt(_allred(st["q"], jnp.add) * (1.0 / C) + EPS)
            ms_ref[j] = _cat([st["s"], rs])
            stats_done.add(j)
            return rs

        return ([functools.partial(sum_step, g) for g in range(0, NG, 12)]
                + [functools.partial(var_step, g) for g in range(0, NG, 6)] + [last_step])

    def wave_steps(lo, hi):
        steps = []
        for j0 in range(lo, hi, 4):
            for grp in zip(*[stats_steps(j) for j in range(j0, j0 + 4)]):
                steps += grp
        return steps

    def normed(j, blk, k=0):
        assert j in stats_done
        m, rs = ms_ref[j, 0:8, :], ms_ref[j, 8:16, :]
        return _cat([(x - m) * rs for x in ld_x0(j, k, range(8 * blk, 8 * blk + 8))])

    t_done = {}

    def put_t(dst, tiles):
        tt = pltpu.bitcast(jnp.concatenate(tiles, axis=1).astype(BF16).T, U32)
        for i, (u, e) in enumerate(dst):
            t_ref[u, e] = tt[64 * i:64 * i + 64]
        t_done[len(t_done)] = pltpu.bitcast(tt[120:128], F32)

    def t_first(u):
        ja, jb = 2 * u, 2 * u + 1
        bx = normed(jb, 0)
        put_t([(u, 0), (u, 2)], [_cat([normed(ja, 0) - bx, normed(ja, 1)]), _cat([bx, normed(ja, 2)])])

    def t_second(r):
        put_t([(u, 1) for u in (2 * r, 2 * r + 1)],
              [_cat([normed(2 * u + 1, 1), normed(2 * u + 1, 2) - normed(2 * u, 2, 1)])
               for u in (2 * r, 2 * r + 1)])

    t_items = []
    for r in range(WS):
        t_items += [functools.partial(t_first, 2 * r), functools.partial(t_first, 2 * r + 1),
                    functools.partial(t_second, r)]

    def qkv_chunk(us, n, steps):
        lhs = {i: [b for u in us for b in _blocks(t_ref[u, i])] for i in range(3)}
        for q, step in enumerate(steps):
            tok = pltpu.bitcast(step(), U32)
            q = q * 24 * len(us) // len(steps)
            blks = lhs[(2, 0, 1)[q % 3]]
            blks[q // 3] = jnp.where(mk["never"], tok, blks[q // 3])
        p3 = None
        for i in (2, 0, 1):
            p = _dot(pltpu.bitcast(_cat(lhs[i]), BF16), pltpu.bitcast(ws_ref[i, n], BF16))
            if p3 is None:
                p3 = p
            else:
                p = p + p3
                for e, u in enumerate(us):
                    r, tp = divmod(u, 2)
                    qkv_ref[n, r, pl.ds((2 * tp + i) * LANES, LANES), :] = p[e * LANES:(e + 1) * LANES]

    vr_words = {}
    job_done = {}

    def side_dots(u, n):
        r, tp = divmod(u, 2)
        st = {}

        def one(i, parts=1):
            if parts > 1:
                lhs, rows = t_ref[u, i], 64 // parts
                p = _cat([_dot(pltpu.bitcast(lhs[q * rows:(q + 1) * rows], BF16),
                               pltpu.bitcast(ws_ref[i, n], BF16)) for q in range(parts)])
            elif n == 4:
                p = _dot_nt(pltpu.bitcast(ws_ref[i, 4, 0:32, :], BF16), pltpu.bitcast(t_ref[u, i], BF16))
            else:
                p = _dot(pltpu.bitcast(t_ref[u, i], BF16), pltpu.bitcast(ws_ref[i, n], BF16))
            st[i] = p if i == 2 else p + st[2]
            if n < 4 and i < 2:
                qkv_ref[n, r, pl.ds((2 * tp + i) * LANES, LANES), :] = st[i]
            elif i == 1:
                vr_words[u] = (_round_bits(st[0]) >> 16) | _hi(_round_bits(st[1]))

        return [(64 if n == 4 else LANES, (u, n, i), functools.partial(one, i)) for i in (2, 0, 1)]

    def vr_store(u):
        r, tp = divmod(u, 2)
        w = pltpu.bitcast(vr_words[u], F32)
        wt = pltpu.bitcast(_cat([w, w]).T, U32)
        job_done["v", u] = pltpu.bitcast(wt[120:128], F32)
        for j in range(2):
            qkv_ref[4, r, pl.ds((2 * tp + j) * LANES, LANES), :] = _halves(wt)[j]

    zero8 = jnp.zeros((8, LANES), F32)

    def gather(n, off):
        return [qkv_ref[n, r, pl.ds(off, 8), :] for r in range(WS)]

    def softmax_t(st):
        rows = _blocks(st)
        m = functools.reduce(jnp.maximum, rows)
        m = _allred(jnp.where(mk["key"], m, -jnp.inf), jnp.maximum)
        p = [jnp.exp2(x - m) for x in rows]
        return p, functools.reduce(jnp.add, p)

    def s2_pair(pi, offa):
        single = pi == 0
        offb = offa if single else offa + WS
        st = {}

        def vprep():
            g = [gather(n, a) + gather(n, b) for n in range(5)
                 for a, b in [(offa + dyn0 * 3, offb + dyn0 * 3) if n in (2, 3) else (offa, offb)]]
            u1 = [jnp.where(mk["left64"], z, jnp.where(mk["v"], x, y)) for x, y, z in zip(g[0], g[1], g[4])]
            u2 = [jnp.where(mk["v"], x, y) for x, y in zip(g[2], g[3])]
            u = jnp.concatenate([_cat(u1 + [zero8, zero8]), _cat(u2 + [zero8, zero8])], axis=1)
            vt = pltpu.bitcast(u.astype(BF16).T, U32)
            vt = _cat([vt[0:64], vt[96:128]])
            if single:
                b = _blocks(vt)
                vt = _cat([jnp.where(mk["left"], b[i], b[i + 3]) for i in (0, 1, 2) * 2 + (6, 7, 8) * 2])
            st["vt"] = [pltpu.bitcast(vt[24 * h:24 * h + 24], BF16) for h in range(NH)]

        def score(i, ties):
            hp, sw = divmod(i, 2)
            lo, hi = mk["lo"], mk["hi%d" % hp]
            ma, mb = (lo, hi) if sw == 0 else (hi, lo)
            q = _cat([jnp.where(ma, v, 0.0) for v in gather(hp, offa)]
                     + [jnp.where(mb, v, 0.0) for v in gather(hp, offb)] + [zero8, zero8])
            ka, kb = gather(2 + hp, offa), gather(2 + hp, offb)
            k = ka if single else [jnp.where(lo, x, y) for x, y in (zip(ka, kb) if sw == 0 else zip(kb, ka))]
            for _, job in ties:
                k[0] = jnp.where(mk["never"], job(), k[0])
            st["p", i] = softmax_t(_dot_nt(_cat(k), q))

        def value(h):
            hp, sw = divmod(h, 2)
            (pa, sa), (pb, sb) = st["p", h], st["p", h if single else 2 * hp + 1 - sw]
            pm = _cat([jnp.where(mk["keep_a"], v, 0.0) for v in pa]
                      + [jnp.where(mk["keep_b"], v, 0.0) for v in pb] + [zero8, zero8])
            den = _allred(jnp.where(mk["keep_a"], sa, jnp.where(mk["keep_b"], sb, 0.0)), jnp.add)
            rec = pl.reciprocal(den, approx=True)
            st["o", h] = [b * rec for b in _blocks(_dot(st["vt"][h], pm))]
            if single:
                st["o", h + 1] = [jnp.where(mk["left"], 0.0, b) for b in st["o", h]]
                st["o", h] = [jnp.where(mk["left"], b, 0.0) for b in st["o", h]]

        def finish():
            o = [_round_bits(b) for h in range(NH) for b in st["o", h]]
            hi = [_hi(b) for b in o[16:24]]
            w = _cat([(b >> 16) | z for b, z in zip(o[0:16], hi + hi)])
            stg_ref[pi] = pltpu.bitcast(w, F32)

        def scatter():
            wt = stg_ref[pi].T
            job_done["s", pi] = wt[104:112]
            if single:
                wt = pltpu.bitcast(pltpu.bitcast(wt[0:SLOTS], U32)
                                   | pltpu.bitcast(wt[SLOTS:2 * SLOTS], U32), F32)
            for i, off in enumerate((offa,) if single else (offa, offb)):
                for r in range(WS):
                    base = i * SLOTS + 8 * r
                    ob_ref[pl.ds(r * WP + off, WS), :] = wt[base:base + WS]

        return vprep, score, value, finish, scatter

    pairs = [s2_pair(p, (2 * p - 2 if p else nwin - 1) * WS) for p in range(npair)]

    def s3_unit(r, tp, ties=()):
        def unpack(t):
            w = pltpu.bitcast(ob_ref[pl.ds(r * WP + t * LANES, LANES), :], U32)
            return [_blocks(v) for v in _halves(w)]

        (la, ha), (lb, hb) = unpack(2 * tp), unpack(2 * tp + 1)
        t3 = [jnp.where(mk["left64"], x, y) for x, y in zip(lb, ha)]
        t1 = _cat([x - y for x, y in zip(la, t3)])
        t2 = _cat([jnp.where(mk["left64"], x, z) - y for x, y, z in zip(hb, ha, lb)])
        t3 = _cat(t3)
        wo = [_blocks(wos_ref[i]) for i in range(3)]
        for q, (e, job) in enumerate(ties):
            blks = wo[(2, 0, 1)[q % 3]]
            blks[e] = jnp.where(mk["never"], pltpu.bitcast(job(), U32), blks[e])
        wo = [pltpu.bitcast(_cat(w), BF16) for w in wo]
        p3 = _dot_nt(wo[2], t3)
        ys = [_dot_nt(wo[i], t) + p3
              + x0_ref[rows_at(sc["prv"], (r * NT + 2 * tp + i) * C, C), :] for i, t in enumerate((t1, t2))]
        n = min(2 * LANES, W - 2 * tp * LANES)
        o_ref[sc["ooff"] + r, :, pl.ds(2 * tp * LANES, n)] = (
            jnp.concatenate(ys, axis=1).astype(o_ref.dtype)[:, :n])

    s3_all = [functools.partial(s3_unit, r, tp) for tp in range(2) for r in range(WS)]

    def block_x():
        new_scalars()
        njob = 28
        steps = wave_steps(0, NSTX)
        chunks = [(u, n) for u in range(NU) for n in range(4)]
        side = side_dots(*chunks.pop())
        for u in range(NU):
            side += side_dots(u, 4)
        for _ in range(8):
            side += side_dots(*chunks.pop())
        merged = []
        for u, n in chunks:
            prev = [c for c in merged if c[1] == n and c[0][0] // 2 == u // 2]
            if prev:
                prev[0][0].append(u)
            else:
                merged.append(([u], n))
        t_conv = (len(chunks) - 7) * LANES
        span = len(chunks) * LANES - t_conv
        plan, t, vr_ready = [], 0, {}
        for k, (us, n) in enumerate(merged):
            dur = LANES * len(us)
            assert not t < t_conv < t + dur
            lo, hi = (max(x - t_conv, 0) * len(steps) // span for x in (t, t + dur))
            plan.append((t, tuple(us), n, list(steps[lo:hi])))
            room = dur
            while side and (room > 0 or k == len(merged) - 1):
                rows, key, f = side.pop(0)
                plan.append((t, f if room > 0 else functools.partial(f, 4), None, []))
                room -= rows
                if key[1:] == (4, 1):
                    vr_ready[key[0]] = t + dur - room + 150
            t += dur
        ci = conv_items(4 * njob)
        fast = (t_conv - 4 * njob * 32.0) / (len(ci) - 4 * njob)
        t_piece = [min(min(j, 4 * njob) * 32.0 + max(j - 4 * njob, 0) * fast, t_conv)
                   for j in range(len(ci) + 1)]
        scat, vrs = list(range(npair)), list(range(NU))
        jobs = []
        for q in range(njob):
            if vrs and vr_ready[vrs[0]] <= t_piece[4 * q + 1]:
                jobs.append((t_piece[4 * q + 1], ("v", vrs[0])))
                ci[4 * q].insert(0, functools.partial(vr_store, vrs.pop(0)))
            elif scat:
                jobs.append((t_piece[4 * q + 1], ("s", scat[0])))
                ci[4 * q].insert(0, pairs[scat.pop(0)][4])
        extra = [(t_piece[j + 1], f) for j, fs in enumerate(ci) for f in fs]
        tail = ([(("v", u), functools.partial(vr_store, u)) for u in vrs]
                + [(("s", p), pairs[p][4]) for p in scat])
        for q, (key, f) in enumerate(tail):
            t_q = max(t_conv + 1 + (q // 3) * 128, vr_ready[key[1]] if key[0] == "v" else 0)
            extra.append((t_q, f))
            jobs.append((t_q, key))
        for t_q, key in jobs:
            later = [e for e in plan if e[2] is not None and e[0] >= t_q + 800]
            if later:
                later[0][3].insert(0, functools.partial(job_done.get, key))
        _run([(t0, u if n is None else functools.partial(qkv_chunk, u, n, st)) for t0, u, n, st in plan],
             extra)

    def block_y():
        new_scalars()
        pattern = "SFFVFFFF" + "SSSSFVVVV" * 8 + "SSSSVVVV"
        load = [0] * 4
        items, cnt = [], {"S": 0, "V": 0, "F": 0}
        for ch in pattern:
            for _ in range(1 if ch == "F" else 4):
                cnt[ch] += 1
                if ch != "F" and cnt[ch] in (2, 4):
                    continue
                items.append((min(load), ch, cnt[ch] - 1, []))
                for x in {"S": [SLOTS], "V": [DH], "F": [C] * 3}[ch]:
                    load[load.index(min(load))] += x
        assert cnt == {"S": 4 * npair, "V": 4 * npair, "F": NU}
        spots = sorted([(it[0], it, 0) for it in items if it[1] == "S"]
                       + [(it[0] + 16 * e, it, e) for it in items if it[1] == "F" for e in range(12)],
                       key=lambda x: x[0])
        steps = wave_steps(NSTX, WS * NT)
        fspots = sorted([x for x in spots if x[1][1] == "F" and x[1][2] < 5],
                        key=lambda x: (x[1][2], x[2]))
        for q, step in enumerate(steps):
            _, it, e = fspots[q * len(fspots) // len(steps)]
            it[3].append((e, step))
        late = sorted([x for x in spots if x[1][1] == "S" and x[1][2] % 16 in (14, 15)],
                      key=lambda x: x[1][2])
        n1 = len(t_items) - len(late)
        extra = []
        for j, f in enumerate(t_items):
            if j < n1:
                t_s, it, e = [x for x in spots if x[0] >= 400 + j * 500 / n1][0]
            else:
                t_s, it, e = late[j - n1]
            it[3].append((e, functools.partial(t_done.get, j)))
            extra.append((min(t_s - 450, it[0]), f))
        prog = []
        for t0, ch, idx, ties in items:
            p, i = divmod(idx, 4)
            if ch == "S":
                if i == 0:
                    prog.append((t0, pairs[p][0]))
                prog.append((t0, functools.partial(pairs[p][1], i, ties)))
            elif ch == "V":
                prog.append((t0, functools.partial(pairs[p][2], i)))
                if i == 3 or idx == 2:
                    extra.append((t0 + DH, pairs[p][3]))
            else:
                prog.append((t0, functools.partial(s3_all[idx], ties)))
        _run(prog, extra)

    if mode != "main":
        new_scalars()

    @when(k_ < nstrip, ("main",))
    def _():
        x_copy(k_).wait()

    @when(k_ < nstrip - 1, ("first", "main"))
    def _():
        x_copy(k_ + 1).start()

    new_masks("x")
    when(k_ <= nstrip, ("main",))(block_x)

    @when(k_ == 0, ("first",))
    def _():
        def body(g, carry):
            x0_copy(g).wait()
            for j in range(FG):
                piece = conv_group(pl.multiple_of((g * FG + j) * 8, 8))[1]
                for r in range(WS):
                    piece(r)
            return carry
        lax.fori_loop(0, NG // FG, body, 0)

    @when(k_ >= 4, ("main", "last"))
    def _():
        o_copy(k_ - 4).wait()

    @when(k_ >= 3, ("main", "last"))
    def _():
        o_copy(k_ - 3).start()

    new_masks("y")
    when((k_ <= nstrip) & (k_ >= 1), ("main",))(block_y)

    @when(k_ == 0, ("first",))
    def _():
        for j in range(WS * NT):
            for f in stats_steps(j):
                f()
        for f in t_items:
            f()

    @when(k_ == nstrip + 1, ("last",))
    def _():
        new_masks("y")
        for p in range(npair):
            pairs[p][4]()
        for q, f in enumerate(s3_all):
            f()
            if q >= WS:
                row_copy(q - WS).start()

    @when(k_ == nstrip + 1, ("last",))
    def _():
        o_copy(k_ - 3).wait()
        for r in range(WS):
            row_copy(r).wait()


@jax.jit
def pallas_standalone__window_attn_davit__vision_kernel(
    x: jax.Array,
    dw_pe: jax.Array,
    w_qkv: jax.Array,
    w_o: jax.Array,
):
    B, H, W, Cx = x.shape
    assert B == 1 and Cx == C and W == WP - 1 and H % WS == 0 and 3 <= H // WS <= 250
    xt = jnp.transpose(x[0], (0, 2, 1))

    vmem = pl.BlockSpec(memory_space=pltpu.VMEM)
    yt = pl.pallas_call(
        functools.partial(_kernel, H=H, W=W),
        in_specs=[pl.BlockSpec(memory_space=pl.ANY), vmem, vmem, vmem],
        out_specs=pl.BlockSpec(memory_space=pl.ANY),
        out_shape=jax.ShapeDtypeStruct((H, C, W), x.dtype),
        scratch_shapes=[
            pltpu.VMEM((2 * (WS + 2), C, W), x.dtype),
            pltpu.VMEM((2 * WS, C, W), x.dtype),
            pltpu.SemaphoreType.DMA((2 + NG // FG,)),
            pltpu.VMEM((X0_ROWS, LANES), F32),
            pltpu.VMEM((WS * WP, LANES), F32),
            pltpu.VMEM((9, C, LANES), F32),
            pltpu.VMEM((3, 5, LANES // 2, LANES), U32),
            pltpu.VMEM((3, C // 2, LANES), U32),
            pltpu.VMEM((5, WS, WP + 8, LANES), F32),
            pltpu.VMEM((NU, 3, LANES // 2, LANES), U32),
            pltpu.VMEM(((W // WS + 1) // 2, LANES, LANES), F32),
            pltpu.VMEM((WS * NT, 16, LANES), F32),
            pltpu.VMEM((C, WP), F32),
        ],
        compiler_params=pltpu.CompilerParams(
            vmem_limit_bytes=64 * 1024 * 1024,
            disable_bounds_checks=True,
        ),
        name="davit_window_attn",
    )(xt, dw_pe, w_qkv, w_o)
    return jnp.transpose(yt, (0, 2, 1))[None]
```

```python
import functools
import math

import jax
import jax.numpy as jnp
from jax import lax
import jax.experimental.pallas as pl
import jax.experimental.pallas.tpu as pltpu

WS = 7
NH = 4
C = 192
DH = C // NH
NG = C // 8
LANES = 128
WP = 512
NT = WP // LANES
NU = WS * NT // 2
SLOTS = 8 * WS
EPS = 1e-5
F32 = jnp.float32
BF16 = jnp.bfloat16
U32 = jnp.uint32

X0_SLOT = WS * NT * C
DW_OFF = 3 * X0_SLOT
X0_ROWS = DW_OFF + 2 * C

FG = 8
NSTX = 24


def _dot(a, b):
    return jnp.dot(a, b, preferred_element_type=F32)


def _dot_nt(a, b):
    return lax.dot_general(a, b, (((1,), (1,)), ((), ())), preferred_element_type=F32)


def _cat(xs):
    return jnp.concatenate(xs, axis=0)


def _blocks(v):
    return [v[i:i + 8] for i in range(0, v.shape[0], 8)]


def _allred(x, op):
    for sh in (4, 2, 1):
        x = op(x, pltpu.roll(x, sh, 0))
    return x


def _round_bits(x):
    return pltpu.bitcast(x, U32) + jnp.uint32(0x8000)


def _hi(w):
    return w & jnp.uint32(0xFFFF0000)


def _halves(w):
    return pltpu.bitcast(w << 16, F32), pltpu.bitcast(_hi(w), F32)


def _run(prog, extra):
    extra = sorted(extra, key=lambda e: e[0])
    j = 0
    for t0, fn in prog:
        while j < len(extra) and extra[j][0] <= t0:
            extra[j][1]()
            j += 1
        fn()
    for e in extra[j:]:
        e[1]()


def _kernel(*refs, H, W):
    nstrip = H // WS
    for lo, hi, mode in ((0, 1, "first"), (1, nstrip + 1, "main"), (nstrip + 1, nstrip + 2, "last")):
        def body(k, carry, mode=mode):
            _step(*refs, H=H, W=W, k_=k, mode=mode)
            return carry
        lax.fori_loop(lo, hi, body, 0)


def _step(x_hbm, dw_ref, wqkv_ref, wo_ref, o_hbm,
          x_ref, o_ref, sems, x0_ref, ob_ref, dws_ref, ws_ref, wos_ref, qkv_ref, t_ref, stg_ref, ms_ref,
          top_ref, *, H, W, k_, mode):
    nstrip, nwin = H // WS, W // WS
    npair = (nwin + 1) // 2

    def x_copy(k):
        return pltpu.make_async_copy(x_hbm.at[pl.ds(jnp.minimum(k * WS, H - WS - 1), WS + 1)],
                                     x_ref.at[pl.ds((k & 1) * (WS + 2), WS + 1)], sems.at[0])

    def o_copy(k):
        return pltpu.make_async_copy(o_ref.at[pl.ds((k & 1) * WS, WS)], o_hbm.at[pl.ds(k * WS, WS)],
                                     sems.at[1])

    def x0_copy(g):
        cs = pl.ds(pl.multiple_of(g * (8 * FG), 8 * FG), 8 * FG)
        return pltpu.make_async_copy(x_hbm.at[pl.ds(0, WS + 1), cs], x_ref.at[pl.ds(0, WS + 1), cs],
                                     sems.at[2 + g])

    def row_copy(r):
        return pltpu.make_async_copy(o_ref.at[sc["ooff"] + r], o_hbm.at[H - WS + r], sems.at[2])

    def when(cond, modes):
        return pl.when(cond) if mode in modes else (lambda f: None)

    sc = {}

    def new_scalars():
        k3 = k_ - 3 * ((k_ * 171) >> 9)
        sc["nxt"] = k3 * X0_SLOT
        sc["prv"] = jnp.where((k3 == 2) | (k_ < 2), 0, sc["nxt"] + X0_SLOT)
        sc["xoff"] = (k_ & 1) * (WS + 2) + jnp.where(k_ >= nstrip - 1, 1, 0)
        sc["ooff"] = (k_ & 1) * WS

    dyn0 = jnp.minimum(k_, 0)

    def rows_at(base, off, n):
        if isinstance(base, int):
            return pl.ds(base + off, n)
        return pl.ds(pl.multiple_of(base + off, 8), n)

    mk = {}

    def new_masks(blk):
        lane = lax.broadcasted_iota(jnp.int32, (8, LANES), 1)
        mk.clear()
        mk["never"] = lane < dyn0
        if blk == "y":
            key_ok = lax.broadcasted_iota(jnp.int32, (8, LANES), 0) < WS
            mk.update(
                lo=lane < DH, hi0=(lane >= DH) & ((lane < 64) | (lane >= 96)),
                hi1=(lane >= DH) & (lane < 96), v=lane < 96, key=key_ok,
                keep_a=key_ok & (lane < SLOTS), keep_b=key_ok & (lane >= SLOTS), left64=lane < 64,
                left=lane < SLOTS)

    conv_done = []

    def conv_group(c0):
        st = {}

        def row(i):
            if i == 0 and i not in st:
                st[i] = top_ref[pl.ds(c0, 8), :]
            if i not in st:
                v = x_ref[sc["xoff"] + (i - 1), pl.ds(c0, 8), :].astype(F32)
                st[i] = jnp.concatenate([v, jnp.zeros((8, WP - W), F32)], axis=1)
                if i == WS:
                    top_ref[pl.ds(c0, 8), :] = st[i]
            return st[i]

        def bc(v):
            return jnp.concatenate([v] * NT, axis=1)

        def taps(r):
            st["tw", r] = [bc(x0_ref[rows_at(c0, DW_OFF + k * C, 8), :]) for k in range(2)]

        def piece(r):
            if "w" not in st:
                st["w"] = [bc(dws_ref[k, pl.ds(c0, 8), :]) for k in range(9)]
            wts = list(st["w"])
            if ("tw", r) in st:
                wts[6], wts[8] = st["tw", r]
            row(r)
            abc = [row(r + 1) * wts[3 + j] + row(r) * wts[j] + row(r + 2) * wts[6 + j] for j in range(3)]
            x0 = pltpu.roll(abc[0], 1, 1) + abc[1] + pltpu.roll(abc[2], WP - 1, 1)
            for t in range(NT):
                x0_ref[rows_at(sc["nxt"], (r * NT + t) * C + c0, 8), :] = x0[:, t * LANES:(t + 1) * LANES]
            conv_done.append(r)

        return taps, piece

    def conv_items(nslow):
        groups = [conv_group(8 * g) for g in range(NG)]
        plist = [(g, r) for g in range(NG) for r in range(WS)]
        items, tap = [], 4
        for k, (g, r) in enumerate(plist):
            fs = []
            while tap <= min(k + (4 if k < nslow else 5), len(plist) - 1):
                fs.append(functools.partial(groups[plist[tap][0]][0], plist[tap][1]))
                tap += 1
            fs.append(functools.partial(groups[g][1], r))
            items.append(fs)
        return items

    @when(k_ == 0, ("first",))
    def _():
        for g in range(NG // FG):
            x0_copy(g).start()
        for k in range(9):
            w = dw_ref[k // 3].astype(F32)[k % 3:k % 3 + 1, :]
            w = jnp.broadcast_to(w, (LANES, C)).T
            dws_ref[k] = w + 1.0 if k == 4 else w
            if k in (6, 8):
                x0_ref[pl.ds(DW_OFF + (k - 6) // 2 * C, C), :] = w
        w = wqkv_ref[...].astype(F32)
        wq = w[:, 0:C] * ((DH ** -0.5) * math.log2(math.e))
        wk, wv = w[:, C:2 * C], w[:, 2 * C:3 * C]
        tiles = [(wq[:, 0:64], wv[:, 64:96], wq[:, 64:96]),
                 (wq[:, 96:192], wv[:, 96:128]),
                 (wk[:, 0:64], wv[:, 128:160], wk[:, 64:96]),
                 (wk[:, 96:192], wv[:, 160:192]),
                 (wv[:, 0:128],)]
        for n, parts in enumerate(tiles):
            w = jnp.concatenate(parts, axis=1)
            for i, wi in enumerate((w[0:128], w[64:192], _cat([w[0:64], w[128:192]]))):
                if n == 4:
                    wi = wi.T
                ws_ref[i, n] = pltpu.bitcast(wi.astype(BF16), U32)
        w = wo_ref[...].astype(F32)
        wx, wy, wz = w[0:64], w[64:128], w[128:192]
        for i, parts in enumerate(((wx, wy), (wz, wy), (wx, wy + wz))):
            wos_ref[i] = pltpu.bitcast(_cat(parts).T.astype(BF16), U32)

        top_ref[...] = jnp.zeros(top_ref.shape, F32)
        for i in (WS + 1, 2 * WS + 3):
            x_ref[i] = jnp.zeros(x_ref.shape[1:], x_ref.dtype)
        for p in range(npair):
            stg_ref[p] = jnp.zeros(stg_ref.shape[1:], F32)
        for r in range(WS):
            ob_ref[pl.ds(r * WP + WP - 8, 8), :] = jnp.zeros((8, LANES), F32)

    def ld_x0(j, k, gs):
        return [x0_ref[rows_at(sc["nxt"] + dyn0 * (8 * k), j * C + 8 * g, 8), :] for g in gs]

    def add2(acc, xs):
        a = functools.reduce(jnp.add, xs[0::2])
        b = functools.reduce(jnp.add, xs[1::2])
        return a + b if acc is None else (acc + a) + b

    stats_done = set()

    def stats_steps(j):
        st = {"q": None}

        def mean_step():
            assert mode != "main" or len(conv_done) == NG * WS
            st["s"] = _allred(add2(None, ld_x0(j, 0, range(NG))), jnp.add) * (1.0 / C)
            return st["s"]

        def var_step(g0):
            d = [x - st["s"] for x in ld_x0(j, 1, range(g0, g0 + 6))]
            st["q"] = add2(st["q"], [x * x for x in d])
            return st["q"]

        def last_step():
            rs = lax.rsqrt(_allred(st["q"], jnp.add) * (1.0 / C) + EPS)
            ms_ref[j] = _cat([st["s"], rs])
            stats_done.add(j)
            return rs

        return [mean_step] + [functools.partial(var_step, g) for g in range(0, NG, 6)] + [last_step]

    def wave_steps(lo, hi):
        steps = []
        for j0 in range(lo, hi, 4):
            for grp in zip(*[stats_steps(j) for j in range(j0, j0 + 4)]):
                steps += grp
        return steps

    def normed(j, blk, k=0):
        assert j in stats_done
        m, rs = ms_ref[j, 0:8, :], ms_ref[j, 8:16, :]
        return _cat([(x - m) * rs for x in ld_x0(j, k, range(8 * blk, 8 * blk + 8))])

    t_done = {}

    def put_t(dst, tiles):
        tt = pltpu.bitcast(jnp.concatenate(tiles, axis=1).astype(BF16).T, U32)
        for i, (u, e) in enumerate(dst):
            t_ref[u, e] = tt[64 * i:64 * i + 64]
        t_done[len(t_done)] = pltpu.bitcast(tt[120:128], F32)

    def t_first(u):
        ja, jb = 2 * u, 2 * u + 1
        bx = normed(jb, 0)
        put_t([(u, 0), (u, 2)], [_cat([normed(ja, 0) - bx, normed(ja, 1)]), _cat([bx, normed(ja, 2)])])

    def t_second(r):
        put_t([(u, 1) for u in (2 * r, 2 * r + 1)],
              [_cat([normed(2 * u + 1, 1), normed(2 * u + 1, 2) - normed(2 * u, 2, 1)])
               for u in (2 * r, 2 * r + 1)])

    t_items = []
    for r in range(WS):
        t_items += [functools.partial(t_first, 2 * r), functools.partial(t_first, 2 * r + 1),
                    functools.partial(t_second, r)]

    def qkv_chunk(us, n, steps):
        lhs = {i: [b for u in us for b in _blocks(t_ref[u, i])] for i in range(3)}
        for q, step in enumerate(steps):
            tok = pltpu.bitcast(step(), U32)
            q = q * 24 * len(us) // len(steps)
            blks = lhs[(2, 0, 1)[q % 3]]
            blks[q // 3] = jnp.where(mk["never"], tok, blks[q // 3])
        p3 = None
        for i in (2, 0, 1):
            p = _dot(pltpu.bitcast(_cat(lhs[i]), BF16), pltpu.bitcast(ws_ref[i, n], BF16))
            if p3 is None:
                p3 = p
            else:
                p = p + p3
                for e, u in enumerate(us):
                    r, tp = divmod(u, 2)
                    qkv_ref[n, r, pl.ds((2 * tp + i) * LANES, LANES), :] = p[e * LANES:(e + 1) * LANES]

    vr_words = {}
    job_done = {}

    def side_dots(u, n):
        r, tp = divmod(u, 2)
        st = {}

        def one(i, parts=1):
            if parts > 1:
                lhs, rows = t_ref[u, i], 64 // parts
                p = _cat([_dot(pltpu.bitcast(lhs[q * rows:(q + 1) * rows], BF16),
                               pltpu.bitcast(ws_ref[i, n], BF16)) for q in range(parts)])
            elif n == 4:
                p = _dot_nt(pltpu.bitcast(ws_ref[i, 4, 0:32, :], BF16), pltpu.bitcast(t_ref[u, i], BF16))
            else:
                p = _dot(pltpu.bitcast(t_ref[u, i], BF16), pltpu.bitcast(ws_ref[i, n], BF16))
            st[i] = p if i == 2 else p + st[2]
            if n < 4 and i < 2:
                qkv_ref[n, r, pl.ds((2 * tp + i) * LANES, LANES), :] = st[i]
            elif i == 1:
                vr_words[u] = (_round_bits(st[0]) >> 16) | _hi(_round_bits(st[1]))

        return [(64 if n == 4 else LANES, (u, n, i), functools.partial(one, i)) for i in (2, 0, 1)]

    def vr_store(u):
        r, tp = divmod(u, 2)
        w = pltpu.bitcast(vr_words[u], F32)
        wt = pltpu.bitcast(_cat([w, w]).T, U32)
        job_done["v", u] = pltpu.bitcast(wt[120:128], F32)
        for j in range(2):
            qkv_ref[4, r, pl.ds((2 * tp + j) * LANES, LANES), :] = _halves(wt)[j]

    zero8 = jnp.zeros((8, LANES), F32)

    def gather(n, off):
        return [qkv_ref[n, r, pl.ds(off, 8), :] for r in range(WS)]

    def softmax_t(st):
        rows = _blocks(st)
        m = functools.reduce(jnp.maximum, rows)
        m = _allred(jnp.where(mk["key"], m, -jnp.inf), jnp.maximum)
        p = [jnp.exp2(x - m) for x in rows]
        return p, functools.reduce(jnp.add, p)

    def s2_pair(pi, offa):
        single = pi == 0
        offb = offa if single else offa + WS
        st = {}

        def vprep():
            g = [gather(n, a) + gather(n, b) for n in range(5)
                 for a, b in [(offa + dyn0 * 3, offb + dyn0 * 3) if n in (2, 3) else (offa, offb)]]
            u1 = [jnp.where(mk["left64"], z, jnp.where(mk["v"], x, y)) for x, y, z in zip(g[0], g[1], g[4])]
            u2 = [jnp.where(mk["v"], x, y) for x, y in zip(g[2], g[3])]
            u = jnp.concatenate([_cat(u1 + [zero8, zero8]), _cat(u2 + [zero8, zero8])], axis=1)
            vt = pltpu.bitcast(u.astype(BF16).T, U32)
            vt = _cat([vt[0:64], vt[96:128]])
            if single:
                b = _blocks(vt)
                vt = _cat([jnp.where(mk["left"], b[i], b[i + 3]) for i in (0, 1, 2) * 2 + (6, 7, 8) * 2])
            st["vt"] = [pltpu.bitcast(vt[24 * h:24 * h + 24], BF16) for h in range(NH)]

        def score(i, ties):
            hp, sw = divmod(i, 2)
            lo, hi = mk["lo"], mk["hi%d" % hp]
            ma, mb = (lo, hi) if sw == 0 else (hi, lo)
            q = _cat([jnp.where(ma, v, 0.0) for v in gather(hp, offa)]
                     + [jnp.where(mb, v, 0.0) for v in gather(hp, offb)] + [zero8, zero8])
            ka, kb = gather(2 + hp, offa), gather(2 + hp, offb)
            k = ka if single else [jnp.where(lo, x, y) for x, y in (zip(ka, kb) if sw == 0 else zip(kb, ka))]
            for _, job in ties:
                k[0] = jnp.where(mk["never"], job(), k[0])
            st["p", i] = softmax_t(_dot_nt(_cat(k), q))

        def value(h):
            hp, sw = divmod(h, 2)
            (pa, sa), (pb, sb) = st["p", h], st["p", h if single else 2 * hp + 1 - sw]
            pm = _cat([jnp.where(mk["keep_a"], v, 0.0) for v in pa]
                      + [jnp.where(mk["keep_b"], v, 0.0) for v in pb] + [zero8, zero8])
            den = _allred(jnp.where(mk["keep_a"], sa, jnp.where(mk["keep_b"], sb, 0.0)), jnp.add)
            rec = pl.reciprocal(den, approx=True)
            st["o", h] = [b * rec for b in _blocks(_dot(st["vt"][h], pm))]
            if single:
                st["o", h + 1] = [jnp.where(mk["left"], 0.0, b) for b in st["o", h]]
                st["o", h] = [jnp.where(mk["left"], b, 0.0) for b in st["o", h]]

        def finish():
            o = [_round_bits(b) for h in range(NH) for b in st["o", h]]
            hi = [_hi(b) for b in o[16:24]]
            w = _cat([(b >> 16) | z for b, z in zip(o[0:16], hi + hi)])
            stg_ref[pi] = pltpu.bitcast(w, F32)

        def scatter():
            wt = stg_ref[pi].T
            job_done["s", pi] = wt[104:112]
            if single:
                wt = pltpu.bitcast(pltpu.bitcast(wt[0:SLOTS], U32)
                                   | pltpu.bitcast(wt[SLOTS:2 * SLOTS], U32), F32)
            for i, off in enumerate((offa,) if single else (offa, offb)):
                for r in range(WS):
                    base = i * SLOTS + 8 * r
                    ob_ref[pl.ds(r * WP + off, WS), :] = wt[base:base + WS]

        return vprep, score, value, finish, scatter

    pairs = [s2_pair(p, (2 * p - 2 if p else nwin - 1) * WS) for p in range(npair)]

    def s3_unit(r, tp, ties=()):
        def unpack(t):
            w = pltpu.bitcast(ob_ref[pl.ds(r * WP + t * LANES, LANES), :], U32)
            return [_blocks(v) for v in _halves(w)]

        (la, ha), (lb, hb) = unpack(2 * tp), unpack(2 * tp + 1)
        t3 = [jnp.where(mk["left64"], x, y) for x, y in zip(lb, ha)]
        t1 = _cat([x - y for x, y in zip(la, t3)])
        t2 = _cat([jnp.where(mk["left64"], x, z) - y for x, y, z in zip(hb, ha, lb)])
        t3 = _cat(t3)
        wo = [_blocks(wos_ref[i]) for i in range(3)]
        for q, (e, job) in enumerate(ties):
            blks = wo[(2, 0, 1)[q % 3]]
            blks[e] = jnp.where(mk["never"], pltpu.bitcast(job(), U32), blks[e])
        wo = [pltpu.bitcast(_cat(w), BF16) for w in wo]
        p3 = _dot_nt(wo[2], t3)
        ys = [_dot_nt(wo[i], t) + p3
              + x0_ref[rows_at(sc["prv"], (r * NT + 2 * tp + i) * C, C), :] for i, t in enumerate((t1, t2))]
        n = min(2 * LANES, W - 2 * tp * LANES)
        o_ref[sc["ooff"] + r, :, pl.ds(2 * tp * LANES, n)] = (
            jnp.concatenate(ys, axis=1).astype(o_ref.dtype)[:, :n])

    s3_all = [functools.partial(s3_unit, r, tp) for tp in range(2) for r in range(WS)]

    def block_x():
        new_scalars()
        njob = 28
        steps = wave_steps(0, NSTX)
        chunks = [(u, n) for u in range(NU) for n in range(4)]
        side = side_dots(*chunks.pop())
        for u in range(NU):
            side += side_dots(u, 4)
        for _ in range(8):
            side += side_dots(*chunks.pop())
        merged = []
        for u, n in chunks:
            prev = [c for c in merged if c[1] == n and c[0][0] // 4 == u // 4]
            if prev:
                prev[0][0].append(u)
            else:
                merged.append(([u], n))
        t_conv = (len(chunks) - 7) * LANES
        span = len(chunks) * LANES - t_conv
        plan, t, vr_ready = [], 0, {}
        for k, (us, n) in enumerate(merged):
            dur = LANES * len(us)
            assert not t < t_conv < t + dur
            lo, hi = (max(x - t_conv, 0) * len(steps) // span for x in (t, t + dur))
            plan.append((t, tuple(us), n, list(steps[lo:hi])))
            room = dur
            while side and (room > 0 or k == len(merged) - 1):
                rows, key, f = side.pop(0)
                plan.append((t, f if room > 0 else functools.partial(f, 4), None, []))
                room -= rows
                if key[1:] == (4, 1):
                    vr_ready[key[0]] = t + dur - room + 350
            t += dur
        ci = conv_items(4 * njob)
        fast = (t_conv - 4 * njob * 31.5) / (len(ci) - 4 * njob)
        t_piece = [min(min(j, 4 * njob) * 31.5 + max(j - 4 * njob, 0) * fast, t_conv)
                   for j in range(len(ci) + 1)]
        scat, vrs = list(range(npair)), list(range(NU))
        jobs = []
        for q in range(njob):
            if vrs and vr_ready[vrs[0]] <= t_piece[4 * q + 1]:
                jobs.append((t_piece[4 * q + 1], ("v", vrs[0])))
                ci[4 * q].insert(0, functools.partial(vr_store, vrs.pop(0)))
            elif scat:
                jobs.append((t_piece[4 * q + 1], ("s", scat[0])))
                ci[4 * q].insert(0, pairs[scat.pop(0)][4])
        extra = [(t_piece[j + 1], f) for j, fs in enumerate(ci) for f in fs]
        tail = ([(("v", u), functools.partial(vr_store, u)) for u in vrs]
                + [(("s", p), pairs[p][4]) for p in scat])
        for q, (key, f) in enumerate(tail):
            t_q = max(t_conv + 1 + (q // 3) * 128, vr_ready[key[1]] if key[0] == "v" else 0)
            extra.append((t_q, f))
            jobs.append((t_q, key))
        for t_q, key in jobs:
            later = [e for e in plan if e[2] is not None and e[0] >= t_q + 800]
            if later:
                later[0][3].insert(0, functools.partial(job_done.get, key))
        _run([(t0, u if n is None else functools.partial(qkv_chunk, u, n, st)) for t0, u, n, st in plan],
             extra)

    def block_y():
        new_scalars()
        pattern = "SFFVFFFF" + "SSSSFVVVV" * 8 + "SSSSVVVV"
        load = [0] * 4
        items, cnt = [], {"S": 0, "V": 0, "F": 0}
        for ch in pattern:
            for _ in range(1 if ch == "F" else 4):
                cnt[ch] += 1
                if ch != "F" and cnt[ch] in (2, 4):
                    continue
                items.append((min(load), ch, cnt[ch] - 1, []))
                for x in {"S": [SLOTS], "V": [DH], "F": [C] * 3}[ch]:
                    load[load.index(min(load))] += x
        assert cnt == {"S": 4 * npair, "V": 4 * npair, "F": NU}
        spots = sorted([(it[0], it, 0) for it in items if it[1] == "S"]
                       + [(it[0] + 16 * e, it, e) for it in items if it[1] == "F" for e in range(12)],
                       key=lambda x: x[0])
        steps = wave_steps(NSTX, WS * NT)
        fspots = sorted([x for x in spots if x[1][1] == "F" and x[1][2] < 5],
                        key=lambda x: (x[1][2], x[2]))
        for q, step in enumerate(steps):
            _, it, e = fspots[q * len(fspots) // len(steps)]
            it[3].append((e, step))
        late = sorted([x for x in spots if x[1][1] == "S" and x[1][2] % 16 in (14, 15)],
                      key=lambda x: x[1][2])
        n1 = len(t_items) - len(late)
        extra = []
        for j, f in enumerate(t_items):
            if j < n1:
                t_s, it, e = [x for x in spots if x[0] >= 400 + j * 500 / n1][0]
            else:
                t_s, it, e = late[j - n1]
            it[3].append((e, functools.partial(t_done.get, j)))
            extra.append((min(t_s - 450, it[0]), f))
        prog = []
        for t0, ch, idx, ties in items:
            p, i = divmod(idx, 4)
            if ch == "S":
                if i == 0:
                    prog.append((t0, pairs[p][0]))
                prog.append((t0, functools.partial(pairs[p][1], i, ties)))
            elif ch == "V":
                prog.append((t0, functools.partial(pairs[p][2], i)))
                if i == 3 or idx == 2:
                    extra.append((t0 + DH, pairs[p][3]))
            else:
                prog.append((t0, functools.partial(s3_all[idx], ties)))
        _run(prog, extra)

    if mode != "main":
        new_scalars()

    @when(k_ < nstrip, ("main",))
    def _():
        x_copy(k_).wait()

    @when(k_ < nstrip - 1, ("first", "main"))
    def _():
        x_copy(k_ + 1).start()

    new_masks("x")
    when(k_ <= nstrip, ("main",))(block_x)

    @when(k_ == 0, ("first",))
    def _():
        def body(g, carry):
            x0_copy(g).wait()
            for j in range(FG):
                piece = conv_group(pl.multiple_of((g * FG + j) * 8, 8))[1]
                for r in range(WS):
                    piece(r)
            return carry
        lax.fori_loop(0, NG // FG, body, 0)

    @when(k_ >= 4, ("main", "last"))
    def _():
        o_copy(k_ - 4).wait()

    @when(k_ >= 3, ("main", "last"))
    def _():
        o_copy(k_ - 3).start()

    new_masks("y")
    when((k_ <= nstrip) & (k_ >= 1), ("main",))(block_y)

    @when(k_ == 0, ("first",))
    def _():
        for j in range(WS * NT):
            for f in stats_steps(j):
                f()
        for f in t_items:
            f()

    @when(k_ == nstrip + 1, ("last",))
    def _():
        new_masks("y")
        for p in range(npair):
            pairs[p][4]()
        for q, f in enumerate(s3_all):
            f()
            if q >= WS:
                row_copy(q - WS).start()

    @when(k_ == nstrip + 1, ("last",))
    def _():
        o_copy(k_ - 3).wait()
        for r in range(WS):
            row_copy(r).wait()


@jax.jit
def pallas_standalone__window_attn_davit__vision_kernel(
    x: jax.Array,
    dw_pe: jax.Array,
    w_qkv: jax.Array,
    w_o: jax.Array,
):
    B, H, W, Cx = x.shape
    assert B == 1 and Cx == C and W == WP - 1 and H % WS == 0 and 3 <= H // WS <= 250
    xt = jnp.transpose(x[0], (0, 2, 1))

    vmem = pl.BlockSpec(memory_space=pltpu.VMEM)
    yt = pl.pallas_call(
        functools.partial(_kernel, H=H, W=W),
        in_specs=[pl.BlockSpec(memory_space=pl.ANY), vmem, vmem, vmem],
        out_specs=pl.BlockSpec(memory_space=pl.ANY),
        out_shape=jax.ShapeDtypeStruct((H, C, W), x.dtype),
        scratch_shapes=[
            pltpu.VMEM((2 * (WS + 2), C, W), x.dtype),
            pltpu.VMEM((2 * WS, C, W), x.dtype),
            pltpu.SemaphoreType.DMA((2 + NG // FG,)),
            pltpu.VMEM((X0_ROWS, LANES), F32),
            pltpu.VMEM((WS * WP, LANES), F32),
            pltpu.VMEM((9, C, LANES), F32),
            pltpu.VMEM((3, 5, LANES // 2, LANES), U32),
            pltpu.VMEM((3, C // 2, LANES), U32),
            pltpu.VMEM((5, WS, WP + 8, LANES), F32),
            pltpu.VMEM((NU, 3, LANES // 2, LANES), U32),
            pltpu.VMEM(((W // WS + 1) // 2, LANES, LANES), F32),
            pltpu.VMEM((WS * NT, 16, LANES), F32),
            pltpu.VMEM((C, WP), F32),
        ],
        compiler_params=pltpu.CompilerParams(
            vmem_limit_bytes=64 * 1024 * 1024,
            disable_bounds_checks=True,
        ),
        name="davit_window_attn",
    )(xt, dw_pe, w_qkv, w_o)
    return jnp.transpose(yt, (0, 2, 1))[None]
```
